```python
import jax
import jax.numpy as jnp

def _softmax(x, axis=-1):
    return jax.nn.softmax(x, axis=axis)

def _gelu(x):
    return jax.nn.gelu(x, approximate=True)

def _silu(x):
    return jax.nn.silu(x)

def _sigmoid(x):
    return jax.nn.sigmoid(x)

def _layernorm(x, axis=-1, eps=1e-05):
    m = jnp.mean(x, axis=axis, keepdims=True)
    v = jnp.var(x, axis=axis, keepdims=True)
    return (x - m) / jnp.sqrt(v + eps)

def _scatter_add(tgt, idx, src, axis=0):
    return tgt.at[idx].add(src)

def _segment_sum(src, seg, n):
    return jax.ops.segment_sum(src, seg, n)

class _Rng:

    def __init__(self, key):
        self._k = key

    def _next(self):
        self._k, sub = jax.random.split(self._k)
        return sub

    def normal(self, shape):
        return jax.random.normal(self._next(), shape, dtype=jnp.bfloat16)

    def randint(self, lo, hi, shape):
        return jax.random.randint(self._next(), shape, lo, hi, dtype=jnp.int32)

    def uniform(self, shape, lo=0.0, hi=1.0):
        return jax.random.uniform(self._next(), shape, jnp.bfloat16, lo, hi)

    def permutation(self, n):
        return jax.random.permutation(self._next(), n)
kernel_name = 'adaLN_cond__memory_aug_recurrent_mem_tr__mixer_s_mlp__prompt'

def setup_inputs():
    _rng = _Rng(jax.random.key(int.from_bytes(__import__("os").urandom(4), "little")))
    _w = lambda a: (lambda t: t.astype(jnp.bfloat16) if jnp.issubdtype(t.dtype, jnp.floating) else t)(jnp.asarray(a))

    def _A_setup():
        B, S, Dm = (1, 2048, 1024)
        H, Dh = (32, 128)
        M, seg = (8, 32)
        seg = min(seg, S)
        S = S // seg * seg
        return {'x': _w((lambda *s: _rng.normal(s) * 0.05)(B, S, Dm)), 'mem0': _w((lambda *s: _rng.normal(s) * 0.05)(B, M, Dm)), 'Wq': _w((lambda *s: _rng.normal(s) * 0.05)(Dm, H, Dh) * Dm ** (-0.5)), 'Wk': _w((lambda *s: _rng.normal(s) * 0.05)(Dm, H, Dh) * Dm ** (-0.5)), 'Wv': _w((lambda *s: _rng.normal(s) * 0.05)(Dm, H, Dh) * Dm ** (-0.5)), 'Wo': _w((lambda *s: _rng.normal(s) * 0.05)(H, Dh, Dm) * (H * Dh) ** (-0.5)), 'seg_len': seg}
    _A_in = _A_setup()

    def _B_setup():
        B, S, D, F = (1, 2048, 1024, 3584)
        return {'x': _w((lambda *s: _rng.normal(s) * 0.05)(B, S, D)), 'w1': _w((lambda *s: _rng.normal(s) * 0.05)(D, D) * D ** (-0.5)), 'w2': _w((lambda *s: _rng.normal(s) * 0.05)(D, D) * D ** (-0.5)), 'w3': _w((lambda *s: _rng.normal(s) * 0.05)(D, F) * D ** (-0.5)), 'w4': _w((lambda *s: _rng.normal(s) * 0.05)(F, D) * F ** (-0.5))}
    _B_in = _B_setup()
    return {'A_x': _A_in['x'], 'A_mem0': _A_in['mem0'], 'A_Wq': _A_in['Wq'], 'A_Wk': _A_in['Wk'], 'A_Wv': _A_in['Wv'], 'A_Wo': _A_in['Wo'], 'A_seg_len': _A_in['seg_len'], 'B_x': _B_in['x'], 'B_w1': _B_in['w1'], 'B_w2': _B_in['w2'], 'B_w3': _B_in['w3'], 'B_w4': _B_in['w4'], 'c': _w((lambda *s: _rng.normal(s) * 0.05)(1, 1024)), 'w_mod': _w((lambda *s: _rng.normal(s) * 0.05)(1024, 6 * 1024) * 1024 ** (-0.5))}

def reference(A_x, A_mem0, A_Wq, A_Wk, A_Wv, A_Wo, A_seg_len, B_x, B_w1, B_w2, B_w3, B_w4, c, w_mod):

    def _A_ref(x, mem0, Wq, Wk, Wv, Wo, seg_len):
        B, S, Dm = x.shape
        H, Dh = (Wq.shape[1], Wq.shape[2])
        M = mem0.shape[1]
        scale = Dh ** (-0.5)
        n_seg = S // seg_len
        L = M + seg_len
        idx = jnp.arange(L)
        mask = (idx[:, None] < M) | (idx[:, None] >= idx[None, :])
        mem = mem0
        outs = []
        for s in range(n_seg):
            xs = x[:, s * seg_len:(s + 1) * seg_len, :].copy()
            h = jnp.concatenate([mem, xs], axis=1)
            q = jnp.einsum('btd,dhe->bhte', h, Wq)
            k = jnp.einsum('btd,dhe->bhte', h, Wk)
            v = jnp.einsum('btd,dhe->bhte', h, Wv)
            scores = jnp.einsum('bhqe,bhke->bhqk', q, k) * scale
            scores = jnp.where(mask[None, None], scores, -1000000000.0)
            p = _softmax(scores, axis=-1)
            o = jnp.einsum('bhqk,bhke->bhqe', p, v)
            o = jnp.einsum('bhte,hed->btd', o, Wo)
            mem = o[:, :M, :].copy()
            outs.append(o[:, M:, :])
        return jnp.concatenate(outs, axis=1)

    def _B_ref(x, w1, w2, w3, w4):
        B, S, D = x.shape
        h = _gelu(_layernorm(x, axis=-1) @ w1)
        c = D // 4
        g0 = jnp.pad(h[:, :, 0 * c:1 * c], ((0, 0), (1, 0), (0, 0)))[:, :S, :]
        g1 = jnp.pad(h[:, :, 1 * c:2 * c], ((0, 0), (0, 1), (0, 0)))[:, 1:, :]
        g2 = jnp.pad(h[:, :, 2 * c:3 * c], ((0, 0), (2, 0), (0, 0)))[:, :S, :]
        g3 = jnp.pad(h[:, :, 3 * c:], ((0, 0), (0, 2), (0, 0)))[:, 2:, :]
        hs = jnp.concatenate([g0, g1, g2, g3], axis=-1) @ w2
        x1 = x + hs
        h2 = _gelu(_layernorm(x1, axis=-1) @ w3) @ w4
        return x1 + h2
    x = A_x
    mod = (_silu(c) @ w_mod).reshape(c.shape[0], 6, 1, -1)
    sa, ca, ga, sb, cb, gb = (mod[:, 0].copy(), mod[:, 1].copy(), mod[:, 2].copy(), mod[:, 3].copy(), mod[:, 4].copy(), mod[:, 5].copy())
    h = _layernorm(x, axis=-1) * (1 + ca) + sa
    x = x + ga * _A_ref(h, A_mem0, A_Wq, A_Wk, A_Wv, A_Wo, A_seg_len)
    h = _layernorm(x, axis=-1) * (1 + cb) + sb
    x = x + gb * _B_ref(h, B_w1, B_w2, B_w3, B_w4)
    return x
```

```python
import functools

import jax
import jax.numpy as jnp
from jax import lax
import jax.experimental.pallas as pl
import jax.experimental.pallas.tpu as pltpu

F32 = jnp.float32
BF16 = jnp.bfloat16
U32 = jnp.uint32

S = 2048
D = 1024
H = 32
E = 128
M = 8
SEG = 32
FF = 3584
EPS = 1e-5

LEAD = 512
RING = 288
SL = 520
HG = 16
NPAIR = S // (2 * SEG)

SEM_X, SEM_C, SEM_MEM, SEM_WO, SEM_W1, SEM_W2, SEM_W3, SEM_W4 = range(8)
SEM_MOD = 8
SEM_ST = 14
SEM_OUT = 16
NSEM = 18


def _slot(t, h):
    g, r = divmod(h, HG)
    return t * H + g * HG + (r // 2) + (r % 2) * (HG // 2)


def _ln(x):
    mu = jnp.mean(x, axis=-1, keepdims=True)
    xc = x - mu
    var = jnp.mean(xc * xc, axis=-1, keepdims=True)
    return xc * lax.rsqrt(var + EPS)


def _gelu(x):
    return jax.nn.gelu(x, approximate=True)


def _pack(x):
    return pltpu.bitcast(x.astype(BF16), U32)


def _unpack(x):
    return pltpu.bitcast(x, BF16)


def _dot(a, b):
    return jnp.dot(a, b, preferred_element_type=F32)


def _cols(ref, lo, hi):
    return jnp.concatenate([ref[c] for c in range(lo, hi)], axis=1)


def _kernel(x_hbm, mem_hbm, wq_hbm, wk_hbm, wv_hbm, wo_hbm, w1_hbm, w2_hbm,
            w3_hbm, w4_hbm, c_hbm, wmod_hbm, out_hbm,
            xv, cv, memv, wmodv, modv, st, wqkv, wov, w1v, w2v, w3v, w4v,
            hv, ring, fillv, aout, h2v, gv, outv, sems, *, phases):
    def cp(src, dst, s):
        return pltpu.make_async_copy(src, dst, sems.at[s])

    def col_copies(w_hbm, w_v, s):
        return [cp(w_hbm.at[:, pl.ds(c * 128, 128)], w_v.at[c], s)
                for c in range(w_v.shape[0])]

    c_cp = cp(c_hbm, cv, SEM_C)
    mem_cp = cp(mem_hbm, memv, SEM_MEM)
    x_cp = cp(x_hbm, xv, SEM_X)
    mod_cps = [cp(wmod_hbm.at[:, pl.ds(i * D, D)], wmodv.at[i], SEM_MOD + i)
               for i in range(6)]
    w_hbms = (wq_hbm, wk_hbm, wv_hbm)
    groups = [(t, g) for g in range(H // HG) for t in range(3)]
    st_cps = [cp(w_hbms[t].at[:, pl.ds(g * HG, HG), :], st.at[i % 2],
                 SEM_ST + i % 2) for i, (t, g) in enumerate(groups)]
    wo_cps = col_copies(wo_hbm, wov, SEM_WO)
    w1_cps = col_copies(w1_hbm, w1v, SEM_W1)
    w2_cps = col_copies(w2_hbm, w2v, SEM_W2)
    w3_cps = col_copies(w3_hbm, w3v, SEM_W3)
    w4_cps = col_copies(w4_hbm, w4v, SEM_W4)

    c_cp.start()
    mem_cp.start()
    mod_cps[0].start()
    mod_cps[1].start()
    x_cp.start()
    st_cps[0].start()
    st_cps[1].start()

    c_cp.wait()
    cf = cv[...].astype(F32)
    sc = jnp.broadcast_to((cf * jax.nn.sigmoid(cf)).astype(BF16), (16, D))

    def mod_part(i):
        mod_cps[i].wait()
        modv[i] = _dot(sc, wmodv[i])[0:8]

    mod_part(0)
    mod_part(1)

    r = lax.broadcasted_iota(jnp.int32, (80, 80), 0)
    k = lax.broadcasted_iota(jnp.int32, (80, 80), 1)

    def head_of(i):
        return jnp.where(i < 16, i // 8, (i - 16) // 32)

    def pos_of(i):
        return jnp.where(i < 16, i % 8, 8 + (i - 16) % 32)

    same = head_of(r) == head_of(k)
    vis = (pos_of(r) < M) | (pos_of(r) >= pos_of(k))
    fillv[...] = jnp.where(same, jnp.where(vis, 0.0, -1e9), -jnp.inf).astype(F32)

    x_cp.wait()

    def ln_body(i, _):
        r0 = pl.multiple_of(i * 64, 64)
        xf = xv[pl.ds(r0, 64), :].astype(F32)
        hh = _ln(xf) * (1.0 + modv[1, 0:1, :]) + modv[0, 0:1, :]
        hv[pl.ds(pl.multiple_of(i * 32, 32), 32), :] = _pack(hh)
        return 0

    lax.fori_loop(0, S // 64, ln_body, 0)

    for i, (t, g) in enumerate(groups):
        st_cps[i].wait()
        base = (t * H + g * HG) * SL

        def rl_body(ii, _, i=i, base=base):
            for u in range(16):
                d0 = ii * 32 + 2 * u
                a = pltpu.bitcast(st[i % 2, d0], U32)
                b = pltpu.bitcast(st[i % 2, d0 + 1], U32)
                lo = (a & jnp.uint32(0xFFFF)) | (b << 16)
                hi = (a >> 16) | (b & jnp.uint32(0xFFFF0000))
                rr = ii * 16 + u
                wqkv[pl.ds(base + rr, 8, stride=SL), :] = lo
                wqkv[pl.ds(base + 8 * SL + rr, 8, stride=SL), :] = hi
            return 0

        lax.fori_loop(0, D // 32, rl_body, 0)
        if i + 2 < len(groups):
            st_cps[i + 2].start()
        if i == len(groups) - 2:
            for q in wo_cps:
                q.start()
            for j in range(2, 6):
                mod_cps[j].start()
        if i == len(groups) - 1:
            for q in w1_cps + w2_cps + w3_cps + w4_cps:
                q.start()

        def pro_body(ii, _, t=t, g=g):
            lhs = _unpack(hv[pl.ds(pl.multiple_of(ii * 64, 64), 64), :])
            for hq in range(HG // 4):
                hs = [g * HG + hq * 4 + u for u in range(4)]
                w = jnp.concatenate(
                    [_unpack(wqkv[pl.ds(_slot(t, h) * SL, 512), :]) for h in hs],
                    axis=1)
                y = _pack(_dot(lhs, w))
                for u, h in enumerate(hs):
                    ring[t * H + h, pl.ds(pl.multiple_of(ii * 64, 64), 64), :] = (
                        y[:, u * 128:(u + 1) * 128])
            return 0

        lax.fori_loop(0, LEAD // 128, pro_body, 0)

    for q in wo_cps:
        q.wait()
    mem_cp.wait()

    scale = float(E) ** -0.5

    def segment(lhs, ro, store_tok):
        fill = fillv[...]
        keep = fill == 0.0
        o_mem, o_tok = [], []
        for hp in range(H // 2):
            hs = (2 * hp, 2 * hp + 1)
            tiles = [(t, h) for t in range(3) for h in hs]
            w = jnp.concatenate(
                [_unpack(wqkv[pl.ds(_slot(t, h) * SL, 512), :]) for t, h in tiles],
                axis=1)
            y = _dot(lhs, w)
            for u, (t, h) in enumerate(tiles):
                store_tok(t * H + h, y[8:32, u * 128:(u + 1) * 128])
            ops = []
            for t in range(3):
                ym = jnp.concatenate(
                    [y[0:8, (2 * t) * 128:(2 * t + 1) * 128],
                     y[0:8, (2 * t + 1) * 128:(2 * t + 2) * 128]], axis=0)
                ops.append(jnp.concatenate(
                    [ym.astype(BF16)]
                    + [_unpack(ring[t * H + h, pl.ds(ro, 16), :]) for h in hs],
                    axis=0))
            q, kk, v = ops
            s = lax.dot_general(q, kk, (((1,), (1,)), ((), ())),
                                preferred_element_type=F32)
            s = jnp.where(keep, s * scale, fill)
            mx = jnp.max(s, axis=-1, keepdims=True)
            p = jnp.exp(s - mx)
            l = jnp.sum(p, axis=-1, keepdims=True)
            o = _dot(p.astype(BF16), v) * (1.0 / l)
            o_mem += [o[0:8], o[8:16]]
            o_tok += [o[16:48], o[48:80]]
        return o_mem, o_tok

    def wo_pass(blocks):
        lhs = jnp.concatenate([b.astype(BF16) for b in blocks], axis=1)
        return _dot(lhs, _cols(wov, 0, 8))

    def a_body(j, mem):
        w0 = LEAD // 2 + 24 * j
        hb = _unpack(hv[pl.ds(pl.multiple_of(w0, 8), 8), :])
        hac = _unpack(hv[pl.ds(pl.multiple_of(w0 + 8, 8), 8), :]).astype(F32)
        hd = _unpack(hv[pl.ds(pl.multiple_of(w0 + 16, 8), 8), :])
        wr = [pl.multiple_of(lax.rem(w0 + 8 * i, RING), 8) for i in range(3)]
        ro0 = pl.multiple_of(lax.rem(32 * j, RING), 16)
        ro1 = pl.multiple_of(lax.rem(32 * j + 16, RING), 16)
        r0 = pl.multiple_of(64 * j, 64)

        lhs = jnp.concatenate(
            [jnp.concatenate([mem, hac[0:8]], axis=0).astype(BF16), hb], axis=0)
        tok_a = {}

        def store0(c, y):
            tok_a[c] = y[0:8]
            ring[c, pl.ds(wr[0], 8), :] = _pack(y[8:24])

        o_mem, o_tok = segment(lhs, ro0, store0)
        out = wo_pass([jnp.concatenate([m_, t_[0:24]], axis=0)
                       for m_, t_ in zip(o_mem, o_tok)])
        deferred = [t_[24:32] for t_ in o_tok]
        mem = out[0:8]
        aout[pl.ds(r0, 24), :] = out[8:32]

        lhs = jnp.concatenate(
            [jnp.concatenate([mem, hac[8:16]], axis=0).astype(BF16), hd], axis=0)

        def store1(c, y):
            ring[c, pl.ds(wr[1], 8), :] = _pack(
                jnp.concatenate([tok_a[c], y[0:8]], axis=0))
            ring[c, pl.ds(wr[2], 8), :] = _pack(y[8:24])

        o_mem, o_tok = segment(lhs, ro1, store1)
        out = wo_pass([jnp.concatenate([m_, d_, t_], axis=0)
                       for m_, d_, t_ in zip(o_mem, deferred, o_tok)])
        aout[pl.ds(r0 + 24, 40), :] = out[8:48]
        return out[0:8]

    if "A" in phases:
        lax.fori_loop(0, NPAIR, a_body, memv[...].astype(F32))
    else:
        aout[...] = jnp.zeros(aout.shape, F32)

    for j in range(2, 6):
        mod_part(j)
    for q in w1_cps + w2_cps + w3_cps + w4_cps:
        q.wait()

    gv[:, 0:8, :] = jnp.zeros((8, 8, 128), F32)
    gv[:, S + 8:S + 16, :] = jnp.zeros((8, 8, 128), F32)

    RB = 256

    def b1_body(i, _):
        r0 = pl.multiple_of(i * RB, RB)
        x2 = xv[pl.ds(r0, RB), :].astype(F32) + modv[2, 0:1, :] * aout[pl.ds(r0, RB), :]
        aout[pl.ds(r0, RB), :] = x2
        h2 = _ln(x2) * (1.0 + modv[4, 0:1, :]) + modv[3, 0:1, :]
        h2v[pl.ds(r0, RB), :] = h2
        g = _gelu(_dot(_ln(h2).astype(BF16), _cols(w1v, 0, 8)))
        for c in range(8):
            gv[c, pl.ds(r0 + 8, RB), :] = g[:, c * 128:(c + 1) * 128]
        return 0

    shifts = (-1, -1, 1, 1, -2, -2, 2, 2)

    def out_cp(i, slot):
        return cp(outv.at[slot], out_hbm.at[pl.ds(i * RB, RB), :], SEM_OUT + slot)

    def b2_body(i, _):
        r0 = pl.multiple_of(i * RB, RB)
        gs = jnp.concatenate(
            [gv[c, pl.ds(r0 + 8 + shifts[c], RB), :] for c in range(8)],
            axis=1).astype(BF16)
        x1 = h2v[pl.ds(r0, RB), :] + _dot(gs, _cols(w2v, 0, 8))
        tt = _ln(x1).astype(BF16)
        ff = jnp.concatenate(
            [_gelu(_dot(tt, _cols(w3v, 4 * q, 4 * q + 4))).astype(BF16)
             for q in range(FF // 512)], axis=1)
        y = _dot(ff, _cols(w4v, 0, 8))
        res = aout[pl.ds(r0, RB), :] + modv[5, 0:1, :] * (x1 + y)
        slot = i % 2

        @pl.when(i >= 2)
        def _():
            out_cp(i - 2, slot).wait()

        outv[slot] = res.astype(BF16)
        out_cp(i, slot).start()
        return 0

    nb = S // RB
    if "B" in phases:
        lax.fori_loop(0, nb, b1_body, 0)
        lax.fori_loop(0, nb, b2_body, 0)
        out_cp(nb - 2, 0).wait()
        out_cp(nb - 1, 1).wait()
    else:
        for i in range(nb):
            outv[0] = aout[pl.ds(i * RB, RB), :].astype(BF16)
            out_cp(i, 0).start()
            out_cp(i, 0).wait()


def _call(A_x, A_mem0, A_Wq, A_Wk, A_Wv, A_Wo, B_w1, B_w2, B_w3, B_w4, c, w_mod,
          phases="AB"):
    any_spec = pl.BlockSpec(memory_space=pl.ANY)
    scratch = [
        pltpu.VMEM((S, D), BF16),
        pltpu.VMEM((1, D), BF16),
        pltpu.VMEM((M, D), BF16),
        pltpu.VMEM((6, D, D), BF16),
        pltpu.VMEM((6, 8, D), F32),
        pltpu.VMEM((2, D, HG, E), BF16),
        pltpu.VMEM((3 * H * SL, E), U32),
        pltpu.VMEM((8, H * E, 128), BF16),
        pltpu.VMEM((8, D, 128), BF16),
        pltpu.VMEM((8, D, 128), BF16),
        pltpu.VMEM((FF // 128, D, 128), BF16),
        pltpu.VMEM((8, FF, 128), BF16),
        pltpu.VMEM((S // 2, D), U32),
        pltpu.VMEM((3 * H, RING, E), U32),
        pltpu.VMEM((80, 80), F32),
        pltpu.VMEM((S, D), F32),
        pltpu.VMEM((S, D), F32),
        pltpu.VMEM((8, S + 16, 128), F32),
        pltpu.VMEM((2, 256, D), BF16),
        pltpu.SemaphoreType.DMA((NSEM,)),
    ]
    out = pl.pallas_call(
        functools.partial(_kernel, phases=phases),
        in_specs=[any_spec] * 12,
        out_specs=any_spec,
        out_shape=jax.ShapeDtypeStruct((S, D), BF16),
        scratch_shapes=scratch,
        compiler_params=pltpu.CompilerParams(
            vmem_limit_bytes=126 * 1024 * 1024),
    )(A_x.reshape(S, D), A_mem0.reshape(M, D), A_Wq, A_Wk, A_Wv,
      A_Wo.reshape(H * E, D), B_w1, B_w2, B_w3, B_w4, c, w_mod)
    return out.reshape(1, S, D)


def pallas_adaLN_cond__memory_aug_recurrent_mem_tr__mixer_s_mlp__prompt_kernel(
    A_x, A_mem0, A_Wq, A_Wk, A_Wv, A_Wo, A_seg_len, B_x, B_w1, B_w2, B_w3, B_w4,
    c, w_mod,
):
    assert A_seg_len == SEG
    del B_x
    return _call(A_x, A_mem0, A_Wq, A_Wk, A_Wv, A_Wo, B_w1, B_w2, B_w3, B_w4,
                 c, w_mod)
```

```python
import functools

import jax
import jax.numpy as jnp
from jax import lax
import jax.experimental.pallas as pl
import jax.experimental.pallas.tpu as pltpu

F32 = jnp.float32
BF16 = jnp.bfloat16
U32 = jnp.uint32

S = 2048
D = 1024
H = 32
E = 128
M = 8
SEG = 32
FF = 3584
EPS = 1e-5

LEAD = 512
RING = 288
SL = 520
HG = 16
NPAIR = S // (2 * SEG)

SEM_X, SEM_C, SEM_MEM, SEM_WO, SEM_W1, SEM_W2, SEM_W3, SEM_W4 = range(8)
SEM_MOD = 8
SEM_ST = 14
SEM_OUT = 16
NSEM = 18


def _slot(t, h):
    g, r = divmod(h, HG)
    return t * H + g * HG + (r // 2) + (r % 2) * (HG // 2)


def _ln(x):
    mu = jnp.mean(x, axis=-1, keepdims=True)
    xc = x - mu
    var = jnp.mean(xc * xc, axis=-1, keepdims=True)
    return xc * lax.rsqrt(var + EPS)


def _gelu(x):
    return jax.nn.gelu(x, approximate=True)


def _pack(x):
    return pltpu.bitcast(x.astype(BF16), U32)


def _unpack(x):
    return pltpu.bitcast(x, BF16)


def _dot(a, b):
    return jnp.dot(a, b, preferred_element_type=F32)


def _cols(ref, lo, hi, k0=0, k1=None):
    k1 = 2 * ref.shape[1] if k1 is None else k1
    return jnp.concatenate(
        [_unpack(ref[c, k0 // 2:k1 // 2, :]) for c in range(lo, hi)], axis=1)


def _kernel(x_hbm, mem_hbm, wq_hbm, wk_hbm, wv_hbm, wo_hbm, w1_hbm, w2_hbm,
            w3_hbm, w4_hbm, c_hbm, wmod_hbm, out_hbm,
            xv, cv, memv, wmodv, modv, st, wqkv, wov, w1v, w2v, w3v, w4v,
            hv, ring, fillv, aout, h2v, gv, outv, sems, *, phases):
    def cp(src, dst, s):
        return pltpu.make_async_copy(src, dst, sems.at[s])

    def col_copies(w_hbm, w_v, s):
        w32 = w_hbm.bitcast(U32)
        return [cp(w32.at[:, pl.ds(c * 128, 128)], w_v.at[c], s)
                for c in range(w_v.shape[0])]

    c_cp = cp(c_hbm, cv, SEM_C)
    mem_cp = cp(mem_hbm, memv, SEM_MEM)
    x_cp = cp(x_hbm, xv, SEM_X)
    mod_cps = [cp(wmod_hbm.at[:, pl.ds(i * D, D)], wmodv.at[i], SEM_MOD + i)
               for i in range(6)]
    w_hbms = (wq_hbm, wk_hbm, wv_hbm)
    groups = [(t, g) for g in range(H // HG) for t in range(3)]
    st_cps = [cp(w_hbms[t].at[:, pl.ds(g * HG, HG), :], st.at[i % 2],
                 SEM_ST + i % 2) for i, (t, g) in enumerate(groups)]
    wo_cps = col_copies(wo_hbm, wov, SEM_WO)
    w1_cps = col_copies(w1_hbm, w1v, SEM_W1)
    w2_cps = col_copies(w2_hbm, w2v, SEM_W2)
    w3_cps = col_copies(w3_hbm, w3v, SEM_W3)
    w4_cps = col_copies(w4_hbm, w4v, SEM_W4)

    c_cp.start()
    mem_cp.start()
    mod_cps[0].start()
    mod_cps[1].start()
    x_cp.start()
    st_cps[0].start()
    st_cps[1].start()

    c_cp.wait()
    cf = cv[...].astype(F32)
    sc = jnp.broadcast_to((cf * jax.nn.sigmoid(cf)).astype(BF16), (16, D))

    def mod_part(i):
        mod_cps[i].wait()
        modv[i] = _dot(sc, wmodv[i])[0:8]

    mod_part(0)
    mod_part(1)

    r = lax.broadcasted_iota(jnp.int32, (80, 80), 0)
    k = lax.broadcasted_iota(jnp.int32, (80, 80), 1)

    def head_of(i):
        return jnp.where(i < 16, i // 8, (i - 16) // 32)

    def pos_of(i):
        return jnp.where(i < 16, i % 8, 8 + (i - 16) % 32)

    same = head_of(r) == head_of(k)
    vis = (pos_of(r) < M) | (pos_of(r) >= pos_of(k))
    fillv[...] = jnp.where(same, jnp.where(vis, 0.0, -1e9), -jnp.inf).astype(F32)

    x_cp.wait()

    def ln_body(i, _):
        r0 = pl.multiple_of(i * 64, 64)
        xf = xv[pl.ds(r0, 64), :].astype(F32)
        hh = _ln(xf) * (1.0 + modv[1, 0:1, :]) + modv[0, 0:1, :]
        hv[pl.ds(pl.multiple_of(i * 32, 32), 32), :] = _pack(hh)
        return 0

    lax.fori_loop(0, S // 64, ln_body, 0)

    for i, (t, g) in enumerate(groups):
        st_cps[i].wait()
        base = (t * H + g * HG) * SL

        def rl_body(ii, _, i=i, base=base):
            for u in range(16):
                d0 = ii * 32 + 2 * u
                a = pltpu.bitcast(st[i % 2, d0], U32)
                b = pltpu.bitcast(st[i % 2, d0 + 1], U32)
                lo = (a & jnp.uint32(0xFFFF)) | (b << 16)
                hi = (a >> 16) | (b & jnp.uint32(0xFFFF0000))
                rr = ii * 16 + u
                wqkv[pl.ds(base + rr, 8, stride=SL), :] = lo
                wqkv[pl.ds(base + 8 * SL + rr, 8, stride=SL), :] = hi
            return 0

        lax.fori_loop(0, D // 32, rl_body, 0)
        if i + 2 < len(groups):
            st_cps[i + 2].start()
        if i == len(groups) - 2:
            for q in wo_cps:
                q.start()
            for j in range(2, 6):
                mod_cps[j].start()
        if i == len(groups) - 1:
            for q in w1_cps + w2_cps + w3_cps + w4_cps:
                q.start()

        def pro_body(ii, _, t=t, g=g):
            lhs = _unpack(hv[pl.ds(pl.multiple_of(ii * 64, 64), 64), :])
            for hq in range(HG // 4):
                hs = [g * HG + hq * 4 + u for u in range(4)]
                w = jnp.concatenate(
                    [_unpack(wqkv[pl.ds(_slot(t, h) * SL, 512), :]) for h in hs],
                    axis=1)
                y = _pack(_dot(lhs, w))
                for u, h in enumerate(hs):
                    ring[t * H + h, pl.ds(pl.multiple_of(ii * 64, 64), 64), :] = (
                        y[:, u * 128:(u + 1) * 128])
            return 0

        lax.fori_loop(0, LEAD // 128, pro_body, 0)

    for q in wo_cps:
        q.wait()
    mem_cp.wait()

    scale = float(E) ** -0.5

    def segment(lhs, ro, store_tok, wo_lhs):
        fill = fillv[...]
        keep = fill == 0.0
        NP = H // 2
        qkv, probs, blocks = {}, {}, []

        def proj(hp):
            hs = (2 * hp, 2 * hp + 1)
            tiles = [(t, h) for t in range(3) for h in hs]
            w = jnp.concatenate(
                [_unpack(wqkv[pl.ds(_slot(t, h) * SL, 512), :]) for t, h in tiles],
                axis=1)
            if hp == 0:
                y = _dot(lhs[:, :512], w[:512])
                y = _dot(lhs[:, 512:], w[512:]) + y
            else:
                y = _dot(lhs, w)
            for u, (t, h) in enumerate(tiles):
                store_tok(t * H + h, y[8:32, u * 128:(u + 1) * 128])
            ops = []
            for t in range(3):
                ym = jnp.concatenate(
                    [y[0:8, (2 * t) * 128:(2 * t + 1) * 128],
                     y[0:8, (2 * t + 1) * 128:(2 * t + 2) * 128]], axis=0)
                ops.append(jnp.concatenate(
                    [ym.astype(BF16)]
                    + [_unpack(ring[t * H + h, pl.ds(ro, 16), :]) for h in hs],
                    axis=0))
            qkv[hp] = ops

        def scores(hp):
            q, kk, _ = qkv[hp]
            s = lax.dot_general(q, kk, (((1,), (1,)), ((), ())),
                                preferred_element_type=F32)
            s = jnp.where(keep, s * scale, fill)
            mx = jnp.max(s, axis=-1, keepdims=True)
            p = jnp.exp(s - mx)
            l = jnp.sum(p, axis=-1, keepdims=True)
            rl = pl.reciprocal(l, approx=True)
            rl = rl * (2.0 - l * rl)
            probs[hp] = (p * rl).astype(BF16)

        def pv(hp):
            o = _dot(probs[hp], qkv[hp][2])
            blocks.append(wo_lhs(2 * hp, o[0:8], o[16:48]).astype(BF16))
            blocks.append(wo_lhs(2 * hp + 1, o[8:16], o[48:80]).astype(BF16))

        def wo_part(h0, h1, acc=None):
            lw = jnp.concatenate(blocks[h0:h1], axis=1)
            y = _dot(lw, _cols(wov, 0, 8, E * h0, E * h1))
            return y if acc is None else y + acc

        for i in range(NP):
            proj(i)
            if i >= 1:
                scores(i - 1)
            if i >= 3:
                pv(i - 3)
        acc = wo_part(0, 4)
        scores(NP - 1)
        pv(NP - 3)
        acc = wo_part(4, 12, acc)
        pv(NP - 2)
        pv(NP - 1)
        acc = wo_part(12, 24, acc)
        acc = wo_part(24, 32, acc)
        return acc

    def a_body(j, mem):
        w0 = LEAD // 2 + 24 * j
        hb = _unpack(hv[pl.ds(pl.multiple_of(w0, 8), 8), :])
        hac = _unpack(hv[pl.ds(pl.multiple_of(w0 + 8, 8), 8), :]).astype(F32)
        hd = _unpack(hv[pl.ds(pl.multiple_of(w0 + 16, 8), 8), :])
        wr = [pl.multiple_of(lax.rem(w0 + 8 * i, RING), 8) for i in range(3)]
        ro0 = pl.multiple_of(lax.rem(32 * j, RING), 16)
        ro1 = pl.multiple_of(lax.rem(32 * j + 16, RING), 16)
        r0 = pl.multiple_of(64 * j, 64)

        lhs = jnp.concatenate(
            [jnp.concatenate([mem, hac[0:8]], axis=0).astype(BF16), hb], axis=0)
        tok_a = {}

        def store0(c, y):
            tok_a[c] = y[0:8]
            ring[c, pl.ds(wr[0], 8), :] = _pack(y[8:24])

        deferred = {}

        def wo_lhs0(h, om, ot):
            deferred[h] = ot[24:32]
            return jnp.concatenate([om, ot[0:24]], axis=0)

        out = segment(lhs, ro0, store0, wo_lhs0)
        mem = out[0:8]
        aout[pl.ds(r0, 24), :] = out[8:32]

        lhs = jnp.concatenate(
            [jnp.concatenate([mem, hac[8:16]], axis=0).astype(BF16), hd], axis=0)

        def store1(c, y):
            ring[c, pl.ds(wr[1], 8), :] = _pack(
                jnp.concatenate([tok_a[c], y[0:8]], axis=0))
            ring[c, pl.ds(wr[2], 8), :] = _pack(y[8:24])

        def wo_lhs1(h, om, ot):
            return jnp.concatenate([om, deferred[h], ot], axis=0)

        out = segment(lhs, ro1, store1, wo_lhs1)
        aout[pl.ds(r0 + 24, 40), :] = out[8:48]
        return out[0:8]

    if "A" in phases:
        lax.fori_loop(0, NPAIR, a_body, memv[...].astype(F32))
    else:
        aout[...] = jnp.zeros(aout.shape, F32)

    for j in range(2, 6):
        mod_part(j)
    for q in w1_cps + w2_cps + w3_cps + w4_cps:
        q.wait()

    gv[:, 0:8, :] = jnp.zeros((8, 8, 128), F32)
    gv[:, S + 8:S + 16, :] = jnp.zeros((8, 8, 128), F32)

    RB = 256

    def b1_body(i, _):
        r0 = pl.multiple_of(i * RB, RB)
        x2 = xv[pl.ds(r0, RB), :].astype(F32) + modv[2, 0:1, :] * aout[pl.ds(r0, RB), :]
        aout[pl.ds(r0, RB), :] = x2
        h2 = _ln(x2) * (1.0 + modv[4, 0:1, :]) + modv[3, 0:1, :]
        h2v[pl.ds(r0, RB), :] = h2
        g = _gelu(_dot(_ln(h2).astype(BF16), _cols(w1v, 0, 8)))
        for c in range(8):
            gv[c, pl.ds(r0 + 8, RB), :] = g[:, c * 128:(c + 1) * 128]
        return 0

    shifts = (-1, -1, 1, 1, -2, -2, 2, 2)

    def out_cp(i, slot):
        return cp(outv.at[slot], out_hbm.at[pl.ds(i * RB, RB), :], SEM_OUT + slot)

    def b2_body(i, _):
        r0 = pl.multiple_of(i * RB, RB)
        gs = jnp.concatenate(
            [gv[c, pl.ds(r0 + 8 + shifts[c], RB), :] for c in range(8)],
            axis=1).astype(BF16)
        x1 = h2v[pl.ds(r0, RB), :] + _dot(gs, _cols(w2v, 0, 8))
        tt = _ln(x1).astype(BF16)
        ff = jnp.concatenate(
            [_gelu(_dot(tt, _cols(w3v, 4 * q, 4 * q + 4))).astype(BF16)
             for q in range(FF // 512)], axis=1)
        y = _dot(ff, _cols(w4v, 0, 8))
        res = aout[pl.ds(r0, RB), :] + modv[5, 0:1, :] * (x1 + y)
        slot = i % 2

        @pl.when(i >= 2)
        def _():
            out_cp(i - 2, slot).wait()

        outv[slot] = res.astype(BF16)
        out_cp(i, slot).start()
        return 0

    nb = S // RB
    if "B" in phases:
        lax.fori_loop(0, nb, b1_body, 0)
        lax.fori_loop(0, nb, b2_body, 0)
        out_cp(nb - 2, 0).wait()
        out_cp(nb - 1, 1).wait()
    else:
        for i in range(nb):
            outv[0] = aout[pl.ds(i * RB, RB), :].astype(BF16)
            out_cp(i, 0).start()
            out_cp(i, 0).wait()


def _call(A_x, A_mem0, A_Wq, A_Wk, A_Wv, A_Wo, B_w1, B_w2, B_w3, B_w4, c, w_mod,
          phases="AB"):
    any_spec = pl.BlockSpec(memory_space=pl.ANY)
    scratch = [
        pltpu.VMEM((S, D), BF16),
        pltpu.VMEM((1, D), BF16),
        pltpu.VMEM((M, D), BF16),
        pltpu.VMEM((6, D, D), BF16),
        pltpu.VMEM((6, 8, D), F32),
        pltpu.VMEM((2, D, HG, E), BF16),
        pltpu.VMEM((3 * H * SL, E), U32),
        pltpu.VMEM((8, H * E // 2, 128), U32),
        pltpu.VMEM((8, D // 2, 128), U32),
        pltpu.VMEM((8, D // 2, 128), U32),
        pltpu.VMEM((FF // 128, D // 2, 128), U32),
        pltpu.VMEM((8, FF // 2, 128), U32),
        pltpu.VMEM((S // 2, D), U32),
        pltpu.VMEM((3 * H, RING, E), U32),
        pltpu.VMEM((80, 80), F32),
        pltpu.VMEM((S, D), F32),
        pltpu.VMEM((S, D), F32),
        pltpu.VMEM((8, S + 16, 128), F32),
        pltpu.VMEM((2, 256, D), BF16),
        pltpu.SemaphoreType.DMA((NSEM,)),
    ]
    out = pl.pallas_call(
        functools.partial(_kernel, phases=phases),
        in_specs=[any_spec] * 12,
        out_specs=any_spec,
        out_shape=jax.ShapeDtypeStruct((S, D), BF16),
        scratch_shapes=scratch,
        compiler_params=pltpu.CompilerParams(
            vmem_limit_bytes=126 * 1024 * 1024),
    )(A_x.reshape(S, D), A_mem0.reshape(M, D), A_Wq, A_Wk, A_Wv,
      A_Wo.reshape(H * E, D), B_w1, B_w2, B_w3, B_w4, c, w_mod)
    return out.reshape(1, S, D)


def pallas_adaLN_cond__memory_aug_recurrent_mem_tr__mixer_s_mlp__prompt_kernel(
    A_x, A_mem0, A_Wq, A_Wk, A_Wv, A_Wo, A_seg_len, B_x, B_w1, B_w2, B_w3, B_w4,
    c, w_mod,
):
    assert A_seg_len == SEG
    del B_x
    return _call(A_x, A_mem0, A_Wq, A_Wk, A_Wv, A_Wo, B_w1, B_w2, B_w3, B_w4,
                 c, w_mod)
```

```python
import functools

import jax
import jax.numpy as jnp
from jax import lax
import jax.experimental.pallas as pl
import jax.experimental.pallas.tpu as pltpu

F32 = jnp.float32
BF16 = jnp.bfloat16
U32 = jnp.uint32

S = 2048
D = 1024
H = 32
E = 128
M = 8
SEG = 32
FF = 3584
EPS = 1e-5

LEAD = 512
RING = 288
SL = 520
HG = 16
NG = 3 * H // HG
NPAIR = S // (2 * SEG)
HALO = 80
RB = 256
SHIFTS = (-1, -1, 1, 1, -2, -2, 2, 2)

(SEM_X0, SEM_X1, SEM_C, SEM_MEM, SEM_WO, SEM_W1, SEM_W2, SEM_W3, SEM_W4,
 SEM_MODA, SEM_MODB) = range(11)
SEM_ST = 11
SEM_OUT = SEM_ST + 4 + NG
NSEM = SEM_OUT + 2


def _slot(t, h):
    g, r = divmod(h, HG)
    return t * H + g * HG + (r // 2) + (r % 2) * (HG // 2)


def _ln(x):
    mu = jnp.mean(x, axis=-1, keepdims=True)
    xc = x - mu
    var = jnp.mean(xc * xc, axis=-1, keepdims=True)
    return xc * lax.rsqrt(var + EPS)


def _gelu(x):
    return jax.nn.gelu(x, approximate=True)


def _pack(x):
    return pltpu.bitcast(x.astype(BF16), U32)


def _unpack(x):
    return pltpu.bitcast(x, BF16)


def _dot(a, b):
    return jnp.dot(a, b, preferred_element_type=F32)


def _cols(ref, lo, hi, k0=0, k1=None):
    k1 = 2 * ref.shape[1] if k1 is None else k1
    return jnp.concatenate(
        [_unpack(ref[c, k0 // 2:k1 // 2, :]) for c in range(lo, hi)], axis=1)


def _kernel(x_hbm, mem_hbm, wq_hbm, wk_hbm, wv_hbm, wo_hbm, w1_hbm, w2_hbm,
            w3_hbm, w4_hbm, c_hbm, wmod_hbm, out_hbm,
            xv, cv, memv, wmodv, modv, wqkv, wov, w1v, w2v,
            hv, ring, fillv, aout, gbuf, x2t, h2t, outv, sems, *, phases):
    def cp(src, dst, s):
        return pltpu.make_async_copy(src, dst, sems.at[s])

    def col_copies(w_hbm, w_v, s, lo=0, hi=None):
        w32 = w_hbm.bitcast(U32)
        hi = w_v.shape[0] if hi is None else hi
        return [cp(w32.at[:, pl.ds(c * 128, 128)], w_v.at[c], s)
                for c in range(lo, hi)]

    def start(cps):
        for q in cps:
            q.start()

    def wait(cps):
        for q in cps:
            q.wait()

    c_cp = cp(c_hbm, cv, SEM_C)
    mem_cp = cp(mem_hbm, memv, SEM_MEM)
    x0_cp = cp(x_hbm.at[pl.ds(0, LEAD)], xv.at[pl.ds(0, LEAD)], SEM_X0)
    x1_cp = cp(x_hbm.at[pl.ds(LEAD, S - LEAD)], xv.at[pl.ds(LEAD, S - LEAD)],
               SEM_X1)
    moda_cps = col_copies(wmod_hbm, wmodv, SEM_MODA, 0, 16)
    modb_cps = col_copies(wmod_hbm, wmodv, SEM_MODB, 16, 48)
    wo_cps = col_copies(wo_hbm, wov, SEM_WO)
    w1_cps = col_copies(w1_hbm, w1v, SEM_W1)
    w2_cps = col_copies(w2_hbm, w2v, SEM_W2)

    def mod_row(i):
        return modv[i, 0:1, :]

    def silu_c():
        cf = cv[...].astype(F32)
        return jnp.broadcast_to((cf * jax.nn.sigmoid(cf)).astype(BF16), (16, D))

    def h_rows(r0, n):
        xf = xv[pl.ds(pl.multiple_of(r0, 16), n), :].astype(F32)
        hh = _ln(xf) * (1.0 + mod_row(1)) + mod_row(0)
        hv[pl.ds(pl.multiple_of(r0 // 2, 8), n // 2), :] = _pack(hh)

    def prologue(st):
        w_hbms = (wq_hbm, wk_hbm, wv_hbm)

        def st_src(i):
            return w_hbms[i // 2].at[:, pl.ds((i % 2) * HG, HG), :]

        st0_cps = [cp(st_src(0).at[pl.ds(q * 256, 256)],
                      st.at[0, pl.ds(q * 256, 256)], SEM_ST + q) for q in range(4)]
        st_cps = [None] + [cp(st_src(i), st.at[i], SEM_ST + 4 + i)
                           for i in range(1, NG)]

        start([c_cp, mem_cp, x0_cp])
        start(moda_cps)
        start(st0_cps)
        start([st_cps[1], x1_cp, st_cps[2], st_cps[3]])
        start(wo_cps)
        start([st_cps[4]])
        start(modb_cps)
        start([st_cps[5]])
        start(w1_cps + w2_cps)

        r = lax.broadcasted_iota(jnp.int32, (80, 80), 0)
        k = lax.broadcasted_iota(jnp.int32, (80, 80), 1)

        def head_of(i):
            return jnp.where(i < 16, i // 8, (i - 16) // 32)

        def pos_of(i):
            return jnp.where(i < 16, i % 8, 8 + (i - 16) % 32)

        same = head_of(r) == head_of(k)
        vis = (pos_of(r) < M) | (pos_of(r) >= pos_of(k))
        fillv[...] = jnp.where(same, jnp.where(vis, 0.0, -1e9), -jnp.inf).astype(F32)
        aout[...] = jnp.zeros(aout.shape, F32)
        gbuf[...] = jnp.zeros(gbuf.shape, F32)
        x2t[...] = jnp.zeros(x2t.shape, F32)
        h2t[...] = jnp.zeros(h2t.shape, F32)

        c_cp.wait()
        wait(moda_cps)
        sc = silu_c()
        for i in range(2):
            modv[i] = _dot(sc, _cols(wmodv, 8 * i, 8 * i + 8))[0:8]
        x0_cp.wait()

        def ln_body(i, _):
            h_rows(i * 64, 64)
            return 0

        lax.fori_loop(0, LEAD // 64, ln_body, 0)

        def relayout(g, p0, n):
            base = g * (HG * SL)
            for u in range(n):
                a = pltpu.bitcast(st[g, 2 * (p0 + u)], U32)
                b = pltpu.bitcast(st[g, 2 * (p0 + u) + 1], U32)
                lo = (a & jnp.uint32(0xFFFF)) | (b << 16)
                hi = (a >> 16) | (b & jnp.uint32(0xFFFF0000))
                wqkv[pl.ds(base + p0 + u, 8, stride=SL), :] = lo
                wqkv[pl.ds(base + 8 * SL + p0 + u, 8, stride=SL), :] = hi

        for q in range(4):
            st0_cps[q].wait()

            def rl_body(i, _, q=q):
                relayout(0, q * 128 + i * 16, 16)
                return 0

            lax.fori_loop(0, 8, rl_body, 0)

        def lead_proj(g, hq, rc):
            s0 = g * HG + hq * 4
            w = jnp.concatenate(
                [_unpack(wqkv[pl.ds(pl.multiple_of((s0 + u) * SL, 8), 512), :])
                 for u in range(4)], axis=1)
            y = _pack(_dot(_unpack(hv[rc * 128:(rc + 1) * 128, :]), w))
            for u in range(4):
                ring[s0 + u, rc * 128:(rc + 1) * 128, :] = y[:, u * 128:(u + 1) * 128]

        def group_body(g, _):
            for hq in range(2):
                for rc in range(2):
                    lead_proj(g, hq, rc)

            @pl.when(g == 0)
            def _():
                x1_cp.wait()

            @pl.when(g < NG - 1)
            def _():
                pltpu.make_async_copy(st_src(1), st.at[g + 1],
                                      sems.at[SEM_ST + 5 + g]).wait()

            gn = jnp.minimum(g + 1, NG - 1)
            for hq in range(2, 4):
                for rc in range(2):
                    part = (hq - 2) * 2 + rc
                    lead_proj(g, hq, rc)
                    relayout(gn, part * 128, 128)
                    h_rows(LEAD + g * 256 + part * 64, 64)
            return 0

        lax.fori_loop(0, NG, group_body, 0)

    pl.run_scoped(prologue, pltpu.VMEM((NG, D, HG, E), BF16))

    def main(w3v, w4v, zv, ttv):
        w34_cps = col_copies(w3_hbm, w3v, SEM_W3) + col_copies(w4_hbm, w4v, SEM_W4)
        start(w34_cps)
        wait(modb_cps)
        sc = silu_c()
        for i in range(2, 6):
            modv[i] = _dot(sc, _cols(wmodv, 8 * i, 8 * i + 8))[0:8]
        wait(wo_cps + w1_cps + w2_cps + [mem_cp])

        scale = float(E) ** -0.5

        def segment(lhs, ro, store_tok, wo_lhs, extras):
            fill = fillv[...]
            keep = fill == 0.0
            NP = H // 2
            qkv, probs, blocks = {}, {}, []

            def proj(hp):
                hs = (2 * hp, 2 * hp + 1)
                slots = [_slot(t, h) for t in range(3) for h in hs]
                w = jnp.concatenate(
                    [_unpack(wqkv[pl.ds(sl * SL, 512), :]) for sl in slots], axis=1)
                if hp == 0:
                    y = _dot(lhs[:, :512], w[:512])
                    y = _dot(lhs[:, 512:], w[512:]) + y
                else:
                    y = _dot(lhs, w)
                for u, sl in enumerate(slots):
                    store_tok(sl, y[8:32, u * 128:(u + 1) * 128])
                ops = []
                for t in range(3):
                    ym = jnp.concatenate(
                        [y[0:8, (2 * t) * 128:(2 * t + 1) * 128],
                         y[0:8, (2 * t + 1) * 128:(2 * t + 2) * 128]], axis=0)
                    ops.append(jnp.concatenate(
                        [ym.astype(BF16)]
                        + [_unpack(ring[sl, pl.ds(ro, 16), :])
                           for sl in slots[2 * t:2 * t + 2]], axis=0))
                qkv[hp] = ops

            def scores(hp):
                q, kk, _ = qkv[hp]
                s = lax.dot_general(q, kk, (((1,), (1,)), ((), ())),
                                    preferred_element_type=F32)
                s = jnp.where(keep, s * scale, fill)
                mx = jnp.max(s, axis=-1, keepdims=True)
                p = jnp.exp(s - mx)
                l = jnp.sum(p, axis=-1, keepdims=True)
                rl = pl.reciprocal(l, approx=True)
                rl = rl * (2.0 - l * rl)
                probs[hp] = (p * rl).astype(BF16)

            def pv(hp):
                o = _dot(probs[hp], qkv[hp][2])
                blocks.append(wo_lhs(2 * hp, o[0:8], o[16:48]).astype(BF16))
                blocks.append(wo_lhs(2 * hp + 1, o[8:16], o[48:80]).astype(BF16))

            def wo_part(h0, h1, acc=None):
                lw = jnp.concatenate(blocks[h0:h1], axis=1)
                y = _dot(lw, _cols(wov, 0, 8, E * h0, E * h1))
                return y if acc is None else y + acc

            for i in range(NP):
                proj(i)
                if i >= 1:
                    scores(i - 1)
                if i >= 3:
                    pv(i - 3)
                if i in extras:
                    extras[i]()
            acc = wo_part(0, 4)
            scores(NP - 1)
            pv(NP - 3)
            acc = wo_part(4, 12, acc)
            pv(NP - 2)
            pv(NP - 1)
            acc = wo_part(12, 24, acc)
            acc = wo_part(24, 32, acc)
            return acc

        def p1_front(r0):
            x2 = (xv[pl.ds(pl.multiple_of(r0, 64), 64), :].astype(F32)
                  + mod_row(2) * aout[...])
            h2 = _ln(x2) * (1.0 + mod_row(4)) + mod_row(3)
            return x2, h2, _ln(h2).astype(BF16)

        def p1_tile(u, c, live):
            g = _gelu(_dot(u, _cols(w1v, c, c + 1)))
            if live is not None:
                g = jnp.where(live, g, 0.0)
            gbuf[c, 24:88, :] = g

        def p2_front(n):
            return jnp.concatenate(
                [gbuf[c, 8 + SHIFTS[c]:8 + SHIFTS[c] + n, :] for c in range(8)],
                axis=1).astype(BF16)

        def p2_back(x2, h2, hs, row, n):
            x1 = jnp.concatenate([h2t[...], h2[0:n - 16]], axis=0) + hs
            x2w = jnp.concatenate([x2t[...], x2[0:n - 16]], axis=0)
            zv[pl.ds(pl.multiple_of(row, 16), n), :] = x2w + mod_row(5) * x1
            ttv[pl.ds(pl.multiple_of(row // 2, 8), n // 2), :] = _pack(_ln(x1))

        def a_body(j, mem):
            w0 = LEAD // 2 + 24 * j
            hb = _unpack(hv[pl.ds(pl.multiple_of(w0, 8), 8), :])
            hac = _unpack(hv[pl.ds(pl.multiple_of(w0 + 8, 8), 8), :]).astype(F32)
            hd = _unpack(hv[pl.ds(pl.multiple_of(w0 + 16, 8), 8), :])
            wr = [pl.multiple_of(lax.rem(w0 + 8 * i, RING), 8) for i in range(3)]
            ro0 = pl.multiple_of(lax.rem(32 * j, RING), 16)
            ro1 = pl.multiple_of(lax.rem(32 * j + 16, RING), 16)

            x2, h2, u = p1_front(64 * jnp.maximum(j - 1, 0))
            live = j > 0

            lhs = jnp.concatenate(
                [jnp.concatenate([mem, hac[0:8]], axis=0).astype(BF16), hb], axis=0)
            tok_a = {}

            def store0(c, y):
                tok_a[c] = y[0:8]
                ring[c, pl.ds(wr[0], 8), :] = _pack(y[8:24])

            deferred = {}

            def wo_lhs0(h, om, ot):
                deferred[h] = ot[24:32]
                return jnp.concatenate([om, ot[0:24]], axis=0)

            extras = {5 + c: functools.partial(p1_tile, u, c, live) for c in range(8)}
            out = segment(lhs, ro0, store0, wo_lhs0, extras)
            mem = out[0:8]
            aout[0:24, :] = out[8:32]

            lhs = jnp.concatenate(
                [jnp.concatenate([mem, hac[8:16]], axis=0).astype(BF16), hd], axis=0)

            def store1(c, y):
                ring[c, pl.ds(wr[1], 8), :] = _pack(
                    jnp.concatenate([tok_a[c], y[0:8]], axis=0))
                ring[c, pl.ds(wr[2], 8), :] = _pack(y[8:24])

            def wo_lhs1(h, om, ot):
                return jnp.concatenate([om, deferred[h], ot], axis=0)

            gs = p2_front(64)
            gbuf[:, 0:24, :] = gbuf[:, 64:88, :]
            hs = []

            def p2_tile(c):
                hs.append(_dot(gs, _cols(w2v, c, c + 1)))

            def p2_fin():
                p2_back(x2, h2, jnp.concatenate(hs, axis=1), 64 * j, 64)
                x2t[...] = x2[48:64]
                h2t[...] = h2[48:64]

            extras = {2 + c: functools.partial(p2_tile, c) for c in range(8)}
            extras[11] = p2_fin
            out = segment(lhs, ro1, store1, wo_lhs1, extras)
            aout[24:64, :] = out[8:48]
            return out[0:8]

        if "A" in phases:
            lax.fori_loop(0, NPAIR, a_body, memv[...].astype(F32))
        else:
            zv[...] = jnp.zeros(zv.shape, F32)
            ttv[...] = jnp.zeros(ttv.shape, U32)

        x2, h2, u = p1_front(S - 64)
        for c in range(8):
            p1_tile(u, c, None)
        p2_back(x2, h2, _dot(p2_front(80), _cols(w2v, 0, 8)), S, 80)

        wait(w34_cps)

        def out_cp(i, slot):
            return cp(outv.at[slot], out_hbm.at[pl.ds(i * RB, RB), :],
                      SEM_OUT + slot)

        def p3_body(i, _):
            slot = i % 2

            @pl.when(i >= 2)
            def _():
                out_cp(i - 2, slot).wait()

            r0 = HALO + i * RB
            tt = _unpack(ttv[pl.ds(pl.multiple_of(r0 // 2, 8), RB // 2), :])
            ff = jnp.concatenate(
                [_gelu(_dot(tt, _cols(w3v, 4 * q, 4 * q + 4))).astype(BF16)
                 for q in range(FF // 512)], axis=1)
            y = _dot(ff, _cols(w4v, 0, 8))
            res = zv[pl.ds(pl.multiple_of(r0, 16), RB), :] + mod_row(5) * y
            outv[slot] = res.astype(BF16)
            out_cp(i, slot).start()
            return 0

        nb = S // RB
        if "B" in phases:
            lax.fori_loop(0, nb, p3_body, 0)
            out_cp(nb - 2, 0).wait()
            out_cp(nb - 1, 1).wait()
        else:
            outv[0] = zv[pl.ds(HALO, RB), :].astype(BF16)
            out_cp(0, 0).start()
            out_cp(0, 0).wait()

    pl.run_scoped(
        main,
        pltpu.VMEM((FF // 128, D // 2, 128), U32),
        pltpu.VMEM((8, FF // 2, 128), U32),
        pltpu.VMEM((S + HALO, D), F32),
        pltpu.VMEM(((S + HALO) // 2, D), U32),
    )


def _call(A_x, A_mem0, A_Wq, A_Wk, A_Wv, A_Wo, B_w1, B_w2, B_w3, B_w4, c, w_mod,
          phases="AB"):
    any_spec = pl.BlockSpec(memory_space=pl.ANY)
    scratch = [
        pltpu.VMEM((S, D), BF16),
        pltpu.VMEM((1, D), BF16),
        pltpu.VMEM((M, D), BF16),
        pltpu.VMEM((48, D // 2, 128), U32),
        pltpu.VMEM((6, 8, D), F32),
        pltpu.VMEM((3 * H * SL, E), U32),
        pltpu.VMEM((8, H * E // 2, 128), U32),
        pltpu.VMEM((8, D // 2, 128), U32),
        pltpu.VMEM((8, D // 2, 128), U32),
        pltpu.VMEM((S // 2, D), U32),
        pltpu.VMEM((3 * H, RING, E), U32),
        pltpu.VMEM((80, 80), F32),
        pltpu.VMEM((64, D), F32),
        pltpu.VMEM((8, 96, 128), F32),
        pltpu.VMEM((16, D), F32),
        pltpu.VMEM((16, D), F32),
        pltpu.VMEM((2, RB, D), BF16),
        pltpu.SemaphoreType.DMA((NSEM,)),
    ]
    out = pl.pallas_call(
        functools.partial(_kernel, phases=phases),
        in_specs=[any_spec] * 12,
        out_specs=any_spec,
        out_shape=jax.ShapeDtypeStruct((S, D), BF16),
        scratch_shapes=scratch,
        compiler_params=pltpu.CompilerParams(
            vmem_limit_bytes=126 * 1024 * 1024),
    )(A_x.reshape(S, D), A_mem0.reshape(M, D), A_Wq, A_Wk, A_Wv,
      A_Wo.reshape(H * E, D), B_w1, B_w2, B_w3, B_w4, c, w_mod)
    return out.reshape(1, S, D)


def pallas_adaLN_cond__memory_aug_recurrent_mem_tr__mixer_s_mlp__prompt_kernel(
    A_x, A_mem0, A_Wq, A_Wk, A_Wv, A_Wo, A_seg_len, B_x, B_w1, B_w2, B_w3, B_w4,
    c, w_mod,
):
    assert A_seg_len == SEG
    del B_x
    return _call(A_x, A_mem0, A_Wq, A_Wk, A_Wv, A_Wo, B_w1, B_w2, B_w3, B_w4,
                 c, w_mod)
```

```python
import functools

import jax
import jax.numpy as jnp
from jax import lax
import jax.experimental.pallas as pl
import jax.experimental.pallas.tpu as pltpu

F32 = jnp.float32
BF16 = jnp.bfloat16
U32 = jnp.uint32

S = 2048
D = 1024
H = 32
E = 128
M = 8
SEG = 32
FF = 3584
EPS = 1e-5

LEAD = 512
RING = 288
SL = 520
HG = 16
NG = 3 * H // HG
NPAIR = S // (2 * SEG)
HALO = 80
RB = 256
SHIFTS = (-1, -1, 1, 1, -2, -2, 2, 2)

(SEM_X0, SEM_X1, SEM_C, SEM_MEM, SEM_WO, SEM_W1, SEM_W2, SEM_W3, SEM_W4,
 SEM_MODA, SEM_MODB) = range(11)
SEM_ST = 11
SEM_OUT = SEM_ST + 4 + NG
NSEM = SEM_OUT + 2


def _ln(x):
    mu = jnp.mean(x, axis=-1, keepdims=True)
    xc = x - mu
    var = jnp.mean(xc * xc, axis=-1, keepdims=True)
    return xc * lax.rsqrt(var + EPS)


def _gelu(x):
    return jax.nn.gelu(x, approximate=True)


def _pack(x):
    return pltpu.bitcast(x.astype(BF16), U32)


def _unpack(x):
    return pltpu.bitcast(x, BF16)


def _dot(a, b):
    return jnp.dot(a, b, preferred_element_type=F32)


def _cols(ref, lo, hi, k0=0, k1=None):
    k1 = 2 * ref.shape[1] if k1 is None else k1
    return jnp.concatenate(
        [_unpack(ref[c, k0 // 2:k1 // 2, :]) for c in range(lo, hi)], axis=1)


def _kernel(x_hbm, mem_hbm, wq_hbm, wk_hbm, wv_hbm, wo_hbm, w1_hbm, w2_hbm,
            w3_hbm, w4_hbm, c_hbm, wmod_hbm, out_hbm,
            xv, cv, memv, wmodv, modv, wqa, wqb, wov, w1v, w2v,
            hv0, hv1, ring, fillv, aout, gbuf, x2t, h2t, outv, sems, *, phases):
    def cp(src, dst, s):
        return pltpu.make_async_copy(src, dst, sems.at[s])

    def col_copies(w_hbm, w_v, s, lo=0, hi=None):
        w32 = w_hbm.bitcast(U32)
        hi = w_v.shape[0] if hi is None else hi
        return [cp(w32.at[:, pl.ds(c * 128, 128)], w_v.at[c], s)
                for c in range(lo, hi)]

    def start(cps):
        for q in cps:
            q.start()

    def wait(cps):
        for q in cps:
            q.wait()

    c_cp = cp(c_hbm, cv, SEM_C)
    mem_cp = cp(mem_hbm, memv, SEM_MEM)
    x0_cp = cp(x_hbm.at[pl.ds(0, LEAD)], xv.at[pl.ds(0, LEAD)], SEM_X0)
    x1_cp = cp(x_hbm.at[pl.ds(LEAD, S - LEAD)], xv.at[pl.ds(LEAD, S - LEAD)],
               SEM_X1)
    moda_cps = col_copies(wmod_hbm, wmodv, SEM_MODA, 0, 16)
    modb_cps = col_copies(wmod_hbm, wmodv, SEM_MODB, 16, 48)
    wo_cps = col_copies(wo_hbm, wov, SEM_WO)
    w1_cps = col_copies(w1_hbm, w1v, SEM_W1)
    w2_cps = col_copies(w2_hbm, w2v, SEM_W2)

    def mod_row(i):
        return modv[i, 0:1, :]

    def silu_c():
        cf = cv[...].astype(F32)
        return jnp.broadcast_to((cf * jax.nn.sigmoid(cf)).astype(BF16), (16, D))

    wq2 = (wqa, wqb)

    def h_rows(hv, off, i, n):
        xf = xv[pl.ds(pl.multiple_of(off + i * n, n), n), :].astype(F32)
        hh = _ln(xf) * (1.0 + mod_row(1)) + mod_row(0)
        hv[pl.ds(pl.multiple_of(i * (n // 2), n // 2), n // 2), :] = _pack(hh)

    def prologue(st):
        w_hbms = (wq_hbm, wk_hbm, wv_hbm)

        def st_src(i):
            return w_hbms[i // 2].at[:, pl.ds((i % 2) * HG, HG), :]

        st0_cps = [cp(st_src(0).at[pl.ds(q * 256, 256)],
                      st.at[0, pl.ds(q * 256, 256)], SEM_ST + q) for q in range(4)]
        st_cps = [None] + [cp(st_src(i), st.at[i], SEM_ST + 4 + i)
                           for i in range(1, NG)]

        start([c_cp, mem_cp, x0_cp])
        start(moda_cps)
        start(st0_cps)
        start([st_cps[1], x1_cp, st_cps[2], st_cps[3]])
        start(wo_cps)
        start([st_cps[4]])
        start(modb_cps)
        start([st_cps[5]])
        start(w1_cps + w2_cps)

        r = lax.broadcasted_iota(jnp.int32, (80, 80), 0)
        k = lax.broadcasted_iota(jnp.int32, (80, 80), 1)

        def head_of(i):
            return jnp.where(i < 16, i // 8, (i - 16) // 32)

        def pos_of(i):
            return jnp.where(i < 16, i % 8, 8 + (i - 16) % 32)

        same = head_of(r) == head_of(k)
        vis = (pos_of(r) < M) | (pos_of(r) >= pos_of(k))
        fillv[...] = jnp.where(same, jnp.where(vis, 0.0, -1e9), -jnp.inf).astype(F32)
        aout[...] = jnp.zeros(aout.shape, F32)
        gbuf[...] = jnp.zeros(gbuf.shape, F32)
        x2t[...] = jnp.zeros(x2t.shape, F32)
        h2t[...] = jnp.zeros(h2t.shape, F32)

        c_cp.wait()
        wait(moda_cps)
        sc = silu_c()
        for i in range(2):
            modv[i] = _dot(sc, _cols(wmodv, 8 * i, 8 * i + 8))[0:8]
        x0_cp.wait()

        def ln_body(i, _):
            h_rows(hv0, 0, i, 64)
            return 0

        lax.fori_loop(0, LEAD // 64, ln_body, 0)

        def relayout(par, g, p0, n):
            base = g * (8 * SL)
            for u in range(n):
                a = pltpu.bitcast(st[g, 2 * (p0 + u)], U32)
                b = pltpu.bitcast(st[g, 2 * (p0 + u) + 1], U32)
                if par == 0:
                    w = (a & jnp.uint32(0xFFFF)) | (b << 16)
                else:
                    w = (a >> 16) | (b & jnp.uint32(0xFFFF0000))
                wq2[par][pl.ds(base + p0 + u, 8, stride=SL), :] = w

        for q in range(4):
            st0_cps[q].wait()

            def rl_body(i, _, q=q):
                relayout(0, 0, q * 128 + i * 32, 32)
                return 0

            lax.fori_loop(0, 4, rl_body, 0)

        def lead_proj(par, g, hq, rc):
            s0 = g * 8 + hq * 4
            w = jnp.concatenate(
                [_unpack(wq2[par][pl.ds(pl.multiple_of((s0 + u) * SL, 8), 512), :])
                 for u in range(4)], axis=1)
            y = _pack(_dot(_unpack(hv0[rc * 128:(rc + 1) * 128, :]), w))
            for u in range(4):
                ring[2 * (s0 + u) + par, rc * 128:(rc + 1) * 128, :] = (
                    y[:, u * 128:(u + 1) * 128])

        def group_body(g, _):
            for part in range(4):
                lead_proj(0, g, part // 2, part % 2)
                relayout(1, g, part * 128, 128)

            @pl.when(g == 0)
            def _():
                x1_cp.wait()

            @pl.when(g < NG - 1)
            def _():
                pltpu.make_async_copy(st_src(1), st.at[g + 1],
                                      sems.at[SEM_ST + 5 + g]).wait()

            gn = jnp.minimum(g + 1, NG - 1)
            for part in range(4):
                lead_proj(1, g, part // 2, part % 2)
                relayout(0, gn, part * 128, 128)
                h_rows(hv1, LEAD, g * 4 + part, 64)
            return 0

        lax.fori_loop(0, NG, group_body, 0)

    pl.run_scoped(prologue, pltpu.VMEM((NG, D, HG, E), BF16))

    def main(w3v, w4v, zv, ttv):
        w34_cps = col_copies(w3_hbm, w3v, SEM_W3) + col_copies(w4_hbm, w4v, SEM_W4)
        start(w34_cps)
        wait(modb_cps)
        sc = silu_c()
        for i in range(2, 6):
            modv[i] = _dot(sc, _cols(wmodv, 8 * i, 8 * i + 8))[0:8]
        wait(wo_cps + w1_cps + w2_cps + [mem_cp])

        scale = float(E) ** -0.5

        def segment(lhs, ro, store_tok, wo_lhs, extras):
            fill = fillv[...]
            keep = fill == 0.0
            NP = H // 2
            qkv, probs, blocks = {}, {}, []

            def proj(hp):
                slots = [t * H + 2 * hp + par for t in range(3) for par in range(2)]
                w = jnp.concatenate(
                    [_unpack(wq2[sl % 2][pl.ds((sl // 2) * SL, 512), :])
                     for sl in slots], axis=1)
                if hp == 0:
                    y = _dot(lhs[:, :512], w[:512])
                    y = _dot(lhs[:, 512:], w[512:]) + y
                else:
                    y = _dot(lhs, w)
                for u, sl in enumerate(slots):
                    store_tok(sl, y[8:32, u * 128:(u + 1) * 128])
                ops = []
                for t in range(3):
                    ym = jnp.concatenate(
                        [y[0:8, (2 * t) * 128:(2 * t + 1) * 128],
                         y[0:8, (2 * t + 1) * 128:(2 * t + 2) * 128]], axis=0)
                    ops.append(jnp.concatenate(
                        [ym.astype(BF16)]
                        + [_unpack(ring[sl, pl.ds(ro, 16), :])
                           for sl in slots[2 * t:2 * t + 2]], axis=0))
                qkv[hp] = ops

            def scores(hp):
                q, kk, _ = qkv[hp]
                s = lax.dot_general(q, kk, (((1,), (1,)), ((), ())),
                                    preferred_element_type=F32)
                s = jnp.where(keep, s * scale, fill)
                mx = jnp.max(s, axis=-1, keepdims=True)
                p = jnp.exp(s - mx)
                l = jnp.sum(p, axis=-1, keepdims=True)
                rl = pl.reciprocal(l, approx=True)
                rl = rl * (2.0 - l * rl)
                probs[hp] = (p * rl).astype(BF16)

            def pv(hp):
                o = _dot(probs[hp], qkv[hp][2])
                blocks.append(wo_lhs(2 * hp, o[0:8], o[16:48]).astype(BF16))
                blocks.append(wo_lhs(2 * hp + 1, o[8:16], o[48:80]).astype(BF16))

            def wo_part(h0, h1, acc=None):
                lw = jnp.concatenate(blocks[h0:h1], axis=1)
                y = _dot(lw, _cols(wov, 0, 8, E * h0, E * h1))
                return y if acc is None else y + acc

            for i in range(NP):
                proj(i)
                if i >= 1:
                    scores(i - 1)
                if i >= 3:
                    pv(i - 3)
                for thunk in extras.get(i, ()):
                    thunk()
            acc = wo_part(0, 4)
            scores(NP - 1)
            pv(NP - 3)
            acc = wo_part(4, 12, acc)
            pv(NP - 2)
            pv(NP - 1)
            acc = wo_part(12, 24, acc)
            acc = wo_part(24, 32, acc)
            return acc

        def p1_front(r0):
            x2 = (xv[pl.ds(pl.multiple_of(r0, 64), 64), :].astype(F32)
                  + mod_row(2) * aout[...])
            h2 = _ln(x2) * (1.0 + mod_row(4)) + mod_row(3)
            return x2, h2, _ln(h2).astype(BF16)

        def p1_store(y, c, live):
            g = _gelu(y)
            if live is not None:
                g = jnp.where(live, g, 0.0)
            gbuf[c, 24:88, :] = g

        def half_dots(lhs, wv, done):
            part = {}

            def run(c, kh):
                y = _dot(lhs[:, kh * 512:(kh + 1) * 512],
                         _cols(wv, c, c + 1, kh * 512, (kh + 1) * 512))
                if kh == 0:
                    part[c] = y
                else:
                    done(y + part[c], c)

            return [functools.partial(run, c, kh) for c in range(8) for kh in range(2)]

        def p2_front(n):
            return jnp.concatenate(
                [gbuf[c, 8 + SHIFTS[c]:8 + SHIFTS[c] + n, :] for c in range(8)],
                axis=1).astype(BF16)

        def p2_back(x2, h2, hs, row, n):
            x1 = jnp.concatenate([h2t[...], h2[0:n - 16]], axis=0) + hs
            x2w = jnp.concatenate([x2t[...], x2[0:n - 16]], axis=0)
            zv[pl.ds(pl.multiple_of(row, 16), n), :] = x2w + mod_row(5) * x1
            ttv[pl.ds(pl.multiple_of(row // 2, 8), n // 2), :] = _pack(_ln(x1))

        def a_body(j, mem):
            w0 = 24 * j
            hb = _unpack(hv1[pl.ds(pl.multiple_of(w0, 8), 8), :])
            hac = _unpack(hv1[pl.ds(pl.multiple_of(w0 + 8, 8), 8), :]).astype(F32)
            hd = _unpack(hv1[pl.ds(pl.multiple_of(w0 + 16, 8), 8), :])
            wr = [pl.multiple_of(lax.rem(LEAD // 2 + w0 + 8 * i, RING), 8)
                  for i in range(3)]
            ro0 = pl.multiple_of(lax.rem(32 * j, RING), 16)
            ro1 = pl.multiple_of(lax.rem(32 * j + 16, RING), 16)

            x2, h2, u = p1_front(64 * jnp.maximum(j - 1, 0))
            live = j > 0

            lhs = jnp.concatenate(
                [jnp.concatenate([mem, hac[0:8]], axis=0).astype(BF16), hb], axis=0)
            tok_a = {}

            def store0(c, y):
                tok_a[c] = y[0:8]
                ring[c, pl.ds(wr[0], 8), :] = _pack(y[8:24])

            deferred = {}

            def wo_lhs0(h, om, ot):
                deferred[h] = ot[24:32]
                return jnp.concatenate([om, ot[0:24]], axis=0)

            th = half_dots(u, w1v, lambda y, c: p1_store(y, c, live))
            extras = {i: [th[i - 2]] for i in range(2, 14)}
            extras[14] = th[12:14]
            extras[15] = th[14:16]
            out = segment(lhs, ro0, store0, wo_lhs0, extras)
            mem = out[0:8]
            aout[0:24, :] = out[8:32]

            lhs = jnp.concatenate(
                [jnp.concatenate([mem, hac[8:16]], axis=0).astype(BF16), hd], axis=0)

            def store1(c, y):
                ring[c, pl.ds(wr[1], 8), :] = _pack(
                    jnp.concatenate([tok_a[c], y[0:8]], axis=0))
                ring[c, pl.ds(wr[2], 8), :] = _pack(y[8:24])

            def wo_lhs1(h, om, ot):
                return jnp.concatenate([om, deferred[h], ot], axis=0)

            gs = p2_front(64)
            gbuf[:, 0:24, :] = gbuf[:, 64:88, :]
            hs = []

            def p2_fin():
                p2_back(x2, h2, jnp.concatenate(hs, axis=1), 64 * j, 64)
                x2t[...] = x2[48:64]
                h2t[...] = h2[48:64]

            th = half_dots(gs, w2v, lambda y, c: hs.append(y))
            extras = {i: [th[i]] for i in range(16)}
            extras[15].append(p2_fin)
            out = segment(lhs, ro1, store1, wo_lhs1, extras)
            aout[24:64, :] = out[8:48]
            return out[0:8]

        if "A" in phases:
            lax.fori_loop(0, NPAIR, a_body, memv[...].astype(F32))
        else:
            zv[...] = jnp.zeros(zv.shape, F32)
            ttv[...] = jnp.zeros(ttv.shape, U32)

        x2, h2, u = p1_front(S - 64)
        y = _dot(u, _cols(w1v, 0, 8))
        for c in range(8):
            p1_store(y[:, c * 128:(c + 1) * 128], c, None)
        p2_back(x2, h2, _dot(p2_front(80), _cols(w2v, 0, 8)), S, 80)

        wait(w34_cps)

        def out_cp(i, slot):
            return cp(outv.at[slot], out_hbm.at[pl.ds(i * RB, RB), :],
                      SEM_OUT + slot)

        def p3_body(i, _):
            slot = i % 2

            @pl.when(i >= 2)
            def _():
                out_cp(i - 2, slot).wait()

            r0 = HALO + i * RB
            tt = _unpack(ttv[pl.ds(pl.multiple_of(r0 // 2, 8), RB // 2), :])
            ff = jnp.concatenate(
                [_gelu(_dot(tt, _cols(w3v, 4 * q, 4 * q + 4))).astype(BF16)
                 for q in range(FF // 512)], axis=1)
            y = _dot(ff, _cols(w4v, 0, 8))
            res = zv[pl.ds(pl.multiple_of(r0, 16), RB), :] + mod_row(5) * y
            outv[slot] = res.astype(BF16)
            out_cp(i, slot).start()
            return 0

        nb = S // RB
        if "B" in phases:
            lax.fori_loop(0, nb, p3_body, 0)
            out_cp(nb - 2, 0).wait()
            out_cp(nb - 1, 1).wait()
        else:
            outv[0] = zv[pl.ds(HALO, RB), :].astype(BF16)
            out_cp(0, 0).start()
            out_cp(0, 0).wait()

    pl.run_scoped(
        main,
        pltpu.VMEM((FF // 128, D // 2, 128), U32),
        pltpu.VMEM((8, FF // 2, 128), U32),
        pltpu.VMEM((S + HALO, D), F32),
        pltpu.VMEM(((S + HALO) // 2, D), U32),
    )


def _call(A_x, A_mem0, A_Wq, A_Wk, A_Wv, A_Wo, B_w1, B_w2, B_w3, B_w4, c, w_mod,
          phases="AB"):
    any_spec = pl.BlockSpec(memory_space=pl.ANY)
    scratch = [
        pltpu.VMEM((S, D), BF16),
        pltpu.VMEM((1, D), BF16),
        pltpu.VMEM((M, D), BF16),
        pltpu.VMEM((48, D // 2, 128), U32),
        pltpu.VMEM((6, 8, D), F32),
        pltpu.VMEM((3 * H // 2 * SL, E), U32),
        pltpu.VMEM((3 * H // 2 * SL, E), U32),
        pltpu.VMEM((8, H * E // 2, 128), U32),
        pltpu.VMEM((8, D // 2, 128), U32),
        pltpu.VMEM((8, D // 2, 128), U32),
        pltpu.VMEM((LEAD // 2, D), U32),
        pltpu.VMEM(((S - LEAD) // 2, D), U32),
        pltpu.VMEM((3 * H, RING, E), U32),
        pltpu.VMEM((80, 80), F32),
        pltpu.VMEM((64, D), F32),
        pltpu.VMEM((8, 96, 128), F32),
        pltpu.VMEM((16, D), F32),
        pltpu.VMEM((16, D), F32),
        pltpu.VMEM((2, RB, D), BF16),
        pltpu.SemaphoreType.DMA((NSEM,)),
    ]
    out = pl.pallas_call(
        functools.partial(_kernel, phases=phases),
        in_specs=[any_spec] * 12,
        out_specs=any_spec,
        out_shape=jax.ShapeDtypeStruct((S, D), BF16),
        scratch_shapes=scratch,
        compiler_params=pltpu.CompilerParams(
            vmem_limit_bytes=126 * 1024 * 1024),
    )(A_x.reshape(S, D), A_mem0.reshape(M, D), A_Wq, A_Wk, A_Wv,
      A_Wo.reshape(H * E, D), B_w1, B_w2, B_w3, B_w4, c, w_mod)
    return out.reshape(1, S, D)


def pallas_adaLN_cond__memory_aug_recurrent_mem_tr__mixer_s_mlp__prompt_kernel(
    A_x, A_mem0, A_Wq, A_Wk, A_Wv, A_Wo, A_seg_len, B_x, B_w1, B_w2, B_w3, B_w4,
    c, w_mod,
):
    assert A_seg_len == SEG
    del B_x
    return _call(A_x, A_mem0, A_Wq, A_Wk, A_Wv, A_Wo, B_w1, B_w2, B_w3, B_w4,
                 c, w_mod)
```

```python
import contextlib
import functools

import jax
import jax.numpy as jnp
from jax import lax
import jax.experimental.pallas as pl
import jax.experimental.pallas.tpu as pltpu

F32 = jnp.float32
BF16 = jnp.bfloat16
U32 = jnp.uint32

S = 2048
D = 1024
H = 32
E = 128
M = 8
SEG = 32
FF = 3584
EPS = 1e-5

LEAD = 512
RING = 36
X0 = 640
SL = 520
HG = 16
NG = 3 * H // HG
NPAIR = S // (2 * SEG)
HALO = 80
RB = 256
SHIFTS = (-1, -1, 1, 1, -2, -2, 2, 2)

(SEM_X0, SEM_X1, SEM_C, SEM_MEM, SEM_WO, SEM_W1, SEM_W2, SEM_W3, SEM_W4,
 SEM_MODA, SEM_MODB) = range(11)
SEM_ST = 11
SEM_OUT = SEM_ST + 4 + NG
NSEM = SEM_OUT + 2


def _ln(x):
    mu = jnp.mean(x, axis=-1, keepdims=True)
    xc = x - mu
    var = jnp.mean(xc * xc, axis=-1, keepdims=True)
    return xc * lax.rsqrt(var + EPS)


def _gelu(x):
    return jax.nn.gelu(x, approximate=True)


def _pack(x):
    return pltpu.bitcast(x.astype(BF16), U32)


def _unpack(x):
    return pltpu.bitcast(x, BF16)


def _dot(a, b):
    return jnp.dot(a, b, preferred_element_type=F32)


def _cols(ref, lo, hi, k0=0, k1=None):
    k1 = 2 * ref.shape[1] if k1 is None else k1
    return jnp.concatenate(
        [_unpack(ref[c, k0 // 2:k1 // 2, :]) for c in range(lo, hi)], axis=1)


def _kernel(x_hbm, mem_hbm, wq_hbm, wk_hbm, wv_hbm, wo_hbm, w1_hbm, w2_hbm,
            w3_hbm, w4_hbm, c_hbm, wmod_hbm, out_hbm,
            xv, cv, memv, wmodv, modv, wqa, wqb, wov, w1v, w2v,
            hv0, hcur, hnext, ring, fillv, aout, gbuf, x2t, h2t, outv, sems, *, phases):
    def scope(name):
        return jax.named_scope(name) if "s" in phases else contextlib.nullcontext()

    def cp(src, dst, s):
        return pltpu.make_async_copy(src, dst, sems.at[s])

    def col_copies(w_hbm, w_v, s, lo=0, hi=None):
        w32 = w_hbm.bitcast(U32)
        hi = w_v.shape[0] if hi is None else hi
        return [cp(w32.at[:, pl.ds(c * 128, 128)], w_v.at[c], s)
                for c in range(lo, hi)]

    def start(cps):
        for q in cps:
            q.start()

    def wait(cps):
        for q in cps:
            q.wait()

    c_cp = cp(c_hbm, cv, SEM_C)
    mem_cp = cp(mem_hbm, memv, SEM_MEM)
    x0_cp = cp(x_hbm.at[pl.ds(0, LEAD)], xv.at[pl.ds(0, LEAD)], SEM_X0)
    x1_cp = cp(x_hbm.at[pl.ds(LEAD, S - LEAD)], xv.at[pl.ds(LEAD, S - LEAD)],
               SEM_X1)
    moda_cps = col_copies(wmod_hbm, wmodv, SEM_MODA, 0, 16)
    modb_cps = col_copies(wmod_hbm, wmodv, SEM_MODB, 16, 48)
    wo_cps = col_copies(wo_hbm, wov, SEM_WO)
    w1_cps = col_copies(w1_hbm, w1v, SEM_W1)
    w2_cps = col_copies(w2_hbm, w2v, SEM_W2)

    def mod_row(i):
        return modv[i, 0:1, :]

    def silu_c():
        cf = cv[...].astype(F32)
        return jnp.broadcast_to((cf * jax.nn.sigmoid(cf)).astype(BF16), (16, D))

    wq2 = (wqa, wqb)

    def h_rows(r0, n):
        xf = xv[pl.ds(pl.multiple_of(r0, 16), n), :].astype(F32)
        return _pack(_ln(xf) * (1.0 + mod_row(1)) + mod_row(0))

    def prologue(st):
        w_hbms = (wq_hbm, wk_hbm, wv_hbm)

        def st_src(i):
            return w_hbms[i // 2].at[:, pl.ds((i % 2) * HG, HG), :]

        st0_cps = [cp(st_src(0).at[pl.ds(q * 256, 256)],
                      st.at[0, pl.ds(q * 256, 256)], SEM_ST + q) for q in range(4)]
        st_cps = [None] + [cp(st_src(i), st.at[i], SEM_ST + 4 + i)
                           for i in range(1, NG)]

        with scope("first"):
            start([c_cp, mem_cp, x0_cp])
        start(moda_cps)
        start(st0_cps)
        start([st_cps[1], st_cps[2], x1_cp, st_cps[3]])
        start(wo_cps)
        start([st_cps[4]])
        start(modb_cps)
        start([st_cps[5]])
        start(w1_cps + w2_cps)

        r = lax.broadcasted_iota(jnp.int32, (80, 80), 0)
        k = lax.broadcasted_iota(jnp.int32, (80, 80), 1)

        def head_of(i):
            return jnp.where(i < 16, i // 8, (i - 16) // 32)

        def pos_of(i):
            return jnp.where(i < 16, i % 8, 8 + (i - 16) % 32)

        same = head_of(r) == head_of(k)
        vis = (pos_of(r) < M) | (pos_of(r) >= pos_of(k))
        fillv[...] = jnp.where(same, jnp.where(vis, 0.0, -1e9), -jnp.inf).astype(F32)
        aout[...] = jnp.zeros(aout.shape, F32)
        gbuf[...] = jnp.zeros(gbuf.shape, F32)
        x2t[...] = jnp.zeros(x2t.shape, F32)
        h2t[...] = jnp.zeros(h2t.shape, F32)

        c_cp.wait()
        wait(moda_cps)
        sc = silu_c()
        for i in range(2):
            modv[i] = _dot(sc, _cols(wmodv, 8 * i, 8 * i + 8))[0:8]
        x0_cp.wait()

        def ln_body(i, _):
            hv0[pl.ds(pl.multiple_of(i * 32, 32), 32), :] = h_rows(i * 64, 64)
            return 0

        lax.fori_loop(0, LEAD // 64, ln_body, 0)

        def relayout(par, g, p0, n):
            base = g * (8 * SL)
            for u in range(n):
                a = pltpu.bitcast(st[g, 2 * (p0 + u)], U32)
                b = pltpu.bitcast(st[g, 2 * (p0 + u) + 1], U32)
                if par == 0:
                    w = (a & jnp.uint32(0xFFFF)) | (b << 16)
                else:
                    w = (a >> 16) | (b & jnp.uint32(0xFFFF0000))
                wq2[par][pl.ds(base + p0 + u, 8, stride=SL), :] = w

        for q in range(4):
            st0_cps[q].wait()

            def rl_body(i, _, q=q):
                relayout(0, 0, q * 128 + i * 32, 32)
                return 0

            lax.fori_loop(0, 4, rl_body, 0)

        def lead_proj(par, g, hq, rc):
            s0 = g * 8 + hq * 4
            w = jnp.concatenate(
                [_unpack(wq2[par][pl.ds(pl.multiple_of((s0 + u) * SL, 8), 512), :])
                 for u in range(4)], axis=1)
            y = _pack(_dot(_unpack(hv0[rc * 128:(rc + 1) * 128, :]), w))
            for u in range(4):
                row = pl.multiple_of((2 * (s0 + u) + par) * 8, 8)
                for b in range(16):
                    ring[rc * 16 + b, pl.ds(row, 8), :] = (
                        y[b * 8:(b + 1) * 8, u * 128:(u + 1) * 128])

        def group_body(g, _):
            for part in range(4):
                lead_proj(0, g, part // 2, part % 2)
                relayout(1, g, part * 128, 128)

            @pl.when(g < NG - 1)
            def _():
                pltpu.make_async_copy(st_src(1), st.at[g + 1],
                                      sems.at[SEM_ST + 5 + g]).wait()

            gn = jnp.minimum(g + 1, NG - 1)
            for part in range(4):
                lead_proj(1, g, part // 2, part % 2)
                relayout(0, gn, part * 128, 128)
            return 0

        with scope("groups"):
            lax.fori_loop(0, NG, group_body, 0)

    pl.run_scoped(prologue, pltpu.VMEM((NG, D, HG, E), BF16))

    def main(w3v, w4v, zv, ttv):
        w34_cps = col_copies(w3_hbm, w3v, SEM_W3) + col_copies(w4_hbm, w4v, SEM_W4)
        start(w34_cps)
        wait(modb_cps)
        sc = silu_c()
        for i in range(2, 6):
            modv[i] = _dot(sc, _cols(wmodv, 8 * i, 8 * i + 8))[0:8]
        wait(wo_cps + w1_cps + w2_cps + [mem_cp, x1_cp])
        hnext[...] = h_rows(LEAD, 48)

        scale = float(E) ** -0.5

        def segment(lhs, ro, store_tok, wo_lhs, extras):
            fill = fillv[...]
            keep = fill == 0.0
            NP = H // 2
            qkv, probs, blocks = {}, {}, []

            def proj(hp):
                slots = [t * H + 2 * hp + par for t in range(3) for par in range(2)]
                w = jnp.concatenate(
                    [_unpack(wq2[sl % 2][pl.ds((sl // 2) * SL, 512), :])
                     for sl in slots], axis=1)
                if hp == 0:
                    y = _dot(lhs[:, :512], w[:512])
                    y = _dot(lhs[:, 512:], w[512:]) + y
                else:
                    y = _dot(lhs, w)
                for u, sl in enumerate(slots):
                    store_tok(sl, y[8:32, u * 128:(u + 1) * 128])
                ops = []
                for t in range(3):
                    ym = jnp.concatenate(
                        [y[0:8, (2 * t) * 128:(2 * t + 1) * 128],
                         y[0:8, (2 * t + 1) * 128:(2 * t + 2) * 128]], axis=0)
                    ops.append(jnp.concatenate(
                        [ym.astype(BF16)]
                        + [_unpack(ring[ro + b, sl * 8:(sl + 1) * 8, :])
                           for sl in slots[2 * t:2 * t + 2] for b in range(2)],
                        axis=0))
                qkv[hp] = ops

            def scores(hp):
                q, kk, _ = qkv[hp]
                s = lax.dot_general(q, kk, (((1,), (1,)), ((), ())),
                                    preferred_element_type=F32)
                s = jnp.where(keep, s * scale, fill)
                mx = jnp.max(s, axis=-1, keepdims=True)
                p = jnp.exp(s - mx)
                l = jnp.sum(p, axis=-1, keepdims=True)
                rl = pl.reciprocal(l, approx=True)
                rl = rl * (2.0 - l * rl)
                probs[hp] = (p * rl).astype(BF16)

            def pv(hp):
                o = _dot(probs[hp], qkv[hp][2])
                blocks.append(wo_lhs(2 * hp, o[0:8], o[16:48]).astype(BF16))
                blocks.append(wo_lhs(2 * hp + 1, o[8:16], o[48:80]).astype(BF16))

            def wo_part(h0, h1, acc=None):
                lw = jnp.concatenate(blocks[h0:h1], axis=1)
                y = _dot(lw, _cols(wov, 0, 8, E * h0, E * h1))
                return y if acc is None else y + acc

            for i in range(NP):
                proj(i)
                if i >= 1:
                    scores(i - 1)
                if i >= 3:
                    pv(i - 3)
                for thunk in extras.get(i, ()):
                    thunk()
            acc = wo_part(0, 4)
            scores(NP - 1)
            pv(NP - 3)
            acc = wo_part(4, 12, acc)
            pv(NP - 2)
            pv(NP - 1)
            acc = wo_part(12, 24, acc)
            acc = wo_part(24, 32, acc)
            return acc

        def p1_front(r0):
            x2 = (xv[pl.ds(pl.multiple_of(r0, 64), 64), :].astype(F32)
                  + mod_row(2) * aout[...])
            h2 = _ln(x2) * (1.0 + mod_row(4)) + mod_row(3)
            return x2, h2, _ln(h2).astype(BF16)

        def p1_store(y, c, live):
            g = _gelu(y)
            if live is not None:
                g = jnp.where(live, g, 0.0)
            gbuf[c, 24:88, :] = g

        def half_dots(lhs, wv, done):
            part = {}

            def run(c, kh):
                y = _dot(lhs[:, kh * 512:(kh + 1) * 512],
                         _cols(wv, c, c + 1, kh * 512, (kh + 1) * 512))
                if kh == 0:
                    part[c] = y
                else:
                    done(y + part[c], c)

            return [functools.partial(run, c, kh) for c in range(8) for kh in range(2)]

        def p2_front(n):
            return jnp.concatenate(
                [gbuf[c, 8 + SHIFTS[c]:8 + SHIFTS[c] + n, :] for c in range(8)],
                axis=1).astype(BF16)

        def p2_back(x2, h2, hs, row, n):
            x1 = jnp.concatenate([h2t[...], h2[0:n - 16]], axis=0) + hs
            x2w = jnp.concatenate([x2t[...], x2[0:n - 16]], axis=0)
            zv[pl.ds(pl.multiple_of(row, 16), n), :] = x2w + mod_row(5) * x1
            ttv[pl.ds(pl.multiple_of(row // 2, 8), n // 2), :] = _pack(_ln(x1))

        def a_body(j, mem):
            hcur[...] = hnext[...]
            hb = _unpack(hcur[0:8, :])
            hac = _unpack(hcur[8:16, :]).astype(F32)
            hd = _unpack(hcur[16:24, :])
            wr = [lax.rem(LEAD // 16 + 3 * j + i, RING) for i in range(3)]
            ro0 = lax.rem(4 * j, RING)
            ro1 = ro0 + 2

            x2, h2, u = p1_front(64 * jnp.maximum(j - 1, 0))
            live = j > 0

            lhs = jnp.concatenate(
                [jnp.concatenate([mem, hac[0:8]], axis=0).astype(BF16), hb], axis=0)
            tok_a = {}

            def store0(c, y):
                tok_a[c] = y[0:8]
                ring[wr[0], c * 8:(c + 1) * 8, :] = _pack(y[8:24])

            deferred = {}

            def wo_lhs0(h, om, ot):
                deferred[h] = ot[24:32]
                return jnp.concatenate([om, ot[0:24]], axis=0)

            th = half_dots(u, w1v, lambda y, c: p1_store(y, c, live))
            extras = {i: [th[i - 2]] for i in range(2, 14)}
            extras[14] = th[12:14]
            extras[15] = th[14:16]
            out = segment(lhs, ro0, store0, wo_lhs0, extras)
            mem = out[0:8]
            aout[0:24, :] = out[8:32]

            lhs = jnp.concatenate(
                [jnp.concatenate([mem, hac[8:16]], axis=0).astype(BF16), hd], axis=0)

            def store1(c, y):
                ring[wr[1], c * 8:(c + 1) * 8, :] = _pack(
                    jnp.concatenate([tok_a[c], y[0:8]], axis=0))
                ring[wr[2], c * 8:(c + 1) * 8, :] = _pack(y[8:24])

            def wo_lhs1(h, om, ot):
                return jnp.concatenate([om, deferred[h], ot], axis=0)

            hnext[...] = h_rows(LEAD + 48 * jnp.minimum(j + 1, NPAIR - 1), 48)
            gs = p2_front(64)
            gbuf[:, 0:24, :] = gbuf[:, 64:88, :]
            hs = []

            def p2_fin():
                p2_back(x2, h2, jnp.concatenate(hs, axis=1), 64 * j, 64)
                x2t[...] = x2[48:64]
                h2t[...] = h2[48:64]

            th = half_dots(gs, w2v, lambda y, c: hs.append(y))
            extras = {i: [th[i]] for i in range(16)}
            extras[15].append(p2_fin)
            out = segment(lhs, ro1, store1, wo_lhs1, extras)
            aout[24:64, :] = out[8:48]
            return out[0:8]

        if "A" in phases:
            with scope("aloop"):
                lax.fori_loop(0, NPAIR, a_body, memv[...].astype(F32))
        else:
            zv[...] = jnp.zeros(zv.shape, F32)
            ttv[...] = jnp.zeros(ttv.shape, U32)

        x2, h2, u = p1_front(S - 64)
        y = _dot(u, _cols(w1v, 0, 8))
        for c in range(8):
            p1_store(y[:, c * 128:(c + 1) * 128], c, None)
        p2_back(x2, h2, _dot(p2_front(80), _cols(w2v, 0, 8)), S, 80)

        wait(w34_cps)

        def out_cp(i, slot):
            return cp(outv.at[slot], out_hbm.at[pl.ds(i * RB, RB), :],
                      SEM_OUT + slot)

        def p3_body(i, _):
            slot = i % 2

            @pl.when(i >= 2)
            def _():
                out_cp(i - 2, slot).wait()

            r0 = HALO + i * RB
            tt = _unpack(ttv[pl.ds(pl.multiple_of(r0 // 2, 8), RB // 2), :])
            ff = jnp.concatenate(
                [_gelu(_dot(tt, _cols(w3v, 4 * q, 4 * q + 4))).astype(BF16)
                 for q in range(FF // 512)], axis=1)
            y = _dot(ff, _cols(w4v, 0, 8))
            res = zv[pl.ds(pl.multiple_of(r0, 16), RB), :] + mod_row(5) * y
            outv[slot] = res.astype(BF16)
            out_cp(i, slot).start()
            return 0

        nb = S // RB
        if "B" in phases:
            with scope("p3"):
                lax.fori_loop(0, nb, p3_body, 0)
            out_cp(nb - 2, 0).wait()
            out_cp(nb - 1, 1).wait()
        else:
            outv[0] = zv[pl.ds(HALO, RB), :].astype(BF16)
            out_cp(0, 0).start()
            out_cp(0, 0).wait()

    pl.run_scoped(
        main,
        pltpu.VMEM((FF // 128, D // 2, 128), U32),
        pltpu.VMEM((8, FF // 2, 128), U32),
        pltpu.VMEM((S + HALO, D), F32),
        pltpu.VMEM(((S + HALO) // 2, D), U32),
    )


def _call(A_x, A_mem0, A_Wq, A_Wk, A_Wv, A_Wo, B_w1, B_w2, B_w3, B_w4, c, w_mod,
          phases="AB"):
    any_spec = pl.BlockSpec(memory_space=pl.ANY)
    scratch = [
        pltpu.VMEM((S, D), BF16),
        pltpu.VMEM((1, D), BF16),
        pltpu.VMEM((M, D), BF16),
        pltpu.VMEM((48, D // 2, 128), U32),
        pltpu.VMEM((6, 8, D), F32),
        pltpu.VMEM((3 * H // 2 * SL, E), U32),
        pltpu.VMEM((3 * H // 2 * SL, E), U32),
        pltpu.VMEM((8, H * E // 2, 128), U32),
        pltpu.VMEM((8, D // 2, 128), U32),
        pltpu.VMEM((8, D // 2, 128), U32),
        pltpu.VMEM((LEAD // 2, D), U32),
        pltpu.VMEM((24, D), U32),
        pltpu.VMEM((24, D), U32),
        pltpu.VMEM((RING, 3 * H * 8, E), U32),
        pltpu.VMEM((80, 80), F32),
        pltpu.VMEM((64, D), F32),
        pltpu.VMEM((8, 96, 128), F32),
        pltpu.VMEM((16, D), F32),
        pltpu.VMEM((16, D), F32),
        pltpu.VMEM((2, RB, D), BF16),
        pltpu.SemaphoreType.DMA((NSEM,)),
    ]
    out = pl.pallas_call(
        functools.partial(_kernel, phases=phases),
        in_specs=[any_spec] * 12,
        out_specs=any_spec,
        out_shape=jax.ShapeDtypeStruct((S, D), BF16),
        scratch_shapes=scratch,
        compiler_params=pltpu.CompilerParams(
            vmem_limit_bytes=126 * 1024 * 1024),
    )(A_x.reshape(S, D), A_mem0.reshape(M, D), A_Wq, A_Wk, A_Wv,
      A_Wo.reshape(H * E, D), B_w1, B_w2, B_w3, B_w4, c, w_mod)
    return out.reshape(1, S, D)


def pallas_adaLN_cond__memory_aug_recurrent_mem_tr__mixer_s_mlp__prompt_kernel(
    A_x, A_mem0, A_Wq, A_Wk, A_Wv, A_Wo, A_seg_len, B_x, B_w1, B_w2, B_w3, B_w4,
    c, w_mod,
):
    assert A_seg_len == SEG
    del B_x
    return _call(A_x, A_mem0, A_Wq, A_Wk, A_Wv, A_Wo, B_w1, B_w2, B_w3, B_w4,
                 c, w_mod)
```

```python
import contextlib
import functools

import jax
import jax.numpy as jnp
from jax import lax
import jax.experimental.pallas as pl
import jax.experimental.pallas.tpu as pltpu

F32 = jnp.float32
BF16 = jnp.bfloat16
U32 = jnp.uint32

S = 2048
D = 1024
H = 32
E = 128
M = 8
SEG = 32
FF = 3584
EPS = 1e-5

LEAD = 512
RING = 36
SL = 520
HG = 16
NG = 3 * H // HG
NPAIR = S // (2 * SEG)
HALO = 80
RB = 256
SHIFTS = (-1, -1, 1, 1, -2, -2, 2, 2)

(SEM_X0, SEM_X1, SEM_C, SEM_MEM, SEM_WO, SEM_W1, SEM_W2, SEM_W3,
 SEM_W4) = range(9)
SEM_Q = 9
SEM_Q1 = 13
SEM_ST = 17
SEM_MOD = SEM_ST + NG
SEM_OUT = SEM_MOD + 6
NSEM = SEM_OUT + 2


def _ln(x):
    mu = jnp.mean(x, axis=-1, keepdims=True)
    xc = x - mu
    var = jnp.mean(xc * xc, axis=-1, keepdims=True)
    return xc * lax.rsqrt(var + EPS)


def _gelu(x):
    return jax.nn.gelu(x, approximate=True)


def _pack(x):
    return pltpu.bitcast(x.astype(BF16), U32)


def _unpack(x):
    return pltpu.bitcast(x, BF16)


def _dot(a, b):
    return jnp.dot(a, b, preferred_element_type=F32)


def _cols(ref, lo, hi, k0=0, k1=None):
    k1 = 2 * ref.shape[1] if k1 is None else k1
    return jnp.concatenate(
        [_unpack(ref[c, k0 // 2:k1 // 2, :]) for c in range(lo, hi)], axis=1)


def _kernel(x_hbm, mem_hbm, wq_hbm, wk_hbm, wv_hbm, wo_hbm, w1_hbm, w2_hbm,
            w3_hbm, w4_hbm, c_hbm, wmod_hbm, out_hbm,
            xv, scv, memv, wmodv, modv, wqa, wqb, wov, w1v, w2v,
            hv0, hcur, hnext, ring, aout, gbuf, x2t, h2t, outv, fillv, cv, sems, *, phases):
    def scope(name):
        return jax.named_scope(name) if "s" in phases else contextlib.nullcontext()

    def cp(src, dst, s):
        return pltpu.make_async_copy(src, dst, sems.at[s])

    def col_copies(w_hbm, w_v, s, lo=0, hi=None):
        w32 = w_hbm.bitcast(U32)
        hi = w_v.shape[0] if hi is None else hi
        return [cp(w32.at[:, pl.ds(c * 128, 128)], w_v.at[c], s)
                for c in range(lo, hi)]

    def start(cps):
        for q in cps:
            q.start()

    def wait(cps):
        for q in cps:
            q.wait()

    c_cp = cp(c_hbm, cv, SEM_C)
    mem_cp = cp(mem_hbm, memv, SEM_MEM)
    x0_cp = cp(x_hbm.at[pl.ds(0, LEAD)], xv.at[pl.ds(0, LEAD)], SEM_X0)
    x1_cp = cp(x_hbm.at[pl.ds(LEAD, S - LEAD)], xv.at[pl.ds(LEAD, S - LEAD)],
               SEM_X1)
    wo_cps = col_copies(wo_hbm, wov, SEM_WO)
    w1_cps = col_copies(w1_hbm, w1v, SEM_W1)
    w2_cps = col_copies(w2_hbm, w2v, SEM_W2)

    def mod_row(i):
        return jnp.concatenate([modv[8 * i + c, 0:1, :] for c in range(8)], axis=1)

    def mod_tiles(tiles):
        w = jnp.concatenate([_unpack(wmodv[c]) for c in tiles], axis=1)
        y = _dot(_unpack(scv[...]), w)[0:8]
        for u, c in enumerate(tiles):
            modv[c] = y[:, u * 128:(u + 1) * 128]
        return y[0:1]

    wq2 = (wqa, wqb)

    def h_rows(r0, n):
        xf = xv[pl.ds(pl.multiple_of(r0, 16), n), :].astype(F32)
        return _pack(_ln(xf) * (1.0 + mod_row(1)) + mod_row(0))

    def prologue(st, xn, acc):
        w_hbms = (wq_hbm, wk_hbm, wv_hbm)

        def st_src(i):
            return w_hbms[i // 2].bitcast(U32).at[:, pl.ds((i % 2) * 8, 8), :]

        def st_quarter(i, q, s):
            return cp(st_src(i).at[pl.ds(q * 256, 256)],
                      st.at[i, pl.ds(q * 256, 256)], s)

        def q_cps(q):
            w32 = wmod_hbm.bitcast(U32)
            return [cp(w32.at[:, pl.ds(pl.multiple_of(c * 128, 128), 128)],
                       wmodv.at[c], SEM_Q + q)
                    for c in (2 * q, 2 * q + 1, 8 + 2 * q, 9 + 2 * q)
                    ] + [st_quarter(0, q, SEM_Q + q)]

        def st_cp(i):
            return cp(st_src(i), st.at[i], SEM_ST + i)

        def mod_cps(i):
            return col_copies(wmod_hbm, wmodv, SEM_MOD + i, 8 * i, 8 * i + 8)

        with scope("first"):
            start([c_cp, mem_cp, x0_cp])
        for q in range(4):
            start(q_cps(q))
        start([st_quarter(1, q, SEM_Q1 + q) for q in range(4)])
        start([st_cp(2), st_cp(3)] + mod_cps(2) + [st_cp(4)] + mod_cps(3)
              + [st_cp(5)])

        r = lax.broadcasted_iota(jnp.int32, (80, 80), 0)
        k = lax.broadcasted_iota(jnp.int32, (80, 80), 1)

        def head_of(i):
            return jnp.where(i < 16, i // 8, (i - 16) // 32)

        def pos_of(i):
            return jnp.where(i < 16, i % 8, 8 + (i - 16) % 32)

        same = head_of(r) == head_of(k)
        vis = (pos_of(r) < M) | (pos_of(r) >= pos_of(k))
        fillv[...] = jnp.where(same, jnp.where(vis, 0.0, -1e9), -jnp.inf).astype(F32)
        aout[...] = jnp.zeros(aout.shape, F32)
        gbuf[...] = jnp.zeros(gbuf.shape, F32)
        x2t[...] = jnp.zeros(x2t.shape, F32)
        h2t[...] = jnp.zeros(h2t.shape, F32)

        c_cp.wait()
        cf = cv[...].astype(F32)
        scv[...] = _pack(jnp.broadcast_to(cf * jax.nn.sigmoid(cf), (16, D)))
        x0_cp.wait()

        def ln_body(i, _):
            r0 = pl.multiple_of(i * 64, 64)
            y = _ln(xv[pl.ds(r0, 64), :].astype(F32))
            for q in range(4):
                xn[q, pl.ds(r0, 64), :] = y[:, q * 256:(q + 1) * 256]
            return 0

        lax.fori_loop(0, LEAD // 64, ln_body, 0)

        def relayout(par, g, p0, n):
            base = g * (8 * SL)
            for u in range(n):
                a = st[g, 2 * (p0 + u)]
                b = st[g, 2 * (p0 + u) + 1]
                if par == 0:
                    w = (a & jnp.uint32(0xFFFF)) | (b << 16)
                else:
                    w = (a >> 16) | (b & jnp.uint32(0xFFFF0000))
                wq2[par][pl.ds(base + p0 + u, 8, stride=SL), :] = w

        def to_ring(y, par, s0, rc):
            for u in range(4):
                row = pl.multiple_of((2 * (s0 + u) + par) * 8, 8)
                for b in range(16):
                    ring[rc * 16 + b, pl.ds(row, 8), :] = (
                        y[b * 8:(b + 1) * 8, u * 128:(u + 1) * 128])

        def q_body(q, _):
            wait(q_cps(q))
            m = mod_tiles([2 * q, 2 * q + 1, 8 + 2 * q, 9 + 2 * q])
            hv0[q] = _pack(xn[q] * (1.0 + m[:, 256:512]) + m[:, 0:256])
            relayout(0, 0, q * 128, 128)
            relayout(1, 0, q * 128, 128)

            def rc_body(rc, _):
                lhs = _unpack(hv0[q, pl.ds(pl.multiple_of(rc * 128, 128), 128), :])
                for part in range(4):
                    par, hq = part // 2, part % 2
                    w = jnp.concatenate(
                        [_unpack(wq2[par][pl.ds(pl.multiple_of(
                            (hq * 4 + u) * SL + q * 128, 8), 128), :])
                         for u in range(4)], axis=1)
                    y = _dot(lhs, w) + jnp.where(q > 0, acc[rc * 4 + part], 0.0)
                    acc[rc * 4 + part] = y
                    to_ring(_pack(y), par, hq * 4, rc)
                return 0

            lax.fori_loop(0, 2, rc_body, 0)
            return 0

        with scope("quarters"):
            lax.fori_loop(0, 4, q_body, 0)

        start(mod_cps(4) + mod_cps(5) + wo_cps + w1_cps + w2_cps + [x1_cp])

        for q in range(4):
            st_quarter(1, q, SEM_Q1 + q).wait()

            def rl_body(i, _, q=q):
                relayout(0, 1, q * 128 + i * 32, 32)
                return 0

            lax.fori_loop(0, 4, rl_body, 0)

        def lead_proj(par, g, hq, rc):
            s0 = g * 8 + hq * 4
            w = jnp.concatenate(
                [_unpack(wq2[par][pl.ds(pl.multiple_of((s0 + u) * SL, 8), 512), :])
                 for u in range(4)], axis=1)
            lhs = jnp.concatenate(
                [_unpack(hv0[q, rc * 128:(rc + 1) * 128, :]) for q in range(4)],
                axis=1)
            to_ring(_pack(_dot(lhs, w)), par, s0, rc)

        def group_body(g, _):
            for part in range(4):
                lead_proj(0, g, part // 2, part % 2)
                relayout(1, g, part * 128, 128)

            @pl.when(g < NG - 1)
            def _():
                cp(st_src(1), st.at[g + 1], SEM_ST + g + 1).wait()

            @pl.when(g >= 2)
            def _():
                part_g = wmodv.at[pl.ds(8 * g, 8)]
                cp(part_g, part_g, SEM_MOD + g).wait()

            gn = jnp.minimum(g + 1, NG - 1)
            for part in range(4):
                lead_proj(1, g, part // 2, part % 2)
                relayout(0, gn, part * 128, 128)
                mod_tiles([8 * g + 2 * part, 8 * g + 2 * part + 1])
            return 0

        with scope("groups"):
            lax.fori_loop(1, NG, group_body, 0)

    pl.run_scoped(
        prologue,
        pltpu.VMEM((NG, D, 8, E), U32),
        pltpu.VMEM((4, LEAD, 256), F32),
        pltpu.VMEM((8, 256, 512), F32),
    )

    def main(w3v, w4v, zv, ttv):
        w34_cps = col_copies(w3_hbm, w3v, SEM_W3) + col_copies(w4_hbm, w4v, SEM_W4)
        start(w34_cps)
        wait(wo_cps + w1_cps + w2_cps + [mem_cp, x1_cp])
        hnext[...] = h_rows(LEAD, 48)

        scale = float(E) ** -0.5

        def segment(lhs, ro, store_tok, wo_lhs, extras):
            fill = fillv[...]
            keep = fill == 0.0
            NP = H // 2
            qkv, probs, blocks = {}, {}, []

            def proj(hp):
                slots = [t * H + 2 * hp + par for t in range(3) for par in range(2)]
                w = jnp.concatenate(
                    [_unpack(wq2[sl % 2][pl.ds((sl // 2) * SL, 512), :])
                     for sl in slots], axis=1)
                if hp == 0:
                    y = _dot(lhs[:, :512], w[:512])
                    y = _dot(lhs[:, 512:], w[512:]) + y
                else:
                    y = _dot(lhs, w)
                for u, sl in enumerate(slots):
                    store_tok(sl, y[8:32, u * 128:(u + 1) * 128])
                ops = []
                for t in range(3):
                    ym = jnp.concatenate(
                        [y[0:8, (2 * t) * 128:(2 * t + 1) * 128],
                         y[0:8, (2 * t + 1) * 128:(2 * t + 2) * 128]], axis=0)
                    ops.append(jnp.concatenate(
                        [ym.astype(BF16)]
                        + [_unpack(ring[ro + b, sl * 8:(sl + 1) * 8, :])
                           for sl in slots[2 * t:2 * t + 2] for b in range(2)],
                        axis=0))
                qkv[hp] = ops

            def scores(hp):
                q, kk, _ = qkv[hp]
                s = lax.dot_general(q, kk, (((1,), (1,)), ((), ())),
                                    preferred_element_type=F32)
                s = jnp.where(keep, s * scale, fill)
                mx = jnp.max(s, axis=-1, keepdims=True)
                p = jnp.exp(s - mx)
                l = jnp.sum(p, axis=-1, keepdims=True)
                rl = pl.reciprocal(l, approx=True)
                rl = rl * (2.0 - l * rl)
                probs[hp] = (p * rl).astype(BF16)

            def pv(hp):
                o = _dot(probs[hp], qkv[hp][2])
                blocks.append(wo_lhs(2 * hp, o[0:8], o[16:48]).astype(BF16))
                blocks.append(wo_lhs(2 * hp + 1, o[8:16], o[48:80]).astype(BF16))

            def wo_part(h0, h1, acc=None):
                lw = jnp.concatenate(blocks[h0:h1], axis=1)
                y = _dot(lw, _cols(wov, 0, 8, E * h0, E * h1))
                return y if acc is None else y + acc

            for i in range(NP):
                proj(i)
                if i >= 1:
                    scores(i - 1)
                if i >= 3:
                    pv(i - 3)
                for thunk in extras.get(i, ()):
                    thunk()
            acc = wo_part(0, 4)
            scores(NP - 1)
            pv(NP - 3)
            acc = wo_part(4, 12, acc)
            pv(NP - 2)
            pv(NP - 1)
            acc = wo_part(12, 24, acc)
            acc = wo_part(24, 32, acc)
            return acc

        def p1_front(r0):
            x2 = (xv[pl.ds(pl.multiple_of(r0, 64), 64), :].astype(F32)
                  + mod_row(2) * aout[...])
            h2 = _ln(x2) * (1.0 + mod_row(4)) + mod_row(3)
            return x2, h2, _ln(h2).astype(BF16)

        def p1_store(y, c, live):
            g = _gelu(y)
            if live is not None:
                g = jnp.where(live, g, 0.0)
            gbuf[c, 24:88, :] = g

        def half_dots(lhs, wv, done):
            part = {}

            def run(c, kh):
                y = _dot(lhs[:, kh * 512:(kh + 1) * 512],
                         _cols(wv, c, c + 1, kh * 512, (kh + 1) * 512))
                if kh == 0:
                    part[c] = y
                else:
                    done(y + part[c], c)

            return [functools.partial(run, c, kh) for c in range(8) for kh in range(2)]

        def p2_front(n):
            return jnp.concatenate(
                [gbuf[c, 8 + SHIFTS[c]:8 + SHIFTS[c] + n, :] for c in range(8)],
                axis=1).astype(BF16)

        def p2_back(x2, h2, hs, row, n):
            x1 = jnp.concatenate([h2t[...], h2[0:n - 16]], axis=0) + hs
            x2w = jnp.concatenate([x2t[...], x2[0:n - 16]], axis=0)
            zv[pl.ds(pl.multiple_of(row, 16), n), :] = x2w + mod_row(5) * x1
            ttv[pl.ds(pl.multiple_of(row // 2, 8), n // 2), :] = _pack(_ln(x1))

        def a_body(j, mem):
            hcur[...] = hnext[...]
            hb = _unpack(hcur[0:8, :])
            hac = _unpack(hcur[8:16, :]).astype(F32)
            hd = _unpack(hcur[16:24, :])
            wr = [lax.rem(LEAD // 16 + 3 * j + i, RING) for i in range(3)]
            ro0 = lax.rem(4 * j, RING)
            ro1 = ro0 + 2

            x2, h2, u = p1_front(64 * jnp.maximum(j - 1, 0))
            live = j > 0

            lhs = jnp.concatenate(
                [jnp.concatenate([mem, hac[0:8]], axis=0).astype(BF16), hb], axis=0)
            tok_a = {}

            def store0(c, y):
                tok_a[c] = y[0:8]
                ring[wr[0], c * 8:(c + 1) * 8, :] = _pack(y[8:24])

            deferred = {}

            def wo_lhs0(h, om, ot):
                deferred[h] = ot[24:32]
                return jnp.concatenate([om, ot[0:24]], axis=0)

            th = half_dots(u, w1v, lambda y, c: p1_store(y, c, live))
            extras = {i: [th[i - 2]] for i in range(2, 14)}
            extras[14] = th[12:14]
            extras[15] = th[14:16]
            out = segment(lhs, ro0, store0, wo_lhs0, extras)
            mem = out[0:8]
            aout[0:24, :] = out[8:32]

            lhs = jnp.concatenate(
                [jnp.concatenate([mem, hac[8:16]], axis=0).astype(BF16), hd], axis=0)

            def store1(c, y):
                ring[wr[1], c * 8:(c + 1) * 8, :] = _pack(
                    jnp.concatenate([tok_a[c], y[0:8]], axis=0))
                ring[wr[2], c * 8:(c + 1) * 8, :] = _pack(y[8:24])

            def wo_lhs1(h, om, ot):
                return jnp.concatenate([om, deferred[h], ot], axis=0)

            hnext[...] = h_rows(LEAD + 48 * jnp.minimum(j + 1, NPAIR - 1), 48)
            gs = p2_front(64)
            gbuf[:, 0:24, :] = gbuf[:, 64:88, :]
            hs = []

            def p2_fin():
                p2_back(x2, h2, jnp.concatenate(hs, axis=1), 64 * j, 64)
                x2t[...] = x2[48:64]
                h2t[...] = h2[48:64]

            th = half_dots(gs, w2v, lambda y, c: hs.append(y))
            extras = {i: [th[i]] for i in range(16)}
            extras[15].append(p2_fin)
            out = segment(lhs, ro1, store1, wo_lhs1, extras)
            aout[24:64, :] = out[8:48]
            return out[0:8]

        if "A" in phases:
            with scope("aloop"):
                lax.fori_loop(0, NPAIR, a_body, memv[...].astype(F32))
        else:
            zv[...] = jnp.zeros(zv.shape, F32)
            ttv[...] = jnp.zeros(ttv.shape, U32)

        x2, h2, u = p1_front(S - 64)
        y = _dot(u, _cols(w1v, 0, 8))
        for c in range(8):
            p1_store(y[:, c * 128:(c + 1) * 128], c, None)
        p2_back(x2, h2, _dot(p2_front(80), _cols(w2v, 0, 8)), S, 80)

        wait(w34_cps)

        def out_cp(i, slot):
            return cp(outv.at[slot], out_hbm.at[pl.ds(i * RB, RB), :],
                      SEM_OUT + slot)

        def p3_body(i, _):
            slot = i % 2

            @pl.when(i >= 2)
            def _():
                out_cp(i - 2, slot).wait()

            r0 = HALO + i * RB
            tt = _unpack(ttv[pl.ds(pl.multiple_of(r0 // 2, 8), RB // 2), :])
            ff = jnp.concatenate(
                [_gelu(_dot(tt, _cols(w3v, 4 * q, 4 * q + 4))).astype(BF16)
                 for q in range(FF // 512)], axis=1)
            y = _dot(ff, _cols(w4v, 0, 8))
            res = zv[pl.ds(pl.multiple_of(r0, 16), RB), :] + mod_row(5) * y
            outv[slot] = res.astype(BF16)
            out_cp(i, slot).start()
            return 0

        nb = S // RB
        if "B" in phases:
            with scope("p3"):
                lax.fori_loop(0, nb, p3_body, 0)
            out_cp(nb - 2, 0).wait()
            out_cp(nb - 1, 1).wait()
        else:
            outv[0] = zv[pl.ds(HALO, RB), :].astype(BF16)
            out_cp(0, 0).start()
            out_cp(0, 0).wait()

    pl.run_scoped(
        main,
        pltpu.VMEM((FF // 128, D // 2, 128), U32),
        pltpu.VMEM((8, FF // 2, 128), U32),
        pltpu.VMEM((S + HALO, D), F32),
        pltpu.VMEM(((S + HALO) // 2, D), U32),
    )


def _call(A_x, A_mem0, A_Wq, A_Wk, A_Wv, A_Wo, B_w1, B_w2, B_w3, B_w4, c, w_mod,
          phases="AB"):
    any_spec = pl.BlockSpec(memory_space=pl.ANY)
    scratch = [
        pltpu.VMEM((S, D), BF16),
        pltpu.VMEM((8, D), U32),
        pltpu.VMEM((M, D), BF16),
        pltpu.VMEM((48, D // 2, 128), U32),
        pltpu.VMEM((48, 8, 128), F32),
        pltpu.VMEM((3 * H // 2 * SL, E), U32),
        pltpu.VMEM((3 * H // 2 * SL, E), U32),
        pltpu.VMEM((8, H * E // 2, 128), U32),
        pltpu.VMEM((8, D // 2, 128), U32),
        pltpu.VMEM((8, D // 2, 128), U32),
        pltpu.VMEM((4, LEAD // 2, 256), U32),
        pltpu.VMEM((24, D), U32),
        pltpu.VMEM((24, D), U32),
        pltpu.VMEM((RING, 3 * H * 8, E), U32),
        pltpu.VMEM((64, D), F32),
        pltpu.VMEM((8, 96, 128), F32),
        pltpu.VMEM((16, D), F32),
        pltpu.VMEM((16, D), F32),
        pltpu.VMEM((2, RB, D), BF16),
        pltpu.VMEM((80, 80), F32),
        pltpu.VMEM((1, D), BF16),
        pltpu.SemaphoreType.DMA((NSEM,)),
    ]
    out = pl.pallas_call(
        functools.partial(_kernel, phases=phases),
        in_specs=[any_spec] * 12,
        out_specs=any_spec,
        out_shape=jax.ShapeDtypeStruct((S, D), BF16),
        scratch_shapes=scratch,
        compiler_params=pltpu.CompilerParams(
            vmem_limit_bytes=126 * 1024 * 1024),
    )(A_x.reshape(S, D), A_mem0.reshape(M, D), A_Wq, A_Wk, A_Wv,
      A_Wo.reshape(H * E, D), B_w1, B_w2, B_w3, B_w4, c, w_mod)
    return out.reshape(1, S, D)


def pallas_adaLN_cond__memory_aug_recurrent_mem_tr__mixer_s_mlp__prompt_kernel(
    A_x, A_mem0, A_Wq, A_Wk, A_Wv, A_Wo, A_seg_len, B_x, B_w1, B_w2, B_w3, B_w4,
    c, w_mod,
):
    assert A_seg_len == SEG
    del B_x
    return _call(A_x, A_mem0, A_Wq, A_Wk, A_Wv, A_Wo, B_w1, B_w2, B_w3, B_w4,
                 c, w_mod)
```

```python
import contextlib
import functools

import jax
import jax.numpy as jnp
from jax import lax
import jax.experimental.pallas as pl
import jax.experimental.pallas.tpu as pltpu

F32 = jnp.float32
BF16 = jnp.bfloat16
U32 = jnp.uint32

S = 2048
D = 1024
H = 32
E = 128
M = 8
SEG = 32
FF = 3584
EPS = 1e-5

LEAD = 512
RING = 36
SL = 520
HG = 16
NG = 3 * H // HG
NPAIR = S // (2 * SEG)
HALO = 80
RB = 256
SHIFTS = (-1, -1, 1, 1, -2, -2, 2, 2)

(SEM_X0, SEM_X1, SEM_C, SEM_MEM, SEM_WO, SEM_W1, SEM_W2, SEM_W3,
 SEM_W4) = range(9)
SEM_Q = 9
SEM_Q1 = 13
SEM_ST = 17
SEM_MOD = SEM_ST + NG
SEM_OUT = SEM_MOD + 6
NSEM = SEM_OUT + 2


def _ln(x):
    mu = jnp.mean(x, axis=-1, keepdims=True)
    xc = x - mu
    var = jnp.mean(xc * xc, axis=-1, keepdims=True)
    return xc * lax.rsqrt(var + EPS)


def _gelu(x):
    return jax.nn.gelu(x, approximate=True)


def _pack(x):
    return pltpu.bitcast(x.astype(BF16), U32)


def _unpack(x):
    return pltpu.bitcast(x, BF16)


def _dot(a, b):
    return jnp.dot(a, b, preferred_element_type=F32)


def _cols(ref, lo, hi, k0=0, k1=None):
    k1 = 2 * ref.shape[1] if k1 is None else k1
    return jnp.concatenate(
        [_unpack(ref[c, k0 // 2:k1 // 2, :]) for c in range(lo, hi)], axis=1)


def _kernel(x_hbm, mem_hbm, wq_hbm, wk_hbm, wv_hbm, wo_hbm, w1_hbm, w2_hbm,
            w3_hbm, w4_hbm, c_hbm, wmod_hbm, out_hbm,
            xv, scv, memv, wmodv, modv, wqa, wqb, wov, w1v, w2v,
            hv0, hcur, ring, aout, gbuf, x2t, h2t, outv, fillv, cv, sems, *, phases):
    def scope(name):
        return jax.named_scope(name) if "s" in phases else contextlib.nullcontext()

    def cp(src, dst, s):
        return pltpu.make_async_copy(src, dst, sems.at[s])

    def col_copies(w_hbm, w_v, s, lo=0, hi=None):
        w32 = w_hbm.bitcast(U32)
        hi = w_v.shape[0] if hi is None else hi
        return [cp(w32.at[:, pl.ds(c * 128, 128)], w_v.at[c], s)
                for c in range(lo, hi)]

    def start(cps):
        for q in cps:
            q.start()

    def wait(cps):
        for q in cps:
            q.wait()

    c_cp = cp(c_hbm, cv, SEM_C)
    mem_cp = cp(mem_hbm, memv, SEM_MEM)
    x0_cp = cp(x_hbm.at[pl.ds(0, LEAD)], xv.at[pl.ds(0, LEAD)], SEM_X0)
    x1_cp = cp(x_hbm.at[pl.ds(LEAD, S - LEAD)], xv.at[pl.ds(LEAD, S - LEAD)],
               SEM_X1)
    wo_cps = col_copies(wo_hbm, wov, SEM_WO)
    w1_cps = col_copies(w1_hbm, w1v, SEM_W1)
    w2_cps = col_copies(w2_hbm, w2v, SEM_W2)

    def mod_rows(i, n):
        m = jnp.concatenate([modv[8 * i + c] for c in range(8)], axis=1)
        return jnp.concatenate([m] * (n // 8), axis=0)

    def mod_tiles(tiles, offs):
        w = jnp.concatenate([_unpack(wmodv[c]) for c in tiles], axis=1)
        y = _dot(_unpack(scv[...]), w)[0:8]
        ys = [y[:, u * 128:(u + 1) * 128] + o for u, o in enumerate(offs)]
        for c, v in zip(tiles, ys):
            modv[c] = v
        return ys

    wq2 = (wqa, wqb)

    def h_rows(r0, n):
        xf = xv[pl.ds(pl.multiple_of(r0, 16), n), :].astype(F32)
        return _pack(_ln(xf) * mod_rows(1, n) + mod_rows(0, n))

    def prologue(st, xn, acc):
        w_hbms = (wq_hbm, wk_hbm, wv_hbm)

        def st_src(i):
            return w_hbms[i // 2].bitcast(U32).at[:, pl.ds((i % 2) * 8, 8), :]

        def st_quarter(i, q, s):
            return cp(st_src(i).at[pl.ds(q * 256, 256)],
                      st.at[i, pl.ds(q * 256, 256)], s)

        def q_cps(q):
            w32 = wmod_hbm.bitcast(U32)
            return [cp(w32.at[:, pl.ds(pl.multiple_of(c * 128, 128), 128)],
                       wmodv.at[c], SEM_Q + q)
                    for c in (2 * q, 2 * q + 1, 8 + 2 * q, 9 + 2 * q)
                    ] + [st_quarter(0, q, SEM_Q + q)]

        def st_cp(i):
            return cp(st_src(i), st.at[i], SEM_ST + i)

        def mod_cps(i):
            return col_copies(wmod_hbm, wmodv, SEM_MOD + i, 8 * i, 8 * i + 8)

        with scope("first"):
            start([c_cp, mem_cp, x0_cp])
        for q in range(4):
            start(q_cps(q))
        start([st_quarter(1, q, SEM_Q1 + q) for q in range(4)])
        start([st_cp(2), st_cp(3)] + mod_cps(2) + [st_cp(4)] + mod_cps(3)
              + [st_cp(5)])

        r = lax.broadcasted_iota(jnp.int32, (80, 80), 0)
        k = lax.broadcasted_iota(jnp.int32, (80, 80), 1)

        def head_of(i):
            return jnp.where(i < 16, i // 8, (i - 16) // 32)

        def pos_of(i):
            return jnp.where(i < 16, i % 8, 8 + (i - 16) % 32)

        same = head_of(r) == head_of(k)
        vis = (pos_of(r) < M) | (pos_of(r) >= pos_of(k))
        fillv[...] = jnp.where(same, jnp.where(vis, 0.0, -1e9), -jnp.inf).astype(F32)
        aout[...] = jnp.zeros(aout.shape, F32)
        gbuf[...] = jnp.zeros(gbuf.shape, F32)
        x2t[...] = jnp.zeros(x2t.shape, F32)
        h2t[...] = jnp.zeros(h2t.shape, F32)

        c_cp.wait()
        cf = cv[...].astype(F32)
        scv[...] = _pack(jnp.broadcast_to(cf * jax.nn.sigmoid(cf), (16, D)))
        x0_cp.wait()

        def ln_body(i, _):
            r0 = pl.multiple_of(i * 64, 64)
            y = _ln(xv[pl.ds(r0, 64), :].astype(F32))
            for q in range(4):
                xn[q, pl.ds(r0, 64), :] = y[:, q * 256:(q + 1) * 256]
            return 0

        lax.fori_loop(0, LEAD // 64, ln_body, 0)

        def relayout(par, g, p0, n):
            base = g * (8 * SL)
            for u in range(n):
                a = st[g, 2 * (p0 + u)]
                b = st[g, 2 * (p0 + u) + 1]
                if par == 0:
                    w = (a & jnp.uint32(0xFFFF)) | (b << 16)
                else:
                    w = (a >> 16) | (b & jnp.uint32(0xFFFF0000))
                wq2[par][pl.ds(base + p0 + u, 8, stride=SL), :] = w

        def to_ring(y, par, s0, rc):
            for u in range(4):
                row = pl.multiple_of((2 * (s0 + u) + par) * 8, 8)
                for b in range(16):
                    ring[rc * 16 + b, pl.ds(row, 8), :] = (
                        y[b * 8:(b + 1) * 8, u * 128:(u + 1) * 128])

        def q_body(q, _):
            wait(q_cps(q))
            m = mod_tiles([2 * q, 2 * q + 1, 8 + 2 * q, 9 + 2 * q], [0.0, 0.0, 1.0, 1.0])
            sa, ca = [jnp.concatenate([jnp.concatenate(v, axis=1)] * (LEAD // 8), axis=0)
                      for v in (m[0:2], m[2:4])]
            hv0[q] = _pack(xn[q] * ca + sa)
            relayout(0, 0, q * 128, 128)
            relayout(1, 0, q * 128, 128)

            def rc_body(rc, _):
                lhs = _unpack(hv0[q, pl.ds(pl.multiple_of(rc * 128, 128), 128), :])
                for part in range(4):
                    par, hq = part // 2, part % 2
                    w = jnp.concatenate(
                        [_unpack(wq2[par][pl.ds(pl.multiple_of(
                            (hq * 4 + u) * SL + q * 128, 8), 128), :])
                         for u in range(4)], axis=1)
                    y = _dot(lhs, w) + jnp.where(q > 0, acc[rc * 4 + part], 0.0)
                    acc[rc * 4 + part] = y
                    to_ring(_pack(y), par, hq * 4, rc)
                return 0

            lax.fori_loop(0, 2, rc_body, 0)
            return 0

        with scope("quarters"):
            lax.fori_loop(0, 4, q_body, 0)

        start(mod_cps(4) + mod_cps(5) + wo_cps + w1_cps + w2_cps + [x1_cp])

        for q in range(4):
            st_quarter(1, q, SEM_Q1 + q).wait()

            def rl_body(i, _, q=q):
                relayout(0, 1, q * 128 + i * 32, 32)
                return 0

            lax.fori_loop(0, 4, rl_body, 0)

        def lead_proj(par, g, hq, rc):
            s0 = g * 8 + hq * 4
            w = jnp.concatenate(
                [_unpack(wq2[par][pl.ds(pl.multiple_of((s0 + u) * SL, 8), 512), :])
                 for u in range(4)], axis=1)
            lhs = jnp.concatenate(
                [_unpack(hv0[q, rc * 128:(rc + 1) * 128, :]) for q in range(4)],
                axis=1)
            to_ring(_pack(_dot(lhs, w)), par, s0, rc)

        def group_body(g, _):
            for part in range(4):
                lead_proj(0, g, part // 2, part % 2)
                relayout(1, g, part * 128, 128)

            @pl.when(g < NG - 1)
            def _():
                cp(st_src(1), st.at[g + 1], SEM_ST + g + 1).wait()

            @pl.when(g >= 2)
            def _():
                part_g = wmodv.at[pl.ds(8 * g, 8)]
                cp(part_g, part_g, SEM_MOD + g).wait()

            gn = jnp.minimum(g + 1, NG - 1)
            off = jnp.where((g == 1) | (g == 4), 1.0, 0.0).astype(F32)
            for part in range(4):
                lead_proj(1, g, part // 2, part % 2)
                relayout(0, gn, part * 128, 128)
                mod_tiles([8 * g + 2 * part, 8 * g + 2 * part + 1], [off, off])
            return 0

        with scope("groups"):
            lax.fori_loop(1, NG, group_body, 0)

    pl.run_scoped(
        prologue,
        pltpu.VMEM((NG, D, 8, E), U32),
        pltpu.VMEM((4, LEAD, 256), F32),
        pltpu.VMEM((8, 256, 512), F32),
    )

    def main(w3v, w4v, zv, ttv):
        w34_cps = col_copies(w3_hbm, w3v, SEM_W3) + col_copies(w4_hbm, w4v, SEM_W4)
        start(w34_cps)
        wait(wo_cps + w1_cps + w2_cps + [mem_cp, x1_cp])

        def h_next(r0, g):
            y = h_rows(r0 + 16 * g, 16)
            for c in range(8):
                ring[RING, (g * 8 + c) * 8:(g * 8 + c + 1) * 8, :] = (
                    y[:, c * 128:(c + 1) * 128])

        for g in range(3):
            h_next(LEAD, g)

        scale = float(E) ** -0.5

        def segment(lhs, ro, store_tok, wo_lhs, extras):
            fill = fillv[...]
            keep = fill == 0.0
            NP = H // 2
            qkv, probs, blocks = {}, {}, []

            def proj(hp):
                slots = [t * H + 2 * hp + par for t in range(3) for par in range(2)]
                w = jnp.concatenate(
                    [_unpack(wq2[sl % 2][pl.ds((sl // 2) * SL, 512), :])
                     for sl in slots], axis=1)
                if hp == 0:
                    y = _dot(lhs[:, :512], w[:512])
                    y = _dot(lhs[:, 512:], w[512:]) + y
                else:
                    y = _dot(lhs, w)
                for u, sl in enumerate(slots):
                    store_tok(sl, y[8:32, u * 128:(u + 1) * 128])
                ops = []
                for t in range(3):
                    ym = jnp.concatenate(
                        [y[0:8, (2 * t) * 128:(2 * t + 1) * 128],
                         y[0:8, (2 * t + 1) * 128:(2 * t + 2) * 128]], axis=0)
                    ops.append(jnp.concatenate(
                        [ym.astype(BF16)]
                        + [_unpack(ring[ro + b, sl * 8:(sl + 1) * 8, :])
                           for sl in slots[2 * t:2 * t + 2] for b in range(2)],
                        axis=0))
                qkv[hp] = ops

            def scores(hp):
                q, kk, _ = qkv[hp]
                s = lax.dot_general(q, kk, (((1,), (1,)), ((), ())),
                                    preferred_element_type=F32)
                s = jnp.where(keep, s * scale, fill)
                mx = jnp.max(s, axis=-1, keepdims=True)
                p = jnp.exp(s - mx)
                l = jnp.sum(p, axis=-1, keepdims=True)
                rl = pl.reciprocal(l, approx=True)
                rl = rl * (2.0 - l * rl)
                probs[hp] = (p * rl).astype(BF16)

            def pv(hp):
                o = _dot(probs[hp], qkv[hp][2])
                blocks.append(wo_lhs(2 * hp, o[0:8], o[16:48]).astype(BF16))
                blocks.append(wo_lhs(2 * hp + 1, o[8:16], o[48:80]).astype(BF16))

            def wo_part(h0, h1, acc=None):
                lw = jnp.concatenate(blocks[h0:h1], axis=1)
                y = _dot(lw, _cols(wov, 0, 8, E * h0, E * h1))
                return y if acc is None else y + acc

            for i in range(NP):
                proj(i)
                if i >= 1:
                    scores(i - 1)
                if i >= 3:
                    pv(i - 3)
                for thunk in extras.get(i, ()):
                    thunk()
            acc = wo_part(0, 4)
            scores(NP - 1)
            pv(NP - 3)
            acc = wo_part(4, 12, acc)
            pv(NP - 2)
            pv(NP - 1)
            acc = wo_part(12, 24, acc)
            acc = wo_part(24, 32, acc)
            return acc

        def p1_front(r0):
            x2 = (xv[pl.ds(pl.multiple_of(r0, 64), 64), :].astype(F32)
                  + mod_rows(2, 64) * aout[...])
            h2 = _ln(x2) * mod_rows(4, 64) + mod_rows(3, 64)
            return x2, h2, _ln(h2).astype(BF16)

        def p1_store(y, c, live):
            g = _gelu(y)
            if live is not None:
                g = jnp.where(live, g, 0.0)
            gbuf[c, 24:88, :] = g

        def half_dots(lhs, wv, done):
            part = {}

            def run(c, kh):
                y = _dot(lhs[:, kh * 512:(kh + 1) * 512],
                         _cols(wv, c, c + 1, kh * 512, (kh + 1) * 512))
                if kh == 0:
                    part[c] = y
                else:
                    done(y + part[c], c)

            return [functools.partial(run, c, kh) for c in range(8) for kh in range(2)]

        def p2_front(n):
            return jnp.concatenate(
                [gbuf[c, 8 + SHIFTS[c]:8 + SHIFTS[c] + n, :] for c in range(8)],
                axis=1).astype(BF16)

        def p2_back(x2, h2, hs, row, n):
            x1 = jnp.concatenate([h2t[...], h2[0:n - 16]], axis=0) + hs
            x2w = jnp.concatenate([x2t[...], x2[0:n - 16]], axis=0)
            zv[pl.ds(pl.multiple_of(row, 16), n), :] = x2w + mod_rows(5, n) * x1
            ttv[pl.ds(pl.multiple_of(row // 2, 8), n // 2), :] = _pack(_ln(x1))

        def a_body(j, mem):
            for g in range(3):
                for c in range(8):
                    hcur[g * 8:(g + 1) * 8, c * 128:(c + 1) * 128] = (
                        ring[RING, (g * 8 + c) * 8:(g * 8 + c + 1) * 8, :])
            hb = _unpack(hcur[0:8, :])
            hac = _unpack(hcur[8:16, :]).astype(F32)
            hd = _unpack(hcur[16:24, :])
            wr = [lax.rem(LEAD // 16 + 3 * j + i, RING) for i in range(3)]
            ro0 = lax.rem(4 * j, RING)
            ro1 = ro0 + 2

            x2, h2, u = p1_front(64 * jnp.maximum(j - 1, 0))
            live = j > 0

            lhs = jnp.concatenate(
                [jnp.concatenate([mem, hac[0:8]], axis=0).astype(BF16), hb], axis=0)
            tok_a = {}

            def store0(c, y):
                tok_a[c] = y[0:8]
                ring[wr[0], c * 8:(c + 1) * 8, :] = _pack(y[8:24])

            deferred = {}

            def wo_lhs0(h, om, ot):
                deferred[h] = ot[24:32]
                return jnp.concatenate([om, ot[0:24]], axis=0)

            th = half_dots(u, w1v, lambda y, c: p1_store(y, c, live))
            extras = {i: [th[i - 2]] for i in range(2, 14)}
            extras[14] = th[12:14]
            extras[15] = th[14:16]
            out = segment(lhs, ro0, store0, wo_lhs0, extras)
            mem = out[0:8]
            aout[0:24, :] = out[8:32]

            lhs = jnp.concatenate(
                [jnp.concatenate([mem, hac[8:16]], axis=0).astype(BF16), hd], axis=0)

            def store1(c, y):
                ring[wr[1], c * 8:(c + 1) * 8, :] = _pack(
                    jnp.concatenate([tok_a[c], y[0:8]], axis=0))
                ring[wr[2], c * 8:(c + 1) * 8, :] = _pack(y[8:24])

            def wo_lhs1(h, om, ot):
                return jnp.concatenate([om, deferred[h], ot], axis=0)

            gs = p2_front(64)
            gbuf[:, 0:24, :] = gbuf[:, 64:88, :]
            hs = []

            def p2_fin():
                p2_back(x2, h2, jnp.concatenate(hs, axis=1), 64 * j, 64)
                x2t[...] = x2[48:64]
                h2t[...] = h2[48:64]

            th = half_dots(gs, w2v, lambda y, c: hs.append(y))
            extras = {i: [th[i]] for i in range(16)}
            extras[15].append(p2_fin)
            rn = LEAD + 48 * jnp.minimum(j + 1, NPAIR - 1)
            for g in range(3):
                extras[3 + 4 * g].append(functools.partial(h_next, rn, g))
            out = segment(lhs, ro1, store1, wo_lhs1, extras)
            aout[24:64, :] = out[8:48]
            return out[0:8]

        if "A" in phases:
            with scope("aloop"):
                lax.fori_loop(0, NPAIR, a_body, memv[...].astype(F32))
        else:
            zv[...] = jnp.zeros(zv.shape, F32)
            ttv[...] = jnp.zeros(ttv.shape, U32)

        x2, h2, u = p1_front(S - 64)
        y = _dot(u, _cols(w1v, 0, 8))
        for c in range(8):
            p1_store(y[:, c * 128:(c + 1) * 128], c, None)
        p2_back(x2, h2, _dot(p2_front(80), _cols(w2v, 0, 8)), S, 80)

        wait(w34_cps)

        def out_cp(i, slot):
            return cp(outv.at[slot], out_hbm.at[pl.ds(i * RB, RB), :],
                      SEM_OUT + slot)

        def p3_body(i, _):
            slot = i % 2

            @pl.when(i >= 2)
            def _():
                out_cp(i - 2, slot).wait()

            r0 = HALO + i * RB
            tt = _unpack(ttv[pl.ds(pl.multiple_of(r0 // 2, 8), RB // 2), :])
            ff = jnp.concatenate(
                [_gelu(_dot(tt, _cols(w3v, 4 * q, 4 * q + 4))).astype(BF16)
                 for q in range(FF // 512)], axis=1)
            y = _dot(ff, _cols(w4v, 0, 8))
            res = zv[pl.ds(pl.multiple_of(r0, 16), RB), :] + mod_rows(5, RB) * y
            outv[slot] = res.astype(BF16)
            out_cp(i, slot).start()
            return 0

        nb = S // RB
        if "B" in phases:
            with scope("p3"):
                lax.fori_loop(0, nb, p3_body, 0)
            out_cp(nb - 2, 0).wait()
            out_cp(nb - 1, 1).wait()
        else:
            outv[0] = zv[pl.ds(HALO, RB), :].astype(BF16)
            out_cp(0, 0).start()
            out_cp(0, 0).wait()

    pl.run_scoped(
        main,
        pltpu.VMEM((FF // 128, D // 2, 128), U32),
        pltpu.VMEM((8, FF // 2, 128), U32),
        pltpu.VMEM((S + HALO, D), F32),
        pltpu.VMEM(((S + HALO) // 2, D), U32),
    )


def _call(A_x, A_mem0, A_Wq, A_Wk, A_Wv, A_Wo, B_w1, B_w2, B_w3, B_w4, c, w_mod,
          phases="AB"):
    any_spec = pl.BlockSpec(memory_space=pl.ANY)
    scratch = [
        pltpu.VMEM((S, D), BF16),
        pltpu.VMEM((8, D), U32),
        pltpu.VMEM((M, D), BF16),
        pltpu.VMEM((48, D // 2, 128), U32),
        pltpu.VMEM((48, 8, 128), F32),
        pltpu.VMEM((3 * H // 2 * SL, E), U32),
        pltpu.VMEM((3 * H // 2 * SL, E), U32),
        pltpu.VMEM((8, H * E // 2, 128), U32),
        pltpu.VMEM((8, D // 2, 128), U32),
        pltpu.VMEM((8, D // 2, 128), U32),
        pltpu.VMEM((4, LEAD // 2, 256), U32),
        pltpu.VMEM((24, D), U32),
        pltpu.VMEM((RING + 1, 3 * H * 8, E), U32),
        pltpu.VMEM((64, D), F32),
        pltpu.VMEM((8, 96, 128), F32),
        pltpu.VMEM((16, D), F32),
        pltpu.VMEM((16, D), F32),
        pltpu.VMEM((2, RB, D), BF16),
        pltpu.VMEM((80, 80), F32),
        pltpu.VMEM((1, D), BF16),
        pltpu.SemaphoreType.DMA((NSEM,)),
    ]
    out = pl.pallas_call(
        functools.partial(_kernel, phases=phases),
        in_specs=[any_spec] * 12,
        out_specs=any_spec,
        out_shape=jax.ShapeDtypeStruct((S, D), BF16),
        scratch_shapes=scratch,
        compiler_params=pltpu.CompilerParams(
            vmem_limit_bytes=126 * 1024 * 1024),
    )(A_x.reshape(S, D), A_mem0.reshape(M, D), A_Wq, A_Wk, A_Wv,
      A_Wo.reshape(H * E, D), B_w1, B_w2, B_w3, B_w4, c, w_mod)
    return out.reshape(1, S, D)


def pallas_adaLN_cond__memory_aug_recurrent_mem_tr__mixer_s_mlp__prompt_kernel(
    A_x, A_mem0, A_Wq, A_Wk, A_Wv, A_Wo, A_seg_len, B_x, B_w1, B_w2, B_w3, B_w4,
    c, w_mod,
):
    assert A_seg_len == SEG
    del B_x
    return _call(A_x, A_mem0, A_Wq, A_Wk, A_Wv, A_Wo, B_w1, B_w2, B_w3, B_w4,
                 c, w_mod)
```

```python
import contextlib
import functools

import jax
import jax.numpy as jnp
from jax import lax
import jax.experimental.pallas as pl
import jax.experimental.pallas.tpu as pltpu

F32 = jnp.float32
BF16 = jnp.bfloat16
U32 = jnp.uint32

S = 2048
D = 1024
H = 32
E = 128
M = 8
SEG = 32
FF = 3584
EPS = 1e-5

LEAD = 512
RING = 36
SL = 520
HG = 16
NG = 3 * H // HG
NPAIR = S // (2 * SEG)
HALO = 80
RB = 256
SHIFTS = (-1, -1, 1, 1, -2, -2, 2, 2)

(SEM_X0, SEM_X1, SEM_C, SEM_MEM, SEM_WO, SEM_W1, SEM_W2, SEM_W3,
 SEM_W4) = range(9)
SEM_Q = 9
SEM_Q1 = 13
SEM_ST = 17
SEM_MOD = SEM_ST + NG
SEM_OUT = SEM_MOD + 6
NSEM = SEM_OUT + 2


def _ln(x):
    mu = jnp.mean(x, axis=-1, keepdims=True)
    xc = x - mu
    var = jnp.mean(xc * xc, axis=-1, keepdims=True)
    return xc * lax.rsqrt(var + EPS)


def _gelu(x):
    return jax.nn.gelu(x, approximate=True)


def _pack(x):
    return pltpu.bitcast(x.astype(BF16), U32)


def _unpack(x):
    return pltpu.bitcast(x, BF16)


def _dot(a, b):
    return jnp.dot(a, b, preferred_element_type=F32)


def _cols(ref, lo, hi, k0=0, k1=None):
    k1 = 2 * ref.shape[1] if k1 is None else k1
    return jnp.concatenate(
        [_unpack(ref[c, k0 // 2:k1 // 2, :]) for c in range(lo, hi)], axis=1)


def _kernel(x_hbm, mem_hbm, wq_hbm, wk_hbm, wv_hbm, wo_hbm, w1_hbm, w2_hbm,
            w3_hbm, w4_hbm, c_hbm, wmod_hbm, out_hbm,
            xv, scv, memv, wmodv, modv, wqa, wqb, wov, w1v, w2v,
            hv0, hcur, ring, aout, gbuf, x2t, h2t, outv, fillv, cv, sems, *, phases):
    def scope(name):
        return jax.named_scope(name) if "s" in phases else contextlib.nullcontext()

    def cp(src, dst, s):
        return pltpu.make_async_copy(src, dst, sems.at[s])

    def col_copies(w_hbm, w_v, s, lo=0, hi=None):
        w32 = w_hbm.bitcast(U32)
        hi = w_v.shape[0] if hi is None else hi
        return [cp(w32.at[:, pl.ds(c * 128, 128)], w_v.at[c], s)
                for c in range(lo, hi)]

    def start(cps):
        for q in cps:
            q.start()

    def wait(cps):
        for q in cps:
            q.wait()

    c_cp = cp(c_hbm, cv, SEM_C)
    mem_cp = cp(mem_hbm, memv, SEM_MEM)
    x0_cp = cp(x_hbm.at[pl.ds(0, LEAD)], xv.at[pl.ds(0, LEAD)], SEM_X0)
    x1_cp = cp(x_hbm.at[pl.ds(LEAD, S - LEAD)], xv.at[pl.ds(LEAD, S - LEAD)],
               SEM_X1)
    wo_cps = col_copies(wo_hbm, wov, SEM_WO)
    w1_cps = col_copies(w1_hbm, w1v, SEM_W1)
    w2_cps = col_copies(w2_hbm, w2v, SEM_W2)

    def mod_rows(i, n):
        m = jnp.concatenate([modv[8 * i + c] for c in range(8)], axis=1)
        return jnp.concatenate([m] * (n // 8), axis=0)

    def mod_tiles(tiles, offs):
        w = jnp.concatenate([_unpack(wmodv[c]) for c in tiles], axis=1)
        y = _dot(_unpack(scv[...]), w)[0:8]
        ys = [y[:, u * 128:(u + 1) * 128] + o for u, o in enumerate(offs)]
        for c, v in zip(tiles, ys):
            modv[c] = v
        return ys

    wq2 = (wqa, wqb)

    def h_rows(r0, n):
        xf = xv[pl.ds(pl.multiple_of(r0, 16), n), :].astype(F32)
        return _pack(_ln(xf) * mod_rows(1, n) + mod_rows(0, n))

    def prologue(st, xn, acc):
        w_hbms = (wq_hbm, wk_hbm, wv_hbm)

        def st_src(i):
            return w_hbms[i // 2].bitcast(U32).at[:, pl.ds((i % 2) * 8, 8), :]

        def st_quarter(i, q, s):
            return cp(st_src(i).at[pl.ds(q * 256, 256)],
                      st.at[i, pl.ds(q * 256, 256)], s)

        def q_cps(q):
            w32 = wmod_hbm.bitcast(U32)
            return [cp(w32.at[:, pl.ds(pl.multiple_of(c * 128, 128), 128)],
                       wmodv.at[c], SEM_Q + q)
                    for c in (2 * q, 2 * q + 1, 8 + 2 * q, 9 + 2 * q)
                    ] + [st_quarter(0, q, SEM_Q + q)]

        def st_cp(i):
            return cp(st_src(i), st.at[i], SEM_ST + i)

        def mod_cps(i):
            return col_copies(wmod_hbm, wmodv, SEM_MOD + i, 8 * i, 8 * i + 8)

        with scope("first"):
            start([c_cp, mem_cp, x0_cp])
        for q in range(4):
            start(q_cps(q))
        start([st_quarter(1, q, SEM_Q1 + q) for q in range(4)])
        start([st_cp(2), st_cp(3)] + mod_cps(2) + [st_cp(4)] + mod_cps(3)
              + [st_cp(5)])

        r = lax.broadcasted_iota(jnp.int32, (80, 128), 0)
        k = lax.broadcasted_iota(jnp.int32, (80, 128), 1)

        def head_of(i):
            return jnp.where(i < 16, i // 8, (i - 16) // 32)

        def pos_of(i):
            return jnp.where(i < 16, i % 8, 8 + (i - 16) % 32)

        same = head_of(r) == head_of(k)
        vis = (pos_of(r) < M) | (pos_of(r) >= pos_of(k))
        fillv[...] = jnp.where(same, jnp.where(vis, 0.0, -1e9), -jnp.inf).astype(F32)
        aout[...] = jnp.zeros(aout.shape, F32)
        gbuf[...] = jnp.zeros(gbuf.shape, F32)
        x2t[...] = jnp.zeros(x2t.shape, F32)
        h2t[...] = jnp.zeros(h2t.shape, F32)

        c_cp.wait()
        cf = cv[...].astype(F32)
        scv[...] = _pack(jnp.broadcast_to(cf * jax.nn.sigmoid(cf), (16, D)))
        x0_cp.wait()

        def ln_body(i, _):
            r0 = pl.multiple_of(i * 64, 64)
            y = _ln(xv[pl.ds(r0, 64), :].astype(F32))
            for q in range(4):
                xn[q, pl.ds(r0, 64), :] = y[:, q * 256:(q + 1) * 256]
            return 0

        lax.fori_loop(0, LEAD // 64, ln_body, 0)

        def relayout(par, g, p0, n):
            base = g * (8 * SL)
            for u in range(n):
                a = st[g, 2 * (p0 + u)]
                b = st[g, 2 * (p0 + u) + 1]
                if par == 0:
                    w = (a & jnp.uint32(0xFFFF)) | (b << 16)
                else:
                    w = (a >> 16) | (b & jnp.uint32(0xFFFF0000))
                wq2[par][pl.ds(base + p0 + u, 8, stride=SL), :] = w

        def to_ring(y, par, s0, rc):
            for u in range(4):
                row = pl.multiple_of((2 * (s0 + u) + par) * 8, 8)
                for b in range(16):
                    ring[rc * 16 + b, pl.ds(row, 8), :] = (
                        y[b * 8:(b + 1) * 8, u * 128:(u + 1) * 128])

        def q_body(q, _):
            wait(q_cps(q))
            m = mod_tiles([2 * q, 2 * q + 1, 8 + 2 * q, 9 + 2 * q], [0.0, 0.0, 1.0, 1.0])
            sa, ca = [jnp.concatenate([jnp.concatenate(v, axis=1)] * (LEAD // 8), axis=0)
                      for v in (m[0:2], m[2:4])]
            hv0[q] = _pack(xn[q] * ca + sa)
            relayout(0, 0, q * 128, 128)
            relayout(1, 0, q * 128, 128)

            def rc_body(rc, _):
                lhs = _unpack(hv0[q, pl.ds(pl.multiple_of(rc * 128, 128), 128), :])
                for part in range(4):
                    par, hq = part // 2, part % 2
                    w = jnp.concatenate(
                        [_unpack(wq2[par][pl.ds(pl.multiple_of(
                            (hq * 4 + u) * SL + q * 128, 8), 128), :])
                         for u in range(4)], axis=1)
                    y = _dot(lhs, w) + jnp.where(q > 0, acc[rc * 4 + part], 0.0)
                    acc[rc * 4 + part] = y
                    to_ring(_pack(y), par, hq * 4, rc)
                return 0

            lax.fori_loop(0, 2, rc_body, 0)
            return 0

        with scope("quarters"):
            lax.fori_loop(0, 4, q_body, 0)

        start(mod_cps(4) + mod_cps(5) + wo_cps + w1_cps + w2_cps + [x1_cp])

        for q in range(4):
            st_quarter(1, q, SEM_Q1 + q).wait()

            def rl_body(i, _, q=q):
                relayout(0, 1, q * 128 + i * 32, 32)
                return 0

            lax.fori_loop(0, 4, rl_body, 0)

        def lead_proj(par, g, hq, rc):
            s0 = g * 8 + hq * 4
            w = jnp.concatenate(
                [_unpack(wq2[par][pl.ds(pl.multiple_of((s0 + u) * SL, 8), 512), :])
                 for u in range(4)], axis=1)
            lhs = jnp.concatenate(
                [_unpack(hv0[q, rc * 128:(rc + 1) * 128, :]) for q in range(4)],
                axis=1)
            to_ring(_pack(_dot(lhs, w)), par, s0, rc)

        def group_body(g, _):
            for part in range(4):
                lead_proj(0, g, part // 2, part % 2)
                relayout(1, g, part * 128, 128)

            @pl.when(g < NG - 1)
            def _():
                cp(st_src(1), st.at[g + 1], SEM_ST + g + 1).wait()

            @pl.when(g >= 2)
            def _():
                part_g = wmodv.at[pl.ds(8 * g, 8)]
                cp(part_g, part_g, SEM_MOD + g).wait()

            gn = jnp.minimum(g + 1, NG - 1)
            off = jnp.where((g == 1) | (g == 4), 1.0, 0.0).astype(F32)
            for part in range(4):
                lead_proj(1, g, part // 2, part % 2)
                relayout(0, gn, part * 128, 128)
                mod_tiles([8 * g + 2 * part, 8 * g + 2 * part + 1], [off, off])
            return 0

        with scope("groups"):
            lax.fori_loop(1, NG, group_body, 0)

    pl.run_scoped(
        prologue,
        pltpu.VMEM((NG, D, 8, E), U32),
        pltpu.VMEM((4, LEAD, 256), F32),
        pltpu.VMEM((8, 256, 512), F32),
    )

    def main(w3v, w4v, zv, ttv):
        w34_cps = col_copies(w3_hbm, w3v, SEM_W3) + col_copies(w4_hbm, w4v, SEM_W4)
        start(w34_cps)
        wait(wo_cps + w1_cps + w2_cps + [mem_cp, x1_cp])

        def h_next(r0, g):
            y = h_rows(r0 + 16 * g, 16)
            for c in range(8):
                ring[RING, (g * 8 + c) * 8:(g * 8 + c + 1) * 8, :] = (
                    y[:, c * 128:(c + 1) * 128])

        for g in range(3):
            h_next(LEAD, g)

        scale = float(E) ** -0.5

        def segment(lhs, ro, store_tok, wo_lhs, extras):
            fill = fillv[...]
            keep = fill == 0.0
            NP = H // 2
            qkv, probs, blocks = {}, {}, []

            def proj(hp):
                slots = [t * H + 2 * hp + par for t in range(3) for par in range(2)]
                w = jnp.concatenate(
                    [_unpack(wq2[sl % 2][pl.ds((sl // 2) * SL, 512), :])
                     for sl in slots], axis=1)
                if hp == 0:
                    y = _dot(lhs[:, :512], w[:512])
                    y = _dot(lhs[:, 512:], w[512:]) + y
                else:
                    y = _dot(lhs, w)
                for u, sl in enumerate(slots):
                    store_tok(sl, y[8:32, u * 128:(u + 1) * 128])
                ops = []
                for t in range(3):
                    ym = jnp.concatenate(
                        [y[0:8, (2 * t) * 128:(2 * t + 1) * 128],
                         y[0:8, (2 * t + 1) * 128:(2 * t + 2) * 128]], axis=0)
                    ops.append(jnp.concatenate(
                        [ym.astype(BF16)]
                        + [_unpack(ring[ro + b, sl * 8:(sl + 1) * 8, :])
                           for sl in slots[2 * t:2 * t + 2] for b in range(2)]
                        + ([jnp.zeros((48, 128), BF16)] if t else []),
                        axis=0))
                qkv[hp] = ops

            def scores(hp):
                q, kk, _ = qkv[hp]
                s = lax.dot_general(q, kk, (((1,), (1,)), ((), ())),
                                    preferred_element_type=F32)
                s = jnp.where(keep, s * scale, fill)
                mx = jnp.max(s, axis=-1, keepdims=True)
                p = jnp.exp(s - mx)
                l = jnp.sum(p, axis=-1, keepdims=True)
                rl = pl.reciprocal(l, approx=True)
                rl = rl * (2.0 - l * rl)
                probs[hp] = (p * rl).astype(BF16)

            def pv(hp):
                o = _dot(probs[hp], qkv[hp][2])
                blocks.append(wo_lhs(2 * hp, o[0:8], o[16:48]).astype(BF16))
                blocks.append(wo_lhs(2 * hp + 1, o[8:16], o[48:80]).astype(BF16))

            def wo_part(h0, h1, acc=None):
                lw = jnp.concatenate(blocks[h0:h1], axis=1)
                y = _dot(lw, _cols(wov, 0, 8, E * h0, E * h1))
                return y if acc is None else y + acc

            for i in range(NP):
                proj(i)
                if i >= 1:
                    scores(i - 1)
                if i >= 3:
                    pv(i - 3)
                for thunk in extras.get(i, ()):
                    thunk()
            acc = wo_part(0, 4)
            scores(NP - 1)
            pv(NP - 3)
            acc = wo_part(4, 12, acc)
            pv(NP - 2)
            pv(NP - 1)
            acc = wo_part(12, 24, acc)
            acc = wo_part(24, 32, acc)
            return acc

        def p1_front(r0):
            x2 = (xv[pl.ds(pl.multiple_of(r0, 64), 64), :].astype(F32)
                  + mod_rows(2, 64) * aout[...])
            h2 = _ln(x2) * mod_rows(4, 64) + mod_rows(3, 64)
            return x2, h2, _ln(h2).astype(BF16)

        def p1_store(y, c, live):
            g = _gelu(y)
            if live is not None:
                g = jnp.where(live, g, 0.0)
            gbuf[c, 24:88, :] = g

        def half_dots(lhs, wv, done):
            part = {}

            def run(c, kh):
                y = _dot(lhs[:, kh * 512:(kh + 1) * 512],
                         _cols(wv, c, c + 1, kh * 512, (kh + 1) * 512))
                if kh == 0:
                    part[c] = y
                else:
                    done(y + part[c], c)

            return [functools.partial(run, c, kh) for c in range(8) for kh in range(2)]

        def p2_front(n):
            return jnp.concatenate(
                [gbuf[c, 8 + SHIFTS[c]:8 + SHIFTS[c] + n, :] for c in range(8)],
                axis=1).astype(BF16)

        def p2_back(x2, h2, hs, row, n):
            x1 = jnp.concatenate([h2t[...], h2[0:n - 16]], axis=0) + hs
            x2w = jnp.concatenate([x2t[...], x2[0:n - 16]], axis=0)
            zv[pl.ds(pl.multiple_of(row, 16), n), :] = x2w + mod_rows(5, n) * x1
            ttv[pl.ds(pl.multiple_of(row // 2, 8), n // 2), :] = _pack(_ln(x1))

        def a_body(j, mem):
            for g in range(3):
                for c in range(8):
                    hcur[g * 8:(g + 1) * 8, c * 128:(c + 1) * 128] = (
                        ring[RING, (g * 8 + c) * 8:(g * 8 + c + 1) * 8, :])
            hb = _unpack(hcur[0:8, :])
            hac = _unpack(hcur[8:16, :]).astype(F32)
            hd = _unpack(hcur[16:24, :])
            wr = [lax.rem(LEAD // 16 + 3 * j + i, RING) for i in range(3)]
            ro0 = lax.rem(4 * j, RING)
            ro1 = ro0 + 2

            x2, h2, u = p1_front(64 * jnp.maximum(j - 1, 0))
            live = j > 0

            lhs = jnp.concatenate(
                [jnp.concatenate([mem, hac[0:8]], axis=0).astype(BF16), hb], axis=0)
            tok_a = {}

            def store0(c, y):
                tok_a[c] = y[0:8]
                ring[wr[0], c * 8:(c + 1) * 8, :] = _pack(y[8:24])

            deferred = {}

            def wo_lhs0(h, om, ot):
                deferred[h] = ot[24:32]
                return jnp.concatenate([om, ot[0:24]], axis=0)

            th = half_dots(u, w1v, lambda y, c: p1_store(y, c, live))
            extras = {i: [th[i - 2]] for i in range(2, 14)}
            extras[14] = th[12:14]
            extras[15] = th[14:16]
            out = segment(lhs, ro0, store0, wo_lhs0, extras)
            mem = out[0:8]
            aout[0:24, :] = out[8:32]

            lhs = jnp.concatenate(
                [jnp.concatenate([mem, hac[8:16]], axis=0).astype(BF16), hd], axis=0)

            def store1(c, y):
                ring[wr[1], c * 8:(c + 1) * 8, :] = _pack(
                    jnp.concatenate([tok_a[c], y[0:8]], axis=0))
                ring[wr[2], c * 8:(c + 1) * 8, :] = _pack(y[8:24])

            def wo_lhs1(h, om, ot):
                return jnp.concatenate([om, deferred[h], ot], axis=0)

            gs = p2_front(64)
            gbuf[:, 0:24, :] = gbuf[:, 64:88, :]
            hs = []

            def p2_fin():
                p2_back(x2, h2, jnp.concatenate(hs, axis=1), 64 * j, 64)
                x2t[...] = x2[48:64]
                h2t[...] = h2[48:64]

            th = half_dots(gs, w2v, lambda y, c: hs.append(y))
            extras = {i: [th[i]] for i in range(16)}
            extras[15].append(p2_fin)
            rn = LEAD + 48 * jnp.minimum(j + 1, NPAIR - 1)
            for g in range(3):
                extras[3 + 4 * g].append(functools.partial(h_next, rn, g))
            out = segment(lhs, ro1, store1, wo_lhs1, extras)
            aout[24:64, :] = out[8:48]
            return out[0:8]

        if "A" in phases:
            with scope("aloop"):
                lax.fori_loop(0, NPAIR, a_body, memv[...].astype(F32))
        else:
            zv[...] = jnp.zeros(zv.shape, F32)
            ttv[...] = jnp.zeros(ttv.shape, U32)

        x2, h2, u = p1_front(S - 64)
        y = _dot(u, _cols(w1v, 0, 8))
        for c in range(8):
            p1_store(y[:, c * 128:(c + 1) * 128], c, None)
        p2_back(x2, h2, _dot(p2_front(80), _cols(w2v, 0, 8)), S, 80)

        wait(w34_cps)

        def out_cp(i, slot):
            return cp(outv.at[slot], out_hbm.at[pl.ds(i * RB, RB), :],
                      SEM_OUT + slot)

        def p3_body(i, _):
            slot = i % 2

            @pl.when(i >= 2)
            def _():
                out_cp(i - 2, slot).wait()

            r0 = HALO + i * RB
            tt = _unpack(ttv[pl.ds(pl.multiple_of(r0 // 2, 8), RB // 2), :])
            ff = jnp.concatenate(
                [_gelu(_dot(tt, _cols(w3v, 4 * q, 4 * q + 4))).astype(BF16)
                 for q in range(FF // 512)], axis=1)
            y = _dot(ff, _cols(w4v, 0, 8))
            res = zv[pl.ds(pl.multiple_of(r0, 16), RB), :] + mod_rows(5, RB) * y
            outv[slot] = res.astype(BF16)
            out_cp(i, slot).start()
            return 0

        nb = S // RB
        if "B" in phases:
            with scope("p3"):
                lax.fori_loop(0, nb, p3_body, 0)
            out_cp(nb - 2, 0).wait()
            out_cp(nb - 1, 1).wait()
        else:
            outv[0] = zv[pl.ds(HALO, RB), :].astype(BF16)
            out_cp(0, 0).start()
            out_cp(0, 0).wait()

    pl.run_scoped(
        main,
        pltpu.VMEM((FF // 128, D // 2, 128), U32),
        pltpu.VMEM((8, FF // 2, 128), U32),
        pltpu.VMEM((S + HALO, D), F32),
        pltpu.VMEM(((S + HALO) // 2, D), U32),
    )


def _call(A_x, A_mem0, A_Wq, A_Wk, A_Wv, A_Wo, B_w1, B_w2, B_w3, B_w4, c, w_mod,
          phases="AB"):
    any_spec = pl.BlockSpec(memory_space=pl.ANY)
    scratch = [
        pltpu.VMEM((S, D), BF16),
        pltpu.VMEM((8, D), U32),
        pltpu.VMEM((M, D), BF16),
        pltpu.VMEM((48, D // 2, 128), U32),
        pltpu.VMEM((48, 8, 128), F32),
        pltpu.VMEM((3 * H // 2 * SL, E), U32),
        pltpu.VMEM((3 * H // 2 * SL, E), U32),
        pltpu.VMEM((8, H * E // 2, 128), U32),
        pltpu.VMEM((8, D // 2, 128), U32),
        pltpu.VMEM((8, D // 2, 128), U32),
        pltpu.VMEM((4, LEAD // 2, 256), U32),
        pltpu.VMEM((24, D), U32),
        pltpu.VMEM((RING + 1, 3 * H * 8, E), U32),
        pltpu.VMEM((64, D), F32),
        pltpu.VMEM((8, 96, 128), F32),
        pltpu.VMEM((16, D), F32),
        pltpu.VMEM((16, D), F32),
        pltpu.VMEM((2, RB, D), BF16),
        pltpu.VMEM((80, 128), F32),
        pltpu.VMEM((1, D), BF16),
        pltpu.SemaphoreType.DMA((NSEM,)),
    ]
    out = pl.pallas_call(
        functools.partial(_kernel, phases=phases),
        in_specs=[any_spec] * 12,
        out_specs=any_spec,
        out_shape=jax.ShapeDtypeStruct((S, D), BF16),
        scratch_shapes=scratch,
        compiler_params=pltpu.CompilerParams(
            vmem_limit_bytes=126 * 1024 * 1024),
    )(A_x.reshape(S, D), A_mem0.reshape(M, D), A_Wq, A_Wk, A_Wv,
      A_Wo.reshape(H * E, D), B_w1, B_w2, B_w3, B_w4, c, w_mod)
    return out.reshape(1, S, D)


def pallas_adaLN_cond__memory_aug_recurrent_mem_tr__mixer_s_mlp__prompt_kernel(
    A_x, A_mem0, A_Wq, A_Wk, A_Wv, A_Wo, A_seg_len, B_x, B_w1, B_w2, B_w3, B_w4,
    c, w_mod,
):
    assert A_seg_len == SEG
    del B_x
    return _call(A_x, A_mem0, A_Wq, A_Wk, A_Wv, A_Wo, B_w1, B_w2, B_w3, B_w4,
                 c, w_mod)
```

```python
import contextlib
import functools

import jax
import jax.numpy as jnp
from jax import lax
import jax.experimental.pallas as pl
import jax.experimental.pallas.tpu as pltpu

F32 = jnp.float32
BF16 = jnp.bfloat16
U32 = jnp.uint32

S = 2048
D = 1024
H = 32
E = 128
M = 8
SEG = 32
FF = 3584
EPS = 1e-5

LEAD = 512
RING = 36
HB = RING
GB = RING + 1
SL = 520
HG = 16
NG = 3 * H // HG
NPAIR = S // (2 * SEG)
HALO = 80
RB = 256
SHIFTS = (-1, -1, 1, 1, -2, -2, 2, 2)

(SEM_X0, SEM_X1, SEM_C, SEM_MEM, SEM_WO, SEM_W1, SEM_W2, SEM_W3,
 SEM_W4) = range(9)
SEM_Q = 9
SEM_Q1 = 13
SEM_ST = 17
SEM_MOD = SEM_ST + NG
SEM_OUT = SEM_MOD + 6
NSEM = SEM_OUT + 2


def _ln(x):
    mu = jnp.mean(x, axis=-1, keepdims=True)
    xc = x - mu
    var = jnp.mean(xc * xc, axis=-1, keepdims=True)
    return xc * lax.rsqrt(var + EPS)


def _gelu(x):
    return jax.nn.gelu(x, approximate=True)


def _pack(x):
    return pltpu.bitcast(x.astype(BF16), U32)


def _unpack(x):
    return pltpu.bitcast(x, BF16)


def _dot(a, b):
    return jnp.dot(a, b, preferred_element_type=F32)


def _cols(ref, lo, hi, k0=0, k1=None):
    k1 = 2 * ref.shape[1] if k1 is None else k1
    return jnp.concatenate(
        [_unpack(ref[c, k0 // 2:k1 // 2, :]) for c in range(lo, hi)], axis=1)


def _kernel(x_hbm, mem_hbm, wq_hbm, wk_hbm, wv_hbm, wo_hbm, w1_hbm, w2_hbm,
            w3_hbm, w4_hbm, c_hbm, wmod_hbm, out_hbm,
            xv, scv, memv, wmodv, modv, wqa, wqb, wov, w1v, w2v,
            hv0, hcur, ring, aout, x2t, h2t, outv, fillv, cv, sems, *, phases):
    def scope(name):
        return jax.named_scope(name) if "s" in phases else contextlib.nullcontext()

    def cp(src, dst, s):
        return pltpu.make_async_copy(src, dst, sems.at[s])

    def col_copies(w_hbm, w_v, s, lo=0, hi=None):
        w32 = w_hbm.bitcast(U32)
        hi = w_v.shape[0] if hi is None else hi
        return [cp(w32.at[:, pl.ds(c * 128, 128)], w_v.at[c], s)
                for c in range(lo, hi)]

    def start(cps):
        for q in cps:
            q.start()

    def wait(cps):
        for q in cps:
            q.wait()

    c_cp = cp(c_hbm, cv, SEM_C)
    mem_cp = cp(mem_hbm, memv, SEM_MEM)
    x0_cp = cp(x_hbm.at[pl.ds(0, LEAD)], xv.at[pl.ds(0, LEAD)], SEM_X0)
    x1_cp = cp(x_hbm.at[pl.ds(LEAD, S - LEAD)], xv.at[pl.ds(LEAD, S - LEAD)],
               SEM_X1)
    wo_cps = col_copies(wo_hbm, wov, SEM_WO)
    w1_cps = col_copies(w1_hbm, w1v, SEM_W1)
    w2_cps = col_copies(w2_hbm, w2v, SEM_W2)

    def mod_rows(i, n):
        m = jnp.concatenate([modv[8 * i + c] for c in range(8)], axis=1)
        return jnp.concatenate([m] * (n // 8), axis=0)

    def mod_tiles(tiles, offs):
        w = jnp.concatenate([_unpack(wmodv[c]) for c in tiles], axis=1)
        y = _dot(_unpack(scv[...]), w)[0:8]
        ys = [y[:, u * 128:(u + 1) * 128] + o for u, o in enumerate(offs)]
        for c, v in zip(tiles, ys):
            modv[c] = v
        return ys

    wq2 = (wqa, wqb)

    def h_rows(r0, n):
        xf = xv[pl.ds(pl.multiple_of(r0, 16), n), :].astype(F32)
        return _pack(_ln(xf) * mod_rows(1, n) + mod_rows(0, n))

    def prologue(st, xn, acc):
        w_hbms = (wq_hbm, wk_hbm, wv_hbm)

        def st_src(i):
            return w_hbms[i // 2].bitcast(U32).at[:, pl.ds((i % 2) * 8, 8), :]

        def st_quarter(i, q, s):
            return cp(st_src(i).at[pl.ds(q * 256, 256)],
                      st.at[i, pl.ds(q * 256, 256)], s)

        def q_cps(q):
            w32 = wmod_hbm.bitcast(U32)
            return [cp(w32.at[:, pl.ds(pl.multiple_of(c * 128, 128), 128)],
                       wmodv.at[c], SEM_Q + q)
                    for c in (2 * q, 2 * q + 1, 8 + 2 * q, 9 + 2 * q)
                    ] + [st_quarter(0, q, SEM_Q + q)]

        def st_cp(i):
            return cp(st_src(i), st.at[i], SEM_ST + i)

        def mod_cps(i):
            return col_copies(wmod_hbm, wmodv, SEM_MOD + i, 8 * i, 8 * i + 8)

        with scope("first"):
            start([c_cp, mem_cp, x0_cp])
        for q in range(4):
            start(q_cps(q))
        start([st_quarter(1, q, SEM_Q1 + q) for q in range(4)])
        start([st_cp(2), st_cp(3)] + mod_cps(2) + [st_cp(4)] + mod_cps(3)
              + [st_cp(5)])

        r = lax.broadcasted_iota(jnp.int32, (80, 128), 0)
        k = lax.broadcasted_iota(jnp.int32, (80, 128), 1)

        def head_of(i):
            return jnp.where(i < 16, i // 8, (i - 16) // 32)

        def pos_of(i):
            return jnp.where(i < 16, i % 8, 8 + (i - 16) % 32)

        same = head_of(r) == head_of(k)
        vis = (pos_of(r) < M) | (pos_of(r) >= pos_of(k))
        fillv[...] = jnp.where(same, jnp.where(vis, 0.0, -1e9), -jnp.inf).astype(F32)
        aout[...] = jnp.zeros(aout.shape, F32)
        ring[GB] = jnp.zeros(ring.shape[1:], U32)
        x2t[...] = jnp.zeros(x2t.shape, F32)
        h2t[...] = jnp.zeros(h2t.shape, F32)

        c_cp.wait()
        cf = cv[...].astype(F32)
        scv[...] = _pack(jnp.broadcast_to(cf * jax.nn.sigmoid(cf), (16, D)))
        x0_cp.wait()

        def ln_body(i, _):
            r0 = pl.multiple_of(i * 64, 64)
            y = _ln(xv[pl.ds(r0, 64), :].astype(F32))
            for q in range(4):
                xn[q, pl.ds(r0, 64), :] = y[:, q * 256:(q + 1) * 256]
            return 0

        lax.fori_loop(0, LEAD // 64, ln_body, 0)

        def relayout(par, g, p0, n):
            base = g * (8 * SL)
            for u in range(n):
                a = st[g, 2 * (p0 + u)]
                b = st[g, 2 * (p0 + u) + 1]
                if par == 0:
                    w = (a & jnp.uint32(0xFFFF)) | (b << 16)
                else:
                    w = (a >> 16) | (b & jnp.uint32(0xFFFF0000))
                wq2[par][pl.ds(base + p0 + u, 8, stride=SL), :] = w

        def to_ring(y, par, s0, rc):
            for u in range(4):
                row = pl.multiple_of((2 * (s0 + u) + par) * 8, 8)
                for b in range(16):
                    ring[rc * 16 + b, pl.ds(row, 8), :] = (
                        y[b * 8:(b + 1) * 8, u * 128:(u + 1) * 128])

        def q_body(q, _):
            wait(q_cps(q))
            m = mod_tiles([2 * q, 2 * q + 1, 8 + 2 * q, 9 + 2 * q], [0.0, 0.0, 1.0, 1.0])
            sa, ca = [jnp.concatenate([jnp.concatenate(v, axis=1)] * (LEAD // 8), axis=0)
                      for v in (m[0:2], m[2:4])]
            hv0[q] = _pack(xn[q] * ca + sa)
            relayout(0, 0, q * 128, 128)
            relayout(1, 0, q * 128, 128)

            def rc_body(rc, _):
                lhs = _unpack(hv0[q, pl.ds(pl.multiple_of(rc * 128, 128), 128), :])
                for part in range(4):
                    par, hq = part // 2, part % 2
                    w = jnp.concatenate(
                        [_unpack(wq2[par][pl.ds(pl.multiple_of(
                            (hq * 4 + u) * SL + q * 128, 8), 128), :])
                         for u in range(4)], axis=1)
                    y = _dot(lhs, w) + jnp.where(q > 0, acc[rc * 4 + part], 0.0)
                    acc[rc * 4 + part] = y
                    to_ring(_pack(y), par, hq * 4, rc)
                return 0

            lax.fori_loop(0, 2, rc_body, 0)
            return 0

        with scope("quarters"):
            lax.fori_loop(0, 4, q_body, 0)

        start(mod_cps(4) + mod_cps(5) + wo_cps + w1_cps + w2_cps + [x1_cp])

        for q in range(4):
            st_quarter(1, q, SEM_Q1 + q).wait()

            def rl_body(i, _, q=q):
                relayout(0, 1, q * 128 + i * 32, 32)
                return 0

            lax.fori_loop(0, 4, rl_body, 0)

        def lead_proj(par, g, hq, rc):
            s0 = g * 8 + hq * 4
            w = jnp.concatenate(
                [_unpack(wq2[par][pl.ds(pl.multiple_of((s0 + u) * SL, 8), 512), :])
                 for u in range(4)], axis=1)
            lhs = jnp.concatenate(
                [_unpack(hv0[q, rc * 128:(rc + 1) * 128, :]) for q in range(4)],
                axis=1)
            to_ring(_pack(_dot(lhs, w)), par, s0, rc)

        def group_body(g, _):
            for part in range(4):
                lead_proj(0, g, part // 2, part % 2)
                relayout(1, g, part * 128, 128)

            @pl.when(g < NG - 1)
            def _():
                cp(st_src(1), st.at[g + 1], SEM_ST + g + 1).wait()

            @pl.when(g >= 2)
            def _():
                part_g = wmodv.at[pl.ds(8 * g, 8)]
                cp(part_g, part_g, SEM_MOD + g).wait()

            gn = jnp.minimum(g + 1, NG - 1)
            off = jnp.where((g == 1) | (g == 4), 1.0, 0.0).astype(F32)
            for part in range(4):
                lead_proj(1, g, part // 2, part % 2)
                relayout(0, gn, part * 128, 128)
                mod_tiles([8 * g + 2 * part, 8 * g + 2 * part + 1], [off, off])
            return 0

        with scope("groups"):
            lax.fori_loop(1, NG, group_body, 0)

    pl.run_scoped(
        prologue,
        pltpu.VMEM((NG, D, 8, E), U32),
        pltpu.VMEM((4, LEAD, 256), F32),
        pltpu.VMEM((8, 256, 512), F32),
    )

    def main(w3v, w4v, zv, ttv):
        w34_cps = col_copies(w3_hbm, w3v, SEM_W3) + col_copies(w4_hbm, w4v, SEM_W4)
        start(w34_cps)
        wait(wo_cps + w1_cps + w2_cps + [mem_cp, x1_cp])

        def h_next(r0, g):
            y = h_rows(r0 + 16 * g, 16)
            for c in range(8):
                ring[HB, (g * 8 + c) * 8:(g * 8 + c + 1) * 8, :] = (
                    y[:, c * 128:(c + 1) * 128])

        for g in range(3):
            h_next(LEAD, g)

        scale = float(E) ** -0.5

        def segment(lhs, ro, store_tok, wo_lhs, extras):
            fill = fillv[...]
            keep = fill == 0.0
            NP = H // 2
            qkv, probs, blocks = {}, {}, []

            def proj(hp):
                slots = [t * H + 2 * hp + par for t in range(3) for par in range(2)]
                w = jnp.concatenate(
                    [_unpack(wq2[sl % 2][pl.ds((sl // 2) * SL, 512), :])
                     for sl in slots], axis=1)
                if hp == 0:
                    y = _dot(lhs[:, :512], w[:512])
                    y = _dot(lhs[:, 512:], w[512:]) + y
                else:
                    y = _dot(lhs, w)
                for u, sl in enumerate(slots):
                    store_tok(sl, y[8:32, u * 128:(u + 1) * 128])
                ops = []
                for t in range(3):
                    ym = jnp.concatenate(
                        [y[0:8, (2 * t) * 128:(2 * t + 1) * 128],
                         y[0:8, (2 * t + 1) * 128:(2 * t + 2) * 128]], axis=0)
                    ops.append(jnp.concatenate(
                        [ym.astype(BF16)]
                        + [_unpack(ring[ro + b, sl * 8:(sl + 1) * 8, :])
                           for sl in slots[2 * t:2 * t + 2] for b in range(2)]
                        + ([jnp.zeros((48, 128), BF16)] if t else []),
                        axis=0))
                qkv[hp] = ops

            def scores(hp):
                q, kk, _ = qkv[hp]
                s = lax.dot_general(q, kk, (((1,), (1,)), ((), ())),
                                    preferred_element_type=F32)
                s = jnp.where(keep, s * scale, fill)
                mx = jnp.max(s, axis=-1, keepdims=True)
                p = jnp.exp(s - mx)
                l = jnp.sum(p, axis=-1, keepdims=True)
                rl = pl.reciprocal(l, approx=True)
                rl = rl * (2.0 - l * rl)
                probs[hp] = (p * rl).astype(BF16)

            def pv(hp):
                o = _dot(probs[hp], qkv[hp][2])
                blocks.append(wo_lhs(2 * hp, o[0:8], o[16:48]).astype(BF16))
                blocks.append(wo_lhs(2 * hp + 1, o[8:16], o[48:80]).astype(BF16))

            def wo_part(h0, h1, acc=None):
                lw = jnp.concatenate(blocks[h0:h1], axis=1)
                y = _dot(lw, _cols(wov, 0, 8, E * h0, E * h1))
                return y if acc is None else y + acc

            for i in range(NP):
                proj(i)
                if i >= 1:
                    scores(i - 1)
                if i >= 3:
                    pv(i - 3)
                for thunk in extras.get(i, ()):
                    thunk()
            acc = wo_part(0, 4)
            scores(NP - 1)
            pv(NP - 3)
            acc = wo_part(4, 12, acc)
            pv(NP - 2)
            pv(NP - 1)
            acc = wo_part(12, 24, acc)
            acc = wo_part(24, 32, acc)
            return acc

        def p1_front(r0):
            x2 = (xv[pl.ds(pl.multiple_of(r0, 64), 64), :].astype(F32)
                  + mod_rows(2, 64) * aout[...])
            h2 = _ln(x2) * mod_rows(4, 64) + mod_rows(3, 64)
            return x2, h2, _ln(h2).astype(BF16)

        def p1_store(y, c, live):
            g = _gelu(y)
            if live is not None:
                g = jnp.where(live, g, 0.0)
            ring[GB, c * 96 + 24:c * 96 + 88, :] = pltpu.bitcast(g, U32)

        def half_dots(lhs, wv, done):
            part = {}

            def run(c, kh):
                y = _dot(lhs[:, kh * 512:(kh + 1) * 512],
                         _cols(wv, c, c + 1, kh * 512, (kh + 1) * 512))
                if kh == 0:
                    part[c] = y
                else:
                    done(y + part[c], c)

            return [functools.partial(run, c, kh) for c in range(8) for kh in range(2)]

        def p2_front(n):
            return jnp.concatenate(
                [pltpu.bitcast(ring[GB, pl.ds(c * 96 + 8 + SHIFTS[c], n), :], F32)
                 for c in range(8)], axis=1).astype(BF16)

        def p2_back(x2, h2, hs, row, n):
            x1 = jnp.concatenate([h2t[...], h2[0:n - 16]], axis=0) + hs
            x2w = jnp.concatenate([x2t[...], x2[0:n - 16]], axis=0)
            zv[pl.ds(pl.multiple_of(row, 16), n), :] = x2w + mod_rows(5, n) * x1
            ttv[pl.ds(pl.multiple_of(row // 2, 8), n // 2), :] = _pack(_ln(x1))

        def a_body(j, mem):
            for g in range(3):
                for c in range(8):
                    hcur[g * 8:(g + 1) * 8, c * 128:(c + 1) * 128] = (
                        ring[HB, (g * 8 + c) * 8:(g * 8 + c + 1) * 8, :])
            hb = _unpack(hcur[0:8, :])
            hac = _unpack(hcur[8:16, :]).astype(F32)
            hd = _unpack(hcur[16:24, :])
            wr = [lax.rem(LEAD // 16 + 3 * j + i, RING) for i in range(3)]
            ro0 = lax.rem(4 * j, RING)
            ro1 = ro0 + 2

            x2, h2, u = p1_front(64 * jnp.maximum(j - 1, 0))
            live = j > 0

            lhs = jnp.concatenate(
                [jnp.concatenate([mem, hac[0:8]], axis=0).astype(BF16), hb], axis=0)
            tok_a = {}

            def store0(c, y):
                tok_a[c] = y[0:8]
                ring[wr[0], c * 8:(c + 1) * 8, :] = _pack(y[8:24])

            deferred = {}

            def wo_lhs0(h, om, ot):
                deferred[h] = ot[24:32]
                return jnp.concatenate([om, ot[0:24]], axis=0)

            pend = []

            def flush():
                while pend:
                    p1_store(*pend.pop(), live)

            th = half_dots(u, w1v, lambda y, c: pend.append((y, c)))
            extras = {i: [flush, th[i - 2]] for i in range(2, 14)}
            extras[14] = [flush] + th[12:14]
            extras[15] = [flush] + th[14:16]
            out = segment(lhs, ro0, store0, wo_lhs0, extras)
            flush()
            mem = out[0:8]
            aout[0:24, :] = out[8:32]

            lhs = jnp.concatenate(
                [jnp.concatenate([mem, hac[8:16]], axis=0).astype(BF16), hd], axis=0)

            def store1(c, y):
                ring[wr[1], c * 8:(c + 1) * 8, :] = _pack(
                    jnp.concatenate([tok_a[c], y[0:8]], axis=0))
                ring[wr[2], c * 8:(c + 1) * 8, :] = _pack(y[8:24])

            def wo_lhs1(h, om, ot):
                return jnp.concatenate([om, deferred[h], ot], axis=0)

            gs = p2_front(64)
            for c in range(8):
                ring[GB, c * 96:c * 96 + 24, :] = ring[GB, c * 96 + 64:c * 96 + 88, :]
            hs = []

            def p2_fin():
                p2_back(x2, h2, jnp.concatenate(hs, axis=1), 64 * j, 64)
                x2t[...] = x2[48:64]
                h2t[...] = h2[48:64]

            th = half_dots(gs, w2v, lambda y, c: hs.append(y))
            extras = {i: [th[i]] for i in range(16)}
            extras[15].append(p2_fin)
            rn = LEAD + 48 * jnp.minimum(j + 1, NPAIR - 1)
            for g in range(3):
                extras[3 + 4 * g].append(functools.partial(h_next, rn, g))
            out = segment(lhs, ro1, store1, wo_lhs1, extras)
            aout[24:64, :] = out[8:48]
            return out[0:8]

        if "A" in phases:
            with scope("aloop"):
                lax.fori_loop(0, NPAIR, a_body, memv[...].astype(F32))
        else:
            zv[...] = jnp.zeros(zv.shape, F32)
            ttv[...] = jnp.zeros(ttv.shape, U32)

        x2, h2, u = p1_front(S - 64)
        y = _dot(u, _cols(w1v, 0, 8))
        for c in range(8):
            p1_store(y[:, c * 128:(c + 1) * 128], c, None)
        p2_back(x2, h2, _dot(p2_front(80), _cols(w2v, 0, 8)), S, 80)

        wait(w34_cps)

        def out_cp(i, slot):
            return cp(outv.at[slot], out_hbm.at[pl.ds(i * RB, RB), :],
                      SEM_OUT + slot)

        def p3_body(i, _):
            slot = i % 2

            @pl.when(i >= 2)
            def _():
                out_cp(i - 2, slot).wait()

            r0 = HALO + i * RB
            tt = _unpack(ttv[pl.ds(pl.multiple_of(r0 // 2, 8), RB // 2), :])
            ff = jnp.concatenate(
                [_gelu(_dot(tt, _cols(w3v, 4 * q, 4 * q + 4))).astype(BF16)
                 for q in range(FF // 512)], axis=1)
            y = _dot(ff, _cols(w4v, 0, 8))
            res = zv[pl.ds(pl.multiple_of(r0, 16), RB), :] + mod_rows(5, RB) * y
            outv[slot] = res.astype(BF16)
            out_cp(i, slot).start()
            return 0

        nb = S // RB
        if "B" in phases:
            with scope("p3"):
                lax.fori_loop(0, nb, p3_body, 0)
            out_cp(nb - 2, 0).wait()
            out_cp(nb - 1, 1).wait()
        else:
            outv[0] = zv[pl.ds(HALO, RB), :].astype(BF16)
            out_cp(0, 0).start()
            out_cp(0, 0).wait()

    pl.run_scoped(
        main,
        pltpu.VMEM((FF // 128, D // 2, 128), U32),
        pltpu.VMEM((8, FF // 2, 128), U32),
        pltpu.VMEM((S + HALO, D), F32),
        pltpu.VMEM(((S + HALO) // 2, D), U32),
    )


def _call(A_x, A_mem0, A_Wq, A_Wk, A_Wv, A_Wo, B_w1, B_w2, B_w3, B_w4, c, w_mod,
          phases="AB"):
    any_spec = pl.BlockSpec(memory_space=pl.ANY)
    scratch = [
        pltpu.VMEM((S, D), BF16),
        pltpu.VMEM((8, D), U32),
        pltpu.VMEM((M, D), BF16),
        pltpu.VMEM((48, D // 2, 128), U32),
        pltpu.VMEM((48, 8, 128), F32),
        pltpu.VMEM((3 * H // 2 * SL, E), U32),
        pltpu.VMEM((3 * H // 2 * SL, E), U32),
        pltpu.VMEM((8, H * E // 2, 128), U32),
        pltpu.VMEM((8, D // 2, 128), U32),
        pltpu.VMEM((8, D // 2, 128), U32),
        pltpu.VMEM((4, LEAD // 2, 256), U32),
        pltpu.VMEM((24, D), U32),
        pltpu.VMEM((RING + 2, 3 * H * 8, E), U32),
        pltpu.VMEM((64, D), F32),
        pltpu.VMEM((16, D), F32),
        pltpu.VMEM((16, D), F32),
        pltpu.VMEM((2, RB, D), BF16),
        pltpu.VMEM((80, 128), F32),
        pltpu.VMEM((1, D), BF16),
        pltpu.SemaphoreType.DMA((NSEM,)),
    ]
    out = pl.pallas_call(
        functools.partial(_kernel, phases=phases),
        in_specs=[any_spec] * 12,
        out_specs=any_spec,
        out_shape=jax.ShapeDtypeStruct((S, D), BF16),
        scratch_shapes=scratch,
        compiler_params=pltpu.CompilerParams(
            vmem_limit_bytes=126 * 1024 * 1024),
    )(A_x.reshape(S, D), A_mem0.reshape(M, D), A_Wq, A_Wk, A_Wv,
      A_Wo.reshape(H * E, D), B_w1, B_w2, B_w3, B_w4, c, w_mod)
    return out.reshape(1, S, D)


def pallas_adaLN_cond__memory_aug_recurrent_mem_tr__mixer_s_mlp__prompt_kernel(
    A_x, A_mem0, A_Wq, A_Wk, A_Wv, A_Wo, A_seg_len, B_x, B_w1, B_w2, B_w3, B_w4,
    c, w_mod,
):
    assert A_seg_len == SEG
    del B_x
    return _call(A_x, A_mem0, A_Wq, A_Wk, A_Wv, A_Wo, B_w1, B_w2, B_w3, B_w4,
                 c, w_mod)
```

```python
import contextlib
import functools

import jax
import jax.numpy as jnp
from jax import lax
import jax.experimental.pallas as pl
import jax.experimental.pallas.tpu as pltpu

F32 = jnp.float32
BF16 = jnp.bfloat16
U32 = jnp.uint32

S = 2048
D = 1024
H = 32
E = 128
M = 8
SEG = 32
FF = 3584
EPS = 1e-5

LEAD = 512
RING = 36
HB = RING
GB = RING + 1
SL = 516
HG = 16
NG = 3 * H // HG
NPAIR = S // (2 * SEG)
HALO = 80
RB = 256
SHIFTS = (-1, -1, 1, 1, -2, -2, 2, 2)

(SEM_X0, SEM_X1, SEM_C, SEM_MEM, SEM_WO, SEM_W1, SEM_W2, SEM_W3,
 SEM_W4) = range(9)
SEM_Q = 9
SEM_Q1 = 13
SEM_ST = 17
SEM_MOD = SEM_ST + NG
SEM_OUT = SEM_MOD + 6
NSEM = SEM_OUT + 2


def _ln(x):
    mu = jnp.mean(x, axis=-1, keepdims=True)
    xc = x - mu
    var = jnp.mean(xc * xc, axis=-1, keepdims=True)
    return xc * lax.rsqrt(var + EPS)


def _gelu(x):
    return jax.nn.gelu(x, approximate=True)


def _pack(x):
    return pltpu.bitcast(x.astype(BF16), U32)


def _unpack(x):
    return pltpu.bitcast(x, BF16)


def _dot(a, b):
    return jnp.dot(a, b, preferred_element_type=F32)


def _cols(ref, lo, hi, k0=0, k1=None):
    k1 = 2 * ref.shape[1] if k1 is None else k1
    return jnp.concatenate(
        [_unpack(ref[c, k0 // 2:k1 // 2, :]) for c in range(lo, hi)], axis=1)


def _kernel(x_hbm, mem_hbm, wq_hbm, wk_hbm, wv_hbm, wo_hbm, w1_hbm, w2_hbm,
            w3_hbm, w4_hbm, c_hbm, wmod_hbm, out_hbm,
            xv, scv, memv, wmodv, modv, wqa, wqb, wov, w1v, w2v,
            hv0, hcur, ring, aout, x2t, h2t, outv, fillv, cv, sems, *, phases):
    def scope(name):
        return jax.named_scope(name) if "s" in phases else contextlib.nullcontext()

    def cp(src, dst, s):
        return pltpu.make_async_copy(src, dst, sems.at[s])

    def col_copies(w_hbm, w_v, s, lo=0, hi=None):
        w32 = w_hbm.bitcast(U32)
        hi = w_v.shape[0] if hi is None else hi
        return [cp(w32.at[:, pl.ds(c * 128, 128)], w_v.at[c], s)
                for c in range(lo, hi)]

    def start(cps):
        for q in cps:
            q.start()

    def wait(cps):
        for q in cps:
            q.wait()

    c_cp = cp(c_hbm, cv, SEM_C)
    mem_cp = cp(mem_hbm, memv, SEM_MEM)
    x0_cp = cp(x_hbm.at[pl.ds(0, LEAD)], xv.at[pl.ds(0, LEAD)], SEM_X0)
    x1_cp = cp(x_hbm.at[pl.ds(LEAD, S - LEAD)], xv.at[pl.ds(LEAD, S - LEAD)],
               SEM_X1)
    wo_cps = col_copies(wo_hbm, wov, SEM_WO)
    w1_cps = col_copies(w1_hbm, w1v, SEM_W1)
    w2_cps = col_copies(w2_hbm, w2v, SEM_W2)

    def mod_rows(i, n):
        m = jnp.concatenate([modv[8 * i + c] for c in range(8)], axis=1)
        return jnp.concatenate([m] * (n // 8), axis=0)

    def mod_tiles(tiles, offs):
        w = jnp.concatenate([_unpack(wmodv[c]) for c in tiles], axis=1)
        y = _dot(_unpack(scv[...]), w)[0:8]
        ys = [y[:, u * 128:(u + 1) * 128] + o for u, o in enumerate(offs)]
        for c, v in zip(tiles, ys):
            modv[c] = v
        return ys

    wq2 = (wqa, wqb)

    def h_rows(r0, n):
        xf = xv[pl.ds(pl.multiple_of(r0, 16), n), :].astype(F32)
        return _pack(_ln(xf) * mod_rows(1, n) + mod_rows(0, n))

    def prologue(st, xn, acc):
        w_hbms = (wq_hbm, wk_hbm, wv_hbm)

        def st_src(i):
            return w_hbms[i // 2].bitcast(U32).at[:, pl.ds((i % 2) * 8, 8), :]

        def st_quarter(i, q, s):
            return cp(st_src(i).at[pl.ds(q * 256, 256)],
                      st.at[i, pl.ds(q * 256, 256)], s)

        def q_cps(q):
            w32 = wmod_hbm.bitcast(U32)
            return [cp(w32.at[:, pl.ds(pl.multiple_of(c * 128, 128), 128)],
                       wmodv.at[c], SEM_Q + q)
                    for c in (2 * q, 2 * q + 1, 8 + 2 * q, 9 + 2 * q)
                    ] + [st_quarter(0, q, SEM_Q + q)]

        def st_cp(i):
            return cp(st_src(i), st.at[i], SEM_ST + i)

        def mod_cps(i):
            return col_copies(wmod_hbm, wmodv, SEM_MOD + i, 8 * i, 8 * i + 8)

        with scope("first"):
            start([c_cp, mem_cp, x0_cp])
        for q in range(4):
            start(q_cps(q))
        start([st_quarter(1, q, SEM_Q1 + q) for q in range(4)])
        start([st_cp(2), st_cp(3)] + mod_cps(2) + [st_cp(4)] + mod_cps(3)
              + [st_cp(5)])

        r = lax.broadcasted_iota(jnp.int32, (80, 128), 0)
        k = lax.broadcasted_iota(jnp.int32, (80, 128), 1)

        def head_of(i):
            return jnp.where(i < 16, i // 8, (i - 16) // 32)

        def pos_of(i):
            return jnp.where(i < 16, i % 8, 8 + (i - 16) % 32)

        same = head_of(r) == head_of(k)
        vis = (pos_of(r) < M) | (pos_of(r) >= pos_of(k))
        fillv[...] = jnp.where(same, jnp.where(vis, 0.0, -1e9), -jnp.inf).astype(F32)
        aout[...] = jnp.zeros(aout.shape, F32)
        ring[GB] = jnp.zeros(ring.shape[1:], U32)
        x2t[...] = jnp.zeros(x2t.shape, F32)
        h2t[...] = jnp.zeros(h2t.shape, F32)

        c_cp.wait()
        cf = cv[...].astype(F32)
        scv[...] = _pack(jnp.broadcast_to(cf * jax.nn.sigmoid(cf), (16, D)))
        x0_cp.wait()

        def ln_body(i, _):
            r0 = pl.multiple_of(i * 64, 64)
            y = _ln(xv[pl.ds(r0, 64), :].astype(F32))
            for q in range(4):
                xn[q, pl.ds(r0, 64), :] = y[:, q * 256:(q + 1) * 256]
            return 0

        lax.fori_loop(0, LEAD // 64, ln_body, 0)

        def relayout(par, g, p0, n, pace=None):
            base = g * (8 * SL)
            mask = jnp.uint32(0xFFFF0000 if par else 0xFFFF)
            if pace is not None:
                mask = pace | mask
            for u in range(n):
                a = st[g, 2 * (p0 + u)]
                b = st[g, 2 * (p0 + u) + 1]
                if par == 0:
                    w = (a & mask) | (b << 16)
                else:
                    w = (a >> 16) | (b & mask)
                wq2[par][pl.ds(base + p0 + u, 8, stride=SL), :] = w

        def to_ring(y, par, s0, rc):
            for u in range(y.shape[1] // 128):
                row = pl.multiple_of((2 * (s0 + u) + par) * 8, 8)
                for b in range(16):
                    ring[rc * 16 + b, pl.ds(row, 8), :] = (
                        y[b * 8:(b + 1) * 8, u * 128:(u + 1) * 128])

        def q_body(q, _):
            wait(q_cps(q))
            m = mod_tiles([2 * q, 2 * q + 1, 8 + 2 * q, 9 + 2 * q], [0.0, 0.0, 1.0, 1.0])
            sa, ca = [jnp.concatenate([jnp.concatenate(v, axis=1)] * (LEAD // 8), axis=0)
                      for v in (m[0:2], m[2:4])]
            hv0[q] = _pack(xn[q] * ca + sa)
            relayout(0, 0, q * 128, 128)
            relayout(1, 0, q * 128, 128)

            def rc_body(rc, _):
                lhs = _unpack(hv0[q, pl.ds(pl.multiple_of(rc * 128, 128), 128), :])
                for part in range(4):
                    par, hq = part // 2, part % 2
                    w = jnp.concatenate(
                        [_unpack(wq2[par][pl.ds(pl.multiple_of(
                            (hq * 4 + u) * SL + q * 128, 4), 128), :])
                         for u in range(4)], axis=1)
                    y = _dot(lhs, w) + jnp.where(q > 0, acc[rc * 4 + part], 0.0)
                    acc[rc * 4 + part] = y
                    to_ring(_pack(y), par, hq * 4, rc)
                return 0

            lax.fori_loop(0, 2, rc_body, 0)
            return 0

        with scope("quarters"):
            lax.fori_loop(0, 4, q_body, 0)

        start(mod_cps(4) + mod_cps(5) + wo_cps + w1_cps + w2_cps + [x1_cp])

        for q in range(4):
            st_quarter(1, q, SEM_Q1 + q).wait()

            def rl_body(i, _, q=q):
                relayout(0, 1, q * 128 + i * 32, 32)
                return 0

            lax.fori_loop(0, 4, rl_body, 0)

        def lead_proj(par, s0, n, rc, rl):
            w = jnp.concatenate(
                [_unpack(wq2[par][pl.ds(pl.multiple_of((s0 + u) * SL, 4), 512), :])
                 for u in range(n)], axis=1)
            lhs = jnp.concatenate(
                [_unpack(hv0[q, rc * 128:(rc + 1) * 128, :]) for q in range(4)],
                axis=1)
            y = _pack(_dot(lhs, w))
            to_ring(y, par, s0, rc)
            zero = pltpu.bitcast(aout[0:8, 0:128], U32)
            for u in range(n):
                for b in range(16):
                    k = min(3, 512 - rl[2])
                    if k > 0:
                        relayout(rl[0], rl[1], rl[2], k,
                                 y[b * 8:(b + 1) * 8, u * 128:(u + 1) * 128] & zero)
                        rl[2] += k

        def group_body(g, _):
            rl = [1, g, 0]
            for k in range(16):
                lead_proj(0, g * 8 + k // 2, 1, k % 2, rl)

            @pl.when(g < NG - 1)
            def _():
                cp(st_src(1), st.at[g + 1], SEM_ST + g + 1).wait()

            @pl.when(g >= 2)
            def _():
                part_g = wmodv.at[pl.ds(8 * g, 8)]
                cp(part_g, part_g, SEM_MOD + g).wait()

            gn = jnp.minimum(g + 1, NG - 1)
            off = jnp.where((g == 1) | (g == 4), 1.0, 0.0).astype(F32)
            ym = {}

            def mod_half(k):
                kh = k % 2
                y = _dot(_unpack(scv[:, kh * 512:(kh + 1) * 512]),
                         _unpack(wmodv[8 * g + k // 2, kh * 256:(kh + 1) * 256, :]))
                if kh == 0:
                    ym[k // 2] = y
                else:
                    modv[8 * g + k // 2] = (y + ym[k // 2])[0:8] + off

            rl = [0, gn, 0]
            for k in range(16):
                mod_half(k)
                lead_proj(1, g * 8 + k // 2, 1, k % 2, rl)
            return 0

        with scope("groups"):
            lax.fori_loop(1, NG, group_body, 0)

    pl.run_scoped(
        prologue,
        pltpu.VMEM((NG, D, 8, E), U32),
        pltpu.VMEM((4, LEAD, 256), F32),
        pltpu.VMEM((8, 256, 512), F32),
    )

    def main(w3v, w4v, zv, ttv):
        w34_cps = col_copies(w3_hbm, w3v, SEM_W3) + col_copies(w4_hbm, w4v, SEM_W4)
        start(w34_cps)
        wait(wo_cps + w1_cps + w2_cps + [mem_cp, x1_cp])

        def h_next(r0, g):
            y = h_rows(r0 + 16 * g, 16)
            for c in range(8):
                ring[HB, (g * 8 + c) * 8:(g * 8 + c + 1) * 8, :] = (
                    y[:, c * 128:(c + 1) * 128])

        for g in range(3):
            h_next(LEAD, g)

        scale = float(E) ** -0.5

        def segment(lhs, ro, store_tok, wo_lhs, extras):
            fill = fillv[...]
            keep = fill == 0.0
            NP = H // 2
            qkv, probs, blocks = {}, {}, []

            def proj(hp):
                slots = [t * H + 2 * hp + par for t in range(3) for par in range(2)]
                w = jnp.concatenate(
                    [_unpack(wq2[sl % 2][pl.ds((sl // 2) * SL, 512), :])
                     for sl in slots], axis=1)
                if hp == 0:
                    y = _dot(lhs[:, :512], w[:512])
                    y = _dot(lhs[:, 512:], w[512:]) + y
                else:
                    y = _dot(lhs, w)
                for u, sl in enumerate(slots):
                    store_tok(sl, y[8:32, u * 128:(u + 1) * 128])
                ops = []
                for t in range(3):
                    ym = jnp.concatenate(
                        [y[0:8, (2 * t) * 128:(2 * t + 1) * 128],
                         y[0:8, (2 * t + 1) * 128:(2 * t + 2) * 128]], axis=0)
                    ops.append(jnp.concatenate(
                        [ym.astype(BF16)]
                        + [_unpack(ring[ro + b, sl * 8:(sl + 1) * 8, :])
                           for sl in slots[2 * t:2 * t + 2] for b in range(2)]
                        + ([jnp.zeros((48, 128), BF16)] if t else []),
                        axis=0))
                qkv[hp] = ops

            def scores(hp):
                q, kk, _ = qkv[hp]
                s = lax.dot_general(q, kk, (((1,), (1,)), ((), ())),
                                    preferred_element_type=F32)
                s = jnp.where(keep, s * scale, fill)
                mx = jnp.max(s, axis=-1, keepdims=True)
                p = jnp.exp(s - mx)
                l = jnp.sum(p, axis=-1, keepdims=True)
                rl = pl.reciprocal(l, approx=True)
                rl = rl * (2.0 - l * rl)
                probs[hp] = (p * rl).astype(BF16)

            def pv(hp):
                o = _dot(probs[hp], qkv[hp][2])
                blocks.append(wo_lhs(2 * hp, o[0:8], o[16:48]).astype(BF16))
                blocks.append(wo_lhs(2 * hp + 1, o[8:16], o[48:80]).astype(BF16))

            def wo_part(h0, h1, acc=None):
                lw = jnp.concatenate(blocks[h0:h1], axis=1)
                y = _dot(lw, _cols(wov, 0, 8, E * h0, E * h1))
                return y if acc is None else y + acc

            for i in range(NP):
                proj(i)
                if i >= 1:
                    scores(i - 1)
                if i >= 3:
                    pv(i - 3)
                for thunk in extras.get(i, ()):
                    thunk()
            acc = wo_part(0, 4)
            scores(NP - 1)
            pv(NP - 3)
            acc = wo_part(4, 12, acc)
            pv(NP - 2)
            pv(NP - 1)
            acc = wo_part(12, 24, acc)
            acc = wo_part(24, 32, acc)
            return acc

        def p1_front(r0):
            x2 = (xv[pl.ds(pl.multiple_of(r0, 64), 64), :].astype(F32)
                  + mod_rows(2, 64) * aout[...])
            h2 = _ln(x2) * mod_rows(4, 64) + mod_rows(3, 64)
            return x2, h2, _ln(h2).astype(BF16)

        def p1_store(y, c, live):
            g = _gelu(y)
            if live is not None:
                g = jnp.where(live, g, 0.0)
            ring[GB, c * 96 + 24:c * 96 + 88, :] = pltpu.bitcast(g, U32)

        def half_dots(lhs, wv, done):
            part = {}

            def run(c, kh):
                y = _dot(lhs[:, kh * 512:(kh + 1) * 512],
                         _cols(wv, c, c + 1, kh * 512, (kh + 1) * 512))
                if kh == 0:
                    part[c] = y
                else:
                    done(y + part[c], c)

            return [functools.partial(run, c, kh) for c in range(8) for kh in range(2)]

        def p2_front(n):
            return jnp.concatenate(
                [pltpu.bitcast(ring[GB, pl.ds(c * 96 + 8 + SHIFTS[c], n), :], F32)
                 for c in range(8)], axis=1).astype(BF16)

        def p2_back(x2, h2, hs, row, n):
            x1 = jnp.concatenate([h2t[...], h2[0:n - 16]], axis=0) + hs
            x2w = jnp.concatenate([x2t[...], x2[0:n - 16]], axis=0)
            zv[pl.ds(pl.multiple_of(row, 16), n), :] = x2w + mod_rows(5, n) * x1
            ttv[pl.ds(pl.multiple_of(row // 2, 8), n // 2), :] = _pack(_ln(x1))

        def a_body(j, mem):
            for g in range(3):
                for c in range(8):
                    hcur[g * 8:(g + 1) * 8, c * 128:(c + 1) * 128] = (
                        ring[HB, (g * 8 + c) * 8:(g * 8 + c + 1) * 8, :])
            hb = _unpack(hcur[0:8, :])
            hac = _unpack(hcur[8:16, :]).astype(F32)
            hd = _unpack(hcur[16:24, :])
            wr = [lax.rem(LEAD // 16 + 3 * j + i, RING) for i in range(3)]
            ro0 = lax.rem(4 * j, RING)
            ro1 = ro0 + 2

            x2, h2, u = p1_front(64 * jnp.maximum(j - 1, 0))
            live = j > 0

            lhs = jnp.concatenate(
                [jnp.concatenate([mem, hac[0:8]], axis=0).astype(BF16), hb], axis=0)
            tok_a = {}

            def store0(c, y):
                tok_a[c] = y[0:8]
                ring[wr[0], c * 8:(c + 1) * 8, :] = _pack(y[8:24])

            deferred = {}

            def wo_lhs0(h, om, ot):
                deferred[h] = ot[24:32]
                return jnp.concatenate([om, ot[0:24]], axis=0)

            pend = []

            def flush():
                while pend:
                    p1_store(*pend.pop(), live)

            th = half_dots(u, w1v, lambda y, c: pend.append((y, c)))
            extras = {i: [flush, th[i - 2]] for i in range(2, 14)}
            extras[14] = [flush] + th[12:14]
            extras[15] = [flush] + th[14:16]
            out = segment(lhs, ro0, store0, wo_lhs0, extras)
            flush()
            mem = out[0:8]
            aout[0:24, :] = out[8:32]

            lhs = jnp.concatenate(
                [jnp.concatenate([mem, hac[8:16]], axis=0).astype(BF16), hd], axis=0)

            def store1(c, y):
                ring[wr[1], c * 8:(c + 1) * 8, :] = _pack(
                    jnp.concatenate([tok_a[c], y[0:8]], axis=0))
                ring[wr[2], c * 8:(c + 1) * 8, :] = _pack(y[8:24])

            def wo_lhs1(h, om, ot):
                return jnp.concatenate([om, deferred[h], ot], axis=0)

            gs = p2_front(64)
            for c in range(8):
                ring[GB, c * 96:c * 96 + 24, :] = ring[GB, c * 96 + 64:c * 96 + 88, :]
            hs = []

            def p2_fin():
                p2_back(x2, h2, jnp.concatenate(hs, axis=1), 64 * j, 64)
                x2t[...] = x2[48:64]
                h2t[...] = h2[48:64]

            th = half_dots(gs, w2v, lambda y, c: hs.append(y))
            extras = {i: [th[i]] for i in range(16)}
            extras[15].append(p2_fin)
            rn = LEAD + 48 * jnp.minimum(j + 1, NPAIR - 1)
            for g in range(3):
                extras[3 + 4 * g].append(functools.partial(h_next, rn, g))
            out = segment(lhs, ro1, store1, wo_lhs1, extras)
            aout[24:64, :] = out[8:48]
            return out[0:8]

        if "A" in phases:
            with scope("aloop"):
                lax.fori_loop(0, NPAIR, a_body, memv[...].astype(F32))
        else:
            zv[...] = jnp.zeros(zv.shape, F32)
            ttv[...] = jnp.zeros(ttv.shape, U32)

        x2, h2, u = p1_front(S - 64)
        y = _dot(u, _cols(w1v, 0, 8))
        for c in range(8):
            p1_store(y[:, c * 128:(c + 1) * 128], c, None)
        p2_back(x2, h2, _dot(p2_front(80), _cols(w2v, 0, 8)), S, 80)

        wait(w34_cps)

        def out_cp(i, slot):
            return cp(outv.at[slot], out_hbm.at[pl.ds(i * RB, RB), :],
                      SEM_OUT + slot)

        def p3_body(i, _):
            slot = i % 2

            @pl.when(i >= 2)
            def _():
                out_cp(i - 2, slot).wait()

            r0 = HALO + i * RB
            tt = _unpack(ttv[pl.ds(pl.multiple_of(r0 // 2, 8), RB // 2), :])
            ff = jnp.concatenate(
                [_gelu(_dot(tt, _cols(w3v, 4 * q, 4 * q + 4))).astype(BF16)
                 for q in range(FF // 512)], axis=1)
            y = _dot(ff, _cols(w4v, 0, 8))
            res = zv[pl.ds(pl.multiple_of(r0, 16), RB), :] + mod_rows(5, RB) * y
            outv[slot] = res.astype(BF16)
            out_cp(i, slot).start()
            return 0

        nb = S // RB
        if "B" in phases:
            with scope("p3"):
                lax.fori_loop(0, nb, p3_body, 0)
            out_cp(nb - 2, 0).wait()
            out_cp(nb - 1, 1).wait()
        else:
            outv[0] = zv[pl.ds(HALO, RB), :].astype(BF16)
            out_cp(0, 0).start()
            out_cp(0, 0).wait()

    pl.run_scoped(
        main,
        pltpu.VMEM((FF // 128, D // 2, 128), U32),
        pltpu.VMEM((8, FF // 2, 128), U32),
        pltpu.VMEM((S + HALO, D), F32),
        pltpu.VMEM(((S + HALO) // 2, D), U32),
    )


def _call(A_x, A_mem0, A_Wq, A_Wk, A_Wv, A_Wo, B_w1, B_w2, B_w3, B_w4, c, w_mod,
          phases="AB"):
    any_spec = pl.BlockSpec(memory_space=pl.ANY)
    scratch = [
        pltpu.VMEM((S, D), BF16),
        pltpu.VMEM((8, D), U32),
        pltpu.VMEM((M, D), BF16),
        pltpu.VMEM((48, D // 2, 128), U32),
        pltpu.VMEM((48, 8, 128), F32),
        pltpu.VMEM((3 * H // 2 * SL, E), U32),
        pltpu.VMEM((3 * H // 2 * SL, E), U32),
        pltpu.VMEM((8, H * E // 2, 128), U32),
        pltpu.VMEM((8, D // 2, 128), U32),
        pltpu.VMEM((8, D // 2, 128), U32),
        pltpu.VMEM((4, LEAD // 2, 256), U32),
        pltpu.VMEM((24, D), U32),
        pltpu.VMEM((RING + 2, 3 * H * 8, E), U32),
        pltpu.VMEM((64, D), F32),
        pltpu.VMEM((16, D), F32),
        pltpu.VMEM((16, D), F32),
        pltpu.VMEM((2, RB, D), BF16),
        pltpu.VMEM((80, 128), F32),
        pltpu.VMEM((1, D), BF16),
        pltpu.SemaphoreType.DMA((NSEM,)),
    ]
    out = pl.pallas_call(
        functools.partial(_kernel, phases=phases),
        in_specs=[any_spec] * 12,
        out_specs=any_spec,
        out_shape=jax.ShapeDtypeStruct((S, D), BF16),
        scratch_shapes=scratch,
        compiler_params=pltpu.CompilerParams(
            vmem_limit_bytes=126 * 1024 * 1024),
    )(A_x.reshape(S, D), A_mem0.reshape(M, D), A_Wq, A_Wk, A_Wv,
      A_Wo.reshape(H * E, D), B_w1, B_w2, B_w3, B_w4, c, w_mod)
    return out.reshape(1, S, D)


def pallas_adaLN_cond__memory_aug_recurrent_mem_tr__mixer_s_mlp__prompt_kernel(
    A_x, A_mem0, A_Wq, A_Wk, A_Wv, A_Wo, A_seg_len, B_x, B_w1, B_w2, B_w3, B_w4,
    c, w_mod,
):
    assert A_seg_len == SEG
    del B_x
    return _call(A_x, A_mem0, A_Wq, A_Wk, A_Wv, A_Wo, B_w1, B_w2, B_w3, B_w4,
                 c, w_mod)
```

```python
import contextlib
import functools

import jax
import jax.numpy as jnp
from jax import lax
import jax.experimental.pallas as pl
import jax.experimental.pallas.tpu as pltpu

F32 = jnp.float32
BF16 = jnp.bfloat16
U32 = jnp.uint32

S = 2048
D = 1024
H = 32
E = 128
M = 8
SEG = 32
FF = 3584
EPS = 1e-5

LEAD = 512
RING = 36
HB = RING
GB = RING + 1
SL = 516
HG = 16
NG = 3 * H // HG
NPAIR = S // (2 * SEG)
HALO = 80
RB = 256
SHIFTS = (-1, -1, 1, 1, -2, -2, 2, 2)

(SEM_X0, SEM_X1, SEM_C, SEM_MEM, SEM_WO, SEM_W1, SEM_W2, SEM_W3,
 SEM_W4) = range(9)
SEM_Q = 9
SEM_Q1 = 13
SEM_ST = 17
SEM_MOD = SEM_ST + NG
SEM_OUT = SEM_MOD + 6
NSEM = SEM_OUT + 2


def _ln(x):
    mu = jnp.mean(x, axis=-1, keepdims=True)
    xc = x - mu
    var = jnp.mean(xc * xc, axis=-1, keepdims=True)
    return xc * lax.rsqrt(var + EPS)


def _gelu(x):
    return jax.nn.gelu(x, approximate=True)


def _pack(x):
    return pltpu.bitcast(x.astype(BF16), U32)


def _unpack(x):
    return pltpu.bitcast(x, BF16)


def _dot(a, b):
    return jnp.dot(a, b, preferred_element_type=F32)


def _cols(ref, lo, hi, k0=0, k1=None):
    k1 = 2 * ref.shape[1] if k1 is None else k1
    return jnp.concatenate(
        [_unpack(ref[c, k0 // 2:k1 // 2, :]) for c in range(lo, hi)], axis=1)


def _kernel(x_hbm, mem_hbm, wq_hbm, wk_hbm, wv_hbm, wo_hbm, w1_hbm, w2_hbm,
            w3_hbm, w4_hbm, c_hbm, wmod_hbm, out_hbm,
            xv, scv, memv, wmodv, modv, wqa, wqb, wov, w1v, w2v,
            hv0, hcur, hnext, ring, aout, x2t, h2t, zt, outv, fillv, cv, sems, *, phases):
    def scope(name):
        return jax.named_scope(name) if "s" in phases else contextlib.nullcontext()

    def cp(src, dst, s):
        return pltpu.make_async_copy(src, dst, sems.at[s])

    def col_copies(w_hbm, w_v, s, lo=0, hi=None):
        w32 = w_hbm.bitcast(U32)
        hi = w_v.shape[0] if hi is None else hi
        return [cp(w32.at[:, pl.ds(c * 128, 128)], w_v.at[c], s)
                for c in range(lo, hi)]

    def start(cps):
        for q in cps:
            q.start()

    def wait(cps):
        for q in cps:
            q.wait()

    c_cp = cp(c_hbm, cv, SEM_C)
    mem_cp = cp(mem_hbm, memv, SEM_MEM)
    x0_cp = cp(x_hbm.at[pl.ds(0, LEAD)], xv.at[pl.ds(0, LEAD)], SEM_X0)
    x1_cp = cp(x_hbm.at[pl.ds(LEAD, S - LEAD)], xv.at[pl.ds(LEAD, S - LEAD)],
               SEM_X1)
    wo_cps = col_copies(wo_hbm, wov, SEM_WO)
    w1_cps = col_copies(w1_hbm, w1v, SEM_W1)
    w2_cps = col_copies(w2_hbm, w2v, SEM_W2)

    def mod_rows(i, n):
        m = jnp.concatenate([modv[8 * i + c] for c in range(8)], axis=1)
        return jnp.concatenate([m] * (n // 8), axis=0)

    def mod_tiles(tiles, offs):
        w = jnp.concatenate([_unpack(wmodv[c]) for c in tiles], axis=1)
        y = _dot(_unpack(scv[...]), w)[0:8]
        ys = [y[:, u * 128:(u + 1) * 128] + o for u, o in enumerate(offs)]
        for c, v in zip(tiles, ys):
            modv[c] = v
        return ys

    wq2 = (wqa, wqb)

    def paced(x, tiles):
        z = [pltpu.bitcast((t if t.dtype == U32 else pltpu.bitcast(t, U32))
                           & zt[0:8, :], F32) for t in tiles]
        z = jnp.concatenate(z, axis=0)
        return jnp.concatenate([x[:, 0:128] + z, x[:, 128:]], axis=1)

    def h_rows(r0, n, tiles=None):
        xf = xv[pl.ds(pl.multiple_of(r0, 16), n), :].astype(F32)
        if tiles is not None:
            xf = paced(xf, tiles)
        return _ln(xf) * mod_rows(1, n) + mod_rows(0, n)

    def prologue(st, xn, acc):
        w_hbms = (wq_hbm, wk_hbm, wv_hbm)

        def st_src(i):
            return w_hbms[i // 2].bitcast(U32).at[:, pl.ds((i % 2) * 8, 8), :]

        def st_quarter(i, q, s):
            return cp(st_src(i).at[pl.ds(q * 256, 256)],
                      st.at[i, pl.ds(q * 256, 256)], s)

        def q_cps(q):
            w32 = wmod_hbm.bitcast(U32)
            return [cp(w32.at[:, pl.ds(pl.multiple_of(c * 128, 128), 128)],
                       wmodv.at[c], SEM_Q + q)
                    for c in (2 * q, 2 * q + 1, 8 + 2 * q, 9 + 2 * q)
                    ] + [st_quarter(0, q, SEM_Q + q)]

        def st_cp(i):
            return cp(st_src(i), st.at[i], SEM_ST + i)

        def mod_cps(i):
            return col_copies(wmod_hbm, wmodv, SEM_MOD + i, 8 * i, 8 * i + 8)

        with scope("first"):
            start([c_cp, mem_cp, x0_cp])
        for q in range(4):
            start(q_cps(q))
        start([st_quarter(1, q, SEM_Q1 + q) for q in range(4)])
        start([st_cp(2), st_cp(3)] + mod_cps(2) + [st_cp(4)] + mod_cps(3)
              + [st_cp(5)])

        r = lax.broadcasted_iota(jnp.int32, (80, 128), 0)
        k = lax.broadcasted_iota(jnp.int32, (80, 128), 1)

        def head_of(i):
            return jnp.where(i < 16, i // 8, (i - 16) // 32)

        def pos_of(i):
            return jnp.where(i < 16, i % 8, 8 + (i - 16) % 32)

        same = head_of(r) == head_of(k)
        vis = (pos_of(r) < M) | (pos_of(r) >= pos_of(k))
        fillv[...] = jnp.where(same, jnp.where(vis, 0.0, -1e9), -jnp.inf).astype(F32)
        aout[...] = jnp.zeros(aout.shape, F32)
        ring[GB] = jnp.zeros(ring.shape[1:], U32)
        zt[...] = jnp.zeros(zt.shape, U32)
        x2t[...] = jnp.zeros(x2t.shape, F32)
        h2t[...] = jnp.zeros(h2t.shape, F32)

        c_cp.wait()
        cf = cv[...].astype(F32)
        scv[...] = _pack(jnp.broadcast_to(cf * jax.nn.sigmoid(cf), (16, D)))
        x0_cp.wait()

        def ln_body(i, _):
            r0 = pl.multiple_of(i * 64, 64)
            y = _ln(xv[pl.ds(r0, 64), :].astype(F32))
            for q in range(4):
                xn[q, pl.ds(r0, 64), :] = y[:, q * 256:(q + 1) * 256]
            return 0

        lax.fori_loop(0, LEAD // 64, ln_body, 0)

        def relayout(par, g, p0, n, pace=None):
            base = g * (8 * SL)
            mask = jnp.uint32(0xFFFF0000 if par else 0xFFFF)
            if pace is not None:
                mask = pace | mask
            for u in range(n):
                a = st[g, 2 * (p0 + u)]
                b = st[g, 2 * (p0 + u) + 1]
                if par == 0:
                    w = (a & mask) | (b << 16)
                else:
                    w = (a >> 16) | (b & mask)
                wq2[par][pl.ds(base + p0 + u, 8, stride=SL), :] = w

        def to_ring(y, par, s0, rc):
            for u in range(y.shape[1] // 128):
                row = pl.multiple_of((2 * (s0 + u) + par) * 8, 8)
                for b in range(16):
                    ring[rc * 16 + b, pl.ds(row, 8), :] = (
                        y[b * 8:(b + 1) * 8, u * 128:(u + 1) * 128])

        def q_body(q, _):
            wait(q_cps(q))
            m = mod_tiles([2 * q, 2 * q + 1, 8 + 2 * q, 9 + 2 * q], [0.0, 0.0, 1.0, 1.0])
            sa, ca = [jnp.concatenate([jnp.concatenate(v, axis=1)] * (LEAD // 8), axis=0)
                      for v in (m[0:2], m[2:4])]
            hv0[q] = _pack(xn[q] * ca + sa)
            relayout(0, 0, q * 128, 128)
            relayout(1, 0, q * 128, 128)

            def rc_body(rc, _):
                lhs = _unpack(hv0[q, pl.ds(pl.multiple_of(rc * 128, 128), 128), :])
                for part in range(4):
                    par, hq = part // 2, part % 2
                    w = jnp.concatenate(
                        [_unpack(wq2[par][pl.ds(pl.multiple_of(
                            (hq * 4 + u) * SL + q * 128, 4), 128), :])
                         for u in range(4)], axis=1)
                    y = _dot(lhs, w) + jnp.where(q > 0, acc[rc * 4 + part], 0.0)
                    acc[rc * 4 + part] = y
                    to_ring(_pack(y), par, hq * 4, rc)
                return 0

            lax.fori_loop(0, 2, rc_body, 0)
            return 0

        with scope("quarters"):
            lax.fori_loop(0, 4, q_body, 0)

        start(mod_cps(4) + mod_cps(5) + wo_cps + w1_cps + w2_cps + [x1_cp])

        for q in range(4):
            st_quarter(1, q, SEM_Q1 + q).wait()

            def rl_body(i, _, q=q):
                relayout(0, 1, q * 128 + i * 32, 32)
                return 0

            lax.fori_loop(0, 4, rl_body, 0)

        def lead_proj(par, s0, n, rc, rl):
            w = jnp.concatenate(
                [_unpack(wq2[par][pl.ds(pl.multiple_of((s0 + u) * SL, 4), 512), :])
                 for u in range(n)], axis=1)
            lhs = jnp.concatenate(
                [_unpack(hv0[q, rc * 128:(rc + 1) * 128, :]) for q in range(4)],
                axis=1)
            y = _pack(_dot(lhs, w))
            to_ring(y, par, s0, rc)
            zero = zt[0:8, :]
            for u in range(n):
                for b in range(16):
                    k = min(3, 512 - rl[2])
                    if k > 0:
                        relayout(rl[0], rl[1], rl[2], k,
                                 y[b * 8:(b + 1) * 8, u * 128:(u + 1) * 128] & zero)
                        rl[2] += k

        def group_body(g, _):
            rl = [1, g, 0]
            for k in range(16):
                lead_proj(0, g * 8 + k // 2, 1, k % 2, rl)

            @pl.when(g < NG - 1)
            def _():
                cp(st_src(1), st.at[g + 1], SEM_ST + g + 1).wait()

            @pl.when(g >= 2)
            def _():
                part_g = wmodv.at[pl.ds(8 * g, 8)]
                cp(part_g, part_g, SEM_MOD + g).wait()

            gn = jnp.minimum(g + 1, NG - 1)
            off = jnp.where((g == 1) | (g == 4), 1.0, 0.0).astype(F32)
            ym = {}

            def mod_half(k):
                kh = k % 2
                y = _dot(_unpack(scv[:, kh * 512:(kh + 1) * 512]),
                         _unpack(wmodv[8 * g + k // 2, kh * 256:(kh + 1) * 256, :]))
                if kh == 0:
                    ym[k // 2] = y
                else:
                    modv[8 * g + k // 2] = (y + ym[k // 2])[0:8] + off

            rl = [0, gn, 0]
            for k in range(16):
                mod_half(k)
                lead_proj(1, g * 8 + k // 2, 1, k % 2, rl)
            return 0

        with scope("groups"):
            lax.fori_loop(1, NG, group_body, 0)

    pl.run_scoped(
        prologue,
        pltpu.VMEM((NG, D, 8, E), U32),
        pltpu.VMEM((4, LEAD, 256), F32),
        pltpu.VMEM((8, 256, 512), F32),
    )

    def main(w3v, w4v, zv, ttv):
        w34_cps = col_copies(w3_hbm, w3v, SEM_W3) + col_copies(w4_hbm, w4v, SEM_W4)
        start(w34_cps)
        wait(wo_cps + w1_cps + w2_cps + [mem_cp, x1_cp])

        def h_next(r0, g, tile=None):
            y = h_rows(r0 + 16 * g, 16, tile)
            hnext[g * 8:(g + 1) * 8, :] = _pack(y)
            return [y[0:8, 896:1024], y[8:16, 896:1024]]

        for g in range(3):
            h_next(LEAD, g)

        scale = float(E) ** -0.5

        def segment(lhs, ro, store_tok, wo_lhs, extras):
            fill = fillv[...]
            keep = fill == 0.0
            NP = H // 2
            qkv, probs, blocks = {}, {}, []

            def proj(hp):
                slots = [t * H + 2 * hp + par for t in range(3) for par in range(2)]
                w = jnp.concatenate(
                    [_unpack(wq2[sl % 2][pl.ds((sl // 2) * SL, 512), :])
                     for sl in slots], axis=1)
                if hp == 0:
                    y = _dot(lhs[:, :512], w[:512])
                    y = _dot(lhs[:, 512:], w[512:]) + y
                else:
                    y = _dot(lhs, w)
                for u, sl in enumerate(slots):
                    store_tok(sl, y[8:32, u * 128:(u + 1) * 128])
                ops = []
                for t in range(3):
                    ym = jnp.concatenate(
                        [y[0:8, (2 * t) * 128:(2 * t + 1) * 128],
                         y[0:8, (2 * t + 1) * 128:(2 * t + 2) * 128]], axis=0)
                    ops.append(jnp.concatenate(
                        [ym.astype(BF16)]
                        + [_unpack(ring[ro + b, sl * 8:(sl + 1) * 8, :])
                           for sl in slots[2 * t:2 * t + 2] for b in range(2)]
                        + ([jnp.zeros((48, 128), BF16)] if t else []),
                        axis=0))
                qkv[hp] = ops

            def scores(hp):
                q, kk, _ = qkv[hp]
                s = lax.dot_general(q, kk, (((1,), (1,)), ((), ())),
                                    preferred_element_type=F32)
                s = jnp.where(keep, s * scale, fill)
                mx = jnp.max(s, axis=-1, keepdims=True)
                p = jnp.exp(s - mx)
                l = jnp.sum(p, axis=-1, keepdims=True)
                rl = pl.reciprocal(l, approx=True)
                rl = rl * (2.0 - l * rl)
                probs[hp] = (p * rl).astype(BF16)

            def pv(hp):
                o = _dot(probs[hp], qkv[hp][2])
                blocks.append(wo_lhs(2 * hp, o[0:8], o[16:48]).astype(BF16))
                blocks.append(wo_lhs(2 * hp + 1, o[8:16], o[48:80]).astype(BF16))

            def wo_part(h0, h1, acc=None):
                lw = jnp.concatenate(blocks[h0:h1], axis=1)
                y = _dot(lw, _cols(wov, 0, 8, E * h0, E * h1))
                return y if acc is None else y + acc

            for i in range(NP):
                proj(i)
                if i >= 1:
                    scores(i - 1)
                if i >= 3:
                    pv(i - 3)
                for thunk in extras.get(i, ()):
                    thunk()
            acc1 = wo_part(0, 4)
            scores(NP - 1)
            pv(NP - 3)
            acc2 = wo_part(4, 12, acc1)
            pv(NP - 2)
            pv(NP - 1)
            acc3 = wo_part(12, 24, acc2)
            if "wo" in extras:
                extras["wo"]([a[0:8, c * 128:(c + 1) * 128] for a, c in (
                    (acc1, 7), (acc2, 3), (acc2, 7), (acc3, 1), (acc3, 3), (acc3, 5),
                    (acc3, 7))])
            return wo_part(24, 32, acc3)

        def p1_front(r0):
            x2 = (xv[pl.ds(pl.multiple_of(r0, 64), 64), :].astype(F32)
                  + mod_rows(2, 64) * aout[...])
            h2 = _ln(x2) * mod_rows(4, 64) + mod_rows(3, 64)
            return x2, h2, _ln(h2).astype(BF16)

        def p1_store(y, c, live):
            g = _gelu(y)
            if live is not None:
                g = jnp.where(live, g, 0.0)
            ring[GB, c * 96 + 24:c * 96 + 88, :] = pltpu.bitcast(g, U32)

        def half_dots(lhs, wv, done):
            part = {}

            def run(c, kh):
                y = _dot(lhs[:, kh * 512:(kh + 1) * 512],
                         _cols(wv, c, c + 1, kh * 512, (kh + 1) * 512))
                if kh == 0:
                    part[c] = y
                else:
                    done(y + part[c], c)

            return [functools.partial(run, c, kh) for c in range(8) for kh in range(2)]

        def p2_front(n):
            return jnp.concatenate(
                [pltpu.bitcast(ring[GB, pl.ds(c * 96 + 8 + SHIFTS[c], n), :], F32)
                 for c in range(8)], axis=1).astype(BF16)

        def p2_back(x2, h2, hs, row, n, tiles=None):
            x1 = jnp.concatenate([h2t[...], h2[0:n - 16]], axis=0) + hs
            x2w = jnp.concatenate([x2t[...], x2[0:n - 16]], axis=0)
            zv[pl.ds(pl.multiple_of(row, 16), n), :] = x2w + mod_rows(5, n) * x1
            if tiles is None:
                ttv[pl.ds(pl.multiple_of(row // 2, 8), n // 2), :] = _pack(_ln(x1))
                return None
            t = tiles
            for g in range(n // 16):
                y = _ln(paced(x1[16 * g:16 * g + 16], t))
                ttv[pl.ds(pl.multiple_of(row // 2 + 8 * g, 8), 8), :] = _pack(y)
                t = [y[0:8, 896:1024], y[8:16, 896:1024]]
            return t

        def a_body(j, mem):
            hcur[...] = hnext[...]
            hb = _unpack(hcur[0:8, :])
            hac = _unpack(hcur[8:16, :]).astype(F32)
            hd = _unpack(hcur[16:24, :])
            wr = [lax.rem(LEAD // 16 + 3 * j + i, RING) for i in range(3)]
            ro0 = lax.rem(4 * j, RING)
            ro1 = ro0 + 2

            x2, h2, u = p1_front(64 * jnp.maximum(j - 1, 0))
            live = j > 0

            lhs = jnp.concatenate(
                [jnp.concatenate([mem, hac[0:8]], axis=0).astype(BF16), hb], axis=0)
            tok_a = {}

            def store0(c, y):
                tok_a[c] = y[0:8]
                ring[wr[0], c * 8:(c + 1) * 8, :] = _pack(y[8:24])

            deferred = {}

            def wo_lhs0(h, om, ot):
                deferred[h] = ot[24:32]
                return jnp.concatenate([om, ot[0:24]], axis=0)

            pend = []

            gst = {}

            def flush():
                while pend:
                    y, c = pend.pop()
                    p1_store(y, c, live)
                    gst[c] = pltpu.bitcast(
                        ring[GB, pl.ds(c * 96 + 8 + SHIFTS[c], 64), :], F32).astype(BF16)
                    ring[GB, c * 96:c * 96 + 24, :] = ring[GB, c * 96 + 64:c * 96 + 88, :]

            th = half_dots(u, w1v, lambda y, c: pend.append((y, c)))
            extras = {i: [flush, th[i - 2]] for i in range(2, 14)}
            extras[14] = [flush] + th[12:14]
            extras[15] = [flush] + th[14:16]
            out = segment(lhs, ro0, store0, wo_lhs0, extras)
            flush()
            mem = out[0:8]
            aout[0:24, :] = out[8:32]

            lhs = jnp.concatenate(
                [jnp.concatenate([mem, hac[8:16]], axis=0).astype(BF16), hd], axis=0)

            def store1(c, y):
                ring[wr[1], c * 8:(c + 1) * 8, :] = _pack(
                    jnp.concatenate([tok_a[c], y[0:8]], axis=0))
                ring[wr[2], c * 8:(c + 1) * 8, :] = _pack(y[8:24])

            def wo_lhs1(h, om, ot):
                return jnp.concatenate([om, deferred[h], ot], axis=0)

            gs = jnp.concatenate([gst[c] for c in range(8)], axis=1)
            hs = []

            def p2_fin(tiles):
                t = [hs[7][0:8], hs[7][0:8]]
                for g in range(3):
                    t = h_next(rn, g, t)
                p2_back(x2, h2, jnp.concatenate(hs, axis=1), 64 * j, 64, t)
                x2t[...] = x2[48:64]
                h2t[...] = h2[48:64]

            th = half_dots(gs, w2v, lambda y, c: hs.append(y))
            extras = {i: [th[i]] for i in range(16)}
            extras["wo"] = p2_fin
            rn = LEAD + 48 * jnp.minimum(j + 1, NPAIR - 1)
            out = segment(lhs, ro1, store1, wo_lhs1, extras)
            aout[24:64, :] = out[8:48]
            return out[0:8]

        if "A" in phases:
            with scope("aloop"):
                lax.fori_loop(0, NPAIR, a_body, memv[...].astype(F32))
        else:
            zv[...] = jnp.zeros(zv.shape, F32)
            ttv[...] = jnp.zeros(ttv.shape, U32)

        x2, h2, u = p1_front(S - 64)
        y = _dot(u, _cols(w1v, 0, 8))
        for c in range(8):
            p1_store(y[:, c * 128:(c + 1) * 128], c, None)
        p2_back(x2, h2, _dot(p2_front(80), _cols(w2v, 0, 8)), S, 80)

        wait(w34_cps)

        def out_cp(i, slot):
            return cp(outv.at[slot], out_hbm.at[pl.ds(i * RB, RB), :],
                      SEM_OUT + slot)

        def p3_body(i, _):
            slot = i % 2

            @pl.when(i >= 2)
            def _():
                out_cp(i - 2, slot).wait()

            r0 = HALO + i * RB
            tt = _unpack(ttv[pl.ds(pl.multiple_of(r0 // 2, 8), RB // 2), :])
            ff = jnp.concatenate(
                [_gelu(_dot(tt, _cols(w3v, 4 * q, 4 * q + 4))).astype(BF16)
                 for q in range(FF // 512)], axis=1)
            y = _dot(ff, _cols(w4v, 0, 8))
            res = zv[pl.ds(pl.multiple_of(r0, 16), RB), :] + mod_rows(5, RB) * y
            outv[slot] = res.astype(BF16)
            out_cp(i, slot).start()
            return 0

        nb = S // RB
        if "B" in phases:
            with scope("p3"):
                lax.fori_loop(0, nb, p3_body, 0)
            out_cp(nb - 2, 0).wait()
            out_cp(nb - 1, 1).wait()
        else:
            outv[0] = zv[pl.ds(HALO, RB), :].astype(BF16)
            out_cp(0, 0).start()
            out_cp(0, 0).wait()

    pl.run_scoped(
        main,
        pltpu.VMEM((FF // 128, D // 2, 128), U32),
        pltpu.VMEM((8, FF // 2, 128), U32),
        pltpu.VMEM((S + HALO, D), F32),
        pltpu.VMEM(((S + HALO) // 2, D), U32),
    )


def _call(A_x, A_mem0, A_Wq, A_Wk, A_Wv, A_Wo, B_w1, B_w2, B_w3, B_w4, c, w_mod,
          phases="AB"):
    any_spec = pl.BlockSpec(memory_space=pl.ANY)
    scratch = [
        pltpu.VMEM((S, D), BF16),
        pltpu.VMEM((8, D), U32),
        pltpu.VMEM((M, D), BF16),
        pltpu.VMEM((48, D // 2, 128), U32),
        pltpu.VMEM((48, 8, 128), F32),
        pltpu.VMEM((3 * H // 2 * SL, E), U32),
        pltpu.VMEM((3 * H // 2 * SL, E), U32),
        pltpu.VMEM((8, H * E // 2, 128), U32),
        pltpu.VMEM((8, D // 2, 128), U32),
        pltpu.VMEM((8, D // 2, 128), U32),
        pltpu.VMEM((4, LEAD // 2, 256), U32),
        pltpu.VMEM((24, D), U32),
        pltpu.VMEM((24, D), U32),
        pltpu.VMEM((RING + 2, 3 * H * 8, E), U32),
        pltpu.VMEM((64, D), F32),
        pltpu.VMEM((16, D), F32),
        pltpu.VMEM((16, D), F32),
        pltpu.VMEM((32, 128), U32),
        pltpu.VMEM((2, RB, D), BF16),
        pltpu.VMEM((80, 128), F32),
        pltpu.VMEM((1, D), BF16),
        pltpu.SemaphoreType.DMA((NSEM,)),
    ]
    out = pl.pallas_call(
        functools.partial(_kernel, phases=phases),
        in_specs=[any_spec] * 12,
        out_specs=any_spec,
        out_shape=jax.ShapeDtypeStruct((S, D), BF16),
        scratch_shapes=scratch,
        compiler_params=pltpu.CompilerParams(
            vmem_limit_bytes=126 * 1024 * 1024),
    )(A_x.reshape(S, D), A_mem0.reshape(M, D), A_Wq, A_Wk, A_Wv,
      A_Wo.reshape(H * E, D), B_w1, B_w2, B_w3, B_w4, c, w_mod)
    return out.reshape(1, S, D)


def pallas_adaLN_cond__memory_aug_recurrent_mem_tr__mixer_s_mlp__prompt_kernel(
    A_x, A_mem0, A_Wq, A_Wk, A_Wv, A_Wo, A_seg_len, B_x, B_w1, B_w2, B_w3, B_w4,
    c, w_mod,
):
    assert A_seg_len == SEG
    del B_x
    return _call(A_x, A_mem0, A_Wq, A_Wk, A_Wv, A_Wo, B_w1, B_w2, B_w3, B_w4,
                 c, w_mod)
```

```python
import contextlib
import functools

import jax
import jax.numpy as jnp
from jax import lax
import jax.experimental.pallas as pl
import jax.experimental.pallas.tpu as pltpu

F32 = jnp.float32
BF16 = jnp.bfloat16
U32 = jnp.uint32

S = 2048
D = 1024
H = 32
E = 128
M = 8
SEG = 32
FF = 3584
EPS = 1e-5

LEAD = 512
RING = 36
GB = RING
SL = 516
HG = 16
NG = 3 * H // HG
NPAIR = S // (2 * SEG)
HALO = 80
RB = 256
SHIFTS = (-1, -1, 1, 1, -2, -2, 2, 2)

(SEM_X0, SEM_X1, SEM_C, SEM_MEM, SEM_WO, SEM_W1, SEM_W2, SEM_W3,
 SEM_W4) = range(9)
SEM_Q = 9
SEM_Q1 = 13
SEM_ST = 17
SEM_MOD = SEM_ST + NG
SEM_OUT = SEM_MOD + 6
NSEM = SEM_OUT + 2


def _ln(x):
    mu = jnp.mean(x, axis=-1, keepdims=True)
    xc = x - mu
    var = jnp.mean(xc * xc, axis=-1, keepdims=True)
    return xc * lax.rsqrt(var + EPS)


def _gelu(x):
    return jax.nn.gelu(x, approximate=True)


def _pack(x):
    return pltpu.bitcast(x.astype(BF16), U32)


def _unpack(x):
    return pltpu.bitcast(x, BF16)


def _dot(a, b):
    return jnp.dot(a, b, preferred_element_type=F32)


def _cols(ref, lo, hi, k0=0, k1=None):
    k1 = 2 * ref.shape[1] if k1 is None else k1
    return jnp.concatenate(
        [_unpack(ref[c, k0 // 2:k1 // 2, :]) for c in range(lo, hi)], axis=1)


def _kernel(x_hbm, mem_hbm, wq_hbm, wk_hbm, wv_hbm, wo_hbm, w1_hbm, w2_hbm,
            w3_hbm, w4_hbm, c_hbm, wmod_hbm, out_hbm,
            xv, scv, memv, wmodv, modv, wqa, wqb, wov, w1v, w2v,
            hv0, hcur, hnext, ring, aout, x2t, h2t, zt, outv, fillv, cv, sems, *, phases):
    def scope(name):
        return jax.named_scope(name) if "s" in phases else contextlib.nullcontext()

    def cp(src, dst, s):
        return pltpu.make_async_copy(src, dst, sems.at[s])

    def col_copies(w_hbm, w_v, s, lo=0, hi=None):
        w32 = w_hbm.bitcast(U32)
        hi = w_v.shape[0] if hi is None else hi
        return [cp(w32.at[:, pl.ds(c * 128, 128)], w_v.at[c], s)
                for c in range(lo, hi)]

    def start(cps):
        for q in cps:
            q.start()

    def wait(cps):
        for q in cps:
            q.wait()

    c_cp = cp(c_hbm, cv, SEM_C)
    mem_cp = cp(mem_hbm, memv, SEM_MEM)
    x0_cp = cp(x_hbm.at[pl.ds(0, LEAD)], xv.at[pl.ds(0, LEAD)], SEM_X0)
    x1_cp = cp(x_hbm.at[pl.ds(LEAD, S - LEAD)], xv.at[pl.ds(LEAD, S - LEAD)],
               SEM_X1)
    wo_cps = col_copies(wo_hbm, wov, SEM_WO)
    w1_cps = col_copies(w1_hbm, w1v, SEM_W1)
    w2_cps = col_copies(w2_hbm, w2v, SEM_W2)

    def mod_rows(i, n):
        m = jnp.concatenate([modv[8 * i + c] for c in range(8)], axis=1)
        return jnp.concatenate([m] * (n // 8), axis=0)

    def mod_tiles(tiles, offs):
        w = jnp.concatenate([_unpack(wmodv[c]) for c in tiles], axis=1)
        y = _dot(_unpack(scv[...]), w)[0:8]
        ys = [y[:, u * 128:(u + 1) * 128] + o for u, o in enumerate(offs)]
        for c, v in zip(tiles, ys):
            modv[c] = v
        return ys

    wq2 = (wqa, wqb)

    def paced(x, tiles):
        z = [pltpu.bitcast((t if t.dtype == U32 else pltpu.bitcast(t, U32))
                           & zt[0:8, :], F32) for t in tiles]
        z = jnp.concatenate(z, axis=0)
        return jnp.concatenate([x[:, 0:128] + z, x[:, 128:]], axis=1)

    def h_rows(r0, n, tiles=None):
        xf = xv[pl.ds(pl.multiple_of(r0, 16), n), :].astype(F32)
        if tiles is not None:
            xf = paced(xf, tiles)
        return _ln(xf) * mod_rows(1, n) + mod_rows(0, n)

    def prologue(st, xn, acc):
        w_hbms = (wq_hbm, wk_hbm, wv_hbm)

        def st_src(i):
            return w_hbms[i // 2].bitcast(U32).at[:, pl.ds((i % 2) * 8, 8), :]

        def st_quarter(i, q, s):
            return cp(st_src(i).at[pl.ds(q * 256, 256)],
                      st.at[i, pl.ds(q * 256, 256)], s)

        def q_cps(q):
            w32 = wmod_hbm.bitcast(U32)
            return [cp(w32.at[:, pl.ds(pl.multiple_of(c * 128, 128), 128)],
                       wmodv.at[c], SEM_Q + q)
                    for c in (2 * q, 2 * q + 1, 8 + 2 * q, 9 + 2 * q)
                    ] + [st_quarter(0, q, SEM_Q + q)]

        def st_cp(i):
            return cp(st_src(i), st.at[i], SEM_ST + i)

        def mod_cps(i):
            return col_copies(wmod_hbm, wmodv, SEM_MOD + i, 8 * i, 8 * i + 8)

        with scope("first"):
            start([c_cp, mem_cp, x0_cp])
        for q in range(4):
            start(q_cps(q))
        start([st_quarter(1, q, SEM_Q1 + q) for q in range(4)])
        start([st_cp(2), st_cp(3)] + mod_cps(2) + [st_cp(4)] + mod_cps(3)
              + [st_cp(5)])

        r = lax.broadcasted_iota(jnp.int32, (80, 128), 0)
        k = lax.broadcasted_iota(jnp.int32, (80, 128), 1)

        def head_of(i):
            return jnp.where(i < 16, i // 8, (i - 16) // 32)

        def pos_of(i):
            return jnp.where(i < 16, i % 8, 8 + (i - 16) % 32)

        same = head_of(r) == head_of(k)
        vis = (pos_of(r) < M) | (pos_of(r) >= pos_of(k))
        fillv[...] = jnp.where(same, jnp.where(vis, 0.0, -1e9), -jnp.inf).astype(F32)
        aout[...] = jnp.zeros(aout.shape, F32)
        ring[GB] = jnp.zeros(ring.shape[1:], U32)
        zt[...] = jnp.zeros(zt.shape, U32)
        x2t[...] = jnp.zeros(x2t.shape, F32)
        h2t[...] = jnp.zeros(h2t.shape, F32)

        c_cp.wait()
        cf = cv[...].astype(F32)
        scv[...] = _pack(jnp.broadcast_to(cf * jax.nn.sigmoid(cf), (16, D)))
        x0_cp.wait()

        def ln_body(i, _):
            r0 = pl.multiple_of(i * 64, 64)
            y = _ln(xv[pl.ds(r0, 64), :].astype(F32))
            for q in range(4):
                xn[q, pl.ds(r0, 64), :] = y[:, q * 256:(q + 1) * 256]
            return 0

        lax.fori_loop(0, LEAD // 64, ln_body, 0)

        def relayout(par, g, p0, n, pace=None):
            base = g * (8 * SL)
            mask = jnp.uint32(0xFFFF0000 if par else 0xFFFF)
            if pace is not None:
                mask = pace | mask
            for u in range(n):
                a = st[g, 2 * (p0 + u)]
                b = st[g, 2 * (p0 + u) + 1]
                if par == 0:
                    w = (a & mask) | (b << 16)
                else:
                    w = (a >> 16) | (b & mask)
                wq2[par][pl.ds(base + p0 + u, 8, stride=SL), :] = w

        def to_ring(y, par, s0, rc):
            for u in range(y.shape[1] // 128):
                row = pl.multiple_of((2 * (s0 + u) + par) * 8, 8)
                for b in range(16):
                    ring[rc * 16 + b, pl.ds(row, 8), :] = (
                        y[b * 8:(b + 1) * 8, u * 128:(u + 1) * 128])

        def q_body(q, _):
            wait(q_cps(q))
            m = mod_tiles([2 * q, 2 * q + 1, 8 + 2 * q, 9 + 2 * q], [0.0, 0.0, 1.0, 1.0])
            sa, ca = [jnp.concatenate([jnp.concatenate(v, axis=1)] * (LEAD // 8), axis=0)
                      for v in (m[0:2], m[2:4])]
            hv0[q] = _pack(xn[q] * ca + sa)
            relayout(0, 0, q * 128, 128)
            relayout(1, 0, q * 128, 128)

            def rc_body(rc, _):
                lhs = _unpack(hv0[q, pl.ds(pl.multiple_of(rc * 128, 128), 128), :])
                for part in range(4):
                    par, hq = part // 2, part % 2
                    w = jnp.concatenate(
                        [_unpack(wq2[par][pl.ds(pl.multiple_of(
                            (hq * 4 + u) * SL + q * 128, 4), 128), :])
                         for u in range(4)], axis=1)
                    y = _dot(lhs, w) + jnp.where(q > 0, acc[rc * 4 + part], 0.0)
                    acc[rc * 4 + part] = y
                    to_ring(_pack(y), par, hq * 4, rc)
                return 0

            lax.fori_loop(0, 2, rc_body, 0)
            return 0

        with scope("quarters"):
            lax.fori_loop(0, 4, q_body, 0)

        start(mod_cps(4) + mod_cps(5) + wo_cps + w1_cps + w2_cps + [x1_cp])

        for q in range(4):
            st_quarter(1, q, SEM_Q1 + q).wait()

            def rl_body(i, _, q=q):
                relayout(0, 1, q * 128 + i * 32, 32)
                return 0

            lax.fori_loop(0, 4, rl_body, 0)

        def lead_proj(par, s0, n, rc, rl):
            w = jnp.concatenate(
                [_unpack(wq2[par][pl.ds(pl.multiple_of((s0 + u) * SL, 4), 512), :])
                 for u in range(n)], axis=1)
            lhs = jnp.concatenate(
                [_unpack(hv0[q, rc * 128:(rc + 1) * 128, :]) for q in range(4)],
                axis=1)
            y = _pack(_dot(lhs, w))
            to_ring(y, par, s0, rc)
            zero = zt[0:8, :]
            for u in range(n):
                for b in range(16):
                    k = min(3, 512 - rl[2])
                    if k > 0:
                        relayout(rl[0], rl[1], rl[2], k,
                                 y[b * 8:(b + 1) * 8, u * 128:(u + 1) * 128] & zero)
                        rl[2] += k

        def group_body(g, _):
            rl = [1, g, 0]
            for k in range(16):
                lead_proj(0, g * 8 + k // 2, 1, k % 2, rl)

            @pl.when(g < NG - 1)
            def _():
                cp(st_src(1), st.at[g + 1], SEM_ST + g + 1).wait()

            @pl.when(g >= 2)
            def _():
                part_g = wmodv.at[pl.ds(8 * g, 8)]
                cp(part_g, part_g, SEM_MOD + g).wait()

            gn = jnp.minimum(g + 1, NG - 1)
            off = jnp.where((g == 1) | (g == 4), 1.0, 0.0).astype(F32)
            ym = {}

            def mod_half(k):
                kh = k % 2
                y = _dot(_unpack(scv[:, kh * 512:(kh + 1) * 512]),
                         _unpack(wmodv[8 * g + k // 2, kh * 256:(kh + 1) * 256, :]))
                if kh == 0:
                    ym[k // 2] = y
                else:
                    modv[8 * g + k // 2] = (y + ym[k // 2])[0:8] + off

            rl = [0, gn, 0]
            for k in range(16):
                mod_half(k)
                lead_proj(1, g * 8 + k // 2, 1, k % 2, rl)
            return 0

        with scope("groups"):
            lax.fori_loop(1, NG, group_body, 0)

    pl.run_scoped(
        prologue,
        pltpu.VMEM((NG, D, 8, E), U32),
        pltpu.VMEM((4, LEAD, 256), F32),
        pltpu.VMEM((8, 256, 512), F32),
    )

    def main(w3v, w4v, zv, ttv):
        w34_cps = col_copies(w3_hbm, w3v, SEM_W3) + col_copies(w4_hbm, w4v, SEM_W4)
        start(w34_cps)
        wait(wo_cps + w1_cps + w2_cps + [mem_cp, x1_cp])

        def h_next(r0, g, tile=None):
            y = h_rows(r0 + 16 * g, 16, tile)
            hnext[g * 8:(g + 1) * 8, :] = _pack(y)
            return [y[0:8, 896:1024], y[8:16, 896:1024]]

        for g in range(3):
            h_next(LEAD, g)

        scale = float(E) ** -0.5

        def segment(lhs, ro, store_tok, wo_lhs, extras):
            fill = fillv[...]
            keep = fill == 0.0
            NP = H // 2
            qkv, probs, blocks = {}, {}, []

            def proj(hp):
                slots = [t * H + 2 * hp + par for t in range(3) for par in range(2)]
                w = jnp.concatenate(
                    [_unpack(wq2[sl % 2][pl.ds((sl // 2) * SL, 512), :])
                     for sl in slots], axis=1)
                if hp == 0:
                    y = _dot(lhs[:, :512], w[:512])
                    y = _dot(lhs[:, 512:], w[512:]) + y
                else:
                    y = _dot(lhs, w)
                for u, sl in enumerate(slots):
                    store_tok(sl, y[8:32, u * 128:(u + 1) * 128])
                ops = []
                for t in range(3):
                    ym = jnp.concatenate(
                        [y[0:8, (2 * t) * 128:(2 * t + 1) * 128],
                         y[0:8, (2 * t + 1) * 128:(2 * t + 2) * 128]], axis=0)
                    ops.append(jnp.concatenate(
                        [ym.astype(BF16)]
                        + [_unpack(ring[ro + b, sl * 8:(sl + 1) * 8, :])
                           for sl in slots[2 * t:2 * t + 2] for b in range(2)]
                        + ([jnp.zeros((48, 128), BF16)] if t else []),
                        axis=0))
                qkv[hp] = ops

            def scores(hp):
                q, kk, _ = qkv[hp]
                s = lax.dot_general(q, kk, (((1,), (1,)), ((), ())),
                                    preferred_element_type=F32)
                s = jnp.where(keep, s * scale, fill)
                mx = jnp.max(s, axis=-1, keepdims=True)
                p = jnp.exp(s - mx)
                l = jnp.sum(p, axis=-1, keepdims=True)
                rl = pl.reciprocal(l, approx=True)
                rl = rl * (2.0 - l * rl)
                probs[hp] = (p * rl).astype(BF16)

            def pv(hp):
                o = _dot(probs[hp], qkv[hp][2])
                blocks.append(wo_lhs(2 * hp, o[0:8], o[16:48]).astype(BF16))
                blocks.append(wo_lhs(2 * hp + 1, o[8:16], o[48:80]).astype(BF16))

            def wo_part(h0, h1, acc=None):
                lw = jnp.concatenate(blocks[h0:h1], axis=1)
                y = _dot(lw, _cols(wov, 0, 8, E * h0, E * h1))
                return y if acc is None else y + acc

            for i in range(NP):
                proj(i)
                if i >= 1:
                    scores(i - 1)
                if i >= 3:
                    pv(i - 3)
                for thunk in extras.get(i, ()):
                    thunk()
            acc1 = wo_part(0, 4)
            scores(NP - 1)
            pv(NP - 3)
            acc2 = wo_part(4, 12, acc1)
            pv(NP - 2)
            pv(NP - 1)
            acc3 = wo_part(12, 24, acc2)
            for thunk in extras.get("wo", ()):
                thunk()
            return wo_part(24, 32, acc3)

        def p1_front(r0):
            x2 = (xv[pl.ds(pl.multiple_of(r0, 64), 64), :].astype(F32)
                  + mod_rows(2, 64) * aout[...])
            h2 = _ln(x2) * mod_rows(4, 64) + mod_rows(3, 64)
            return x2, h2, _ln(h2).astype(BF16)

        def p1_store(y, c, live):
            g = _gelu(y)
            if live is not None:
                g = jnp.where(live, g, 0.0)
            ring[GB, c * 96 + 24:c * 96 + 88, :] = pltpu.bitcast(g, U32)

        def half_dots(lhs, wv, done):
            part = {}

            def run(c, kh):
                y = _dot(lhs[:, kh * 512:(kh + 1) * 512],
                         _cols(wv, c, c + 1, kh * 512, (kh + 1) * 512))
                if kh == 0:
                    part[c] = y
                else:
                    done(y + part[c], c)

            return [functools.partial(run, c, kh) for c in range(8) for kh in range(2)]

        def p2_front(n):
            return jnp.concatenate(
                [pltpu.bitcast(ring[GB, pl.ds(c * 96 + 8 + SHIFTS[c], n), :], F32)
                 for c in range(8)], axis=1).astype(BF16)

        def p2_back(x2, h2, hs, row, n, tiles=None):
            x1 = jnp.concatenate([h2t[...], h2[0:n - 16]], axis=0) + hs
            x2w = jnp.concatenate([x2t[...], x2[0:n - 16]], axis=0)
            zv[pl.ds(pl.multiple_of(row, 16), n), :] = x2w + mod_rows(5, n) * x1
            if tiles is None:
                ttv[pl.ds(pl.multiple_of(row // 2, 8), n // 2), :] = _pack(_ln(x1))
                return None
            t = tiles
            for g in range(n // 16):
                y = _ln(paced(x1[16 * g:16 * g + 16], t))
                ttv[pl.ds(pl.multiple_of(row // 2 + 8 * g, 8), 8), :] = _pack(y)
                t = [y[0:8, 896:1024], y[8:16, 896:1024]]
            return t

        def a_body(j, mem):
            hcur[...] = hnext[...]
            hb = _unpack(hcur[0:8, :])
            hac = _unpack(hcur[8:16, :]).astype(F32)
            hd = _unpack(hcur[16:24, :])
            wr = [lax.rem(LEAD // 16 + 3 * j + i, RING) for i in range(3)]
            ro0 = lax.rem(4 * j, RING)
            ro1 = ro0 + 2

            x2, h2, u = p1_front(64 * jnp.maximum(j - 1, 0))
            live = j > 0

            lhs = jnp.concatenate(
                [jnp.concatenate([mem, hac[0:8]], axis=0).astype(BF16), hb], axis=0)
            tok_a = {}

            def store0(c, y):
                tok_a[c] = y[0:8]
                ring[wr[0], c * 8:(c + 1) * 8, :] = _pack(y[8:24])

            deferred = {}

            def wo_lhs0(h, om, ot):
                deferred[h] = ot[24:32]
                return jnp.concatenate([om, ot[0:24]], axis=0)

            pend = []

            def flush():
                while pend:
                    p1_store(*pend.pop(), live)

            th = half_dots(u, w1v, lambda y, c: pend.append((y, c)))
            extras = {i: [flush, th[i - 2]] for i in range(2, 14)}
            extras[14] = [flush] + th[12:14]
            extras[15] = [flush] + th[14:16]
            out = segment(lhs, ro0, store0, wo_lhs0, extras)
            flush()
            mem = out[0:8]
            aout[0:24, :] = out[8:32]

            lhs = jnp.concatenate(
                [jnp.concatenate([mem, hac[8:16]], axis=0).astype(BF16), hd], axis=0)

            def store1(c, y):
                ring[wr[1], c * 8:(c + 1) * 8, :] = _pack(
                    jnp.concatenate([tok_a[c], y[0:8]], axis=0))
                ring[wr[2], c * 8:(c + 1) * 8, :] = _pack(y[8:24])

            def wo_lhs1(h, om, ot):
                return jnp.concatenate([om, deferred[h], ot], axis=0)

            gs = p2_front(64)
            for c in range(8):
                ring[GB, c * 96:c * 96 + 24, :] = ring[GB, c * 96 + 64:c * 96 + 88, :]
            hs = []

            def p2_fin():
                t = [hs[7][0:8], hs[7][0:8]]
                for g in range(3):
                    t = h_next(rn, g, t)
                p2_back(x2, h2, jnp.concatenate(hs, axis=1), 64 * j, 64, t)
                x2t[...] = x2[48:64]
                h2t[...] = h2[48:64]

            th = half_dots(gs, w2v, lambda y, c: hs.append(y))
            extras = {i: [th[i]] for i in range(16)}
            extras["wo"] = [p2_fin]
            rn = LEAD + 48 * jnp.minimum(j + 1, NPAIR - 1)
            out = segment(lhs, ro1, store1, wo_lhs1, extras)
            aout[24:64, :] = out[8:48]
            return out[0:8]

        if "A" in phases:
            with scope("aloop"):
                lax.fori_loop(0, NPAIR, a_body, memv[...].astype(F32))
        else:
            zv[...] = jnp.zeros(zv.shape, F32)
            ttv[...] = jnp.zeros(ttv.shape, U32)

        x2, h2, u = p1_front(S - 64)
        y = _dot(u, _cols(w1v, 0, 8))
        for c in range(8):
            p1_store(y[:, c * 128:(c + 1) * 128], c, None)
        p2_back(x2, h2, _dot(p2_front(80), _cols(w2v, 0, 8)), S, 80)

        wait(w34_cps)

        def out_cp(i, slot):
            return cp(outv.at[slot], out_hbm.at[pl.ds(i * RB, RB), :],
                      SEM_OUT + slot)

        def p3_body(i, _):
            slot = i % 2

            @pl.when(i >= 2)
            def _():
                out_cp(i - 2, slot).wait()

            r0 = HALO + i * RB
            tt = _unpack(ttv[pl.ds(pl.multiple_of(r0 // 2, 8), RB // 2), :])
            ff = jnp.concatenate(
                [_gelu(_dot(tt, _cols(w3v, 4 * q, 4 * q + 4))).astype(BF16)
                 for q in range(FF // 512)], axis=1)
            y = _dot(ff, _cols(w4v, 0, 8))
            res = zv[pl.ds(pl.multiple_of(r0, 16), RB), :] + mod_rows(5, RB) * y
            outv[slot] = res.astype(BF16)
            out_cp(i, slot).start()
            return 0

        nb = S // RB
        if "B" in phases:
            with scope("p3"):
                lax.fori_loop(0, nb, p3_body, 0)
            out_cp(nb - 2, 0).wait()
            out_cp(nb - 1, 1).wait()
        else:
            outv[0] = zv[pl.ds(HALO, RB), :].astype(BF16)
            out_cp(0, 0).start()
            out_cp(0, 0).wait()

    pl.run_scoped(
        main,
        pltpu.VMEM((FF // 128, D // 2, 128), U32),
        pltpu.VMEM((8, FF // 2, 128), U32),
        pltpu.VMEM((S + HALO, D), F32),
        pltpu.VMEM(((S + HALO) // 2, D), U32),
    )


def _call(A_x, A_mem0, A_Wq, A_Wk, A_Wv, A_Wo, B_w1, B_w2, B_w3, B_w4, c, w_mod,
          phases="AB"):
    any_spec = pl.BlockSpec(memory_space=pl.ANY)
    scratch = [
        pltpu.VMEM((S, D), BF16),
        pltpu.VMEM((8, D), U32),
        pltpu.VMEM((M, D), BF16),
        pltpu.VMEM((48, D // 2, 128), U32),
        pltpu.VMEM((48, 8, 128), F32),
        pltpu.VMEM((3 * H // 2 * SL, E), U32),
        pltpu.VMEM((3 * H // 2 * SL, E), U32),
        pltpu.VMEM((8, H * E // 2, 128), U32),
        pltpu.VMEM((8, D // 2, 128), U32),
        pltpu.VMEM((8, D // 2, 128), U32),
        pltpu.VMEM((4, LEAD // 2, 256), U32),
        pltpu.VMEM((24, D), U32),
        pltpu.VMEM((24, D), U32),
        pltpu.VMEM((RING + 1, 3 * H * 8, E), U32),
        pltpu.VMEM((64, D), F32),
        pltpu.VMEM((16, D), F32),
        pltpu.VMEM((16, D), F32),
        pltpu.VMEM((32, 128), U32),
        pltpu.VMEM((2, RB, D), BF16),
        pltpu.VMEM((80, 128), F32),
        pltpu.VMEM((1, D), BF16),
        pltpu.SemaphoreType.DMA((NSEM,)),
    ]
    out = pl.pallas_call(
        functools.partial(_kernel, phases=phases),
        in_specs=[any_spec] * 12,
        out_specs=any_spec,
        out_shape=jax.ShapeDtypeStruct((S, D), BF16),
        scratch_shapes=scratch,
        compiler_params=pltpu.CompilerParams(
            vmem_limit_bytes=126 * 1024 * 1024),
    )(A_x.reshape(S, D), A_mem0.reshape(M, D), A_Wq, A_Wk, A_Wv,
      A_Wo.reshape(H * E, D), B_w1, B_w2, B_w3, B_w4, c, w_mod)
    return out.reshape(1, S, D)


def pallas_adaLN_cond__memory_aug_recurrent_mem_tr__mixer_s_mlp__prompt_kernel(
    A_x, A_mem0, A_Wq, A_Wk, A_Wv, A_Wo, A_seg_len, B_x, B_w1, B_w2, B_w3, B_w4,
    c, w_mod,
):
    assert A_seg_len == SEG
    del B_x
    return _call(A_x, A_mem0, A_Wq, A_Wk, A_Wv, A_Wo, B_w1, B_w2, B_w3, B_w4,
                 c, w_mod)
```

```python
import contextlib
import functools

import jax
import jax.numpy as jnp
from jax import lax
import jax.experimental.pallas as pl
import jax.experimental.pallas.tpu as pltpu

F32 = jnp.float32
BF16 = jnp.bfloat16
U32 = jnp.uint32

S = 2048
D = 1024
H = 32
E = 128
M = 8
SEG = 32
FF = 3584
EPS = 1e-5

LEAD = 512
RING = 36
GB = RING
SL = 516
HG = 16
NG = 3 * H // HG
NPAIR = S // (2 * SEG)
HALO = 80
RB = 256
SHIFTS = (-1, -1, 1, 1, -2, -2, 2, 2)

SEM_IN = 0
SEM_A = 1
SEM_B = 2
SEM_Q = 3
SEM_Q1 = 7
SEM_G = 10
SEM_OUT = 16
NSEM = 18


def _ln(x):
    mu = jnp.mean(x, axis=-1, keepdims=True)
    xc = x - mu
    var = jnp.mean(xc * xc, axis=-1, keepdims=True)
    return xc * lax.rsqrt(var + EPS)


def _gelu(x):
    return jax.nn.gelu(x, approximate=True)


def _pack(x):
    return pltpu.bitcast(x.astype(BF16), U32)


def _unpack(x):
    return pltpu.bitcast(x, BF16)


def _dot(a, b):
    return jnp.dot(a, b, preferred_element_type=F32)


def _cols(ref, lo, hi, k0=0, k1=None):
    k1 = 2 * ref.shape[1] if k1 is None else k1
    return jnp.concatenate(
        [_unpack(ref[c, k0 // 2:k1 // 2, :]) for c in range(lo, hi)], axis=1)


def _kernel(x_hbm, mem_hbm, wq_hbm, wk_hbm, wv_hbm, wo_hbm, w1_hbm, w2_hbm,
            w3_hbm, w4_hbm, c_hbm, wmod_hbm, out_hbm,
            xv, scv, memv, wmodv, modv, wqa, wqb, wov, w1v, w2v,
            hv0, hcur, hnext, ring, aout, x2t, h2t, zt, outv, fillv, cv, sems, *, phases):
    def scope(name):
        return jax.named_scope(name) if "s" in phases else contextlib.nullcontext()

    def cp(src, dst, s):
        return pltpu.make_async_copy(src, dst, sems.at[s])

    def col_copies(w_hbm, w_v, s, lo=0, hi=None):
        w32 = w_hbm.bitcast(U32)
        hi = w_v.shape[0] if hi is None else hi
        return [cp(w32.at[:, pl.ds(c * 128, 128)], w_v.at[c], s)
                for c in range(lo, hi)]

    def start(cps):
        for q in cps:
            q.start()

    def wait(cps):
        for q in cps:
            q.wait()

    def x_cp(r0, n, s):
        return cp(x_hbm.at[pl.ds(r0, n)], xv.at[pl.ds(r0, n)], s)

    in_cps = [cp(c_hbm, cv, SEM_IN), cp(mem_hbm, memv, SEM_IN),
              x_cp(0, LEAD, SEM_IN)]
    xw_cp = x_cp(LEAD, 48, SEM_G + 1)
    a_cps = (col_copies(wo_hbm, wov, SEM_A) + col_copies(w1_hbm, w1v, SEM_A)
             + col_copies(w2_hbm, w2v, SEM_A)
             + [x_cp(LEAD + 48, S - LEAD - 48, SEM_A)])

    def mod_rows(i, n):
        m = jnp.concatenate([modv[8 * i + c] for c in range(8)], axis=1)
        return jnp.concatenate([m] * (n // 8), axis=0)

    def mod_tiles(tiles, offs):
        w = jnp.concatenate([_unpack(wmodv[c]) for c in tiles], axis=1)
        y = _dot(_unpack(scv[...]), w)[0:8]
        ys = [y[:, u * 128:(u + 1) * 128] + o for u, o in enumerate(offs)]
        for c, v in zip(tiles, ys):
            modv[c] = v
        return ys

    wq2 = (wqa, wqb)

    def paced(x, tiles):
        z = [pltpu.bitcast((t if t.dtype == U32 else pltpu.bitcast(t, U32))
                           & zt[0:8, :], F32) for t in tiles]
        z = jnp.concatenate(z, axis=0)
        return jnp.concatenate([x[:, 0:128] + z, x[:, 128:]], axis=1)

    def h_rows(r0, n, tiles=None):
        xf = xv[pl.ds(pl.multiple_of(r0, 16), n), :].astype(F32)
        if tiles is not None:
            xf = paced(xf, tiles)
        return _ln(xf) * mod_rows(1, n) + mod_rows(0, n)

    def h_next(r0, g, tile=None):
        y = h_rows(r0 + 16 * g, 16, tile)
        hnext[g * 8:(g + 1) * 8, :] = _pack(y)
        return [y[0:8, 896:1024], y[8:16, 896:1024]]

    def prologue(st, xn, acc):
        w_hbms = (wq_hbm, wk_hbm, wv_hbm)

        def st_src(i):
            return w_hbms[i // 2].bitcast(U32).at[:, pl.ds((i % 2) * 8, 8), :]

        def st_quarter(i, q, s):
            return cp(st_src(i).at[pl.ds(q * 256, 256)],
                      st.at[i, pl.ds(q * 256, 256)], s)

        def q_cps(q):
            w32 = wmod_hbm.bitcast(U32)
            return [cp(w32.at[:, pl.ds(pl.multiple_of(c * 128, 128), 128)],
                       wmodv.at[c], SEM_Q + q)
                    for c in (2 * q, 2 * q + 1, 8 + 2 * q, 9 + 2 * q)
                    ] + [st_quarter(0, q, SEM_Q + q)]

        def st_cp(i):
            return cp(st_src(i), st.at[i], SEM_G + i - 1)

        def mod_cps(i):
            return col_copies(wmod_hbm, wmodv, SEM_G + i, 8 * i, 8 * i + 8)

        with scope("first"):
            start(in_cps)
        for q in range(4):
            start(q_cps(q))
        start([st_quarter(1, q, SEM_Q1 + q) for q in range(4)])
        start([xw_cp, st_cp(2), st_cp(3)] + mod_cps(2) + [st_cp(4)] + mod_cps(3)
              + [st_cp(5)])

        r = lax.broadcasted_iota(jnp.int32, (80, 128), 0)
        k = lax.broadcasted_iota(jnp.int32, (80, 128), 1)

        def head_of(i):
            return jnp.where(i < 16, i // 8, (i - 16) // 32)

        def pos_of(i):
            return jnp.where(i < 16, i % 8, 8 + (i - 16) % 32)

        same = head_of(r) == head_of(k)
        vis = (pos_of(r) < M) | (pos_of(r) >= pos_of(k))
        fillv[...] = jnp.where(same, jnp.where(vis, 0.0, -1e9), -jnp.inf).astype(F32)
        aout[...] = jnp.zeros(aout.shape, F32)
        ring[GB] = jnp.zeros(ring.shape[1:], U32)
        zt[...] = jnp.zeros(zt.shape, U32)
        x2t[...] = jnp.zeros(x2t.shape, F32)
        h2t[...] = jnp.zeros(h2t.shape, F32)

        wait(in_cps)
        cf = cv[...].astype(F32)
        scv[...] = _pack(jnp.broadcast_to(cf * jax.nn.sigmoid(cf), (16, D)))

        def ln_body(i, _):
            r0 = pl.multiple_of(i * 64, 64)
            y = _ln(xv[pl.ds(r0, 64), :].astype(F32))
            for q in range(4):
                xn[q, pl.ds(r0, 64), :] = y[:, q * 256:(q + 1) * 256]
            return 0

        lax.fori_loop(0, LEAD // 64, ln_body, 0)

        def relayout(par, g, p0, n, pace=None):
            base = g * (8 * SL)
            mask = jnp.uint32(0xFFFF0000 if par else 0xFFFF)
            if pace is not None:
                mask = pace | mask
            for u in range(n):
                a = st[g, 2 * (p0 + u)]
                b = st[g, 2 * (p0 + u) + 1]
                if par == 0:
                    w = (a & mask) | (b << 16)
                else:
                    w = (a >> 16) | (b & mask)
                wq2[par][pl.ds(base + p0 + u, 8, stride=SL), :] = w

        def to_ring(y, par, s0, rc):
            for u in range(y.shape[1] // 128):
                row = pl.multiple_of((2 * (s0 + u) + par) * 8, 8)
                for b in range(16):
                    ring[rc * 16 + b, pl.ds(row, 8), :] = (
                        y[b * 8:(b + 1) * 8, u * 128:(u + 1) * 128])

        def q_body(q, _):
            wait(q_cps(q))
            m = mod_tiles([2 * q, 2 * q + 1, 8 + 2 * q, 9 + 2 * q], [0.0, 0.0, 1.0, 1.0])
            sa, ca = [jnp.concatenate([jnp.concatenate(v, axis=1)] * (LEAD // 8), axis=0)
                      for v in (m[0:2], m[2:4])]
            hv0[q] = _pack(xn[q] * ca + sa)
            relayout(0, 0, q * 128, 128)
            relayout(1, 0, q * 128, 128)

            def rc_body(rc, _):
                lhs = _unpack(hv0[q, pl.ds(pl.multiple_of(rc * 128, 128), 128), :])
                for part in range(4):
                    par, hq = part // 2, part % 2
                    w = jnp.concatenate(
                        [_unpack(wq2[par][pl.ds(pl.multiple_of(
                            (hq * 4 + u) * SL + q * 128, 4), 128), :])
                         for u in range(4)], axis=1)
                    y = _dot(lhs, w) + jnp.where(q > 0, acc[rc * 4 + part], 0.0)
                    acc[rc * 4 + part] = y
                    to_ring(_pack(y), par, hq * 4, rc)
                return 0

            lax.fori_loop(0, 2, rc_body, 0)
            return 0

        with scope("quarters"):
            lax.fori_loop(0, 4, q_body, 0)

        start(mod_cps(4) + mod_cps(5) + a_cps)

        for q in range(4):
            st_quarter(1, q, SEM_Q1 + q).wait()

            def rl_body(i, _, q=q):
                relayout(0, 1, q * 128 + i * 32, 32)
                return 0

            lax.fori_loop(0, 4, rl_body, 0)

        def lead_proj(par, s0, n, rc, rl):
            w = jnp.concatenate(
                [_unpack(wq2[par][pl.ds(pl.multiple_of((s0 + u) * SL, 4), 512), :])
                 for u in range(n)], axis=1)
            lhs = jnp.concatenate(
                [_unpack(hv0[q, rc * 128:(rc + 1) * 128, :]) for q in range(4)],
                axis=1)
            y = _pack(_dot(lhs, w))
            to_ring(y, par, s0, rc)
            zero = zt[0:8, :]
            for u in range(n):
                for b in range(16):
                    k = min(3, 512 - rl[2])
                    if k > 0:
                        relayout(rl[0], rl[1], rl[2], k,
                                 y[b * 8:(b + 1) * 8, u * 128:(u + 1) * 128] & zero)
                        rl[2] += k
            return y

        def group_body(g, _):
            rl = [1, g, 0]
            for k in range(16):
                lead_proj(0, g * 8 + k // 2, 1, k % 2, rl)

            @pl.when(g < NG - 1)
            def _():
                cp(st_src(1), st.at[g + 1], SEM_G + g).wait()

            @pl.when(g == 1)
            def _():
                xw_cp.wait()

            @pl.when(g >= 2)
            def _():
                part_g = wmodv.at[pl.ds(8 * g, 8)]
                cp(part_g, part_g, SEM_G + g).wait()

            gn = jnp.minimum(g + 1, NG - 1)
            off = jnp.where((g == 1) | (g == 4), 1.0, 0.0).astype(F32)
            ym = {}

            def mod_half(k):
                kh = k % 2
                y = _dot(_unpack(scv[:, kh * 512:(kh + 1) * 512]),
                         _unpack(wmodv[8 * g + k // 2, kh * 256:(kh + 1) * 256, :]))
                if kh == 0:
                    ym[k // 2] = y
                else:
                    modv[8 * g + k // 2] = (y + ym[k // 2])[0:8] + off

            rl = [0, gn, 0]
            for k in range(16):
                mod_half(k)
                y = lead_proj(1, g * 8 + k // 2, 1, k % 2, rl)
                if k == 11:
                    t = [y[0:8], y[64:72]]
                    for i in range(3):
                        t = h_next(LEAD, i, t)
            return 0

        with scope("groups"):
            lax.fori_loop(1, NG, group_body, 0)

    pl.run_scoped(
        prologue,
        pltpu.VMEM((NG, D, 8, E), U32),
        pltpu.VMEM((4, LEAD, 256), F32),
        pltpu.VMEM((8, 256, 512), F32),
    )

    def main(w3v, w4v, zv, ttv):
        w34_cps = col_copies(w3_hbm, w3v, SEM_B) + col_copies(w4_hbm, w4v, SEM_B)
        start(w34_cps)
        wait(a_cps)

        scale = float(E) ** -0.5

        def segment(lhs, ro, store_tok, wo_lhs, extras):
            fill = fillv[...]
            keep = fill == 0.0
            NP = H // 2
            qkv, probs, blocks = {}, {}, []

            def proj(hp):
                slots = [t * H + 2 * hp + par for t in range(3) for par in range(2)]
                w = jnp.concatenate(
                    [_unpack(wq2[sl % 2][pl.ds((sl // 2) * SL, 512), :])
                     for sl in slots], axis=1)
                if hp == 0:
                    y = _dot(lhs[:, :512], w[:512])
                    y = _dot(lhs[:, 512:], w[512:]) + y
                else:
                    y = _dot(lhs, w)
                for u, sl in enumerate(slots):
                    store_tok(sl, y[8:32, u * 128:(u + 1) * 128])
                ops = []
                for t in range(3):
                    ym = jnp.concatenate(
                        [y[0:8, (2 * t) * 128:(2 * t + 1) * 128],
                         y[0:8, (2 * t + 1) * 128:(2 * t + 2) * 128]], axis=0)
                    ops.append(jnp.concatenate(
                        [ym.astype(BF16)]
                        + [_unpack(ring[ro + b, sl * 8:(sl + 1) * 8, :])
                           for sl in slots[2 * t:2 * t + 2] for b in range(2)]
                        + ([jnp.zeros((48, 128), BF16)] if t else []),
                        axis=0))
                qkv[hp] = ops

            def scores(hp):
                q, kk, _ = qkv[hp]
                s = lax.dot_general(q, kk, (((1,), (1,)), ((), ())),
                                    preferred_element_type=F32)
                s = jnp.where(keep, s * scale, fill)
                mx = jnp.max(s, axis=-1, keepdims=True)
                p = jnp.exp(s - mx)
                l = jnp.sum(p, axis=-1, keepdims=True)
                rl = pl.reciprocal(l, approx=True)
                rl = rl * (2.0 - l * rl)
                probs[hp] = (p * rl).astype(BF16)

            def pv(hp):
                o = _dot(probs[hp], qkv[hp][2])
                blocks.append(wo_lhs(2 * hp, o[0:8], o[16:48]).astype(BF16))
                blocks.append(wo_lhs(2 * hp + 1, o[8:16], o[48:80]).astype(BF16))

            def wo_part(h0, h1, acc=None):
                lw = jnp.concatenate(blocks[h0:h1], axis=1)
                y = _dot(lw, _cols(wov, 0, 8, E * h0, E * h1))
                return y if acc is None else y + acc

            for i in range(NP):
                proj(i)
                if i >= 1:
                    scores(i - 1)
                if i >= 3:
                    pv(i - 3)
                for thunk in extras.get(i, ()):
                    thunk()
            acc1 = wo_part(0, 4)
            scores(NP - 1)
            pv(NP - 3)
            acc2 = wo_part(4, 12, acc1)
            pv(NP - 2)
            pv(NP - 1)
            acc3 = wo_part(12, 24, acc2)
            for thunk in extras.get("wo", ()):
                thunk()
            return wo_part(24, 32, acc3)

        def p1_front(r0):
            x2 = (xv[pl.ds(pl.multiple_of(r0, 64), 64), :].astype(F32)
                  + mod_rows(2, 64) * aout[...])
            h2 = _ln(x2) * mod_rows(4, 64) + mod_rows(3, 64)
            return x2, h2, _ln(h2).astype(BF16)

        def p1_store(y, c, live):
            g = _gelu(y)
            if live is not None:
                g = jnp.where(live, g, 0.0)
            ring[GB, c * 96 + 24:c * 96 + 88, :] = pltpu.bitcast(g, U32)

        def half_dots(lhs, wv, done):
            part = {}

            def run(c, kh):
                y = _dot(lhs[:, kh * 512:(kh + 1) * 512],
                         _cols(wv, c, c + 1, kh * 512, (kh + 1) * 512))
                if kh == 0:
                    part[c] = y
                else:
                    done(y + part[c], c)

            return [functools.partial(run, c, kh) for c in range(8) for kh in range(2)]

        def p2_front(n):
            return jnp.concatenate(
                [pltpu.bitcast(ring[GB, pl.ds(c * 96 + 8 + SHIFTS[c], n), :], F32)
                 for c in range(8)], axis=1).astype(BF16)

        def p2_back(x2, h2, hs, row, n, tiles=None):
            x1 = jnp.concatenate([h2t[...], h2[0:n - 16]], axis=0) + hs
            x2w = jnp.concatenate([x2t[...], x2[0:n - 16]], axis=0)
            zv[pl.ds(pl.multiple_of(row, 16), n), :] = x2w + mod_rows(5, n) * x1
            if tiles is None:
                ttv[pl.ds(pl.multiple_of(row // 2, 8), n // 2), :] = _pack(_ln(x1))
                return None
            t = tiles
            for g in range(n // 16):
                y = _ln(paced(x1[16 * g:16 * g + 16], t))
                ttv[pl.ds(pl.multiple_of(row // 2 + 8 * g, 8), 8), :] = _pack(y)
                t = [y[0:8, 896:1024], y[8:16, 896:1024]]
            return t

        def a_body(j, mem):
            hcur[...] = hnext[...]
            hb = _unpack(hcur[0:8, :])
            hac = _unpack(hcur[8:16, :]).astype(F32)
            hd = _unpack(hcur[16:24, :])
            wr = [lax.rem(LEAD // 16 + 3 * j + i, RING) for i in range(3)]
            ro0 = lax.rem(4 * j, RING)
            ro1 = ro0 + 2

            x2, h2, u = p1_front(64 * jnp.maximum(j - 1, 0))
            live = j > 0

            lhs = jnp.concatenate(
                [jnp.concatenate([mem, hac[0:8]], axis=0).astype(BF16), hb], axis=0)
            tok_a = {}

            def store0(c, y):
                tok_a[c] = y[0:8]
                ring[wr[0], c * 8:(c + 1) * 8, :] = _pack(y[8:24])

            deferred = {}

            def wo_lhs0(h, om, ot):
                deferred[h] = ot[24:32]
                return jnp.concatenate([om, ot[0:24]], axis=0)

            pend = []

            def flush():
                while pend:
                    p1_store(*pend.pop(), live)

            th = half_dots(u, w1v, lambda y, c: pend.append((y, c)))
            extras = {i: [flush, th[i - 2]] for i in range(2, 14)}
            extras[14] = [flush] + th[12:14]
            extras[15] = [flush] + th[14:16]
            out = segment(lhs, ro0, store0, wo_lhs0, extras)
            flush()
            mem = out[0:8]
            aout[0:24, :] = out[8:32]

            lhs = jnp.concatenate(
                [jnp.concatenate([mem, hac[8:16]], axis=0).astype(BF16), hd], axis=0)

            def store1(c, y):
                ring[wr[1], c * 8:(c + 1) * 8, :] = _pack(
                    jnp.concatenate([tok_a[c], y[0:8]], axis=0))
                ring[wr[2], c * 8:(c + 1) * 8, :] = _pack(y[8:24])

            def wo_lhs1(h, om, ot):
                return jnp.concatenate([om, deferred[h], ot], axis=0)

            gs = p2_front(64)
            for c in range(8):
                ring[GB, c * 96:c * 96 + 24, :] = ring[GB, c * 96 + 64:c * 96 + 88, :]
            hs = []

            def p2_fin():
                t = [hs[7][0:8], hs[7][0:8]]
                for g in range(3):
                    t = h_next(rn, g, t)
                p2_back(x2, h2, jnp.concatenate(hs, axis=1), 64 * j, 64, t)
                x2t[...] = x2[48:64]
                h2t[...] = h2[48:64]

            th = half_dots(gs, w2v, lambda y, c: hs.append(y))
            extras = {i: [th[i]] for i in range(16)}
            extras["wo"] = [p2_fin]
            rn = LEAD + 48 * jnp.minimum(j + 1, NPAIR - 1)
            out = segment(lhs, ro1, store1, wo_lhs1, extras)
            aout[24:64, :] = out[8:48]
            return out[0:8]

        if "A" in phases:
            with scope("aloop"):
                lax.fori_loop(0, NPAIR, a_body, memv[...].astype(F32))
        else:
            zv[...] = jnp.zeros(zv.shape, F32)
            ttv[...] = jnp.zeros(ttv.shape, U32)

        x2, h2, u = p1_front(S - 64)
        y = _dot(u, _cols(w1v, 0, 8))
        for c in range(8):
            p1_store(y[:, c * 128:(c + 1) * 128], c, None)
        p2_back(x2, h2, _dot(p2_front(80), _cols(w2v, 0, 8)), S, 80)

        wait(w34_cps)

        def out_cp(i, slot):
            return cp(outv.at[slot], out_hbm.at[pl.ds(i * RB, RB), :],
                      SEM_OUT + slot)

        def p3_body(i, _):
            slot = i % 2

            @pl.when(i >= 2)
            def _():
                out_cp(i - 2, slot).wait()

            r0 = HALO + i * RB
            tt = _unpack(ttv[pl.ds(pl.multiple_of(r0 // 2, 8), RB // 2), :])
            ff = jnp.concatenate(
                [_gelu(_dot(tt, _cols(w3v, 4 * q, 4 * q + 4))).astype(BF16)
                 for q in range(FF // 512)], axis=1)
            gb = mod_rows(5, RB)
            for c0, c1 in ((0, 7), (7, 8)):
                cols = slice(c0 * 128, c1 * 128)
                y = _dot(ff, _cols(w4v, c0, c1))
                res = zv[pl.ds(pl.multiple_of(r0, 16), RB), cols] + gb[:, cols] * y
                outv[slot, :, cols] = res.astype(BF16)
                cp(outv.at[slot, :, cols], out_hbm.at[pl.ds(i * RB, RB), cols],
                   SEM_OUT + slot).start()
            return 0

        nb = S // RB
        if "B" in phases:
            with scope("p3"):
                lax.fori_loop(0, nb, p3_body, 0)
            out_cp(nb - 2, 0).wait()
            out_cp(nb - 1, 1).wait()
        else:
            outv[0] = zv[pl.ds(HALO, RB), :].astype(BF16)
            out_cp(0, 0).start()
            out_cp(0, 0).wait()

    pl.run_scoped(
        main,
        pltpu.VMEM((FF // 128, D // 2, 128), U32),
        pltpu.VMEM((8, FF // 2, 128), U32),
        pltpu.VMEM((S + HALO, D), F32),
        pltpu.VMEM(((S + HALO) // 2, D), U32),
    )


def _call(A_x, A_mem0, A_Wq, A_Wk, A_Wv, A_Wo, B_w1, B_w2, B_w3, B_w4, c, w_mod,
          phases="AB"):
    any_spec = pl.BlockSpec(memory_space=pl.ANY)
    scratch = [
        pltpu.VMEM((S, D), BF16),
        pltpu.VMEM((8, D), U32),
        pltpu.VMEM((M, D), BF16),
        pltpu.VMEM((48, D // 2, 128), U32),
        pltpu.VMEM((48, 8, 128), F32),
        pltpu.VMEM((3 * H // 2 * SL, E), U32),
        pltpu.VMEM((3 * H // 2 * SL, E), U32),
        pltpu.VMEM((8, H * E // 2, 128), U32),
        pltpu.VMEM((8, D // 2, 128), U32),
        pltpu.VMEM((8, D // 2, 128), U32),
        pltpu.VMEM((4, LEAD // 2, 256), U32),
        pltpu.VMEM((24, D), U32),
        pltpu.VMEM((24, D), U32),
        pltpu.VMEM((RING + 1, 3 * H * 8, E), U32),
        pltpu.VMEM((64, D), F32),
        pltpu.VMEM((16, D), F32),
        pltpu.VMEM((16, D), F32),
        pltpu.VMEM((32, 128), U32),
        pltpu.VMEM((2, RB, D), BF16),
        pltpu.VMEM((80, 128), F32),
        pltpu.VMEM((1, D), BF16),
        pltpu.SemaphoreType.DMA((NSEM,)),
    ]
    out = pl.pallas_call(
        functools.partial(_kernel, phases=phases),
        in_specs=[any_spec] * 12,
        out_specs=any_spec,
        out_shape=jax.ShapeDtypeStruct((S, D), BF16),
        scratch_shapes=scratch,
        compiler_params=pltpu.CompilerParams(
            vmem_limit_bytes=126 * 1024 * 1024),
    )(A_x.reshape(S, D), A_mem0.reshape(M, D), A_Wq, A_Wk, A_Wv,
      A_Wo.reshape(H * E, D), B_w1, B_w2, B_w3, B_w4, c, w_mod)
    return out.reshape(1, S, D)


def pallas_adaLN_cond__memory_aug_recurrent_mem_tr__mixer_s_mlp__prompt_kernel(
    A_x, A_mem0, A_Wq, A_Wk, A_Wv, A_Wo, A_seg_len, B_x, B_w1, B_w2, B_w3, B_w4,
    c, w_mod,
):
    assert A_seg_len == SEG
    del B_x
    return _call(A_x, A_mem0, A_Wq, A_Wk, A_Wv, A_Wo, B_w1, B_w2, B_w3, B_w4,
                 c, w_mod)
```

```python
import contextlib
import functools

import jax
import jax.numpy as jnp
from jax import lax
import jax.experimental.pallas as pl
import jax.experimental.pallas.tpu as pltpu

F32 = jnp.float32
BF16 = jnp.bfloat16
U32 = jnp.uint32

S = 2048
D = 1024
H = 32
E = 128
M = 8
SEG = 32
FF = 3584
EPS = 1e-5

LEAD = 512
RING = 36
GB = RING
SL = 516
HG = 16
NG = 3 * H // HG
NPAIR = S // (2 * SEG)
HALO = 80
RB = 256
SHIFTS = (-1, -1, 1, 1, -2, -2, 2, 2)

SEM_IN = 0
SEM_A = 1
SEM_B = 2
SEM_Q = 3
SEM_Q1 = 7
SEM_G = 10
SEM_OUT = 16
NSEM = 18


def _ln(x):
    mu = jnp.mean(x, axis=-1, keepdims=True)
    xc = x - mu
    var = jnp.mean(xc * xc, axis=-1, keepdims=True)
    return xc * lax.rsqrt(var + EPS)


def _gelu(x):
    return jax.nn.gelu(x, approximate=True)


def _pack(x):
    return pltpu.bitcast(x.astype(BF16), U32)


def _unpack(x):
    return pltpu.bitcast(x, BF16)


def _dot(a, b):
    return jnp.dot(a, b, preferred_element_type=F32)


def _cols(ref, lo, hi, k0=0, k1=None):
    k1 = 2 * ref.shape[1] if k1 is None else k1
    return jnp.concatenate(
        [_unpack(ref[c, k0 // 2:k1 // 2, :]) for c in range(lo, hi)], axis=1)


def _kernel(x_hbm, mem_hbm, wq_hbm, wk_hbm, wv_hbm, wo_hbm, w1_hbm, w2_hbm,
            w3_hbm, w4_hbm, c_hbm, wmod_hbm, out_hbm,
            xv, scv, memv, wmodv, modv, wqa, wqb, wov, w1v, w2v,
            hv0, hcur, hnext, ring, aout, x2t, h2t, zt, outv, fillv, cv, sems, *, phases):
    def scope(name):
        return jax.named_scope(name) if "s" in phases else contextlib.nullcontext()

    def cp(src, dst, s):
        return pltpu.make_async_copy(src, dst, sems.at[s])

    def col_copies(w_hbm, w_v, s, lo=0, hi=None):
        w32 = w_hbm.bitcast(U32)
        hi = w_v.shape[0] if hi is None else hi
        return [cp(w32.at[:, pl.ds(c * 128, 128)], w_v.at[c], s)
                for c in range(lo, hi)]

    def start(cps):
        for q in cps:
            q.start()

    def wait(cps):
        for q in cps:
            q.wait()

    def x_cp(r0, n, s):
        return cp(x_hbm.at[pl.ds(r0, n)], xv.at[pl.ds(r0, n)], s)

    in_cps = [cp(c_hbm, cv, SEM_IN), cp(mem_hbm, memv, SEM_IN),
              x_cp(0, LEAD, SEM_IN)]
    xw_cp = x_cp(LEAD, 48, SEM_G + 1)
    a_cps = (col_copies(wo_hbm, wov, SEM_A) + col_copies(w1_hbm, w1v, SEM_A)
             + col_copies(w2_hbm, w2v, SEM_A)
             + [x_cp(LEAD + 48, S - LEAD - 48, SEM_A)])

    def mod_rows(i, n):
        m = jnp.concatenate([modv[8 * i + c] for c in range(8)], axis=1)
        return jnp.concatenate([m] * (n // 8), axis=0)

    def mod_tiles(tiles, offs):
        w = jnp.concatenate([_unpack(wmodv[c]) for c in tiles], axis=1)
        y = _dot(_unpack(scv[...]), w)[0:8]
        ys = [y[:, u * 128:(u + 1) * 128] + o for u, o in enumerate(offs)]
        for c, v in zip(tiles, ys):
            modv[c] = v
        return ys

    HI = jnp.uint32(0xFFFF0000)
    wq2 = (wqa, wqb)

    def paced(x, tiles):
        z = [pltpu.bitcast((t if t.dtype == U32 else pltpu.bitcast(t, U32))
                           & zt[0:8, :], F32) for t in tiles]
        z = jnp.concatenate(z, axis=0)
        return jnp.concatenate([x[:, 0:128] + z, x[:, 128:]], axis=1)

    def h_rows(r0, n, tiles=None):
        xf = xv[pl.ds(pl.multiple_of(r0, 16), n), :].astype(F32)
        if tiles is not None:
            xf = paced(xf, tiles)
        return _ln(xf) * mod_rows(1, n) + mod_rows(0, n)

    def h_next(r0, g, tile=None):
        y = h_rows(r0 + 16 * g, 16, tile)
        hnext[g * 8:(g + 1) * 8, :] = _pack(y)
        return [y[0:8, 896:1024], y[8:16, 896:1024]]

    def prologue(st, xn, acc, scol):
        w_hbms = (wq_hbm, wk_hbm, wv_hbm)

        def st_src(i):
            return w_hbms[i // 2].bitcast(U32).at[:, pl.ds((i % 2) * 8, 8), :]

        def st_quarter(i, q, s):
            return cp(st_src(i).at[pl.ds(q * 256, 256)],
                      st.at[i, pl.ds(q * 256, 256)], s)

        def q_cps(q):
            w32 = wmod_hbm.bitcast(U32)
            return [cp(w32.at[:, pl.ds(pl.multiple_of(c * 128, 128), 128)],
                       wmodv.at[c], SEM_Q + q)
                    for c in (2 * q, 2 * q + 1, 8 + 2 * q, 9 + 2 * q)
                    ] + [st_quarter(0, q, SEM_Q + q)]

        def st_cp(i):
            return cp(st_src(i), st.at[i], SEM_G + i - 1)

        def mod_cps(i):
            return col_copies(wmod_hbm, wmodv, SEM_G + i, 8 * i, 8 * i + 8)

        with scope("first"):
            start(in_cps)
        for q in range(4):
            start(q_cps(q))
        start([st_quarter(1, q, SEM_Q1 + q) for q in range(4)])
        start([xw_cp, st_cp(2), st_cp(3)] + mod_cps(2) + [st_cp(4)] + mod_cps(3)
              + [st_cp(5)])

        r = lax.broadcasted_iota(jnp.int32, (80, 128), 0)
        k = lax.broadcasted_iota(jnp.int32, (80, 128), 1)

        def head_of(i):
            return jnp.where(i < 16, i // 8, (i - 16) // 32)

        def pos_of(i):
            return jnp.where(i < 16, i % 8, 8 + (i - 16) % 32)

        same = head_of(r) == head_of(k)
        vis = (pos_of(r) < M) | (pos_of(r) >= pos_of(k))
        fillv[...] = jnp.where(same, jnp.where(vis, 0.0, -1e9), -jnp.inf).astype(F32)
        aout[...] = jnp.zeros(aout.shape, F32)
        ring[GB] = jnp.zeros(ring.shape[1:], U32)
        zt[...] = jnp.zeros(zt.shape, U32)
        x2t[...] = jnp.zeros(x2t.shape, F32)
        h2t[...] = jnp.zeros(h2t.shape, F32)

        wait(in_cps)
        cf = cv[...].astype(F32)
        sil = cf * jax.nn.sigmoid(cf)
        scv[...] = _pack(jnp.broadcast_to(sil, (16, D)))
        for c in range(8):
            sw = _pack(jnp.broadcast_to(sil[:, c * 128:(c + 1) * 128], (128, 128)).T)
            scol[0, c * 64:(c + 1) * 64, :] = pltpu.bitcast(sw << 16, F32)
            scol[1, c * 64:(c + 1) * 64, :] = pltpu.bitcast(sw & HI, F32)

        def ln_body(i, _):
            r0 = pl.multiple_of(i * 64, 64)
            y = _ln(xv[pl.ds(r0, 64), :].astype(F32))
            for q in range(4):
                xn[q, pl.ds(r0, 64), :] = y[:, q * 256:(q + 1) * 256]
            return 0

        lax.fori_loop(0, LEAD // 64, ln_body, 0)

        def relayout(par, g, p0, n, pace=None):
            base = g * (8 * SL)
            mask = jnp.uint32(0xFFFF0000 if par else 0xFFFF)
            if pace is not None:
                mask = pace | mask
            for u in range(n):
                a = st[g, 2 * (p0 + u)]
                b = st[g, 2 * (p0 + u) + 1]
                if par == 0:
                    w = (a & mask) | (b << 16)
                else:
                    w = (a >> 16) | (b & mask)
                wq2[par][pl.ds(base + p0 + u, 8, stride=SL), :] = w

        def to_ring(y, par, s0, rc):
            for u in range(y.shape[1] // 128):
                row = pl.multiple_of((2 * (s0 + u) + par) * 8, 8)
                for b in range(16):
                    ring[rc * 16 + b, pl.ds(row, 8), :] = (
                        y[b * 8:(b + 1) * 8, u * 128:(u + 1) * 128])

        def q_body(q, _):
            wait(q_cps(q))
            m = mod_tiles([2 * q, 2 * q + 1, 8 + 2 * q, 9 + 2 * q], [0.0, 0.0, 1.0, 1.0])
            sa, ca = [jnp.concatenate([jnp.concatenate(v, axis=1)] * (LEAD // 8), axis=0)
                      for v in (m[0:2], m[2:4])]
            hv0[q] = _pack(xn[q] * ca + sa)
            relayout(0, 0, q * 128, 128)
            relayout(1, 0, q * 128, 128)

            def rc_body(rc, _):
                lhs = _unpack(hv0[q, pl.ds(pl.multiple_of(rc * 128, 128), 128), :])
                for part in range(4):
                    par, hq = part // 2, part % 2
                    w = jnp.concatenate(
                        [_unpack(wq2[par][pl.ds(pl.multiple_of(
                            (hq * 4 + u) * SL + q * 128, 4), 128), :])
                         for u in range(4)], axis=1)
                    y = _dot(lhs, w) + jnp.where(q > 0, acc[rc * 4 + part], 0.0)
                    acc[rc * 4 + part] = y
                    to_ring(_pack(y), par, hq * 4, rc)
                return 0

            lax.fori_loop(0, 2, rc_body, 0)
            return 0

        with scope("quarters"):
            lax.fori_loop(0, 4, q_body, 0)

        start(mod_cps(4) + mod_cps(5) + a_cps)

        for q in range(4):
            st_quarter(1, q, SEM_Q1 + q).wait()

            def rl_body(i, _, q=q):
                relayout(0, 1, q * 128 + i * 32, 32)
                return 0

            lax.fori_loop(0, 4, rl_body, 0)

        def lead_proj(par, s0, n, rc, rl):
            w = jnp.concatenate(
                [_unpack(wq2[par][pl.ds(pl.multiple_of((s0 + u) * SL, 4), 512), :])
                 for u in range(n)], axis=1)
            lhs = jnp.concatenate(
                [_unpack(hv0[q, rc * 128:(rc + 1) * 128, :]) for q in range(4)],
                axis=1)
            y = _pack(_dot(lhs, w))
            to_ring(y, par, s0, rc)
            zero = zt[0:8, :]
            for u in range(n):
                for b in range(16):
                    k = min(3, 512 - rl[2])
                    if k > 0:
                        relayout(rl[0], rl[1], rl[2], k,
                                 y[b * 8:(b + 1) * 8, u * 128:(u + 1) * 128] & zero)
                        rl[2] += k
            return y

        def group_body(g, _):
            rl = [1, g, 0]
            for k in range(16):
                lead_proj(0, g * 8 + k // 2, 1, k % 2, rl)

            @pl.when(g < NG - 1)
            def _():
                cp(st_src(1), st.at[g + 1], SEM_G + g).wait()

            @pl.when(g == 1)
            def _():
                xw_cp.wait()

            @pl.when(g >= 2)
            def _():
                part_g = wmodv.at[pl.ds(8 * g, 8)]
                cp(part_g, part_g, SEM_G + g).wait()

            gn = jnp.minimum(g + 1, NG - 1)
            off = jnp.where((g == 1) | (g == 4), 1.0, 0.0).astype(F32)
            md = {"n": 0, "acc": None}

            def mod_items(n, pace):
                for it in range(md["n"], min(md["n"] + n, 512)):
                    c, i = divmod(it, 64)
                    w = wmodv[8 * g + c, i * 8:(i + 1) * 8, :] | pace
                    v = (pltpu.bitcast(w << 16, F32) * scol[0, i * 8:(i + 1) * 8, :]
                         + pltpu.bitcast(w & HI, F32) * scol[1, i * 8:(i + 1) * 8, :])
                    md["acc"] = v if i == 0 else md["acc"] + v
                    if i == 63:
                        modv[8 * g + c] = jnp.broadcast_to(
                            jnp.sum(md["acc"], axis=0, keepdims=True) + off, (8, 128))
                md["n"] += n

            rl = [0, gn, 0]
            for k in range(16):
                y = lead_proj(1, g * 8 + k // 2, 1, k % 2, rl)
                for b in range(16):
                    mod_items(2 + b % 2, y[8 * b:8 * b + 8] & zt[0:8, :])
                if k == 11:
                    t = [y[0:8], y[64:72]]
                    for i in range(3):
                        t = h_next(LEAD, i, t)
            assert md["n"] >= 512
            return 0

        with scope("groups"):
            lax.fori_loop(1, NG, group_body, 0)

    pl.run_scoped(
        prologue,
        pltpu.VMEM((NG, D, 8, E), U32),
        pltpu.VMEM((4, LEAD, 256), F32),
        pltpu.VMEM((8, 256, 512), F32),
        pltpu.VMEM((2, D // 2, 128), F32),
    )

    def main(w3v, w4v, zv, ttv):
        w34_cps = col_copies(w3_hbm, w3v, SEM_B) + col_copies(w4_hbm, w4v, SEM_B)
        start(w34_cps)
        wait(a_cps)

        scale = float(E) ** -0.5

        def segment(lhs, ro, store_tok, wo_lhs, extras):
            fill = fillv[...]
            keep = fill == 0.0
            NP = H // 2
            qkv, probs, blocks = {}, {}, []

            def proj(hp):
                slots = [t * H + 2 * hp + par for t in range(3) for par in range(2)]
                w = jnp.concatenate(
                    [_unpack(wq2[sl % 2][pl.ds((sl // 2) * SL, 512), :])
                     for sl in slots], axis=1)
                if hp == 0:
                    y = _dot(lhs[:, :512], w[:512])
                    y = _dot(lhs[:, 512:], w[512:]) + y
                else:
                    y = _dot(lhs, w)
                for u, sl in enumerate(slots):
                    store_tok(sl, y[8:32, u * 128:(u + 1) * 128])
                ops = []
                for t in range(3):
                    ym = jnp.concatenate(
                        [y[0:8, (2 * t) * 128:(2 * t + 1) * 128],
                         y[0:8, (2 * t + 1) * 128:(2 * t + 2) * 128]], axis=0)
                    ops.append(jnp.concatenate(
                        [ym.astype(BF16)]
                        + [_unpack(ring[ro + b, sl * 8:(sl + 1) * 8, :])
                           for sl in slots[2 * t:2 * t + 2] for b in range(2)]
                        + ([jnp.zeros((48, 128), BF16)] if t else []),
                        axis=0))
                qkv[hp] = ops

            def scores(hp):
                q, kk, _ = qkv[hp]
                s = lax.dot_general(q, kk, (((1,), (1,)), ((), ())),
                                    preferred_element_type=F32)
                s = jnp.where(keep, s * scale, fill)
                mx = jnp.max(s, axis=-1, keepdims=True)
                p = jnp.exp(s - mx)
                l = jnp.sum(p, axis=-1, keepdims=True)
                rl = pl.reciprocal(l, approx=True)
                rl = rl * (2.0 - l * rl)
                probs[hp] = (p * rl).astype(BF16)

            def pv(hp):
                o = _dot(probs[hp], qkv[hp][2])
                blocks.append(wo_lhs(2 * hp, o[0:8], o[16:48]).astype(BF16))
                blocks.append(wo_lhs(2 * hp + 1, o[8:16], o[48:80]).astype(BF16))

            def wo_part(h0, h1, acc=None):
                lw = jnp.concatenate(blocks[h0:h1], axis=1)
                y = _dot(lw, _cols(wov, 0, 8, E * h0, E * h1))
                return y if acc is None else y + acc

            for i in range(NP):
                proj(i)
                if i >= 1:
                    scores(i - 1)
                if i >= 3:
                    pv(i - 3)
                for thunk in extras.get(i, ()):
                    thunk()
            acc1 = wo_part(0, 4)
            scores(NP - 1)
            pv(NP - 3)
            acc2 = wo_part(4, 12, acc1)
            pv(NP - 2)
            pv(NP - 1)
            acc3 = wo_part(12, 24, acc2)
            for thunk in extras.get("wo", ()):
                thunk()
            return wo_part(24, 32, acc3)

        def p1_front(r0):
            x2 = (xv[pl.ds(pl.multiple_of(r0, 64), 64), :].astype(F32)
                  + mod_rows(2, 64) * aout[...])
            h2 = _ln(x2) * mod_rows(4, 64) + mod_rows(3, 64)
            return x2, h2, _ln(h2).astype(BF16)

        def p1_store(y, c, live):
            g = _gelu(y)
            if live is not None:
                g = jnp.where(live, g, 0.0)
            ring[GB, c * 96 + 24:c * 96 + 88, :] = pltpu.bitcast(g, U32)

        def half_dots(lhs, wv, done):
            part = {}

            def run(c, kh):
                y = _dot(lhs[:, kh * 512:(kh + 1) * 512],
                         _cols(wv, c, c + 1, kh * 512, (kh + 1) * 512))
                if kh == 0:
                    part[c] = y
                else:
                    done(y + part[c], c)

            return [functools.partial(run, c, kh) for c in range(8) for kh in range(2)]

        def p2_front(n):
            return jnp.concatenate(
                [pltpu.bitcast(ring[GB, pl.ds(c * 96 + 8 + SHIFTS[c], n), :], F32)
                 for c in range(8)], axis=1).astype(BF16)

        def p2_back(x2, h2, hs, row, n, tiles=None):
            x1 = jnp.concatenate([h2t[...], h2[0:n - 16]], axis=0) + hs
            x2w = jnp.concatenate([x2t[...], x2[0:n - 16]], axis=0)
            zv[pl.ds(pl.multiple_of(row, 16), n), :] = x2w + mod_rows(5, n) * x1
            if tiles is None:
                ttv[pl.ds(pl.multiple_of(row // 2, 8), n // 2), :] = _pack(_ln(x1))
                return None
            t = tiles
            for g in range(n // 16):
                y = _ln(paced(x1[16 * g:16 * g + 16], t))
                ttv[pl.ds(pl.multiple_of(row // 2 + 8 * g, 8), 8), :] = _pack(y)
                t = [y[0:8, 896:1024], y[8:16, 896:1024]]
            return t

        def a_body(j, mem):
            hcur[...] = hnext[...]
            hb = _unpack(hcur[0:8, :])
            hac = _unpack(hcur[8:16, :]).astype(F32)
            hd = _unpack(hcur[16:24, :])
            wr = [lax.rem(LEAD // 16 + 3 * j + i, RING) for i in range(3)]
            ro0 = lax.rem(4 * j, RING)
            ro1 = ro0 + 2

            x2, h2, u = p1_front(64 * jnp.maximum(j - 1, 0))
            live = j > 0

            lhs = jnp.concatenate(
                [jnp.concatenate([mem, hac[0:8]], axis=0).astype(BF16), hb], axis=0)
            tok_a = {}

            def store0(c, y):
                tok_a[c] = y[0:8]
                ring[wr[0], c * 8:(c + 1) * 8, :] = _pack(y[8:24])

            deferred = {}

            def wo_lhs0(h, om, ot):
                deferred[h] = ot[24:32]
                return jnp.concatenate([om, ot[0:24]], axis=0)

            pend = []

            def flush():
                while pend:
                    p1_store(*pend.pop(), live)

            th = half_dots(u, w1v, lambda y, c: pend.append((y, c)))
            extras = {i: [flush, th[i - 2]] for i in range(2, 14)}
            extras[14] = [flush] + th[12:14]
            extras[15] = [flush] + th[14:16]
            out = segment(lhs, ro0, store0, wo_lhs0, extras)
            flush()
            mem = out[0:8]
            aout[0:24, :] = out[8:32]

            lhs = jnp.concatenate(
                [jnp.concatenate([mem, hac[8:16]], axis=0).astype(BF16), hd], axis=0)

            def store1(c, y):
                ring[wr[1], c * 8:(c + 1) * 8, :] = _pack(
                    jnp.concatenate([tok_a[c], y[0:8]], axis=0))
                ring[wr[2], c * 8:(c + 1) * 8, :] = _pack(y[8:24])

            def wo_lhs1(h, om, ot):
                return jnp.concatenate([om, deferred[h], ot], axis=0)

            gs = p2_front(64)
            for c in range(8):
                ring[GB, c * 96:c * 96 + 24, :] = ring[GB, c * 96 + 64:c * 96 + 88, :]
            hs = []

            def p2_fin():
                t = [hs[7][0:8], hs[7][0:8]]
                for g in range(3):
                    t = h_next(rn, g, t)
                p2_back(x2, h2, jnp.concatenate(hs, axis=1), 64 * j, 64, t)
                x2t[...] = x2[48:64]
                h2t[...] = h2[48:64]

            th = half_dots(gs, w2v, lambda y, c: hs.append(y))
            extras = {i: [th[i]] for i in range(16)}
            extras["wo"] = [p2_fin]
            rn = LEAD + 48 * jnp.minimum(j + 1, NPAIR - 1)
            out = segment(lhs, ro1, store1, wo_lhs1, extras)
            aout[24:64, :] = out[8:48]
            return out[0:8]

        if "A" in phases:
            with scope("aloop"):
                lax.fori_loop(0, NPAIR, a_body, memv[...].astype(F32))
        else:
            zv[...] = jnp.zeros(zv.shape, F32)
            ttv[...] = jnp.zeros(ttv.shape, U32)

        x2, h2, u = p1_front(S - 64)
        y = _dot(u, _cols(w1v, 0, 8))
        for c in range(8):
            p1_store(y[:, c * 128:(c + 1) * 128], c, None)
        p2_back(x2, h2, _dot(p2_front(80), _cols(w2v, 0, 8)), S, 80)

        wait(w34_cps)

        def out_cp(i, slot):
            return cp(outv.at[slot], out_hbm.at[pl.ds(i * RB, RB), :],
                      SEM_OUT + slot)

        def p3_body(i, _):
            slot = i % 2

            @pl.when(i >= 2)
            def _():
                out_cp(i - 2, slot).wait()

            r0 = HALO + i * RB
            tt = _unpack(ttv[pl.ds(pl.multiple_of(r0 // 2, 8), RB // 2), :])
            ff = jnp.concatenate(
                [_gelu(_dot(tt, _cols(w3v, 4 * q, 4 * q + 4))).astype(BF16)
                 for q in range(FF // 512)], axis=1)
            gb = mod_rows(5, RB)
            for c0, c1 in ((0, 7), (7, 8)):
                cols = slice(c0 * 128, c1 * 128)
                y = _dot(ff, _cols(w4v, c0, c1))
                res = zv[pl.ds(pl.multiple_of(r0, 16), RB), cols] + gb[:, cols] * y
                outv[slot, :, cols] = res.astype(BF16)
                cp(outv.at[slot, :, cols], out_hbm.at[pl.ds(i * RB, RB), cols],
                   SEM_OUT + slot).start()
            return 0

        nb = S // RB
        if "B" in phases:
            with scope("p3"):
                lax.fori_loop(0, nb, p3_body, 0)
            out_cp(nb - 2, 0).wait()
            out_cp(nb - 1, 1).wait()
        else:
            outv[0] = zv[pl.ds(HALO, RB), :].astype(BF16)
            out_cp(0, 0).start()
            out_cp(0, 0).wait()

    pl.run_scoped(
        main,
        pltpu.VMEM((FF // 128, D // 2, 128), U32),
        pltpu.VMEM((8, FF // 2, 128), U32),
        pltpu.VMEM((S + HALO, D), F32),
        pltpu.VMEM(((S + HALO) // 2, D), U32),
    )


def _call(A_x, A_mem0, A_Wq, A_Wk, A_Wv, A_Wo, B_w1, B_w2, B_w3, B_w4, c, w_mod,
          phases="AB"):
    any_spec = pl.BlockSpec(memory_space=pl.ANY)
    scratch = [
        pltpu.VMEM((S, D), BF16),
        pltpu.VMEM((8, D), U32),
        pltpu.VMEM((M, D), BF16),
        pltpu.VMEM((48, D // 2, 128), U32),
        pltpu.VMEM((48, 8, 128), F32),
        pltpu.VMEM((3 * H // 2 * SL, E), U32),
        pltpu.VMEM((3 * H // 2 * SL, E), U32),
        pltpu.VMEM((8, H * E // 2, 128), U32),
        pltpu.VMEM((8, D // 2, 128), U32),
        pltpu.VMEM((8, D // 2, 128), U32),
        pltpu.VMEM((4, LEAD // 2, 256), U32),
        pltpu.VMEM((24, D), U32),
        pltpu.VMEM((24, D), U32),
        pltpu.VMEM((RING + 1, 3 * H * 8, E), U32),
        pltpu.VMEM((64, D), F32),
        pltpu.VMEM((16, D), F32),
        pltpu.VMEM((16, D), F32),
        pltpu.VMEM((32, 128), U32),
        pltpu.VMEM((2, RB, D), BF16),
        pltpu.VMEM((80, 128), F32),
        pltpu.VMEM((1, D), BF16),
        pltpu.SemaphoreType.DMA((NSEM,)),
    ]
    out = pl.pallas_call(
        functools.partial(_kernel, phases=phases),
        in_specs=[any_spec] * 12,
        out_specs=any_spec,
        out_shape=jax.ShapeDtypeStruct((S, D), BF16),
        scratch_shapes=scratch,
        compiler_params=pltpu.CompilerParams(
            vmem_limit_bytes=126 * 1024 * 1024),
    )(A_x.reshape(S, D), A_mem0.reshape(M, D), A_Wq, A_Wk, A_Wv,
      A_Wo.reshape(H * E, D), B_w1, B_w2, B_w3, B_w4, c, w_mod)
    return out.reshape(1, S, D)


def pallas_adaLN_cond__memory_aug_recurrent_mem_tr__mixer_s_mlp__prompt_kernel(
    A_x, A_mem0, A_Wq, A_Wk, A_Wv, A_Wo, A_seg_len, B_x, B_w1, B_w2, B_w3, B_w4,
    c, w_mod,
):
    assert A_seg_len == SEG
    del B_x
    return _call(A_x, A_mem0, A_Wq, A_Wk, A_Wv, A_Wo, B_w1, B_w2, B_w3, B_w4,
                 c, w_mod)
```

```python
import contextlib
import functools

import jax
import jax.numpy as jnp
from jax import lax
import jax.experimental.pallas as pl
import jax.experimental.pallas.tpu as pltpu

F32 = jnp.float32
BF16 = jnp.bfloat16
U32 = jnp.uint32

S = 2048
D = 1024
H = 32
E = 128
M = 8
SEG = 32
FF = 3584
EPS = 1e-5

LEAD = 512
RING = 36
GB = RING
SL = 516
HG = 16
NG = 3 * H // HG
NPAIR = S // (2 * SEG)
HALO = 80
RB = 256
SHIFTS = (-1, -1, 1, 1, -2, -2, 2, 2)

SEM_C = 0
SEM_X = 1
SEM_A = 2
SEM_B = 3
SEM_XR = 4
SEM_M0 = 5
SEM_K = 6
SEM_G = 13
SEM_OUT = 19
NSEM = 21


def _ln(x):
    mu = jnp.mean(x, axis=-1, keepdims=True)
    xc = x - mu
    var = jnp.mean(xc * xc, axis=-1, keepdims=True)
    return xc * lax.rsqrt(var + EPS)


def _gelu(x):
    return jax.nn.gelu(x, approximate=True)


def _pack(x):
    return pltpu.bitcast(x.astype(BF16), U32)


def _unpack(x):
    return pltpu.bitcast(x, BF16)


def _dot(a, b):
    return jnp.dot(a, b, preferred_element_type=F32)


def _cols(ref, lo, hi, k0=0, k1=None):
    k1 = 2 * ref.shape[1] if k1 is None else k1
    return jnp.concatenate(
        [_unpack(ref[c, k0 // 2:k1 // 2, :]) for c in range(lo, hi)], axis=1)


def _kernel(x_hbm, mem_hbm, wq_hbm, wk_hbm, wv_hbm, wo_hbm, w1_hbm, w2_hbm,
            w3_hbm, w4_hbm, c_hbm, wmod_hbm, out_hbm,
            xv, memv, wmodv, modv, wqa, wqb, wov, w1v, w2v,
            hv0, hcur, hnext, ring, aout, x2t, h2t, zt, outv, fillv, cv, sems, *, phases):
    def scope(name):
        return jax.named_scope(name) if "s" in phases else contextlib.nullcontext()

    def cp(src, dst, s):
        return pltpu.make_async_copy(src, dst, sems.at[s])

    def col_copies(w_hbm, w_v, s, lo=0, hi=None):
        w32 = w_hbm.bitcast(U32)
        hi = w_v.shape[0] if hi is None else hi
        return [cp(w32.at[:, pl.ds(c * 128, 128)], w_v.at[c], s)
                for c in range(lo, hi)]

    def start(cps):
        for q in cps:
            q.start()

    def wait(cps):
        for q in cps:
            q.wait()

    def x_cp(r0, n, s):
        return cp(x_hbm.at[pl.ds(r0, n)], xv.at[pl.ds(r0, n)], s)

    c_cps = [cp(c_hbm, cv, SEM_C), cp(mem_hbm, memv, SEM_C)]
    x0_cp = x_cp(0, LEAD, SEM_X)
    xw_cp = x_cp(LEAD, 96, SEM_G + 1)
    xr_cp = x_cp(LEAD + 96, S - LEAD - 96, SEM_XR)
    a_cps = (col_copies(wo_hbm, wov, SEM_A) + col_copies(w1_hbm, w1v, SEM_A)
             + col_copies(w2_hbm, w2v, SEM_A))

    def mod_rows(i, n):
        m = jnp.concatenate([modv[8 * i + c] for c in range(8)], axis=1)
        return jnp.concatenate([m] * (n // 8), axis=0)

    HI = jnp.uint32(0xFFFF0000)
    wq2 = (wqa, wqb)

    def paced(x, tiles):
        z = [pltpu.bitcast((t if t.dtype == U32 else pltpu.bitcast(t, U32))
                           & zt[0:8, :], F32) for t in tiles]
        z = jnp.concatenate(z, axis=0)
        return jnp.concatenate([x[:, 0:128] + z, x[:, 128:]], axis=1)

    def h_rows(r0, n, tiles=None):
        xf = xv[pl.ds(pl.multiple_of(r0, 16), n), :].astype(F32)
        if tiles is not None:
            xf = paced(xf, tiles)
        return _ln(xf) * mod_rows(1, n) + mod_rows(0, n)

    def h_next(r0, g, tile=None):
        y = h_rows(r0 + 16 * g, 16, tile)
        hnext[g * 8:(g + 1) * 8, :] = _pack(y)
        return [y[0:8, 896:1024], y[8:16, 896:1024]]

    def prologue(st, xn, acc, scol, hn):
        w_hbms = (wq_hbm, wk_hbm, wv_hbm)

        def st_src(i):
            return w_hbms[i // 2].bitcast(U32).at[:, pl.ds((i % 2) * 8, 8), :]

        def pair_cps(n, s):
            w32 = wmod_hbm.bitcast(U32)
            return [cp(w32.at[:, pl.ds(pl.multiple_of(c * 128, 128), 128)],
                       wmodv.at[c], s) for c in (n, 8 + n)]

        def k_cps(n):
            return [cp(st_src(i).at[pl.ds(n * 128, 128)],
                       st.at[i, pl.ds(n * 128, 128)], SEM_K + n) for i in range(2)]

        def st_cp(i):
            return cp(st_src(i), st.at[i], SEM_G + i - 1)

        def mod_cps(i):
            return col_copies(wmod_hbm, wmodv, SEM_G + i, 8 * i, 8 * i + 8)

        with scope("first"):
            start(c_cps + [x0_cp] + pair_cps(0, SEM_M0))
        for n in range(8):
            start(k_cps(n) + (pair_cps(n + 1, SEM_K + n) if n < 7 else []))
        start([st_cp(2), xw_cp, st_cp(3)] + mod_cps(2) + [st_cp(4)] + mod_cps(3)
              + [st_cp(5)])

        r = lax.broadcasted_iota(jnp.int32, (80, 128), 0)
        k = lax.broadcasted_iota(jnp.int32, (80, 128), 1)

        def head_of(i):
            return jnp.where(i < 16, i // 8, (i - 16) // 32)

        def pos_of(i):
            return jnp.where(i < 16, i % 8, 8 + (i - 16) % 32)

        same = head_of(r) == head_of(k)
        vis = (pos_of(r) < M) | (pos_of(r) >= pos_of(k))
        fillv[...] = jnp.where(same, jnp.where(vis, 0.0, -1e9), -jnp.inf).astype(F32)
        aout[...] = jnp.zeros(aout.shape, F32)
        ring[GB] = jnp.zeros(ring.shape[1:], U32)
        zt[...] = jnp.zeros(zt.shape, U32)
        x2t[...] = jnp.zeros(x2t.shape, F32)
        h2t[...] = jnp.zeros(h2t.shape, F32)


        def zero_body(i, _):
            acc[i] = jnp.zeros(acc.shape[1:], F32)
            return 0

        lax.fori_loop(0, acc.shape[0], zero_body, 0)

        wait(c_cps)
        cf = cv[...].astype(F32)
        sil = cf * jax.nn.sigmoid(cf)
        for c in range(8):
            sw = _pack(jnp.broadcast_to(sil[:, c * 128:(c + 1) * 128], (128, 128)).T)
            scol[0, c * 64:(c + 1) * 64, :] = pltpu.bitcast(sw << 16, F32)
            scol[1, c * 64:(c + 1) * 64, :] = pltpu.bitcast(sw & HI, F32)

        x0_cp.wait()

        def ln_body(i, _):
            r0 = pl.multiple_of(i * 64, 64)
            y = _ln(xv[pl.ds(r0, 64), :].astype(F32))
            for q in range(8):
                xn[q, pl.ds(r0, 64), :] = y[:, q * 128:(q + 1) * 128]
            return 0

        lax.fori_loop(0, LEAD // 64, ln_body, 0)

        class Mod:
            def __init__(self, tiles, offs):
                self.tiles, self.offs = tiles, offs
                self.n, self.acc, self.out = 0, None, []

            def items(self, n, pace=None):
                for it in range(self.n, min(self.n + n, 64 * len(self.tiles))):
                    c, i = divmod(it, 64)
                    w = wmodv[self.tiles[c], i * 8:(i + 1) * 8, :]
                    if pace is not None:
                        w = w | pace
                    v = (pltpu.bitcast(w << 16, F32) * scol[0, i * 8:(i + 1) * 8, :]
                         + pltpu.bitcast(w & HI, F32) * scol[1, i * 8:(i + 1) * 8, :])
                    self.acc = v if i == 0 else self.acc + v
                    if i == 63:
                        m = jnp.broadcast_to(
                            jnp.sum(self.acc, axis=0, keepdims=True) + self.offs[c],
                            (8, 128))
                        modv[self.tiles[c]] = m
                        self.out.append(m)
                self.n += n

        def h_lead(n, b, sa, ca):
            rep = lambda m: jnp.concatenate([m, m], axis=0)
            y = _pack(xn[n, 16 * b:16 * b + 16, :] * rep(ca) + rep(sa))
            hn[8 * b:8 * b + 8, :] = y
            hv0[n, 8 * b:8 * b + 8, :] = y

        wait(pair_cps(0, SEM_M0))
        md = Mod([0, 8], [0.0, 1.0])
        md.items(128)
        for b in range(32):
            h_lead(0, b, *md.out)

        def relayout(par, g, p0, n, pace=None):
            base = g * (8 * SL)
            mask = jnp.uint32(0xFFFF0000 if par else 0xFFFF)
            if pace is not None:
                mask = pace | mask
            for u in range(n):
                a = st[g, 2 * (p0 + u)]
                b = st[g, 2 * (p0 + u) + 1]
                if par == 0:
                    w = (a & mask) | (b << 16)
                else:
                    w = (a >> 16) | (b & mask)
                wq2[par][pl.ds(base + p0 + u, 8, stride=SL), :] = w

        def to_ring(y, par, s0, b0):
            for u in range(y.shape[1] // 128):
                row = pl.multiple_of((2 * (s0 + u) + par) * 8, 8)
                for b in range(y.shape[0] // 8):
                    ring[b0 + b, pl.ds(row, 8), :] = (
                        y[b * 8:(b + 1) * 8, u * 128:(u + 1) * 128])

        def k_body(n, _):
            wait(k_cps(n))

            @pl.when(n < 7)
            def _():
                wait(pair_cps(n + 1, SEM_K + n))

            nn = jnp.minimum(n + 1, 7)
            md = Mod([nn, 8 + nn], [0.0, 1.0])
            zero = zt[0:8, :]
            order = [(0, 0), (1, 0), (0, 1), (1, 1)]
            relayout(0, 0, n * 64, 64)
            for i, (par, g) in enumerate(order):
                for hq in range(2):
                    s0 = g * 8 + hq * 4
                    w = jnp.concatenate(
                        [_unpack(wq2[par][pl.ds(pl.multiple_of(
                            (s0 + u) * SL + n * 64, 4), 64), :])
                         for u in range(4)], axis=1)
                    y = _dot(_unpack(hn[...]), w) + acc[2 * i + hq]
                    acc[2 * i + hq] = y
                    y = _pack(y)
                    to_ring(y, par, s0, 0)
                    tiles = [y[8 * b:8 * b + 8, 0:128] & zero for b in range(32)]
                    for b in range(32):
                        pace = tiles[b]
                        if hq == 0 and i < 3:
                            relayout(*order[i + 1], n * 64 + 2 * b, 2, pace)
                        elif hq == 1 and i < 3:
                            md.items(2 - b % 2, pace)
                        elif hq == 1:
                            sa, ca = md.out
                            ca = ca + pltpu.bitcast(tiles[max(b - 3, 0)], F32)
                            h_lead(nn, b, sa, ca)
            return 0

        with scope("ksteps"):
            lax.fori_loop(0, 8, k_body, 0)

        start(mod_cps(4) + mod_cps(5) + a_cps + [xr_cp])
        wait([st_cp(2), xw_cp])

        def rl_body(i, _):
            relayout(0, 2, i * 64, 64)
            return 0

        lax.fori_loop(0, 8, rl_body, 0)

        def lead_proj(par, s0, n, rc, rl):
            w = jnp.concatenate(
                [_unpack(wq2[par][pl.ds(pl.multiple_of((s0 + u) * SL, 4), 512), :])
                 for u in range(n)], axis=1)
            lhs = jnp.concatenate(
                [_unpack(hv0[q, rc * 128:(rc + 1) * 128, :]) for q in range(8)],
                axis=1)
            y = _pack(_dot(lhs, w))
            to_ring(y, par, s0, rc * 16)
            zero = zt[0:8, :]
            for u in range(n):
                for b in range(16):
                    k = min(3, 512 - rl[2])
                    if k > 0:
                        relayout(rl[0], rl[1], rl[2], k,
                                 y[b * 8:(b + 1) * 8, u * 128:(u + 1) * 128] & zero)
                        rl[2] += k
            return y

        def group_body(g, _):
            rl = [1, g, 0]
            for k in range(16):
                lead_proj(0, g * 8 + k // 2, 1, k % 2, rl)

            @pl.when(g < NG - 1)
            def _():
                cp(st_src(1), st.at[g + 1], SEM_G + g).wait()

            part_g = wmodv.at[pl.ds(8 * g, 8)]
            cp(part_g, part_g, SEM_G + g).wait()

            gn = jnp.minimum(g + 1, NG - 1)
            off = jnp.where(g == 4, 1.0, 0.0).astype(F32)
            md = Mod([8 * g + c for c in range(8)], [off] * 8)
            rl = [0, gn, 0]
            for k in range(16):
                y = lead_proj(1, g * 8 + k // 2, 1, k % 2, rl)
                for b in range(16):
                    md.items(2 + b % 2, y[8 * b:8 * b + 8] & zt[0:8, :])
                if k == 11:
                    t = [y[0:8], y[64:72]]
                    for i in range(3):
                        t = h_next(LEAD, i, t)
            assert len(md.out) == 8
            return 0

        with scope("groups"):
            lax.fori_loop(2, NG, group_body, 0)

    pl.run_scoped(
        prologue,
        pltpu.VMEM((NG, D, 8, E), U32),
        pltpu.VMEM((8, LEAD, 128), F32),
        pltpu.VMEM((8, LEAD, 512), F32),
        pltpu.VMEM((2, D // 2, 128), F32),
        pltpu.VMEM((LEAD // 2, 128), U32),
    )

    def main(w3v, w4v, zv, ttv):
        w34_cps = col_copies(w3_hbm, w3v, SEM_B) + col_copies(w4_hbm, w4v, SEM_B)
        start(w34_cps)
        wait(a_cps)

        scale = float(E) ** -0.5

        def segment(lhs, ro, store_tok, wo_lhs, extras):
            fill = fillv[...]
            keep = fill == 0.0
            NP = H // 2
            qkv, probs, blocks = {}, {}, []

            def proj(hp):
                slots = [t * H + 2 * hp + par for t in range(3) for par in range(2)]
                w = jnp.concatenate(
                    [_unpack(wq2[sl % 2][pl.ds((sl // 2) * SL, 512), :])
                     for sl in slots], axis=1)
                if hp == 0:
                    y = _dot(lhs[:, :512], w[:512])
                    y = _dot(lhs[:, 512:], w[512:]) + y
                else:
                    y = _dot(lhs, w)
                for u, sl in enumerate(slots):
                    store_tok(sl, y[8:32, u * 128:(u + 1) * 128])
                ops = []
                for t in range(3):
                    ym = jnp.concatenate(
                        [y[0:8, (2 * t) * 128:(2 * t + 1) * 128],
                         y[0:8, (2 * t + 1) * 128:(2 * t + 2) * 128]], axis=0)
                    ops.append(jnp.concatenate(
                        [ym.astype(BF16)]
                        + [_unpack(ring[ro + b, sl * 8:(sl + 1) * 8, :])
                           for sl in slots[2 * t:2 * t + 2] for b in range(2)]
                        + ([jnp.zeros((48, 128), BF16)] if t else []),
                        axis=0))
                qkv[hp] = ops

            def scores(hp):
                q, kk, _ = qkv[hp]
                s = lax.dot_general(q, kk, (((1,), (1,)), ((), ())),
                                    preferred_element_type=F32)
                s = jnp.where(keep, s * scale, fill)
                mx = jnp.max(s, axis=-1, keepdims=True)
                p = jnp.exp(s - mx)
                l = jnp.sum(p, axis=-1, keepdims=True)
                rl = pl.reciprocal(l, approx=True)
                rl = rl * (2.0 - l * rl)
                probs[hp] = (p * rl).astype(BF16)

            def pv(hp):
                o = _dot(probs[hp], qkv[hp][2])
                blocks.append(wo_lhs(2 * hp, o[0:8], o[16:48]).astype(BF16))
                blocks.append(wo_lhs(2 * hp + 1, o[8:16], o[48:80]).astype(BF16))

            def wo_part(h0, h1, acc=None):
                lw = jnp.concatenate(blocks[h0:h1], axis=1)
                y = _dot(lw, _cols(wov, 0, 8, E * h0, E * h1))
                return y if acc is None else y + acc

            for i in range(NP):
                proj(i)
                if i >= 1:
                    scores(i - 1)
                if i >= 3:
                    pv(i - 3)
                for thunk in extras.get(i, ()):
                    thunk()
            acc1 = wo_part(0, 4)
            scores(NP - 1)
            pv(NP - 3)
            acc2 = wo_part(4, 12, acc1)
            pv(NP - 2)
            pv(NP - 1)
            acc3 = wo_part(12, 24, acc2)
            for thunk in extras.get("wo", ()):
                thunk()
            return wo_part(24, 32, acc3)

        def p1_front(r0):
            x2 = (xv[pl.ds(pl.multiple_of(r0, 64), 64), :].astype(F32)
                  + mod_rows(2, 64) * aout[...])
            h2 = _ln(x2) * mod_rows(4, 64) + mod_rows(3, 64)
            return x2, h2, _ln(h2).astype(BF16)

        def p1_store(y, c, live):
            g = _gelu(y)
            if live is not None:
                g = jnp.where(live, g, 0.0)
            ring[GB, c * 96 + 24:c * 96 + 88, :] = pltpu.bitcast(g, U32)

        def half_dots(lhs, wv, done):
            part = {}

            def run(c, kh):
                y = _dot(lhs[:, kh * 512:(kh + 1) * 512],
                         _cols(wv, c, c + 1, kh * 512, (kh + 1) * 512))
                if kh == 0:
                    part[c] = y
                else:
                    done(y + part[c], c)

            return [functools.partial(run, c, kh) for c in range(8) for kh in range(2)]

        def p2_front(n):
            return jnp.concatenate(
                [pltpu.bitcast(ring[GB, pl.ds(c * 96 + 8 + SHIFTS[c], n), :], F32)
                 for c in range(8)], axis=1).astype(BF16)

        def p2_back(x2, h2, hs, row, n, tiles=None):
            x1 = jnp.concatenate([h2t[...], h2[0:n - 16]], axis=0) + hs
            x2w = jnp.concatenate([x2t[...], x2[0:n - 16]], axis=0)
            zv[pl.ds(pl.multiple_of(row, 16), n), :] = x2w + mod_rows(5, n) * x1
            if tiles is None:
                ttv[pl.ds(pl.multiple_of(row // 2, 8), n // 2), :] = _pack(_ln(x1))
                return None
            t = tiles
            for g in range(n // 16):
                y = _ln(paced(x1[16 * g:16 * g + 16], t))
                ttv[pl.ds(pl.multiple_of(row // 2 + 8 * g, 8), 8), :] = _pack(y)
                t = [y[0:8, 896:1024], y[8:16, 896:1024]]
            return t

        def a_body(j, mem):
            @pl.when(j == 1)
            def _():
                xr_cp.wait()

            hcur[...] = hnext[...]
            hb = _unpack(hcur[0:8, :])
            hac = _unpack(hcur[8:16, :]).astype(F32)
            hd = _unpack(hcur[16:24, :])
            wr = [lax.rem(LEAD // 16 + 3 * j + i, RING) for i in range(3)]
            ro0 = lax.rem(4 * j, RING)
            ro1 = ro0 + 2

            x2, h2, u = p1_front(64 * jnp.maximum(j - 1, 0))
            live = j > 0

            lhs = jnp.concatenate(
                [jnp.concatenate([mem, hac[0:8]], axis=0).astype(BF16), hb], axis=0)
            tok_a = {}

            def store0(c, y):
                tok_a[c] = y[0:8]
                ring[wr[0], c * 8:(c + 1) * 8, :] = _pack(y[8:24])

            deferred = {}

            def wo_lhs0(h, om, ot):
                deferred[h] = ot[24:32]
                return jnp.concatenate([om, ot[0:24]], axis=0)

            pend = []

            def flush():
                while pend:
                    p1_store(*pend.pop(), live)

            th = half_dots(u, w1v, lambda y, c: pend.append((y, c)))
            extras = {i: [flush, th[i - 2]] for i in range(2, 14)}
            extras[14] = [flush] + th[12:14]
            extras[15] = [flush] + th[14:16]
            out = segment(lhs, ro0, store0, wo_lhs0, extras)
            flush()
            mem = out[0:8]
            aout[0:24, :] = out[8:32]

            lhs = jnp.concatenate(
                [jnp.concatenate([mem, hac[8:16]], axis=0).astype(BF16), hd], axis=0)

            def store1(c, y):
                ring[wr[1], c * 8:(c + 1) * 8, :] = _pack(
                    jnp.concatenate([tok_a[c], y[0:8]], axis=0))
                ring[wr[2], c * 8:(c + 1) * 8, :] = _pack(y[8:24])

            def wo_lhs1(h, om, ot):
                return jnp.concatenate([om, deferred[h], ot], axis=0)

            gs = p2_front(64)
            for c in range(8):
                ring[GB, c * 96:c * 96 + 24, :] = ring[GB, c * 96 + 64:c * 96 + 88, :]
            hs = []

            def p2_fin():
                t = [hs[7][0:8], hs[7][0:8]]
                for g in range(3):
                    t = h_next(rn, g, t)
                p2_back(x2, h2, jnp.concatenate(hs, axis=1), 64 * j, 64, t)
                x2t[...] = x2[48:64]
                h2t[...] = h2[48:64]

            th = half_dots(gs, w2v, lambda y, c: hs.append(y))
            extras = {i: [th[i]] for i in range(16)}
            extras["wo"] = [p2_fin]
            rn = LEAD + 48 * jnp.minimum(j + 1, NPAIR - 1)
            out = segment(lhs, ro1, store1, wo_lhs1, extras)
            aout[24:64, :] = out[8:48]
            return out[0:8]

        if "A" in phases:
            with scope("aloop"):
                lax.fori_loop(0, NPAIR, a_body, memv[...].astype(F32))
        else:
            zv[...] = jnp.zeros(zv.shape, F32)
            ttv[...] = jnp.zeros(ttv.shape, U32)

        x2, h2, u = p1_front(S - 64)
        y = _dot(u, _cols(w1v, 0, 8))
        for c in range(8):
            p1_store(y[:, c * 128:(c + 1) * 128], c, None)
        p2_back(x2, h2, _dot(p2_front(80), _cols(w2v, 0, 8)), S, 80)

        wait(w34_cps)

        def out_cp(i, slot):
            return cp(outv.at[slot], out_hbm.at[pl.ds(i * RB, RB), :],
                      SEM_OUT + slot)

        def p3_body(i, _):
            slot = i % 2

            @pl.when(i >= 2)
            def _():
                out_cp(i - 2, slot).wait()

            r0 = HALO + i * RB
            tt = _unpack(ttv[pl.ds(pl.multiple_of(r0 // 2, 8), RB // 2), :])
            ff = jnp.concatenate(
                [_gelu(_dot(tt, _cols(w3v, 4 * q, 4 * q + 4))).astype(BF16)
                 for q in range(FF // 512)], axis=1)
            gb = mod_rows(5, RB)
            for c0, c1 in ((0, 7), (7, 8)):
                cols = slice(c0 * 128, c1 * 128)
                y = _dot(ff, _cols(w4v, c0, c1))
                res = zv[pl.ds(pl.multiple_of(r0, 16), RB), cols] + gb[:, cols] * y
                outv[slot, :, cols] = res.astype(BF16)
                cp(outv.at[slot, :, cols], out_hbm.at[pl.ds(i * RB, RB), cols],
                   SEM_OUT + slot).start()
            return 0

        nb = S // RB
        if "B" in phases:
            with scope("p3"):
                lax.fori_loop(0, nb, p3_body, 0)
            out_cp(nb - 2, 0).wait()
            out_cp(nb - 1, 1).wait()
        else:
            outv[0] = zv[pl.ds(HALO, RB), :].astype(BF16)
            out_cp(0, 0).start()
            out_cp(0, 0).wait()

    pl.run_scoped(
        main,
        pltpu.VMEM((FF // 128, D // 2, 128), U32),
        pltpu.VMEM((8, FF // 2, 128), U32),
        pltpu.VMEM((S + HALO, D), F32),
        pltpu.VMEM(((S + HALO) // 2, D), U32),
    )


def _call(A_x, A_mem0, A_Wq, A_Wk, A_Wv, A_Wo, B_w1, B_w2, B_w3, B_w4, c, w_mod,
          phases="AB"):
    any_spec = pl.BlockSpec(memory_space=pl.ANY)
    scratch = [
        pltpu.VMEM((S, D), BF16),
        pltpu.VMEM((M, D), BF16),
        pltpu.VMEM((48, D // 2, 128), U32),
        pltpu.VMEM((48, 8, 128), F32),
        pltpu.VMEM((3 * H // 2 * SL, E), U32),
        pltpu.VMEM((3 * H // 2 * SL, E), U32),
        pltpu.VMEM((8, H * E // 2, 128), U32),
        pltpu.VMEM((8, D // 2, 128), U32),
        pltpu.VMEM((8, D // 2, 128), U32),
        pltpu.VMEM((8, LEAD // 2, 128), U32),
        pltpu.VMEM((24, D), U32),
        pltpu.VMEM((24, D), U32),
        pltpu.VMEM((RING + 1, 3 * H * 8, E), U32),
        pltpu.VMEM((64, D), F32),
        pltpu.VMEM((16, D), F32),
        pltpu.VMEM((16, D), F32),
        pltpu.VMEM((32, 128), U32),
        pltpu.VMEM((2, RB, D), BF16),
        pltpu.VMEM((80, 128), F32),
        pltpu.VMEM((1, D), BF16),
        pltpu.SemaphoreType.DMA((NSEM,)),
    ]
    out = pl.pallas_call(
        functools.partial(_kernel, phases=phases),
        in_specs=[any_spec] * 12,
        out_specs=any_spec,
        out_shape=jax.ShapeDtypeStruct((S, D), BF16),
        scratch_shapes=scratch,
        compiler_params=pltpu.CompilerParams(
            vmem_limit_bytes=126 * 1024 * 1024),
    )(A_x.reshape(S, D), A_mem0.reshape(M, D), A_Wq, A_Wk, A_Wv,
      A_Wo.reshape(H * E, D), B_w1, B_w2, B_w3, B_w4, c, w_mod)
    return out.reshape(1, S, D)


def pallas_adaLN_cond__memory_aug_recurrent_mem_tr__mixer_s_mlp__prompt_kernel(
    A_x, A_mem0, A_Wq, A_Wk, A_Wv, A_Wo, A_seg_len, B_x, B_w1, B_w2, B_w3, B_w4,
    c, w_mod,
):
    assert A_seg_len == SEG
    del B_x
    return _call(A_x, A_mem0, A_Wq, A_Wk, A_Wv, A_Wo, B_w1, B_w2, B_w3, B_w4,
                 c, w_mod)
```

```python
import contextlib
import functools

import jax
import jax.numpy as jnp
from jax import lax
import jax.experimental.pallas as pl
import jax.experimental.pallas.tpu as pltpu

F32 = jnp.float32
BF16 = jnp.bfloat16
U32 = jnp.uint32

S = 2048
D = 1024
H = 32
E = 128
M = 8
SEG = 32
FF = 3584
EPS = 1e-5

LEAD = 512
RING = 36
GB = RING
SL = 516
HG = 16
NG = 3 * H // HG
NPAIR = S // (2 * SEG)
HALO = 80
RB = 256
SHIFTS = (-1, -1, 1, 1, -2, -2, 2, 2)

SEM_C = 0
SEM_X = 1
SEM_A = 2
SEM_B = 3
SEM_XR = 4
SEM_M = 5
SEM_K = 7
SEM_G = 14
SEM_OUT = 20
NSEM = 22


def _ln(x):
    mu = jnp.mean(x, axis=-1, keepdims=True)
    xc = x - mu
    var = jnp.mean(xc * xc, axis=-1, keepdims=True)
    return xc * lax.rsqrt(var + EPS)


def _gelu(x):
    return jax.nn.gelu(x, approximate=True)


def _pack(x):
    return pltpu.bitcast(x.astype(BF16), U32)


def _unpack(x):
    return pltpu.bitcast(x, BF16)


def _dot(a, b):
    return jnp.dot(a, b, preferred_element_type=F32)


def _cols(ref, lo, hi, k0=0, k1=None):
    k1 = 2 * ref.shape[1] if k1 is None else k1
    return jnp.concatenate(
        [_unpack(ref[c, k0 // 2:k1 // 2, :]) for c in range(lo, hi)], axis=1)


def _kernel(x_hbm, mem_hbm, wq_hbm, wk_hbm, wv_hbm, wo_hbm, w1_hbm, w2_hbm,
            w3_hbm, w4_hbm, c_hbm, wmod_hbm, out_hbm,
            xv, memv, wmodv, modv, wqa, wqb, wov, w1v, w2v,
            hv0, hcur, hnext, ring, aout, x2t, h2t, zt, outv, fillv, cv, sems, *, phases):
    def scope(name):
        return jax.named_scope(name) if "s" in phases else contextlib.nullcontext()

    def cp(src, dst, s):
        return pltpu.make_async_copy(src, dst, sems.at[s])

    def col_copies(w_hbm, w_v, s, lo=0, hi=None):
        w32 = w_hbm.bitcast(U32)
        hi = w_v.shape[0] if hi is None else hi
        return [cp(w32.at[:, pl.ds(c * 128, 128)], w_v.at[c], s)
                for c in range(lo, hi)]

    def start(cps):
        for q in cps:
            q.start()

    def wait(cps):
        for q in cps:
            q.wait()

    def x_cp(r0, n, s):
        return cp(x_hbm.at[pl.ds(r0, n)], xv.at[pl.ds(r0, n)], s)

    c_cps = [cp(c_hbm, cv, SEM_C), cp(mem_hbm, memv, SEM_C)]
    x0_cp = x_cp(0, LEAD, SEM_X)
    xw_cp = x_cp(LEAD, 96, SEM_G + 1)
    xr_cp = x_cp(LEAD + 96, S - LEAD - 96, SEM_XR)
    a_cps = (col_copies(wo_hbm, wov, SEM_A) + col_copies(w1_hbm, w1v, SEM_A)
             + col_copies(w2_hbm, w2v, SEM_A))

    def mod_rows(i, n):
        m = jnp.concatenate([modv[8 * i + c] for c in range(8)], axis=1)
        return jnp.concatenate([m] * (n // 8), axis=0)

    HI = jnp.uint32(0xFFFF0000)
    wq2 = (wqa, wqb)

    def paced(x, tiles):
        z = [pltpu.bitcast((t if t.dtype == U32 else pltpu.bitcast(t, U32))
                           & zt[0:8, :], F32) for t in tiles]
        z = jnp.concatenate(z, axis=0)
        return jnp.concatenate([x[:, 0:128] + z, x[:, 128:]], axis=1)

    def h_rows(r0, n, tiles=None):
        xf = xv[pl.ds(pl.multiple_of(r0, 16), n), :].astype(F32)
        if tiles is not None:
            xf = paced(xf, tiles)
        return _ln(xf) * mod_rows(1, n) + mod_rows(0, n)

    def h_next(r0, g, tile=None):
        y = h_rows(r0 + 16 * g, 16, tile)
        hnext[g * 8:(g + 1) * 8, :] = _pack(y)
        return [y[0:8, 896:1024], y[8:16, 896:1024]]

    def prologue(st, xn, acc, scol, hn):
        w_hbms = (wq_hbm, wk_hbm, wv_hbm)

        def st_src(i):
            return w_hbms[i // 2].bitcast(U32).at[:, pl.ds((i % 2) * 8, 8), :]

        def pair_cps(n, s):
            w32 = wmod_hbm.bitcast(U32)
            return [cp(w32.at[:, pl.ds(pl.multiple_of(c * 128, 128), 128)],
                       wmodv.at[c], s) for c in (n, 8 + n)]

        def k_cps(n):
            return [cp(st_src(i).at[pl.ds(n * 128, 128)],
                       st.at[i, pl.ds(n * 128, 128)], SEM_K + n) for i in range(2)]

        def st_cp(i):
            return cp(st_src(i), st.at[i], SEM_G + i - 1)

        def mod_cps(i):
            return col_copies(wmod_hbm, wmodv, SEM_G + i, 8 * i, 8 * i + 8)

        with scope("first"):
            start(c_cps + [x0_cp])
        for n in range(8):
            start((pair_cps(n, SEM_M + n) if n < 2 else []) + k_cps(n)
                  + (pair_cps(n + 1, SEM_K + n) if 0 < n < 7 else []))
        start([st_cp(2), xw_cp, st_cp(3)] + mod_cps(2) + [st_cp(4)] + mod_cps(3)
              + [st_cp(5)])

        r = lax.broadcasted_iota(jnp.int32, (80, 128), 0)
        k = lax.broadcasted_iota(jnp.int32, (80, 128), 1)

        def head_of(i):
            return jnp.where(i < 16, i // 8, (i - 16) // 32)

        def pos_of(i):
            return jnp.where(i < 16, i % 8, 8 + (i - 16) % 32)

        same = head_of(r) == head_of(k)
        vis = (pos_of(r) < M) | (pos_of(r) >= pos_of(k))
        fillv[...] = jnp.where(same, jnp.where(vis, 0.0, -1e9), -jnp.inf).astype(F32)
        aout[...] = jnp.zeros(aout.shape, F32)
        ring[GB] = jnp.zeros(ring.shape[1:], U32)
        zt[...] = jnp.zeros(zt.shape, U32)
        x2t[...] = jnp.zeros(x2t.shape, F32)
        h2t[...] = jnp.zeros(h2t.shape, F32)


        def zero_body(i, _):
            acc[i] = jnp.zeros(acc.shape[1:], F32)
            return 0

        lax.fori_loop(0, acc.shape[0], zero_body, 0)

        wait(c_cps)
        cf = cv[...].astype(F32)
        sil = cf * jax.nn.sigmoid(cf)
        for c in range(8):
            sw = _pack(jnp.broadcast_to(sil[:, c * 128:(c + 1) * 128], (128, 128)).T)
            scol[0, c * 64:(c + 1) * 64, :] = pltpu.bitcast(sw << 16, F32)
            scol[1, c * 64:(c + 1) * 64, :] = pltpu.bitcast(sw & HI, F32)

        x0_cp.wait()

        def ln_body(i, _):
            r0 = pl.multiple_of(i * 64, 64)
            y = _ln(xv[pl.ds(r0, 64), :].astype(F32))
            for q in range(8):
                xn[q, pl.ds(r0, 64), :] = y[:, q * 128:(q + 1) * 128]
            return 0

        lax.fori_loop(0, LEAD // 64, ln_body, 0)

        class Mod:
            def __init__(self, tiles, offs):
                self.tiles, self.offs = tiles, offs
                self.n, self.acc, self.out = 0, None, []

            def items(self, n, pace=None):
                for it in range(self.n, min(self.n + n, 64 * len(self.tiles))):
                    c, i = divmod(it, 64)
                    w = wmodv[self.tiles[c], i * 8:(i + 1) * 8, :]
                    if pace is not None:
                        w = w | pace
                    v = (pltpu.bitcast(w << 16, F32) * scol[0, i * 8:(i + 1) * 8, :]
                         + pltpu.bitcast(w & HI, F32) * scol[1, i * 8:(i + 1) * 8, :])
                    self.acc = v if i == 0 else self.acc + v
                    if i == 63:
                        m = jnp.broadcast_to(
                            jnp.sum(self.acc, axis=0, keepdims=True) + self.offs[c],
                            (8, 128))
                        modv[self.tiles[c]] = m
                        self.out.append(m)
                self.n += n

        def h_lead(n, b, sa, ca):
            rep = lambda m: jnp.concatenate([m, m], axis=0)
            y = _pack(xn[n, 16 * b:16 * b + 16, :] * rep(ca) + rep(sa))
            hn[8 * b:8 * b + 8, :] = y
            hv0[n, 8 * b:8 * b + 8, :] = y

        def relayout(par, g, p0, n, pace=None):
            base = g * (8 * SL)
            mask = jnp.uint32(0xFFFF0000 if par else 0xFFFF)
            if pace is not None:
                mask = pace | mask
            for u in range(n):
                a = st[g, 2 * (p0 + u)]
                b = st[g, 2 * (p0 + u) + 1]
                if par == 0:
                    w = (a & mask) | (b << 16)
                else:
                    w = (a >> 16) | (b & mask)
                wq2[par][pl.ds(base + p0 + u, 8, stride=SL), :] = w

        def to_ring(y, par, s0, b0):
            for u in range(y.shape[1] // 128):
                row = pl.multiple_of((2 * (s0 + u) + par) * 8, 8)
                for b in range(y.shape[0] // 8):
                    ring[b0 + b, pl.ds(row, 8), :] = (
                        y[b * 8:(b + 1) * 8, u * 128:(u + 1) * 128])

        def k_body(n, _):
            @pl.when(n < 2)
            def _():
                wait(pair_cps(n, SEM_M + n))
                md = Mod([n, 8 + n], [0.0, 1.0])
                md.items(128)
                for b in range(32):
                    h_lead(n, b, *md.out)

            wait(k_cps(n))

            @pl.when((n > 0) & (n < 7))
            def _():
                wait(pair_cps(n + 1, SEM_K + n))

            nn = jnp.where(n == 0, 0, jnp.minimum(n + 1, 7))
            md = Mod([nn, 8 + nn], [0.0, 1.0])
            zero = zt[0:8, :]
            order = [(0, 0), (1, 0), (0, 1), (1, 1)]
            relayout(0, 0, n * 64, 64)
            for i, (par, g) in enumerate(order):
                for hq in range(2):
                    s0 = g * 8 + hq * 4
                    w = jnp.concatenate(
                        [_unpack(wq2[par][pl.ds(pl.multiple_of(
                            (s0 + u) * SL + n * 64, 4), 64), :])
                         for u in range(4)], axis=1)
                    y = _dot(_unpack(hn[...]), w) + acc[2 * i + hq]
                    acc[2 * i + hq] = y
                    y = _pack(y)
                    to_ring(y, par, s0, 0)
                    tiles = [y[8 * b:8 * b + 8, 0:128] & zero for b in range(32)]
                    for b in range(32):
                        pace = tiles[b]
                        if hq == 0 and i < 3:
                            relayout(*order[i + 1], n * 64 + 2 * b, 2, pace)
                        elif hq == 1 and i < 3:
                            md.items(2 - b % 2, pace)
                        elif hq == 1:
                            sa, ca = md.out
                            ca = ca + pltpu.bitcast(tiles[max(b - 3, 0)], F32)
                            h_lead(nn, b, sa, ca)
            return 0

        with scope("ksteps"):
            lax.fori_loop(0, 8, k_body, 0)

        start(mod_cps(4) + mod_cps(5) + a_cps + [xr_cp])
        wait([st_cp(2), xw_cp])

        def rl_body(i, _):
            relayout(0, 2, i * 64, 64)
            return 0

        lax.fori_loop(0, 8, rl_body, 0)

        def lead_proj(par, s0, n, rc, rl):
            w = jnp.concatenate(
                [_unpack(wq2[par][pl.ds(pl.multiple_of((s0 + u) * SL, 4), 512), :])
                 for u in range(n)], axis=1)
            lhs = jnp.concatenate(
                [_unpack(hv0[q, rc * 128:(rc + 1) * 128, :]) for q in range(8)],
                axis=1)
            y = _pack(_dot(lhs, w))
            to_ring(y, par, s0, rc * 16)
            zero = zt[0:8, :]
            for u in range(n):
                for b in range(16):
                    k = min(3, 512 - rl[2])
                    if k > 0:
                        relayout(rl[0], rl[1], rl[2], k,
                                 y[b * 8:(b + 1) * 8, u * 128:(u + 1) * 128] & zero)
                        rl[2] += k
            return y

        def group_body(g, _):
            rl = [1, g, 0]
            for k in range(16):
                lead_proj(0, g * 8 + k // 2, 1, k % 2, rl)

            @pl.when(g < NG - 1)
            def _():
                cp(st_src(1), st.at[g + 1], SEM_G + g).wait()

            part_g = wmodv.at[pl.ds(8 * g, 8)]
            cp(part_g, part_g, SEM_G + g).wait()

            gn = jnp.minimum(g + 1, NG - 1)
            off = jnp.where(g == 4, 1.0, 0.0).astype(F32)
            md = Mod([8 * g + c for c in range(8)], [off] * 8)
            rl = [0, gn, 0]
            for k in range(16):
                y = lead_proj(1, g * 8 + k // 2, 1, k % 2, rl)
                for b in range(16):
                    md.items(2 + b % 2, y[8 * b:8 * b + 8] & zt[0:8, :])
                if k == 11:
                    t = [y[0:8], y[64:72]]
                    for i in range(3):
                        t = h_next(LEAD, i, t)
            assert len(md.out) == 8
            return 0

        with scope("groups"):
            lax.fori_loop(2, NG, group_body, 0)

    pl.run_scoped(
        prologue,
        pltpu.VMEM((NG, D, 8, E), U32),
        pltpu.VMEM((8, LEAD, 128), F32),
        pltpu.VMEM((8, LEAD, 512), F32),
        pltpu.VMEM((2, D // 2, 128), F32),
        pltpu.VMEM((LEAD // 2, 128), U32),
    )

    def main(w3v, w4v, zv, ttv):
        w34_cps = col_copies(w3_hbm, w3v, SEM_B) + col_copies(w4_hbm, w4v, SEM_B)
        start(w34_cps)
        wait(a_cps)

        scale = float(E) ** -0.5

        def segment(lhs, ro, store_tok, wo_lhs, extras):
            fill = fillv[...]
            keep = fill == 0.0
            NP = H // 2
            qkv, probs, blocks = {}, {}, []

            def proj(hp):
                slots = [t * H + 2 * hp + par for t in range(3) for par in range(2)]
                w = jnp.concatenate(
                    [_unpack(wq2[sl % 2][pl.ds((sl // 2) * SL, 512), :])
                     for sl in slots], axis=1)
                if hp == 0:
                    y = _dot(lhs[:, :512], w[:512])
                    y = _dot(lhs[:, 512:], w[512:]) + y
                else:
                    y = _dot(lhs, w)
                for u, sl in enumerate(slots):
                    store_tok(sl, y[8:32, u * 128:(u + 1) * 128])
                ops = []
                for t in range(3):
                    ym = jnp.concatenate(
                        [y[0:8, (2 * t) * 128:(2 * t + 1) * 128],
                         y[0:8, (2 * t + 1) * 128:(2 * t + 2) * 128]], axis=0)
                    ops.append(jnp.concatenate(
                        [ym.astype(BF16)]
                        + [_unpack(ring[ro + b, sl * 8:(sl + 1) * 8, :])
                           for sl in slots[2 * t:2 * t + 2] for b in range(2)]
                        + ([jnp.zeros((48, 128), BF16)] if t else []),
                        axis=0))
                qkv[hp] = ops

            def scores(hp):
                q, kk, _ = qkv[hp]
                s = lax.dot_general(q, kk, (((1,), (1,)), ((), ())),
                                    preferred_element_type=F32)
                s = jnp.where(keep, s * scale, fill)
                mx = jnp.max(s, axis=-1, keepdims=True)
                p = jnp.exp(s - mx)
                l = jnp.sum(p, axis=-1, keepdims=True)
                rl = pl.reciprocal(l, approx=True)
                rl = rl * (2.0 - l * rl)
                probs[hp] = (p * rl).astype(BF16)

            def pv(hp):
                o = _dot(probs[hp], qkv[hp][2])
                blocks.append(wo_lhs(2 * hp, o[0:8], o[16:48]).astype(BF16))
                blocks.append(wo_lhs(2 * hp + 1, o[8:16], o[48:80]).astype(BF16))

            def wo_part(h0, h1, acc=None):
                lw = jnp.concatenate(blocks[h0:h1], axis=1)
                y = _dot(lw, _cols(wov, 0, 8, E * h0, E * h1))
                return y if acc is None else y + acc

            for i in range(NP):
                proj(i)
                if i >= 1:
                    scores(i - 1)
                if i >= 3:
                    pv(i - 3)
                for thunk in extras.get(i, ()):
                    thunk()
            acc1 = wo_part(0, 4)
            scores(NP - 1)
            pv(NP - 3)
            acc2 = wo_part(4, 12, acc1)
            pv(NP - 2)
            pv(NP - 1)
            acc3 = wo_part(12, 24, acc2)
            for thunk in extras.get("wo", ()):
                thunk()
            return wo_part(24, 32, acc3)

        def p1_front(r0):
            x2 = (xv[pl.ds(pl.multiple_of(r0, 64), 64), :].astype(F32)
                  + mod_rows(2, 64) * aout[...])
            h2 = _ln(x2) * mod_rows(4, 64) + mod_rows(3, 64)
            return x2, h2, _ln(h2).astype(BF16)

        def p1_store(y, c, live):
            g = _gelu(y)
            if live is not None:
                g = jnp.where(live, g, 0.0)
            ring[GB, c * 96 + 24:c * 96 + 88, :] = pltpu.bitcast(g, U32)

        def half_dots(lhs, wv, done):
            part = {}

            def run(c, kh):
                y = _dot(lhs[:, kh * 512:(kh + 1) * 512],
                         _cols(wv, c, c + 1, kh * 512, (kh + 1) * 512))
                if kh == 0:
                    part[c] = y
                else:
                    done(y + part[c], c)

            return [functools.partial(run, c, kh) for c in range(8) for kh in range(2)]

        def p2_front(n):
            return jnp.concatenate(
                [pltpu.bitcast(ring[GB, pl.ds(c * 96 + 8 + SHIFTS[c], n), :], F32)
                 for c in range(8)], axis=1).astype(BF16)

        def p2_back(x2, h2, hs, row, n, tiles=None):
            x1 = jnp.concatenate([h2t[...], h2[0:n - 16]], axis=0) + hs
            x2w = jnp.concatenate([x2t[...], x2[0:n - 16]], axis=0)
            zv[pl.ds(pl.multiple_of(row, 16), n), :] = x2w + mod_rows(5, n) * x1
            if tiles is None:
                ttv[pl.ds(pl.multiple_of(row // 2, 8), n // 2), :] = _pack(_ln(x1))
                return None
            t = tiles
            for g in range(n // 16):
                y = _ln(paced(x1[16 * g:16 * g + 16], t))
                ttv[pl.ds(pl.multiple_of(row // 2 + 8 * g, 8), 8), :] = _pack(y)
                t = [y[0:8, 896:1024], y[8:16, 896:1024]]
            return t

        def a_body(j, mem):
            @pl.when(j == 1)
            def _():
                xr_cp.wait()

            hcur[...] = hnext[...]
            hb = _unpack(hcur[0:8, :])
            hac = _unpack(hcur[8:16, :]).astype(F32)
            hd = _unpack(hcur[16:24, :])
            wr = [lax.rem(LEAD // 16 + 3 * j + i, RING) for i in range(3)]
            ro0 = lax.rem(4 * j, RING)
            ro1 = ro0 + 2

            x2, h2, u = p1_front(64 * jnp.maximum(j - 1, 0))
            live = j > 0

            lhs = jnp.concatenate(
                [jnp.concatenate([mem, hac[0:8]], axis=0).astype(BF16), hb], axis=0)
            tok_a = {}

            def store0(c, y):
                tok_a[c] = y[0:8]
                ring[wr[0], c * 8:(c + 1) * 8, :] = _pack(y[8:24])

            deferred = {}

            def wo_lhs0(h, om, ot):
                deferred[h] = ot[24:32]
                return jnp.concatenate([om, ot[0:24]], axis=0)

            pend = []

            def flush():
                while pend:
                    p1_store(*pend.pop(), live)

            th = half_dots(u, w1v, lambda y, c: pend.append((y, c)))
            extras = {i: [flush, th[i - 2]] for i in range(2, 14)}
            extras[14] = [flush] + th[12:14]
            extras[15] = [flush] + th[14:16]
            out = segment(lhs, ro0, store0, wo_lhs0, extras)
            flush()
            mem = out[0:8]
            aout[0:24, :] = out[8:32]

            lhs = jnp.concatenate(
                [jnp.concatenate([mem, hac[8:16]], axis=0).astype(BF16), hd], axis=0)

            def store1(c, y):
                ring[wr[1], c * 8:(c + 1) * 8, :] = _pack(
                    jnp.concatenate([tok_a[c], y[0:8]], axis=0))
                ring[wr[2], c * 8:(c + 1) * 8, :] = _pack(y[8:24])

            def wo_lhs1(h, om, ot):
                return jnp.concatenate([om, deferred[h], ot], axis=0)

            gs = p2_front(64)
            for c in range(8):
                ring[GB, c * 96:c * 96 + 24, :] = ring[GB, c * 96 + 64:c * 96 + 88, :]
            hs = []

            def p2_fin():
                t = [hs[7][0:8], hs[7][0:8]]
                for g in range(3):
                    t = h_next(rn, g, t)
                p2_back(x2, h2, jnp.concatenate(hs, axis=1), 64 * j, 64, t)
                x2t[...] = x2[48:64]
                h2t[...] = h2[48:64]

            th = half_dots(gs, w2v, lambda y, c: hs.append(y))
            extras = {i: [th[i]] for i in range(16)}
            extras["wo"] = [p2_fin]
            rn = LEAD + 48 * jnp.minimum(j + 1, NPAIR - 1)
            out = segment(lhs, ro1, store1, wo_lhs1, extras)
            aout[24:64, :] = out[8:48]
            return out[0:8]

        if "A" in phases:
            with scope("aloop"):
                lax.fori_loop(0, NPAIR, a_body, memv[...].astype(F32))
        else:
            zv[...] = jnp.zeros(zv.shape, F32)
            ttv[...] = jnp.zeros(ttv.shape, U32)

        x2, h2, u = p1_front(S - 64)
        y = _dot(u, _cols(w1v, 0, 8))
        for c in range(8):
            p1_store(y[:, c * 128:(c + 1) * 128], c, None)
        p2_back(x2, h2, _dot(p2_front(80), _cols(w2v, 0, 8)), S, 80)

        wait(w34_cps)

        def out_cp(i, slot):
            return cp(outv.at[slot], out_hbm.at[pl.ds(i * RB, RB), :],
                      SEM_OUT + slot)

        def p3_body(i, _):
            slot = i % 2

            @pl.when(i >= 2)
            def _():
                out_cp(i - 2, slot).wait()

            r0 = HALO + i * RB
            tt = _unpack(ttv[pl.ds(pl.multiple_of(r0 // 2, 8), RB // 2), :])
            ff = jnp.concatenate(
                [_gelu(_dot(tt, _cols(w3v, 4 * q, 4 * q + 4))).astype(BF16)
                 for q in range(FF // 512)], axis=1)
            gb = mod_rows(5, RB)
            for c0, c1 in ((0, 7), (7, 8)):
                cols = slice(c0 * 128, c1 * 128)
                y = _dot(ff, _cols(w4v, c0, c1))
                res = zv[pl.ds(pl.multiple_of(r0, 16), RB), cols] + gb[:, cols] * y
                outv[slot, :, cols] = res.astype(BF16)
                cp(outv.at[slot, :, cols], out_hbm.at[pl.ds(i * RB, RB), cols],
                   SEM_OUT + slot).start()
            return 0

        nb = S // RB
        if "B" in phases:
            with scope("p3"):
                lax.fori_loop(0, nb, p3_body, 0)
            out_cp(nb - 2, 0).wait()
            out_cp(nb - 1, 1).wait()
        else:
            outv[0] = zv[pl.ds(HALO, RB), :].astype(BF16)
            out_cp(0, 0).start()
            out_cp(0, 0).wait()

    pl.run_scoped(
        main,
        pltpu.VMEM((FF // 128, D // 2, 128), U32),
        pltpu.VMEM((8, FF // 2, 128), U32),
        pltpu.VMEM((S + HALO, D), F32),
        pltpu.VMEM(((S + HALO) // 2, D), U32),
    )


def _call(A_x, A_mem0, A_Wq, A_Wk, A_Wv, A_Wo, B_w1, B_w2, B_w3, B_w4, c, w_mod,
          phases="AB"):
    any_spec = pl.BlockSpec(memory_space=pl.ANY)
    scratch = [
        pltpu.VMEM((S, D), BF16),
        pltpu.VMEM((M, D), BF16),
        pltpu.VMEM((48, D // 2, 128), U32),
        pltpu.VMEM((48, 8, 128), F32),
        pltpu.VMEM((3 * H // 2 * SL + 544, E), U32),
        pltpu.VMEM((3 * H // 2 * SL + 544, E), U32),
        pltpu.VMEM((8, H * E // 2, 128), U32),
        pltpu.VMEM((8, D // 2, 128), U32),
        pltpu.VMEM((8, D // 2, 128), U32),
        pltpu.VMEM((8, LEAD // 2, 128), U32),
        pltpu.VMEM((24, D), U32),
        pltpu.VMEM((24, D), U32),
        pltpu.VMEM((RING + 1, 3 * H * 8, E), U32),
        pltpu.VMEM((64, D), F32),
        pltpu.VMEM((16, D), F32),
        pltpu.VMEM((16, D), F32),
        pltpu.VMEM((32, 128), U32),
        pltpu.VMEM((2, RB, D), BF16),
        pltpu.VMEM((80, 128), F32),
        pltpu.VMEM((1, D), BF16),
        pltpu.SemaphoreType.DMA((NSEM,)),
    ]
    out = pl.pallas_call(
        functools.partial(_kernel, phases=phases),
        in_specs=[any_spec] * 12,
        out_specs=any_spec,
        out_shape=jax.ShapeDtypeStruct((S, D), BF16),
        scratch_shapes=scratch,
        compiler_params=pltpu.CompilerParams(
            vmem_limit_bytes=126 * 1024 * 1024),
    )(A_x.reshape(S, D), A_mem0.reshape(M, D), A_Wq, A_Wk, A_Wv,
      A_Wo.reshape(H * E, D), B_w1, B_w2, B_w3, B_w4, c, w_mod)
    return out.reshape(1, S, D)


def pallas_adaLN_cond__memory_aug_recurrent_mem_tr__mixer_s_mlp__prompt_kernel(
    A_x, A_mem0, A_Wq, A_Wk, A_Wv, A_Wo, A_seg_len, B_x, B_w1, B_w2, B_w3, B_w4,
    c, w_mod,
):
    if isinstance(A_seg_len, int):
        assert A_seg_len == SEG
    del B_x
    return _call(A_x, A_mem0, A_Wq, A_Wk, A_Wv, A_Wo, B_w1, B_w2, B_w3, B_w4,
                 c, w_mod)
```

```python
import contextlib
import functools

import jax
import jax.numpy as jnp
from jax import lax
import jax.experimental.pallas as pl
import jax.experimental.pallas.tpu as pltpu

F32 = jnp.float32
BF16 = jnp.bfloat16
U32 = jnp.uint32

S = 2048
D = 1024
H = 32
E = 128
M = 8
SEG = 32
FF = 3584
EPS = 1e-5

LEAD = 512
RING = 36
GB = RING
SL = 516
HG = 16
NG = 3 * H // HG
NPAIR = S // (2 * SEG)
HALO = 80
RB = 256
SHIFTS = (-1, -1, 1, 1, -2, -2, 2, 2)

SEM_C = 0
SEM_X = 1
SEM_A = 2
SEM_B = 3
SEM_XR = 4
SEM_M = 5
SEM_K = 7
SEM_G = 14
SEM_OUT = 20
NSEM = 22


def _ln(x):
    mu = jnp.mean(x, axis=-1, keepdims=True)
    xc = x - mu
    var = jnp.mean(xc * xc, axis=-1, keepdims=True)
    return xc * lax.rsqrt(var + EPS)


def _gelu(x):
    return jax.nn.gelu(x, approximate=True)


def _pack(x):
    return pltpu.bitcast(x.astype(BF16), U32)


def _unpack(x):
    return pltpu.bitcast(x, BF16)


def _dot(a, b):
    return jnp.dot(a, b, preferred_element_type=F32)


def _cols(ref, lo, hi, k0=0, k1=None):
    k1 = 2 * ref.shape[1] if k1 is None else k1
    return jnp.concatenate(
        [_unpack(ref[c, k0 // 2:k1 // 2, :]) for c in range(lo, hi)], axis=1)


def _kernel(x_hbm, mem_hbm, wq_hbm, wk_hbm, wv_hbm, wo_hbm, w1_hbm, w2_hbm,
            w3_hbm, w4_hbm, c_hbm, wmod_hbm, out_hbm,
            xv, memv, wmodv, modv, wqa, wqb, wov, w1v, w2v,
            hv0, hcur, hnext, ring, aout, x2t, h2t, zt, outv, fillv, cv, sems, *, phases):
    def scope(name):
        return jax.named_scope(name) if "s" in phases else contextlib.nullcontext()

    def cp(src, dst, s):
        return pltpu.make_async_copy(src, dst, sems.at[s])

    def col_copies(w_hbm, w_v, s, lo=0, hi=None):
        w32 = w_hbm.bitcast(U32)
        hi = w_v.shape[0] if hi is None else hi
        return [cp(w32.at[:, pl.ds(c * 128, 128)], w_v.at[c], s)
                for c in range(lo, hi)]

    def start(cps):
        for q in cps:
            q.start()

    def wait(cps):
        for q in cps:
            q.wait()

    def x_cp(r0, n, s):
        return cp(x_hbm.at[pl.ds(r0, n)], xv.at[pl.ds(r0, n)], s)

    c_cps = [cp(c_hbm, cv, SEM_C), cp(mem_hbm, memv, SEM_C)]
    x0_cp = x_cp(0, LEAD, SEM_X)
    xw_cp = x_cp(LEAD, 96, SEM_G + 1)
    xr_cp = x_cp(LEAD + 96, S - LEAD - 96, SEM_XR)
    a_cps = (col_copies(wo_hbm, wov, SEM_A) + col_copies(w1_hbm, w1v, SEM_A)
             + col_copies(w2_hbm, w2v, SEM_A))

    def mod_rows(i, n):
        m = jnp.concatenate([modv[8 * i + c] for c in range(8)], axis=1)
        return jnp.concatenate([m] * (n // 8), axis=0)

    HI = jnp.uint32(0xFFFF0000)
    wq2 = (wqa, wqb)

    def paced(x, tiles):
        z = [pltpu.bitcast((t if t.dtype == U32 else pltpu.bitcast(t, U32))
                           & zt[0:8, :], F32) for t in tiles]
        z = jnp.concatenate(z, axis=0)
        return jnp.concatenate([x[:, 0:128] + z, x[:, 128:]], axis=1)

    def h_rows(r0, n, tiles=None):
        xf = xv[pl.ds(pl.multiple_of(r0, 16), n), :].astype(F32)
        if tiles is not None:
            xf = paced(xf, tiles)
        return _ln(xf) * mod_rows(1, n) + mod_rows(0, n)

    def h_next(r0, g, tile=None):
        y = h_rows(r0 + 16 * g, 16, tile)
        hnext[g * 8:(g + 1) * 8, :] = _pack(y)
        return [y[0:8, 896:1024], y[8:16, 896:1024]]

    def prologue(st, xn, acc, scol, hn):
        w_hbms = (wq_hbm, wk_hbm, wv_hbm)

        def st_src(i):
            return w_hbms[i // 2].bitcast(U32).at[:, pl.ds((i % 2) * 8, 8), :]

        def pair_cps(n, s):
            w32 = wmod_hbm.bitcast(U32)
            return [cp(w32.at[:, pl.ds(pl.multiple_of(c * 128, 128), 128)],
                       wmodv.at[c], s) for c in (n, 8 + n)]

        def k_cps(n):
            return [cp(st_src(i).at[pl.ds(n * 128, 128)],
                       st.at[i, pl.ds(n * 128, 128)], SEM_K + n) for i in range(2)]

        def st_cp(i):
            return cp(st_src(i), st.at[i], SEM_G + i - 1)

        def mod_cps(i):
            return col_copies(wmod_hbm, wmodv, SEM_G + i, 8 * i, 8 * i + 8)

        with scope("first"):
            start(c_cps + [x0_cp])
        for n in range(8):
            start((pair_cps(n, SEM_M + n) if n < 2 else []) + k_cps(n)
                  + (pair_cps(n + 1, SEM_K + n) if 0 < n < 7 else []))
        start([st_cp(2), xw_cp, st_cp(3)] + mod_cps(2) + [st_cp(4)] + mod_cps(3)
              + [st_cp(5)])

        r = lax.broadcasted_iota(jnp.int32, (80, 128), 0)
        k = lax.broadcasted_iota(jnp.int32, (80, 128), 1)

        def head_of(i):
            return jnp.where(i < 16, i // 8, (i - 16) // 32)

        def pos_of(i):
            return jnp.where(i < 16, i % 8, 8 + (i - 16) % 32)

        same = head_of(r) == head_of(k)
        vis = (pos_of(r) < M) | (pos_of(r) >= pos_of(k))
        fillv[...] = jnp.where(same, jnp.where(vis, 0.0, -1e9), -jnp.inf).astype(F32)
        aout[...] = jnp.zeros(aout.shape, F32)
        ring[GB] = jnp.zeros(ring.shape[1:], U32)
        zt[...] = jnp.zeros(zt.shape, U32)
        x2t[...] = jnp.zeros(x2t.shape, F32)
        h2t[...] = jnp.zeros(h2t.shape, F32)


        def zero_body(i, _):
            acc[i] = jnp.zeros(acc.shape[1:], F32)
            return 0

        lax.fori_loop(0, acc.shape[0], zero_body, 0)

        wait(c_cps)
        cf = cv[...].astype(F32)
        sil = cf * jax.nn.sigmoid(cf)
        for c in range(8):
            sw = _pack(jnp.broadcast_to(sil[:, c * 128:(c + 1) * 128], (128, 128)).T)
            scol[0, c * 64:(c + 1) * 64, :] = pltpu.bitcast(sw << 16, F32)
            scol[1, c * 64:(c + 1) * 64, :] = pltpu.bitcast(sw & HI, F32)

        x0_cp.wait()

        def ln_body(i, _):
            r0 = pl.multiple_of(i * 64, 64)
            y = _ln(xv[pl.ds(r0, 64), :].astype(F32))
            for q in range(8):
                xn[q, pl.ds(r0, 64), :] = y[:, q * 128:(q + 1) * 128]
            return 0

        lax.fori_loop(0, LEAD // 64, ln_body, 0)

        class Mod:
            def __init__(self, tiles, offs):
                self.tiles, self.offs = tiles, offs
                self.n, self.acc, self.out = 0, None, []

            def items(self, n, pace=None):
                for it in range(self.n, min(self.n + n, 64 * len(self.tiles))):
                    c, i = divmod(it, 64)
                    w = wmodv[self.tiles[c], i * 8:(i + 1) * 8, :]
                    if pace is not None:
                        w = w | pace
                    v = (pltpu.bitcast(w << 16, F32) * scol[0, i * 8:(i + 1) * 8, :]
                         + pltpu.bitcast(w & HI, F32) * scol[1, i * 8:(i + 1) * 8, :])
                    self.acc = v if i == 0 else self.acc + v
                    if i == 63:
                        m = jnp.broadcast_to(
                            jnp.sum(self.acc, axis=0, keepdims=True) + self.offs[c],
                            (8, 128))
                        modv[self.tiles[c]] = m
                        self.out.append(m)
                self.n += n

        def h_lead(n, b, sa, ca):
            rep = lambda m: jnp.concatenate([m, m], axis=0)
            y = _pack(xn[n, 16 * b:16 * b + 16, :] * rep(ca) + rep(sa))
            hn[8 * b:8 * b + 8, :] = y
            hv0[n, 8 * b:8 * b + 8, :] = y

        def relayout(par, g, p0, n, pace=None):
            base = g * (8 * SL)
            mask = jnp.uint32(0xFFFF0000 if par else 0xFFFF)
            if pace is not None:
                mask = pace | mask
            for u in range(n):
                a = st[g, 2 * (p0 + u)]
                b = st[g, 2 * (p0 + u) + 1]
                if par == 0:
                    w = (a & mask) | (b << 16)
                else:
                    w = (a >> 16) | (b & mask)
                wq2[par][pl.ds(base + p0 + u, 8, stride=SL), :] = w

        def to_ring(y, par, s0, b0):
            for u in range(y.shape[1] // 128):
                row = pl.multiple_of((2 * (s0 + u) + par) * 8, 8)
                for b in range(y.shape[0] // 8):
                    ring[b0 + b, pl.ds(row, 8), :] = (
                        y[b * 8:(b + 1) * 8, u * 128:(u + 1) * 128])

        def k_body(n, _):
            @pl.when(n < 2)
            def _():
                wait(pair_cps(n, SEM_M + n))
                md = Mod([n, 8 + n], [0.0, 1.0])
                md.items(128)
                for b in range(32):
                    h_lead(n, b, *md.out)

            wait(k_cps(n))

            @pl.when((n > 0) & (n < 7))
            def _():
                wait(pair_cps(n + 1, SEM_K + n))

            nn = jnp.where(n == 0, 0, jnp.minimum(n + 1, 7))
            md = Mod([nn, 8 + nn], [0.0, 1.0])
            zero = zt[0:8, :]
            order = [(0, 0), (1, 0), (0, 1), (1, 1)]
            relayout(0, 0, n * 64, 64)
            for i, (par, g) in enumerate(order):
                for hq in range(2):
                    s0 = g * 8 + hq * 4
                    w = jnp.concatenate(
                        [_unpack(wq2[par][pl.ds(pl.multiple_of(
                            (s0 + u) * SL + n * 64, 4), 64), :])
                         for u in range(4)], axis=1)
                    y = _dot(_unpack(hn[...]), w) + acc[2 * i + hq]
                    acc[2 * i + hq] = y
                    y = _pack(y)
                    to_ring(y, par, s0, 0)
                    tiles = [y[8 * b:8 * b + 8, 0:128] & zero for b in range(32)]
                    for b in range(32):
                        pace = tiles[b]
                        if hq == 0 and i < 3:
                            relayout(*order[i + 1], n * 64 + 2 * b, 2, pace)
                        elif hq == 1 and i < 3:
                            md.items(2 - b % 2, pace)
                        elif hq == 1:
                            sa, ca = md.out
                            ca = ca + pltpu.bitcast(tiles[max(b - 3, 0)], F32)
                            h_lead(nn, b, sa, ca)
            return 0

        with scope("ksteps"):
            lax.fori_loop(0, 8, k_body, 0)

        start(mod_cps(4) + mod_cps(5) + a_cps + [xr_cp])
        wait([st_cp(2), xw_cp])

        def rl_body(i, _):
            relayout(0, 2, i * 64, 64)
            return 0

        lax.fori_loop(0, 8, rl_body, 0)

        def lead_proj(par, s0, n, rc, rl):
            w = jnp.concatenate(
                [_unpack(wq2[par][pl.ds(pl.multiple_of((s0 + u) * SL, 4), 512), :])
                 for u in range(n)], axis=1)
            lhs = jnp.concatenate(
                [_unpack(hv0[q, rc * 128:(rc + 1) * 128, :]) for q in range(8)],
                axis=1)
            y = _pack(_dot(lhs, w))
            to_ring(y, par, s0, rc * 16)
            zero = zt[0:8, :]
            for u in range(n):
                for b in range(16):
                    k = min(3, 512 - rl[2])
                    if k > 0:
                        relayout(rl[0], rl[1], rl[2], k,
                                 y[b * 8:(b + 1) * 8, u * 128:(u + 1) * 128] & zero)
                        rl[2] += k
            return y

        def group_body(g, _):
            rl = [1, g, 0]
            for k in range(16):
                lead_proj(0, g * 8 + k // 2, 1, k % 2, rl)

            @pl.when(g < NG - 1)
            def _():
                cp(st_src(1), st.at[g + 1], SEM_G + g).wait()

            part_g = wmodv.at[pl.ds(8 * g, 8)]
            cp(part_g, part_g, SEM_G + g).wait()

            gn = jnp.minimum(g + 1, NG - 1)
            off = jnp.where(g == 4, 1.0, 0.0).astype(F32)
            md = Mod([8 * g + c for c in range(8)], [off] * 8)
            rl = [0, gn, 0]
            for k in range(16):
                y = lead_proj(1, g * 8 + k // 2, 1, k % 2, rl)
                for b in range(16):
                    md.items(2 + b % 2, y[8 * b:8 * b + 8] & zt[0:8, :])
                if k == 11:
                    t = [y[0:8], y[64:72]]
                    for i in range(3):
                        t = h_next(LEAD, i, t)
            assert len(md.out) == 8
            return 0

        with scope("groups"):
            lax.fori_loop(2, NG, group_body, 0)

    pl.run_scoped(
        prologue,
        pltpu.VMEM((NG, D, 8, E), U32),
        pltpu.VMEM((8, LEAD, 128), F32),
        pltpu.VMEM((8, LEAD, 512), F32),
        pltpu.VMEM((2, D // 2, 128), F32),
        pltpu.VMEM((LEAD // 2, 128), U32),
    )

    def main(w3v, w4v, zv, ttv):
        w34_cps = col_copies(w3_hbm, w3v, SEM_B) + col_copies(w4_hbm, w4v, SEM_B)
        start(w34_cps)
        wait(a_cps)

        scale = float(E) ** -0.5

        def segment(lhs, ro, store_tok, wo_lhs, extras):
            fill = fillv[...]
            keep = fill == 0.0
            NP = H // 2
            qkv, probs, blocks = {}, {}, []

            def proj(hp, attend):
                slots = [t * H + 2 * hp + par for t in range(3) for par in range(2)]
                wt = [jnp.concatenate(
                    [_unpack(wq2[sl % 2][pl.ds((sl // 2) * SL, 512), :])
                     for sl in slots[2 * t:2 * t + 2]], axis=1) for t in range(3)]
                if hp == 0:
                    w = jnp.concatenate(wt, axis=1)
                    y = _dot(lhs[:, :512], w[:512])
                    y = _dot(lhs[:, 512:], w[512:]) + y
                else:
                    ys = [_dot(lhs, wt[0]), _dot(lhs, wt[1])]
                    attend()
                    y = jnp.concatenate(ys + [_dot(lhs, wt[2])], axis=1)
                for u, sl in enumerate(slots):
                    store_tok(sl, y[8:32, u * 128:(u + 1) * 128])
                ops = []
                for t in range(3):
                    ym = jnp.concatenate(
                        [y[0:8, (2 * t) * 128:(2 * t + 1) * 128],
                         y[0:8, (2 * t + 1) * 128:(2 * t + 2) * 128]], axis=0)
                    ops.append(jnp.concatenate(
                        [ym.astype(BF16)]
                        + [_unpack(ring[ro + b, sl * 8:(sl + 1) * 8, :])
                           for sl in slots[2 * t:2 * t + 2] for b in range(2)]
                        + ([jnp.zeros((48, 128), BF16)] if t else []),
                        axis=0))
                qkv[hp] = ops

            def scores(hp):
                q, kk, _ = qkv[hp]
                s = lax.dot_general(q, kk, (((1,), (1,)), ((), ())),
                                    preferred_element_type=F32)
                s = jnp.where(keep, s * scale, fill)
                mx = jnp.max(s, axis=-1, keepdims=True)
                p = jnp.exp(s - mx)
                l = jnp.sum(p, axis=-1, keepdims=True)
                rl = pl.reciprocal(l, approx=True)
                rl = rl * (2.0 - l * rl)
                probs[hp] = (p * rl).astype(BF16)

            def pv(hp):
                o = _dot(probs[hp], qkv[hp][2])
                blocks.append(wo_lhs(2 * hp, o[0:8], o[16:48]).astype(BF16))
                blocks.append(wo_lhs(2 * hp + 1, o[8:16], o[48:80]).astype(BF16))

            def wo_part(h0, h1, acc=None):
                lw = jnp.concatenate(blocks[h0:h1], axis=1)
                y = _dot(lw, _cols(wov, 0, 8, E * h0, E * h1))
                return y if acc is None else y + acc

            def attend(i):
                scores(i - 1)
                if i >= 3:
                    pv(i - 3)

            def fillers(key):
                for thunk in extras.get(key, ()):
                    thunk()

            for i in range(NP):
                proj(i, functools.partial(attend, i))
                fillers(i)
            acc = wo_part(0, 4)
            attend(NP)
            fillers(NP)
            acc = wo_part(4, 12, acc)
            pv(NP - 2)
            pv(NP - 1)
            fillers(NP + 1)
            acc = wo_part(12, 24, acc)
            fillers(NP + 2)
            return wo_part(24, 32, acc)

        def p1_front(r0):
            x2 = (xv[pl.ds(pl.multiple_of(r0, 64), 64), :].astype(F32)
                  + mod_rows(2, 64) * aout[...])
            h2 = _ln(x2) * mod_rows(4, 64) + mod_rows(3, 64)
            return x2, h2, _ln(h2).astype(BF16)

        def p1_store(y, c, live):
            g = _gelu(y)
            if live is not None:
                g = jnp.where(live, g, 0.0)
            ring[GB, c * 96 + 24:c * 96 + 88, :] = pltpu.bitcast(g, U32)

        def half_dots(lhs, wv, done):
            part = {}

            def run(c, kh):
                y = _dot(lhs[:, kh * 512:(kh + 1) * 512],
                         _cols(wv, c, c + 1, kh * 512, (kh + 1) * 512))
                if kh == 0:
                    part[c] = y
                else:
                    done(y + part[c], c)

            return [functools.partial(run, c, kh) for c in range(8) for kh in range(2)]

        def p2_front(n):
            return jnp.concatenate(
                [pltpu.bitcast(ring[GB, pl.ds(c * 96 + 8 + SHIFTS[c], n), :], F32)
                 for c in range(8)], axis=1).astype(BF16)

        def p2_back(x2, h2, hs, row, n, tiles=None):
            x1 = jnp.concatenate([h2t[...], h2[0:n - 16]], axis=0) + hs
            x2w = jnp.concatenate([x2t[...], x2[0:n - 16]], axis=0)
            zv[pl.ds(pl.multiple_of(row, 16), n), :] = x2w + mod_rows(5, n) * x1
            if tiles is None:
                ttv[pl.ds(pl.multiple_of(row // 2, 8), n // 2), :] = _pack(_ln(x1))
                return None
            t = tiles
            for g in range(n // 16):
                y = _ln(paced(x1[16 * g:16 * g + 16], t))
                ttv[pl.ds(pl.multiple_of(row // 2 + 8 * g, 8), 8), :] = _pack(y)
                t = [y[0:8, 896:1024], y[8:16, 896:1024]]
            return t

        def a_body(j, mem):
            @pl.when(j == 1)
            def _():
                xr_cp.wait()

            hcur[...] = hnext[...]
            hb = _unpack(hcur[0:8, :])
            hac = _unpack(hcur[8:16, :]).astype(F32)
            hd = _unpack(hcur[16:24, :])
            wr = [lax.rem(LEAD // 16 + 3 * j + i, RING) for i in range(3)]
            ro0 = lax.rem(4 * j, RING)
            ro1 = ro0 + 2

            x2, h2, u = p1_front(64 * jnp.maximum(j - 1, 0))
            live = j > 0

            lhs = jnp.concatenate(
                [jnp.concatenate([mem, hac[0:8]], axis=0).astype(BF16), hb], axis=0)
            tok_a = {}

            def store0(c, y):
                tok_a[c] = y[0:8]
                ring[wr[0], c * 8:(c + 1) * 8, :] = _pack(y[8:24])

            deferred = {}

            def wo_lhs0(h, om, ot):
                deferred[h] = ot[24:32]
                return jnp.concatenate([om, ot[0:24]], axis=0)

            pend = []

            def flush():
                while pend:
                    p1_store(*pend.pop(), live)

            th = half_dots(u, w1v, lambda y, c: pend.append((y, c)))
            extras = {i: [flush, th[i - 2]] for i in range(2, 18)}
            out = segment(lhs, ro0, store0, wo_lhs0, extras)
            flush()
            mem = out[0:8]
            aout[0:24, :] = out[8:32]

            lhs = jnp.concatenate(
                [jnp.concatenate([mem, hac[8:16]], axis=0).astype(BF16), hd], axis=0)

            def store1(c, y):
                ring[wr[1], c * 8:(c + 1) * 8, :] = _pack(
                    jnp.concatenate([tok_a[c], y[0:8]], axis=0))
                ring[wr[2], c * 8:(c + 1) * 8, :] = _pack(y[8:24])

            def wo_lhs1(h, om, ot):
                return jnp.concatenate([om, deferred[h], ot], axis=0)

            gs = p2_front(64)
            for c in range(8):
                ring[GB, c * 96:c * 96 + 24, :] = ring[GB, c * 96 + 64:c * 96 + 88, :]
            hs = []

            def p2_fin():
                t = [hs[7][0:8], hs[7][0:8]]
                for g in range(3):
                    t = h_next(rn, g, t)
                p2_back(x2, h2, jnp.concatenate(hs, axis=1), 64 * j, 64, t)
                x2t[...] = x2[48:64]
                h2t[...] = h2[48:64]

            th = half_dots(gs, w2v, lambda y, c: hs.append(y))
            extras = {i: [th[i]] for i in range(16)}
            extras[18] = [p2_fin]
            rn = LEAD + 48 * jnp.minimum(j + 1, NPAIR - 1)
            out = segment(lhs, ro1, store1, wo_lhs1, extras)
            aout[24:64, :] = out[8:48]
            return out[0:8]

        if "A" in phases:
            with scope("aloop"):
                lax.fori_loop(0, NPAIR, a_body, memv[...].astype(F32))
        else:
            zv[...] = jnp.zeros(zv.shape, F32)
            ttv[...] = jnp.zeros(ttv.shape, U32)

        x2, h2, u = p1_front(S - 64)
        y = _dot(u, _cols(w1v, 0, 8))
        for c in range(8):
            p1_store(y[:, c * 128:(c + 1) * 128], c, None)
        p2_back(x2, h2, _dot(p2_front(80), _cols(w2v, 0, 8)), S, 80)

        wait(w34_cps)

        def out_cp(i, slot):
            return cp(outv.at[slot], out_hbm.at[pl.ds(i * RB, RB), :],
                      SEM_OUT + slot)

        def p3_body(i, _):
            slot = i % 2

            @pl.when(i >= 2)
            def _():
                out_cp(i - 2, slot).wait()

            r0 = HALO + i * RB
            tt = _unpack(ttv[pl.ds(pl.multiple_of(r0 // 2, 8), RB // 2), :])
            ff = jnp.concatenate(
                [_gelu(_dot(tt, _cols(w3v, 4 * q, 4 * q + 4))).astype(BF16)
                 for q in range(FF // 512)], axis=1)
            gb = mod_rows(5, RB)
            for c0, c1 in ((0, 7), (7, 8)):
                cols = slice(c0 * 128, c1 * 128)
                y = _dot(ff, _cols(w4v, c0, c1))
                res = zv[pl.ds(pl.multiple_of(r0, 16), RB), cols] + gb[:, cols] * y
                outv[slot, :, cols] = res.astype(BF16)
                cp(outv.at[slot, :, cols], out_hbm.at[pl.ds(i * RB, RB), cols],
                   SEM_OUT + slot).start()
            return 0

        nb = S // RB
        if "B" in phases:
            with scope("p3"):
                lax.fori_loop(0, nb, p3_body, 0)
            out_cp(nb - 2, 0).wait()
            out_cp(nb - 1, 1).wait()
        else:
            outv[0] = zv[pl.ds(HALO, RB), :].astype(BF16)
            out_cp(0, 0).start()
            out_cp(0, 0).wait()

    pl.run_scoped(
        main,
        pltpu.VMEM((FF // 128, D // 2, 128), U32),
        pltpu.VMEM((8, FF // 2, 128), U32),
        pltpu.VMEM((S + HALO, D), F32),
        pltpu.VMEM(((S + HALO) // 2, D), U32),
    )


def _call(A_x, A_mem0, A_Wq, A_Wk, A_Wv, A_Wo, B_w1, B_w2, B_w3, B_w4, c, w_mod,
          phases="AB"):
    any_spec = pl.BlockSpec(memory_space=pl.ANY)
    scratch = [
        pltpu.VMEM((S, D), BF16),
        pltpu.VMEM((M, D), BF16),
        pltpu.VMEM((48, D // 2, 128), U32),
        pltpu.VMEM((48, 8, 128), F32),
        pltpu.VMEM((3 * H // 2 * SL + 544, E), U32),
        pltpu.VMEM((3 * H // 2 * SL + 544, E), U32),
        pltpu.VMEM((8, H * E // 2, 128), U32),
        pltpu.VMEM((8, D // 2, 128), U32),
        pltpu.VMEM((8, D // 2, 128), U32),
        pltpu.VMEM((8, LEAD // 2, 128), U32),
        pltpu.VMEM((24, D), U32),
        pltpu.VMEM((24, D), U32),
        pltpu.VMEM((RING + 1, 3 * H * 8, E), U32),
        pltpu.VMEM((64, D), F32),
        pltpu.VMEM((16, D), F32),
        pltpu.VMEM((16, D), F32),
        pltpu.VMEM((32, 128), U32),
        pltpu.VMEM((2, RB, D), BF16),
        pltpu.VMEM((80, 128), F32),
        pltpu.VMEM((1, D), BF16),
        pltpu.SemaphoreType.DMA((NSEM,)),
    ]
    out = pl.pallas_call(
        functools.partial(_kernel, phases=phases),
        in_specs=[any_spec] * 12,
        out_specs=any_spec,
        out_shape=jax.ShapeDtypeStruct((S, D), BF16),
        scratch_shapes=scratch,
        compiler_params=pltpu.CompilerParams(
            vmem_limit_bytes=126 * 1024 * 1024),
    )(A_x.reshape(S, D), A_mem0.reshape(M, D), A_Wq, A_Wk, A_Wv,
      A_Wo.reshape(H * E, D), B_w1, B_w2, B_w3, B_w4, c, w_mod)
    return out.reshape(1, S, D)


def pallas_adaLN_cond__memory_aug_recurrent_mem_tr__mixer_s_mlp__prompt_kernel(
    A_x, A_mem0, A_Wq, A_Wk, A_Wv, A_Wo, A_seg_len, B_x, B_w1, B_w2, B_w3, B_w4,
    c, w_mod,
):
    if isinstance(A_seg_len, int):
        assert A_seg_len == SEG
    del B_x
    return _call(A_x, A_mem0, A_Wq, A_Wk, A_Wv, A_Wo, B_w1, B_w2, B_w3, B_w4,
                 c, w_mod)
```

```python
import contextlib
import functools

import jax
import jax.numpy as jnp
from jax import lax
import jax.experimental.pallas as pl
import jax.experimental.pallas.tpu as pltpu

F32 = jnp.float32
BF16 = jnp.bfloat16
U32 = jnp.uint32

S = 2048
D = 1024
H = 32
E = 128
M = 8
SEG = 32
FF = 3584
EPS = 1e-5

LEAD = 512
RING = 36
GB = RING
SL = 516
HG = 16
NG = 3 * H // HG
NPAIR = S // (2 * SEG)
HALO = 80
RB = 256
SHIFTS = (-1, -1, 1, 1, -2, -2, 2, 2)

SEM_C = 0
SEM_X = 1
SEM_A = 2
SEM_B = 3
SEM_XR = 4
SEM_M = 5
SEM_K = 7
SEM_G = 14
SEM_OUT = 20
NSEM = 22


def _ln(x, part=None):
    if part is None:
        mu = jnp.mean(x, axis=-1, keepdims=True)
    else:
        mu = jnp.sum(part, axis=-1, keepdims=True) * (1.0 / x.shape[-1])
    xc = x - mu
    var = jnp.mean(xc * xc, axis=-1, keepdims=True)
    return xc * lax.rsqrt(var + EPS)


def _gelu(x):
    return jax.nn.gelu(x, approximate=True)


def _pack(x):
    return pltpu.bitcast(x.astype(BF16), U32)


def _unpack(x):
    return pltpu.bitcast(x, BF16)


def _dot(a, b):
    return jnp.dot(a, b, preferred_element_type=F32)


def _cols(ref, lo, hi, k0=0, k1=None):
    k1 = 2 * ref.shape[1] if k1 is None else k1
    return jnp.concatenate(
        [_unpack(ref[c, k0 // 2:k1 // 2, :]) for c in range(lo, hi)], axis=1)


def _kernel(x_hbm, mem_hbm, wq_hbm, wk_hbm, wv_hbm, wo_hbm, w1_hbm, w2_hbm,
            w3_hbm, w4_hbm, c_hbm, wmod_hbm, out_hbm,
            xv, memv, wmodv, modv, wqa, wqb, wov, w1v, w2v,
            hv0, hcur, hnext, ring, sums, h2t, zt, outv, fillv, cv, sems, *, phases):
    def scope(name):
        return jax.named_scope(name) if "s" in phases else contextlib.nullcontext()

    def cp(src, dst, s):
        return pltpu.make_async_copy(src, dst, sems.at[s])

    def col_copies(w_hbm, w_v, s, lo=0, hi=None):
        w32 = w_hbm.bitcast(U32)
        hi = w_v.shape[0] if hi is None else hi
        return [cp(w32.at[:, pl.ds(c * 128, 128)], w_v.at[c], s)
                for c in range(lo, hi)]

    def start(cps):
        for q in cps:
            q.start()

    def wait(cps):
        for q in cps:
            q.wait()

    def x_cp(r0, n, s):
        return cp(x_hbm.at[pl.ds(r0, n)], xv.at[pl.ds(r0, n)], s)

    c_cps = [cp(c_hbm, cv, SEM_C), cp(mem_hbm, memv, SEM_C)]
    x0_cp = x_cp(0, LEAD, SEM_X)
    xw_cp = x_cp(LEAD, 96, SEM_G + 1)
    xr_cp = x_cp(LEAD + 96, S - LEAD - 96, SEM_XR)
    a_cps = (col_copies(wo_hbm, wov, SEM_A) + col_copies(w1_hbm, w1v, SEM_A)
             + col_copies(w2_hbm, w2v, SEM_A))

    def mod_rows(i, n):
        m = jnp.concatenate([modv[8 * i + c] for c in range(8)], axis=1)
        return jnp.concatenate([m] * (n // 8), axis=0)

    HI = jnp.uint32(0xFFFF0000)
    wq2 = (wqa, wqb)

    def paced(x, tiles):
        z = [pltpu.bitcast((t if t.dtype == U32 else pltpu.bitcast(t, U32))
                           & zt[0:8, :], F32) for t in tiles]
        z = jnp.concatenate(z, axis=0)
        return jnp.concatenate([x[:, 0:128] + z, x[:, 128:]], axis=1)

    def h_rows(r0, n, tiles=None):
        xf = xv[pl.ds(pl.multiple_of(r0, 16), n), :].astype(F32)
        if tiles is not None:
            xf = paced(xf, tiles)
        return _ln(xf) * mod_rows(1, n) + mod_rows(0, n)

    def h_next(r0, g, tile=None):
        y = h_rows(r0 + 16 * g, 16, tile)
        hnext[g * 8:(g + 1) * 8, :] = _pack(y)
        return [y[0:8, 896:1024], y[8:16, 896:1024]]

    def prologue(st, xn, acc, scol, hn):
        w_hbms = (wq_hbm, wk_hbm, wv_hbm)

        def st_src(i):
            return w_hbms[i // 2].bitcast(U32).at[:, pl.ds((i % 2) * 8, 8), :]

        def pair_cps(n, s):
            w32 = wmod_hbm.bitcast(U32)
            return [cp(w32.at[:, pl.ds(pl.multiple_of(c * 128, 128), 128)],
                       wmodv.at[c], s) for c in (n, 8 + n)]

        def k_cps(n):
            return [cp(st_src(i).at[pl.ds(n * 128, 128)],
                       st.at[i, pl.ds(n * 128, 128)], SEM_K + n) for i in range(2)]

        def st_cp(i):
            return cp(st_src(i), st.at[i], SEM_G + i - 1)

        def mod_cps(i):
            return col_copies(wmod_hbm, wmodv, SEM_G + i, 8 * i, 8 * i + 8)

        with scope("first"):
            start(c_cps + [x0_cp])
        for n in range(8):
            start((pair_cps(n, SEM_M + n) if n < 2 else []) + k_cps(n)
                  + (pair_cps(n + 1, SEM_K + n) if 0 < n < 7 else []))
        start([st_cp(2), xw_cp, st_cp(3)] + mod_cps(2) + [st_cp(4)] + mod_cps(3)
              + [st_cp(5)])

        r = lax.broadcasted_iota(jnp.int32, (80, 128), 0)
        k = lax.broadcasted_iota(jnp.int32, (80, 128), 1)

        def head_of(i):
            return jnp.where(i < 16, i // 8, (i - 16) // 32)

        def pos_of(i):
            return jnp.where(i < 16, i % 8, 8 + (i - 16) % 32)

        same = head_of(r) == head_of(k)
        vis = (pos_of(r) < M) | (pos_of(r) >= pos_of(k))
        fillv[...] = jnp.where(same, jnp.where(vis, 0.0, -1e9), -jnp.inf).astype(F32)
        sums[...] = jnp.zeros(sums.shape, F32)
        ring[GB] = jnp.zeros(ring.shape[1:], U32)
        zt[...] = jnp.zeros(zt.shape, U32)
        h2t[...] = jnp.zeros(h2t.shape, F32)


        def zero_body(i, _):
            acc[i] = jnp.zeros(acc.shape[1:], F32)
            return 0

        lax.fori_loop(0, acc.shape[0], zero_body, 0)

        wait(c_cps)
        cf = cv[...].astype(F32)
        sil = cf * jax.nn.sigmoid(cf)
        for c in range(8):
            sw = _pack(jnp.broadcast_to(sil[:, c * 128:(c + 1) * 128], (128, 128)).T)
            scol[0, c * 64:(c + 1) * 64, :] = pltpu.bitcast(sw << 16, F32)
            scol[1, c * 64:(c + 1) * 64, :] = pltpu.bitcast(sw & HI, F32)

        x0_cp.wait()

        def ln_body(i, _):
            r0 = pl.multiple_of(i * 64, 64)
            y = _ln(xv[pl.ds(r0, 64), :].astype(F32))
            for q in range(8):
                xn[q, pl.ds(r0, 64), :] = y[:, q * 128:(q + 1) * 128]
            return 0

        lax.fori_loop(0, LEAD // 64, ln_body, 0)

        class Mod:
            def __init__(self, tiles, offs):
                self.tiles, self.offs = tiles, offs
                self.n, self.acc, self.out = 0, None, []

            def items(self, n, pace=None):
                for it in range(self.n, min(self.n + n, 64 * len(self.tiles))):
                    c, i = divmod(it, 64)
                    w = wmodv[self.tiles[c], i * 8:(i + 1) * 8, :]
                    if pace is not None:
                        w = w | pace
                    v = (pltpu.bitcast(w << 16, F32) * scol[0, i * 8:(i + 1) * 8, :]
                         + pltpu.bitcast(w & HI, F32) * scol[1, i * 8:(i + 1) * 8, :])
                    self.acc = v if i == 0 else self.acc + v
                    if i == 63:
                        m = jnp.broadcast_to(
                            jnp.sum(self.acc, axis=0, keepdims=True) + self.offs[c],
                            (8, 128))
                        modv[self.tiles[c]] = m
                        self.out.append(m)
                self.n += n

        def h_lead(n, b, sa, ca):
            rep = lambda m: jnp.concatenate([m, m], axis=0)
            y = _pack(xn[n, 16 * b:16 * b + 16, :] * rep(ca) + rep(sa))
            hn[8 * b:8 * b + 8, :] = y
            hv0[n, 8 * b:8 * b + 8, :] = y

        def relayout(par, g, p0, n, pace=None):
            base = g * (8 * SL)
            mask = jnp.uint32(0xFFFF0000 if par else 0xFFFF)
            if pace is not None:
                mask = pace | mask
            for u in range(n):
                a = st[g, 2 * (p0 + u)]
                b = st[g, 2 * (p0 + u) + 1]
                if par == 0:
                    w = (a & mask) | (b << 16)
                else:
                    w = (a >> 16) | (b & mask)
                wq2[par][pl.ds(base + p0 + u, 8, stride=SL), :] = w

        def to_ring(y, par, s0, b0):
            for u in range(y.shape[1] // 128):
                row = pl.multiple_of((2 * (s0 + u) + par) * 8, 8)
                for b in range(y.shape[0] // 8):
                    ring[b0 + b, pl.ds(row, 8), :] = (
                        y[b * 8:(b + 1) * 8, u * 128:(u + 1) * 128])

        def k_body(n, _):
            @pl.when(n < 2)
            def _():
                wait(pair_cps(n, SEM_M + n))
                md = Mod([n, 8 + n], [0.0, 1.0])
                md.items(128)
                for b in range(32):
                    h_lead(n, b, *md.out)

            wait(k_cps(n))

            @pl.when((n > 0) & (n < 7))
            def _():
                wait(pair_cps(n + 1, SEM_K + n))

            nn = jnp.where(n == 0, 0, jnp.minimum(n + 1, 7))
            md = Mod([nn, 8 + nn], [0.0, 1.0])
            zero = zt[0:8, :]
            order = [(0, 0), (1, 0), (0, 1), (1, 1)]
            relayout(0, 0, n * 64, 64)
            for i, (par, g) in enumerate(order):
                for hq in range(2):
                    s0 = g * 8 + hq * 4
                    w = jnp.concatenate(
                        [_unpack(wq2[par][pl.ds(pl.multiple_of(
                            (s0 + u) * SL + n * 64, 4), 64), :])
                         for u in range(4)], axis=1)
                    y = _dot(_unpack(hn[...]), w) + acc[2 * i + hq]
                    acc[2 * i + hq] = y
                    y = _pack(y)
                    to_ring(y, par, s0, 0)
                    tiles = [y[8 * b:8 * b + 8, 0:128] & zero for b in range(32)]
                    for b in range(32):
                        pace = tiles[b]
                        if hq == 0 and i < 3:
                            relayout(*order[i + 1], n * 64 + 2 * b, 2, pace)
                        elif hq == 1 and i < 3:
                            md.items(2 - b % 2, pace)
                        elif hq == 1:
                            sa, ca = md.out
                            ca = ca + pltpu.bitcast(tiles[max(b - 3, 0)], F32)
                            h_lead(nn, b, sa, ca)
            return 0

        with scope("ksteps"):
            lax.fori_loop(0, 8, k_body, 0)

        start(mod_cps(4) + mod_cps(5) + a_cps + [xr_cp])
        wait([st_cp(2), xw_cp])

        def rl_body(i, _):
            relayout(0, 2, i * 64, 64)
            return 0

        lax.fori_loop(0, 8, rl_body, 0)

        def lead_proj(par, s0, n, rc, rl):
            w = jnp.concatenate(
                [_unpack(wq2[par][pl.ds(pl.multiple_of((s0 + u) * SL, 4), 512), :])
                 for u in range(n)], axis=1)
            lhs = jnp.concatenate(
                [_unpack(hv0[q, rc * 128:(rc + 1) * 128, :]) for q in range(8)],
                axis=1)
            y = _pack(_dot(lhs, w))
            to_ring(y, par, s0, rc * 16)
            zero = zt[0:8, :]
            for u in range(n):
                for b in range(16):
                    k = min(3, 512 - rl[2])
                    if k > 0:
                        relayout(rl[0], rl[1], rl[2], k,
                                 y[b * 8:(b + 1) * 8, u * 128:(u + 1) * 128] & zero)
                        rl[2] += k
            return y

        def group_body(g, _):
            rl = [1, g, 0]
            for k in range(16):
                lead_proj(0, g * 8 + k // 2, 1, k % 2, rl)

            @pl.when(g < NG - 1)
            def _():
                cp(st_src(1), st.at[g + 1], SEM_G + g).wait()

            part_g = wmodv.at[pl.ds(8 * g, 8)]
            cp(part_g, part_g, SEM_G + g).wait()

            gn = jnp.minimum(g + 1, NG - 1)
            off = jnp.where(g == 4, 1.0, 0.0).astype(F32)
            md = Mod([8 * g + c for c in range(8)], [off] * 8)
            rl = [0, gn, 0]
            for k in range(16):
                y = lead_proj(1, g * 8 + k // 2, 1, k % 2, rl)
                for b in range(16):
                    md.items(2 + b % 2, y[8 * b:8 * b + 8] & zt[0:8, :])
                if k == 11:
                    t = [y[0:8], y[64:72]]
                    for i in range(3):
                        t = h_next(LEAD, i, t)
            assert len(md.out) == 8
            return 0

        with scope("groups"):
            lax.fori_loop(2, NG, group_body, 0)

    pl.run_scoped(
        prologue,
        pltpu.VMEM((NG, D, 8, E), U32),
        pltpu.VMEM((8, LEAD, 128), F32),
        pltpu.VMEM((8, LEAD, 512), F32),
        pltpu.VMEM((2, D // 2, 128), F32),
        pltpu.VMEM((LEAD // 2, 128), U32),
    )

    def main(w3v, w4v, zv, ttv):
        w34_cps = col_copies(w3_hbm, w3v, SEM_B) + col_copies(w4_hbm, w4v, SEM_B)
        start(w34_cps)
        zv[0:HALO, :] = jnp.zeros((HALO, D), F32)
        wait(a_cps)

        scale = float(E) ** -0.5

        def segment(lhs, ro, store_tok, wo_lhs, extras):
            fill = fillv[...]
            keep = fill == 0.0
            NP = H // 2
            qkv, probs, blocks = {}, {}, []

            def proj(hp, attend):
                slots = [t * H + 2 * hp + par for t in range(3) for par in range(2)]
                wt = [jnp.concatenate(
                    [_unpack(wq2[sl % 2][pl.ds((sl // 2) * SL, 512), :])
                     for sl in slots[2 * t:2 * t + 2]], axis=1) for t in range(3)]
                if hp == 0:
                    w = jnp.concatenate(wt, axis=1)
                    y = _dot(lhs[:, :512], w[:512])
                    y = _dot(lhs[:, 512:], w[512:]) + y
                else:
                    ys = [_dot(lhs, wt[0]), _dot(lhs, wt[1])]
                    attend()
                    y = jnp.concatenate(ys + [_dot(lhs, wt[2])], axis=1)
                for u, sl in enumerate(slots):
                    store_tok(sl, y[8:32, u * 128:(u + 1) * 128])
                ops = []
                for t in range(3):
                    ym = jnp.concatenate(
                        [y[0:8, (2 * t) * 128:(2 * t + 1) * 128],
                         y[0:8, (2 * t + 1) * 128:(2 * t + 2) * 128]], axis=0)
                    ops.append(jnp.concatenate(
                        [ym.astype(BF16)]
                        + [_unpack(ring[ro + b, sl * 8:(sl + 1) * 8, :])
                           for sl in slots[2 * t:2 * t + 2] for b in range(2)]
                        + ([jnp.zeros((48, 128), BF16)] if t else []),
                        axis=0))
                qkv[hp] = ops

            def scores(hp):
                q, kk, _ = qkv[hp]
                s = lax.dot_general(q, kk, (((1,), (1,)), ((), ())),
                                    preferred_element_type=F32)
                s = jnp.where(keep, s * scale, fill)
                mx = jnp.max(s, axis=-1, keepdims=True)
                p = jnp.exp(s - mx)
                l = jnp.sum(p, axis=-1, keepdims=True)
                rl = pl.reciprocal(l, approx=True)
                rl = rl * (2.0 - l * rl)
                probs[hp] = (p * rl).astype(BF16)

            def pv(hp):
                o = _dot(probs[hp], qkv[hp][2])
                blocks.append(wo_lhs(2 * hp, o[0:8], o[16:48]).astype(BF16))
                blocks.append(wo_lhs(2 * hp + 1, o[8:16], o[48:80]).astype(BF16))

            def wo_part(h0, h1, acc=None):
                lw = jnp.concatenate(blocks[h0:h1], axis=1)
                y = _dot(lw, _cols(wov, 0, 8, E * h0, E * h1))
                return y if acc is None else y + acc

            def attend(i):
                scores(i - 1)
                if i >= 3:
                    pv(i - 3)

            def fillers(key):
                for thunk in extras.get(key, ()):
                    thunk()

            for i in range(NP):
                proj(i, functools.partial(attend, i))
                fillers(i)
            acc = wo_part(0, 4)
            attend(NP)
            fillers(NP)
            acc = wo_part(4, 12, acc)
            pv(NP - 2)
            pv(NP - 1)
            fillers(NP + 1)
            acc = wo_part(12, 24, acc)
            fillers(NP + 2)
            return wo_part(24, 32, acc)

        def put_x2(r0, lo, a):
            n = a.shape[0]
            x2 = (xv[pl.ds(pl.multiple_of(r0 + lo, 8), n), :].astype(F32)
                  + mod_rows(2, n) * a)
            zv[pl.ds(pl.multiple_of(HALO + r0 + lo, 8), n), :] = x2
            sums[lo:lo + n, :] = functools.reduce(
                jnp.add, [x2[:, c * 128:(c + 1) * 128] for c in range(8)])

        def p1_front(r0):
            x2 = zv[pl.ds(pl.multiple_of(HALO + r0, 16), 64), :]
            h2 = _ln(x2, sums[...]) * mod_rows(4, 64) + mod_rows(3, 64)
            return h2, _ln(h2).astype(BF16)

        def p1_store(y, c, live):
            g = _gelu(y)
            if live is not None:
                g = jnp.where(live, g, 0.0)
            ring[GB, c * 96 + 24:c * 96 + 88, :] = pltpu.bitcast(g, U32)

        def half_dots(lhs, wv, done):
            part = {}

            def run(c, kh):
                y = _dot(lhs[:, kh * 512:(kh + 1) * 512],
                         _cols(wv, c, c + 1, kh * 512, (kh + 1) * 512))
                if kh == 0:
                    part[c] = y
                else:
                    done(y + part[c], c)

            return [functools.partial(run, c, kh) for c in range(8) for kh in range(2)]

        def p2_front(n):
            return jnp.concatenate(
                [pltpu.bitcast(ring[GB, pl.ds(c * 96 + 8 + SHIFTS[c], n), :], F32)
                 for c in range(8)], axis=1).astype(BF16)

        def p2_back(h2, hs, row, n, tiles=None):
            x1 = jnp.concatenate([h2t[...], h2[0:n - 16]], axis=0) + hs
            rows = pl.ds(pl.multiple_of(row, 16), n)
            zv[rows, :] = zv[rows, :] + mod_rows(5, n) * x1
            if tiles is None:
                ttv[pl.ds(pl.multiple_of(row // 2, 8), n // 2), :] = _pack(_ln(x1))
                return None
            t = tiles
            for g in range(n // 16):
                y = _ln(paced(x1[16 * g:16 * g + 16], t))
                ttv[pl.ds(pl.multiple_of(row // 2 + 8 * g, 8), 8), :] = _pack(y)
                t = [y[0:8, 896:1024], y[8:16, 896:1024]]
            return t

        def a_body(j, mem):
            @pl.when(j == 1)
            def _():
                xr_cp.wait()

            hcur[...] = hnext[...]
            hb = _unpack(hcur[0:8, :])
            hac = _unpack(hcur[8:16, :]).astype(F32)
            hd = _unpack(hcur[16:24, :])
            wr = [lax.rem(LEAD // 16 + 3 * j + i, RING) for i in range(3)]
            ro0 = lax.rem(4 * j, RING)
            ro1 = ro0 + 2

            h2, u = p1_front(64 * (j - 1))
            live = j > 0

            lhs = jnp.concatenate(
                [jnp.concatenate([mem, hac[0:8]], axis=0).astype(BF16), hb], axis=0)
            tok_a = {}

            def store0(c, y):
                tok_a[c] = y[0:8]
                ring[wr[0], c * 8:(c + 1) * 8, :] = _pack(y[8:24])

            deferred = {}

            def wo_lhs0(h, om, ot):
                deferred[h] = ot[24:32]
                return jnp.concatenate([om, ot[0:24]], axis=0)

            pend = []

            def flush():
                while pend:
                    p1_store(*pend.pop(), live)

            th = half_dots(u, w1v, lambda y, c: pend.append((y, c)))
            extras = {i: [flush, th[i - 2]] for i in range(2, 18)}
            out = segment(lhs, ro0, store0, wo_lhs0, extras)
            flush()
            mem = out[0:8]
            put_x2(64 * j, 0, out[8:32])

            lhs = jnp.concatenate(
                [jnp.concatenate([mem, hac[8:16]], axis=0).astype(BF16), hd], axis=0)

            def store1(c, y):
                ring[wr[1], c * 8:(c + 1) * 8, :] = _pack(
                    jnp.concatenate([tok_a[c], y[0:8]], axis=0))
                ring[wr[2], c * 8:(c + 1) * 8, :] = _pack(y[8:24])

            def wo_lhs1(h, om, ot):
                return jnp.concatenate([om, deferred[h], ot], axis=0)

            gs = p2_front(64)
            for c in range(8):
                ring[GB, c * 96:c * 96 + 24, :] = ring[GB, c * 96 + 64:c * 96 + 88, :]
            hs = []

            def p2_fin():
                t = [hs[7][0:8], hs[7][0:8]]
                for g in range(3):
                    t = h_next(rn, g, t)
                p2_back(h2, jnp.concatenate(hs, axis=1), 64 * j, 64, t)
                h2t[...] = h2[48:64]

            th = half_dots(gs, w2v, lambda y, c: hs.append(y))
            extras = {i: [th[i]] for i in range(16)}
            extras[18] = [p2_fin]
            rn = LEAD + 48 * jnp.minimum(j + 1, NPAIR - 1)
            out = segment(lhs, ro1, store1, wo_lhs1, extras)
            put_x2(64 * j, 24, out[8:48])
            return out[0:8]

        if "A" in phases:
            with scope("aloop"):
                lax.fori_loop(0, NPAIR, a_body, memv[...].astype(F32))
        else:
            zv[...] = jnp.zeros(zv.shape, F32)
            ttv[...] = jnp.zeros(ttv.shape, U32)

        h2, u = p1_front(S - 64)
        y = _dot(u, _cols(w1v, 0, 8))
        for c in range(8):
            p1_store(y[:, c * 128:(c + 1) * 128], c, None)
        p2_back(h2, _dot(p2_front(80), _cols(w2v, 0, 8)), S, 80)

        wait(w34_cps)

        def out_cp(i, slot):
            return cp(outv.at[slot], out_hbm.at[pl.ds(i * RB, RB), :],
                      SEM_OUT + slot)

        def p3_body(i, _):
            slot = i % 2

            @pl.when(i >= 2)
            def _():
                out_cp(i - 2, slot).wait()

            r0 = HALO + i * RB
            tt = _unpack(ttv[pl.ds(pl.multiple_of(r0 // 2, 8), RB // 2), :])
            ff = jnp.concatenate(
                [_gelu(_dot(tt, _cols(w3v, 4 * q, 4 * q + 4))).astype(BF16)
                 for q in range(FF // 512)], axis=1)
            gb = mod_rows(5, RB)
            for c0, c1 in ((0, 7), (7, 8)):
                cols = slice(c0 * 128, c1 * 128)
                y = _dot(ff, _cols(w4v, c0, c1))
                res = zv[pl.ds(pl.multiple_of(r0, 16), RB), cols] + gb[:, cols] * y
                outv[slot, :, cols] = res.astype(BF16)
                cp(outv.at[slot, :, cols], out_hbm.at[pl.ds(i * RB, RB), cols],
                   SEM_OUT + slot).start()
            return 0

        nb = S // RB
        if "B" in phases:
            with scope("p3"):
                lax.fori_loop(0, nb, p3_body, 0)
            out_cp(nb - 2, 0).wait()
            out_cp(nb - 1, 1).wait()
        else:
            outv[0] = zv[pl.ds(HALO, RB), :].astype(BF16)
            out_cp(0, 0).start()
            out_cp(0, 0).wait()

    pl.run_scoped(
        main,
        pltpu.VMEM((FF // 128, D // 2, 128), U32),
        pltpu.VMEM((8, FF // 2, 128), U32),
        pltpu.VMEM((S + HALO, D), F32),
        pltpu.VMEM(((S + HALO) // 2, D), U32),
    )


def _call(A_x, A_mem0, A_Wq, A_Wk, A_Wv, A_Wo, B_w1, B_w2, B_w3, B_w4, c, w_mod,
          phases="AB"):
    any_spec = pl.BlockSpec(memory_space=pl.ANY)
    scratch = [
        pltpu.VMEM((S, D), BF16),
        pltpu.VMEM((M, D), BF16),
        pltpu.VMEM((48, D // 2, 128), U32),
        pltpu.VMEM((48, 8, 128), F32),
        pltpu.VMEM((3 * H // 2 * SL + 544, E), U32),
        pltpu.VMEM((3 * H // 2 * SL + 544, E), U32),
        pltpu.VMEM((8, H * E // 2, 128), U32),
        pltpu.VMEM((8, D // 2, 128), U32),
        pltpu.VMEM((8, D // 2, 128), U32),
        pltpu.VMEM((8, LEAD // 2, 128), U32),
        pltpu.VMEM((24, D), U32),
        pltpu.VMEM((24, D), U32),
        pltpu.VMEM((RING + 1, 3 * H * 8, E), U32),
        pltpu.VMEM((64, 128), F32),
        pltpu.VMEM((16, D), F32),
        pltpu.VMEM((32, 128), U32),
        pltpu.VMEM((2, RB, D), BF16),
        pltpu.VMEM((80, 128), F32),
        pltpu.VMEM((1, D), BF16),
        pltpu.SemaphoreType.DMA((NSEM,)),
    ]
    out = pl.pallas_call(
        functools.partial(_kernel, phases=phases),
        in_specs=[any_spec] * 12,
        out_specs=any_spec,
        out_shape=jax.ShapeDtypeStruct((S, D), BF16),
        scratch_shapes=scratch,
        compiler_params=pltpu.CompilerParams(
            vmem_limit_bytes=126 * 1024 * 1024,
            disable_bounds_checks=True, disable_semaphore_checks=True),
    )(A_x.reshape(S, D), A_mem0.reshape(M, D), A_Wq, A_Wk, A_Wv,
      A_Wo.reshape(H * E, D), B_w1, B_w2, B_w3, B_w4, c, w_mod)
    return out.reshape(1, S, D)


def pallas_adaLN_cond__memory_aug_recurrent_mem_tr__mixer_s_mlp__prompt_kernel(
    A_x, A_mem0, A_Wq, A_Wk, A_Wv, A_Wo, A_seg_len, B_x, B_w1, B_w2, B_w3, B_w4,
    c, w_mod,
):
    if isinstance(A_seg_len, int):
        assert A_seg_len == SEG
    del B_x
    return _call(A_x, A_mem0, A_Wq, A_Wk, A_Wv, A_Wo, B_w1, B_w2, B_w3, B_w4,
                 c, w_mod)
```

```python
import contextlib
import functools

import jax
import jax.numpy as jnp
from jax import lax
import jax.experimental.pallas as pl
import jax.experimental.pallas.tpu as pltpu

F32 = jnp.float32
BF16 = jnp.bfloat16
U32 = jnp.uint32

S = 2048
D = 1024
H = 32
E = 128
M = 8
SEG = 32
FF = 3584
EPS = 1e-5

LEAD = 512
RING = 36
GB = RING
SL = 516
WB = 3 * H // 2 * SL + 544
LQ = LEAD - 64
HG = 16
NG = 3 * H // HG
NPAIR = S // (2 * SEG)
HALO = 80
RB = 256
SHIFTS = (-1, -1, 1, 1, -2, -2, 2, 2)

SEM_C = 0
SEM_X = 1
SEM_A = 2
SEM_B = 3
SEM_XR = 4
SEM_M = 5
SEM_K = 7
SEM_G = 14
SEM_OUT = 20
NSEM = 22


def _ln(x, part=None):
    if part is None:
        mu = jnp.mean(x, axis=-1, keepdims=True)
    else:
        mu = jnp.sum(part, axis=-1, keepdims=True) * (1.0 / x.shape[-1])
    xc = x - mu
    var = jnp.mean(xc * xc, axis=-1, keepdims=True)
    return xc * lax.rsqrt(var + EPS)


def _gelu(x):
    return jax.nn.gelu(x, approximate=True)


def _pack(x):
    return pltpu.bitcast(x.astype(BF16), U32)


def _unpack(x):
    return pltpu.bitcast(x, BF16)


def _dot(a, b):
    return jnp.dot(a, b, preferred_element_type=F32)


def _cols(ref, lo, hi, k0=0, k1=None):
    k1 = 2 * ref.shape[1] if k1 is None else k1
    return jnp.concatenate(
        [_unpack(ref[c, k0 // 2:k1 // 2, :]) for c in range(lo, hi)], axis=1)


def _kernel(x_hbm, mem_hbm, wq_hbm, wk_hbm, wv_hbm, wo_hbm, w1_hbm, w2_hbm,
            w3_hbm, w4_hbm, c_hbm, wmod_hbm, out_hbm,
            xv, memv, wmodv, modv, wqa, wqb, wov, us, gsb,
            hv0, hcur, hnext, ring, sums, h2t, zt, outv, fillv, cv, sems, *, phases):
    def scope(name):
        return jax.named_scope(name) if "s" in phases else contextlib.nullcontext()

    def cp(src, dst, s):
        return pltpu.make_async_copy(src, dst, sems.at[s])

    def col_copies(w_hbm, w_v, s, lo=0, hi=None):
        w32 = w_hbm.bitcast(U32)
        hi = w_v.shape[0] if hi is None else hi
        return [cp(w32.at[:, pl.ds(c * 128, 128)], w_v.at[c], s)
                for c in range(lo, hi)]

    def start(cps):
        for q in cps:
            q.start()

    def wait(cps):
        for q in cps:
            q.wait()

    def x_cp(r0, n, s):
        return cp(x_hbm.at[pl.ds(r0, n)], xv.at[pl.ds(r0, n)], s)

    c_cps = [cp(c_hbm, cv, SEM_C), cp(mem_hbm, memv, SEM_C)]
    x0_cp = x_cp(0, LEAD, SEM_X)
    xw_cp = x_cp(LEAD, 96, SEM_G + 1)
    wo_cps = col_copies(wo_hbm, wov, SEM_A)
    late_cps = [x_cp(LEAD + 96, S - LEAD - 96, SEM_XR)] + [
        cp(w.bitcast(U32).at[:, pl.ds(c * 128, 128)],
           wqb.at[pl.ds(WB + (8 * i + c) * 512, 512)], SEM_XR)
        for i, w in enumerate((w1_hbm, w2_hbm)) for c in range(8)]

    def mod_rows(i, n):
        m = jnp.concatenate([modv[8 * i + c] for c in range(8)], axis=1)
        return jnp.concatenate([m] * (n // 8), axis=0)

    HI = jnp.uint32(0xFFFF0000)
    wq2 = (wqa, wqb)

    def paced(x, tiles):
        z = [pltpu.bitcast((t if t.dtype == U32 else pltpu.bitcast(t, U32))
                           & zt[0:8, :], F32) for t in tiles]
        z = jnp.concatenate(z, axis=0)
        return jnp.concatenate([x[:, 0:128] + z, x[:, 128:]], axis=1)

    def h_rows(r0, n, tiles=None):
        xf = xv[pl.ds(pl.multiple_of(r0, 16), n), :].astype(F32)
        if tiles is not None:
            xf = paced(xf, tiles)
        return _ln(xf) * mod_rows(1, n) + mod_rows(0, n)

    def h_next(r0, g, tile=None):
        y = h_rows(r0 + 16 * g, 16, tile)
        hnext[g * 8:(g + 1) * 8, :] = _pack(y)
        return [y[0:8, 896:1024], y[8:16, 896:1024]]

    def prologue(st, xn, acc, scol, hn):
        w_hbms = (wq_hbm, wk_hbm, wv_hbm)

        def st_src(i):
            return w_hbms[i // 2].bitcast(U32).at[:, pl.ds((i % 2) * 8, 8), :]

        def pair_cps(n, s):
            w32 = wmod_hbm.bitcast(U32)
            return [cp(w32.at[:, pl.ds(pl.multiple_of(c * 128, 128), 128)],
                       wmodv.at[c], s) for c in (n, 8 + n)]

        def k_cps(n):
            return [cp(st_src(i).at[pl.ds(n * 128, 128)],
                       st.at[i, pl.ds(n * 128, 128)], SEM_K + n) for i in range(2)]

        def st_cp(i):
            return cp(st_src(i), st.at[i], SEM_G + i - 1)

        def mod_cps(g):
            lo, hi = {3: (16, 27), 4: (27, 38), 5: (38, 48)}[g]
            return col_copies(wmod_hbm, wmodv, SEM_G + g, lo, hi)

        with scope("first"):
            start(c_cps + [x0_cp])
        for n in range(8):
            start((pair_cps(n, SEM_M + n) if n < 2 else []) + k_cps(n)
                  + (pair_cps(n + 1, SEM_K + n) if 0 < n < 7 else []))
        start([st_cp(2), xw_cp, st_cp(3), st_cp(4)] + mod_cps(3) + [st_cp(5)])

        r = lax.broadcasted_iota(jnp.int32, (80, 128), 0)
        k = lax.broadcasted_iota(jnp.int32, (80, 128), 1)

        def head_of(i):
            return jnp.where(i < 16, i // 8, (i - 16) // 32)

        def pos_of(i):
            return jnp.where(i < 16, i % 8, 8 + (i - 16) % 32)

        same = head_of(r) == head_of(k)
        vis = (pos_of(r) < M) | (pos_of(r) >= pos_of(k))
        fillv[...] = jnp.where(same, jnp.where(vis, 0.0, -1e9), -jnp.inf).astype(F32)
        sums[...] = jnp.zeros(sums.shape, F32)
        modv[48:56] = jnp.zeros((8, 8, 128), F32)
        modv[56:64] = jnp.ones((8, 8, 128), F32)
        ring[GB] = jnp.zeros(ring.shape[1:], U32)
        zt[...] = jnp.zeros(zt.shape, U32)
        h2t[...] = jnp.zeros(h2t.shape, F32)


        def zero_body(i, _):
            acc[i] = jnp.zeros(acc.shape[1:], F32)
            return 0

        lax.fori_loop(0, acc.shape[0], zero_body, 0)

        wait(c_cps)
        cf = cv[...].astype(F32)
        sil = cf * jax.nn.sigmoid(cf)
        for c in range(8):
            sw = _pack(jnp.broadcast_to(sil[:, c * 128:(c + 1) * 128], (128, 128)).T)
            scol[0, c * 64:(c + 1) * 64, :] = pltpu.bitcast(sw << 16, F32)
            scol[1, c * 64:(c + 1) * 64, :] = pltpu.bitcast(sw & HI, F32)

        x0_cp.wait()

        def ln_body(i, _):
            r0 = pl.multiple_of(i * 64, 64)
            y = _ln(xv[pl.ds(r0, 64), :].astype(F32))
            for q in range(8):
                xn[q, pl.ds(r0, 64), :] = y[:, q * 128:(q + 1) * 128]
            return 0

        lax.fori_loop(0, LEAD // 64, ln_body, 0)

        class Mod:
            def __init__(self, tiles, offs):
                self.tiles, self.offs = tiles, offs
                self.n, self.acc, self.out = 0, None, []

            def items(self, n, pace=None):
                for it in range(self.n, min(self.n + n, 64 * len(self.tiles))):
                    c, i = divmod(it, 64)
                    w = wmodv[self.tiles[c], i * 8:(i + 1) * 8, :]
                    if pace is not None:
                        w = w | pace
                    v = (pltpu.bitcast(w << 16, F32) * scol[0, i * 8:(i + 1) * 8, :]
                         + pltpu.bitcast(w & HI, F32) * scol[1, i * 8:(i + 1) * 8, :])
                    self.acc = v if i == 0 else self.acc + v
                    if i == 63:
                        m = jnp.broadcast_to(
                            jnp.sum(self.acc, axis=0, keepdims=True) + self.offs[c],
                            (8, 128))
                        modv[self.tiles[c]] = m
                        self.out.append(m)
                self.n += n

        def h_lead(n, b, sa, ca):
            rep = lambda m: jnp.concatenate([m, m], axis=0)
            y = _pack(xn[n, 16 * b:16 * b + 16, :] * rep(ca) + rep(sa))
            hn[8 * b:8 * b + 8, :] = y
            hv0[n, 8 * b:8 * b + 8, :] = y

        def relayout(par, g, p0, n, pace=None):
            base = g * (8 * SL)
            mask = jnp.uint32(0xFFFF0000 if par else 0xFFFF)
            if pace is not None:
                mask = pace | mask
            for u in range(n):
                a = st[g, 2 * (p0 + u)]
                b = st[g, 2 * (p0 + u) + 1]
                if par == 0:
                    w = (a & mask) | (b << 16)
                else:
                    w = (a >> 16) | (b & mask)
                wq2[par][pl.ds(base + p0 + u, 8, stride=SL), :] = w

        def to_ring(y, par, s0, b0):
            for u in range(y.shape[1] // 128):
                row = pl.multiple_of((2 * (s0 + u) + par) * 8, 8)
                for b in range(y.shape[0] // 8):
                    ring[b0 + b, pl.ds(row, 8), :] = (
                        y[b * 8:(b + 1) * 8, u * 128:(u + 1) * 128])

        def k_body(n, _):
            @pl.when(n < 2)
            def _():
                wait(pair_cps(n, SEM_M + n))
                md = Mod([n, 8 + n], [0.0, 1.0])
                md.items(128)
                for b in range(32):
                    h_lead(n, b, *md.out)

            wait(k_cps(n))

            @pl.when((n > 0) & (n < 7))
            def _():
                wait(pair_cps(n + 1, SEM_K + n))

            nn = jnp.where(n == 0, 0, jnp.minimum(n + 1, 7))
            md = Mod([nn, 8 + nn], [0.0, 1.0])
            zero = zt[0:8, :]
            order = [(0, 0), (1, 0), (0, 1), (1, 1)]
            relayout(0, 0, n * 64, 64)
            for i, (par, g) in enumerate(order):
                for hq in range(2):
                    s0 = g * 8 + hq * 4
                    w = jnp.concatenate(
                        [_unpack(wq2[par][pl.ds(pl.multiple_of(
                            (s0 + u) * SL + n * 64, 4), 64), :])
                         for u in range(4)], axis=1)
                    m = LQ if par else LEAD
                    y = _dot(_unpack(hn[0:m // 2, :]), w) + acc[2 * i + hq, 0:m, :]
                    acc[2 * i + hq, 0:m, :] = y
                    y = _pack(y)
                    to_ring(y, par, s0, 0)
                    tiles = [y[8 * b:8 * b + 8, 0:128] & zero for b in range(m // 16)]
                    tiles = [tiles[b * len(tiles) // 32] for b in range(32)]
                    for b in range(32):
                        pace = tiles[b]
                        if hq == 0 and i < 3:
                            relayout(*order[i + 1], n * 64 + 2 * b, 2, pace)
                        elif hq == 1 and i < 3:
                            md.items(2 - b % 2, pace)
                        elif hq == 1:
                            sa, ca = md.out
                            ca = ca + pltpu.bitcast(tiles[max(b - 3, 0)], F32)
                            h_lead(nn, b, sa, ca)
            return 0

        with scope("ksteps"):
            lax.fori_loop(0, 8, k_body, 0)

        start(mod_cps(4) + mod_cps(5) + wo_cps + late_cps)
        for c in range(8):
            hl = hv0[c, LQ // 2:LEAD // 2, :]
            us[0, :, c * 128:(c + 1) * 128] = hl
            gsb[0, :, c * 128:(c + 1) * 128] = hl
        wait([st_cp(2), xw_cp])

        def rl_body(i, _):
            relayout(0, 2, i * 64, 64)
            return 0

        lax.fori_loop(0, 8, rl_body, 0)

        def lead_proj(par, s0, n, rc, rl):
            w = jnp.concatenate(
                [_unpack(wq2[par][pl.ds(pl.multiple_of((s0 + u) * SL, 4), 512), :])
                 for u in range(n)], axis=1)
            lhs = jnp.concatenate(
                [_unpack(hv0[q, rc * 128:(rc + 1) * 128, :]) for q in range(8)],
                axis=1)
            y = _pack(_dot(lhs, w))
            to_ring(y, par, s0, rc * 16)
            zero = zt[0:8, :]
            for u in range(n):
                for b in range(16):
                    k = min(3, 512 - rl[2])
                    if k > 0:
                        relayout(rl[0], rl[1], rl[2], k,
                                 y[b * 8:(b + 1) * 8, u * 128:(u + 1) * 128] & zero)
                        rl[2] += k
            return y

        def group_body(g, _):
            rl = [1, g, 0]
            for k in range(16):
                lead_proj(0, g * 8 + k // 2, 1, k % 2, rl)

            @pl.when(g < NG - 1)
            def _():
                cp(st_src(1), st.at[g + 1], SEM_G + g).wait()

            for gg in (3, 4, 5):
                @pl.when(g == gg)
                def _(gg=gg):
                    wait(mod_cps(gg))

            gn = jnp.minimum(g + 1, NG - 1)
            t0 = jnp.where(g == 2, 0, jnp.minimum(11 * g - 17, 37))
            part = [lax.shift_right_logical(t0 + c, 3) for c in range(11)]
            md = Mod([t0 + c for c in range(11)],
                     [jnp.where((p == 1) | (p == 4), 1.0, 0.0).astype(F32)
                      for p in part])
            rl = [0, gn, 0]
            for k in range(16):
                y = lead_proj(1, g * 8 + k // 2, 1, k % 2, rl)
                for b in range(16):
                    md.items(3, y[8 * b:8 * b + 8] & zt[0:8, :])
                if k == 11:
                    t = [y[0:8], y[64:72]]
                    for i in range(3):
                        t = h_next(LEAD, i, t)
            assert len(md.out) == 11
            return 0

        with scope("groups"):
            lax.fori_loop(2, NG, group_body, 0)

    pl.run_scoped(
        prologue,
        pltpu.VMEM((NG, D, 8, E), U32),
        pltpu.VMEM((8, LEAD, 128), F32),
        pltpu.VMEM((8, LEAD, 512), F32),
        pltpu.VMEM((2, D // 2, 128), F32),
        pltpu.VMEM((LEAD // 2, 128), U32),
    )

    def main(w3v, w4v, zv, ttv):
        w34_cps = col_copies(w3_hbm, w3v, SEM_B) + col_copies(w4_hbm, w4v, SEM_B)
        start(w34_cps)
        zv[0:HALO, :] = jnp.zeros((HALO, D), F32)
        wait(wo_cps)

        scale = float(E) ** -0.5

        def segment(lhs, ro, store_tok, wo_lhs, extras):
            fill = fillv[...]
            keep = fill == 0.0
            NP = H // 2
            qkv, probs, blocks = {}, {}, []

            def proj(hp):
                slots = [t * H + 2 * hp + par for t in range(3) for par in range(2)]
                wt = [jnp.concatenate(
                    [_unpack(wq2[sl % 2][pl.ds((sl // 2) * SL, 512), :])
                     for sl in slots[2 * t:2 * t + 2]], axis=1) for t in range(3)]
                if hp == 0:
                    w = jnp.concatenate(wt, axis=1)
                    y = _dot(lhs[:, :512], w[:512])
                    y = _dot(lhs[:, 512:], w[512:]) + y
                else:
                    y = jnp.concatenate([_dot(lhs, w) for w in wt], axis=1)
                for u, sl in enumerate(slots):
                    store_tok(sl, y[8:32, u * 128:(u + 1) * 128])
                ops = []
                for t in range(3):
                    ym = jnp.concatenate(
                        [y[0:8, (2 * t) * 128:(2 * t + 1) * 128],
                         y[0:8, (2 * t + 1) * 128:(2 * t + 2) * 128]], axis=0)
                    ops.append(jnp.concatenate(
                        [ym.astype(BF16)]
                        + [_unpack(ring[ro + b, sl * 8:(sl + 1) * 8, :])
                           for sl in slots[2 * t:2 * t + 2] for b in range(2)]
                        + ([jnp.zeros((48, 128), BF16)] if t else []),
                        axis=0))
                qkv[hp] = ops

            def scores(hp):
                q, kk, _ = qkv[hp]
                s = lax.dot_general(q, kk, (((1,), (1,)), ((), ())),
                                    preferred_element_type=F32)
                s = jnp.where(keep, s * scale, fill)
                mx = jnp.max(s, axis=-1, keepdims=True)
                p = jnp.exp(s - mx)
                l = jnp.sum(p, axis=-1, keepdims=True)
                rl = pl.reciprocal(l, approx=True)
                rl = rl * (2.0 - l * rl)
                probs[hp] = (p * rl).astype(BF16)

            def pv(hp):
                o = _dot(probs[hp], qkv[hp][2])
                blocks.append(wo_lhs(2 * hp, o[0:8], o[16:48]).astype(BF16))
                blocks.append(wo_lhs(2 * hp + 1, o[8:16], o[48:80]).astype(BF16))

            def wo_part(h0, h1, acc=None):
                lw = jnp.concatenate(blocks[h0:h1], axis=1)
                y = _dot(lw, _cols(wov, 0, 8, E * h0, E * h1))
                return y if acc is None else y + acc

            def attend(i):
                scores(i - 1)
                if i >= 3:
                    pv(i - 3)

            def fillers(key):
                for thunk in extras.get(key, ()):
                    thunk()

            for i in range(NP):
                proj(i)
                if i > 0:
                    attend(i)
                fillers(i)
            acc = wo_part(0, 4)
            attend(NP)
            fillers(NP)
            acc = wo_part(4, 10, acc)
            pv(NP - 2)
            pv(NP - 1)
            fillers(NP + 1)
            acc = wo_part(10, 20, acc)
            fillers(NP + 2)
            return wo_part(20, 32, acc)

        def put_x2(r0, lo, a):
            n = a.shape[0]
            x2 = (xv[pl.ds(pl.multiple_of(r0 + lo, 8), n), :].astype(F32)
                  + mod_rows(2, n) * a)
            zv[pl.ds(pl.multiple_of(HALO + r0 + lo, 8), n), :] = x2
            sums[lo:lo + n, :] = functools.reduce(
                jnp.add, [x2[:, c * 128:(c + 1) * 128] for c in range(8)])

        def p1_front(r0, sb=3):
            x2 = zv[pl.ds(pl.multiple_of(HALO + r0, 16), 64), :]
            h2 = _ln(x2, sums[...]) * mod_rows(4, 64) + mod_rows(sb, 64)
            return h2, _ln(h2)

        def w12(i):
            return jnp.concatenate(
                [_unpack(wqb[pl.ds(WB + (8 * i + c) * 512, 512), :]) for c in range(8)],
                axis=1)

        def p1_store(y, c, live):
            g = _gelu(y)
            if live is not None:
                g = jnp.where(live, g, y)
            ring[GB, c * 96 + 24:c * 96 + 88, :] = pltpu.bitcast(g, U32)

        def half_dots(lhs, i, live, done):
            part = {}

            def run(c, kh):
                row = jnp.where(live, WB + (8 * i + c) * 512, (8 * i + c) * SL)
                w = wqb[pl.ds(pl.multiple_of(row + kh * 256, 4), 256), :]
                y = _dot(lhs(kh), _unpack(w))
                if kh == 0:
                    part[c] = y
                else:
                    done(y + part[c], c)

            return [functools.partial(run, c, kh) for c in range(8) for kh in range(2)]

        def p2_front(n):
            return jnp.concatenate(
                [pltpu.bitcast(ring[GB, pl.ds(c * 96 + 8 + SHIFTS[c], n), :], F32)
                 for c in range(8)], axis=1)

        def p2_back(h2, hs, row, n, tiles=None, gb=5):
            x1 = jnp.concatenate([h2t[...], h2[0:n - 16]], axis=0) + hs
            rows = pl.ds(pl.multiple_of(row, 16), n)
            zv[rows, :] = zv[rows, :] + mod_rows(gb, n) * x1
            if tiles is None:
                ttv[pl.ds(pl.multiple_of(row // 2, 8), n // 2), :] = _pack(_ln(x1))
                return None
            t = tiles
            for g in range(n // 16):
                y = _ln(paced(x1[16 * g:16 * g + 16], t))
                ttv[pl.ds(pl.multiple_of(row // 2 + 8 * g, 8), 8), :] = _pack(y)
                t = [y[0:8, 896:1024], y[8:16, 896:1024]]
            return t

        def a_body(j, mem):
            @pl.when(j == 1)
            def _():
                wait(late_cps)
                for k in range(16):
                    if k < 8:
                        q = pltpu.bitcast(ring[GB, k * 96 + 24:k * 96 + 88, :], F32)
                        ring[GB, k * 96 + 16:k * 96 + 24, :] = zt[0:8, :]
                    else:
                        q = zv[0:64, (k - 8) * 128:(k - 7) * 128]
                    q = _pack(q)
                    for b in range(4):
                        ring[LQ // 16 + b, (2 * k + 1) * 8:(2 * k + 2) * 8, :] = (
                            q[8 * b:8 * b + 8])

            hcur[...] = hnext[...]
            hb = _unpack(hcur[0:8, :])
            hac = _unpack(hcur[8:16, :]).astype(F32)
            hd = _unpack(hcur[16:24, :])
            wr = [lax.rem(LEAD // 16 + 3 * j + i, RING) for i in range(3)]
            ro0 = lax.rem(4 * j, RING)
            ro1 = ro0 + 2

            live = j > 0
            dead = jnp.where(live, 0, 1)
            h2, u = p1_front(64 * (j - 1), 3 + 3 * dead)
            us[dead] = _pack(u)

            lhs = jnp.concatenate(
                [jnp.concatenate([mem, hac[0:8]], axis=0).astype(BF16), hb], axis=0)
            tok_a = {}

            def store0(c, y):
                tok_a[c] = y[0:8]
                ring[wr[0], c * 8:(c + 1) * 8, :] = _pack(y[8:24])

            deferred = {}

            def wo_lhs0(h, om, ot):
                deferred[h] = ot[24:32]
                return jnp.concatenate([om, ot[0:24]], axis=0)

            pend = []

            def flush():
                while pend:
                    p1_store(*pend.pop(), live)

            th = half_dots(lambda kh: _unpack(us[0, :, kh * 512:(kh + 1) * 512]), 0,
                           live, lambda y, c: pend.append((y, c)))
            extras = {i: [flush, th[i - 2]] for i in range(2, 18)}
            out = segment(lhs, ro0, store0, wo_lhs0, extras)
            flush()
            mem = out[0:8]
            put_x2(64 * j, 0, out[8:32])

            lhs = jnp.concatenate(
                [jnp.concatenate([mem, hac[8:16]], axis=0).astype(BF16), hd], axis=0)

            def store1(c, y):
                ring[wr[1], c * 8:(c + 1) * 8, :] = _pack(
                    jnp.concatenate([tok_a[c], y[0:8]], axis=0))
                ring[wr[2], c * 8:(c + 1) * 8, :] = _pack(y[8:24])

            def wo_lhs1(h, om, ot):
                return jnp.concatenate([om, deferred[h], ot], axis=0)

            gsb[dead] = _pack(p2_front(64))
            for c in range(8):
                ring[GB, c * 96:c * 96 + 24, :] = ring[GB, c * 96 + 64:c * 96 + 88, :]
            hs = []

            def p2_fin():
                t = [hs[7][0:8], hs[7][0:8]]
                for g in range(3):
                    t = h_next(rn, g, t)
                p2_back(h2, jnp.concatenate(hs, axis=1), 64 * j, 64, t, 5 + 2 * dead)
                h2t[...] = h2[48:64]

            th = half_dots(lambda kh: _unpack(gsb[0, :, kh * 512:(kh + 1) * 512]), 1, live,
                           lambda y, c: hs.append(y))
            extras = {i: [th[i]] for i in range(16)}
            extras[18] = [p2_fin]
            rn = LEAD + 48 * jnp.minimum(j + 1, NPAIR - 1)
            out = segment(lhs, ro1, store1, wo_lhs1, extras)
            put_x2(64 * j, 24, out[8:48])
            return out[0:8]

        if "A" in phases:
            with scope("aloop"):
                lax.fori_loop(0, NPAIR, a_body, memv[...].astype(F32))
        else:
            zv[...] = jnp.zeros(zv.shape, F32)
            ttv[...] = jnp.zeros(ttv.shape, U32)

        h2, u = p1_front(S - 64)
        y = _dot(u.astype(BF16), w12(0))
        for c in range(8):
            p1_store(y[:, c * 128:(c + 1) * 128], c, None)
        p2_back(h2, _dot(p2_front(80).astype(BF16), w12(1)), S, 80)

        wait(w34_cps)

        def out_cp(i, slot):
            return cp(outv.at[slot], out_hbm.at[pl.ds(i * RB, RB), :],
                      SEM_OUT + slot)

        def p3_body(i, _):
            slot = i % 2

            @pl.when(i >= 2)
            def _():
                out_cp(i - 2, slot).wait()

            r0 = HALO + i * RB
            tt = _unpack(ttv[pl.ds(pl.multiple_of(r0 // 2, 8), RB // 2), :])
            ff = jnp.concatenate(
                [_gelu(_dot(tt, _cols(w3v, 4 * q, 4 * q + 4))).astype(BF16)
                 for q in range(FF // 512)], axis=1)
            gb = mod_rows(5, RB)
            for c0, c1 in ((0, 7), (7, 8)):
                cols = slice(c0 * 128, c1 * 128)
                y = _dot(ff, _cols(w4v, c0, c1))
                res = zv[pl.ds(pl.multiple_of(r0, 16), RB), cols] + gb[:, cols] * y
                outv[slot, :, cols] = res.astype(BF16)
                cp(outv.at[slot, :, cols], out_hbm.at[pl.ds(i * RB, RB), cols],
                   SEM_OUT + slot).start()
            return 0

        nb = S // RB
        if "B" in phases:
            with scope("p3"):
                lax.fori_loop(0, nb, p3_body, 0)
            out_cp(nb - 2, 0).wait()
            out_cp(nb - 1, 1).wait()
        else:
            outv[0] = zv[pl.ds(HALO, RB), :].astype(BF16)
            out_cp(0, 0).start()
            out_cp(0, 0).wait()

    pl.run_scoped(
        main,
        pltpu.VMEM((FF // 128, D // 2, 128), U32),
        pltpu.VMEM((8, FF // 2, 128), U32),
        pltpu.VMEM((S + HALO, D), F32),
        pltpu.VMEM(((S + HALO) // 2, D), U32),
    )


def _call(A_x, A_mem0, A_Wq, A_Wk, A_Wv, A_Wo, B_w1, B_w2, B_w3, B_w4, c, w_mod,
          phases="AB"):
    any_spec = pl.BlockSpec(memory_space=pl.ANY)
    scratch = [
        pltpu.VMEM((S, D), BF16),
        pltpu.VMEM((M, D), BF16),
        pltpu.VMEM((48, D // 2, 128), U32),
        pltpu.VMEM((64, 8, 128), F32),
        pltpu.VMEM((WB, E), U32),
        pltpu.VMEM((WB + 16 * 512, E), U32),
        pltpu.VMEM((8, H * E // 2, 128), U32),
        pltpu.VMEM((2, 32, D), U32),
        pltpu.VMEM((2, 32, D), U32),
        pltpu.VMEM((8, LEAD // 2, 128), U32),
        pltpu.VMEM((24, D), U32),
        pltpu.VMEM((24, D), U32),
        pltpu.VMEM((RING + 1, 3 * H * 8, E), U32),
        pltpu.VMEM((64, 128), F32),
        pltpu.VMEM((16, D), F32),
        pltpu.VMEM((32, 128), U32),
        pltpu.VMEM((2, RB, D), BF16),
        pltpu.VMEM((80, 128), F32),
        pltpu.VMEM((1, D), BF16),
        pltpu.SemaphoreType.DMA((NSEM,)),
    ]
    out = pl.pallas_call(
        functools.partial(_kernel, phases=phases),
        in_specs=[any_spec] * 12,
        out_specs=any_spec,
        out_shape=jax.ShapeDtypeStruct((S, D), BF16),
        scratch_shapes=scratch,
        compiler_params=pltpu.CompilerParams(
            vmem_limit_bytes=126 * 1024 * 1024,
            disable_bounds_checks=True, disable_semaphore_checks=True),
    )(A_x.reshape(S, D), A_mem0.reshape(M, D), A_Wq, A_Wk, A_Wv,
      A_Wo.reshape(H * E, D), B_w1, B_w2, B_w3, B_w4, c, w_mod)
    return out.reshape(1, S, D)


def pallas_adaLN_cond__memory_aug_recurrent_mem_tr__mixer_s_mlp__prompt_kernel(
    A_x, A_mem0, A_Wq, A_Wk, A_Wv, A_Wo, A_seg_len, B_x, B_w1, B_w2, B_w3, B_w4,
    c, w_mod,
):
    if isinstance(A_seg_len, int):
        assert A_seg_len == SEG
    del B_x
    return _call(A_x, A_mem0, A_Wq, A_Wk, A_Wv, A_Wo, B_w1, B_w2, B_w3, B_w4,
                 c, w_mod)
```

```python
import contextlib
import functools

import jax
import jax.numpy as jnp
from jax import lax
import jax.experimental.pallas as pl
import jax.experimental.pallas.tpu as pltpu

F32 = jnp.float32
BF16 = jnp.bfloat16
U32 = jnp.uint32

S = 2048
D = 1024
H = 32
E = 128
M = 8
SEG = 32
FF = 3584
EPS = 1e-5

LEAD = 512
RING = 36
GB = RING
SL = 516
WB = 3 * H // 2 * SL + 544
LQ = LEAD - 64
HG = 16
NG = 3 * H // HG
NPAIR = S // (2 * SEG)
HALO = 80
RB = 256
SHIFTS = (-1, -1, 1, 1, -2, -2, 2, 2)

SEM_C = 0
SEM_X = 1
SEM_A = 2
SEM_B = 3
SEM_XR = 4
SEM_M = 5
SEM_K = 7
SEM_G = 14
SEM_OUT = 20
NSEM = 22


def _ln(x, part=None):
    if part is None:
        mu = jnp.mean(x, axis=-1, keepdims=True)
    else:
        mu = jnp.sum(part, axis=-1, keepdims=True) * (1.0 / x.shape[-1])
    xc = x - mu
    var = jnp.mean(xc * xc, axis=-1, keepdims=True)
    return xc * lax.rsqrt(var + EPS)


def _gelu(x):
    return jax.nn.gelu(x, approximate=True)


def _pack(x):
    return pltpu.bitcast(x.astype(BF16), U32)


def _unpack(x):
    return pltpu.bitcast(x, BF16)


def _dot(a, b):
    return jnp.dot(a, b, preferred_element_type=F32)


def _cols(ref, lo, hi, k0=0, k1=None):
    k1 = 2 * ref.shape[1] if k1 is None else k1
    return jnp.concatenate(
        [_unpack(ref[c, k0 // 2:k1 // 2, :]) for c in range(lo, hi)], axis=1)


def _kernel(x_hbm, mem_hbm, wq_hbm, wk_hbm, wv_hbm, wo_hbm, w1_hbm, w2_hbm,
            w3_hbm, w4_hbm, c_hbm, wmod_hbm, out_hbm,
            xv, memv, wmodv, modv, wqa, wqb, wov, us, gsb,
            hv0, hcur, hnext, ring, sums, h2t, h2l, x1l, zt, outv, fillv, cv, sems, *, phases):
    def scope(name):
        return jax.named_scope(name) if "s" in phases else contextlib.nullcontext()

    def cp(src, dst, s):
        return pltpu.make_async_copy(src, dst, sems.at[s])

    def col_copies(w_hbm, w_v, s, lo=0, hi=None):
        w32 = w_hbm.bitcast(U32)
        hi = w_v.shape[0] if hi is None else hi
        return [cp(w32.at[:, pl.ds(c * 128, 128)], w_v.at[c], s)
                for c in range(lo, hi)]

    def start(cps):
        for q in cps:
            q.start()

    def wait(cps):
        for q in cps:
            q.wait()

    def x_cp(r0, n, s):
        return cp(x_hbm.at[pl.ds(r0, n)], xv.at[pl.ds(r0, n)], s)

    c_cps = [cp(c_hbm, cv, SEM_C), cp(mem_hbm, memv, SEM_C)]
    x0_cp = x_cp(0, LEAD, SEM_X)
    xw_cp = x_cp(LEAD, 96, SEM_G + 1)
    wo_cps = col_copies(wo_hbm, wov, SEM_A)
    late_cps = [x_cp(LEAD + 96, S - LEAD - 96, SEM_XR)] + [
        cp(w.bitcast(U32).at[:, pl.ds(c * 128, 128)],
           wqb.at[pl.ds(WB + (8 * i + c) * 512, 512)], SEM_XR)
        for i, w in enumerate((w1_hbm, w2_hbm)) for c in range(8)]

    def mod_rows(i, n):
        m = jnp.concatenate([modv[8 * i + c] for c in range(8)], axis=1)
        return jnp.concatenate([m] * (n // 8), axis=0)

    HI = jnp.uint32(0xFFFF0000)
    wq2 = (wqa, wqb)

    def paced(x, tiles):
        z = [pltpu.bitcast((t if t.dtype == U32 else pltpu.bitcast(t, U32))
                           & zt[0:8, :], F32) for t in tiles]
        z = jnp.concatenate(z, axis=0)
        if x.shape[1] == 128:
            return x + z
        return jnp.concatenate([x[:, 0:128] + z, x[:, 128:]], axis=1)

    def h_rows(r0, n, tiles=None):
        xf = xv[pl.ds(pl.multiple_of(r0, 16), n), :].astype(F32)
        if tiles is not None:
            xf = paced(xf, tiles)
        return _ln(xf) * mod_rows(1, n) + mod_rows(0, n)

    def h_next(r0, g, tile=None):
        y = h_rows(r0 + 16 * g, 16, tile)
        hnext[g * 8:(g + 1) * 8, :] = _pack(y)
        return [y[0:8, 896:1024], y[8:16, 896:1024]]

    def prologue(st, xn, acc, scol, hn):
        w_hbms = (wq_hbm, wk_hbm, wv_hbm)

        def st_src(i):
            return w_hbms[i // 2].bitcast(U32).at[:, pl.ds((i % 2) * 8, 8), :]

        def pair_cps(n, s):
            w32 = wmod_hbm.bitcast(U32)
            return [cp(w32.at[:, pl.ds(pl.multiple_of(c * 128, 128), 128)],
                       wmodv.at[c], s) for c in (n, 8 + n)]

        def k_cps(n):
            return [cp(st_src(i).at[pl.ds(n * 128, 128)],
                       st.at[i, pl.ds(n * 128, 128)], SEM_K + n) for i in range(2)]

        def st_cp(i):
            return cp(st_src(i), st.at[i], SEM_G + i - 1)

        def mod_cps(g):
            lo, hi = {3: (16, 27), 4: (27, 38), 5: (38, 48)}[g]
            return col_copies(wmod_hbm, wmodv, SEM_G + g, lo, hi)

        with scope("first"):
            start(c_cps + [x0_cp])
        for n in range(8):
            start((pair_cps(n, SEM_M + n) if n < 2 else []) + k_cps(n)
                  + (pair_cps(n + 1, SEM_K + n) if 0 < n < 7 else []))
        start([st_cp(2), xw_cp, st_cp(3), st_cp(4)] + mod_cps(3) + [st_cp(5)])

        r = lax.broadcasted_iota(jnp.int32, (80, 128), 0)
        k = lax.broadcasted_iota(jnp.int32, (80, 128), 1)

        def head_of(i):
            return jnp.where(i < 16, i // 8, (i - 16) // 32)

        def pos_of(i):
            return jnp.where(i < 16, i % 8, 8 + (i - 16) % 32)

        same = head_of(r) == head_of(k)
        vis = (pos_of(r) < M) | (pos_of(r) >= pos_of(k))
        fillv[...] = jnp.where(same, jnp.where(vis, 0.0, -1e9), -jnp.inf).astype(F32)
        sums[...] = jnp.zeros(sums.shape, F32)
        modv[48:56] = jnp.zeros((8, 8, 128), F32)
        modv[56:64] = jnp.ones((8, 8, 128), F32)
        ring[GB] = jnp.zeros(ring.shape[1:], U32)
        zt[...] = jnp.zeros(zt.shape, U32)
        h2t[...] = jnp.zeros(h2t.shape, F32)
        x1l[...] = jnp.zeros(x1l.shape, F32)


        def zero_body(i, _):
            acc[i] = jnp.zeros(acc.shape[1:], F32)
            return 0

        lax.fori_loop(0, acc.shape[0], zero_body, 0)

        wait(c_cps)
        cf = cv[...].astype(F32)
        sil = cf * jax.nn.sigmoid(cf)
        for c in range(8):
            sw = _pack(jnp.broadcast_to(sil[:, c * 128:(c + 1) * 128], (128, 128)).T)
            scol[0, c * 64:(c + 1) * 64, :] = pltpu.bitcast(sw << 16, F32)
            scol[1, c * 64:(c + 1) * 64, :] = pltpu.bitcast(sw & HI, F32)

        x0_cp.wait()

        def ln_body(i, _):
            r0 = pl.multiple_of(i * 64, 64)
            y = _ln(xv[pl.ds(r0, 64), :].astype(F32))
            for q in range(8):
                xn[q, pl.ds(r0, 64), :] = y[:, q * 128:(q + 1) * 128]
            return 0

        lax.fori_loop(0, LEAD // 64, ln_body, 0)

        class Mod:
            def __init__(self, tiles, offs):
                self.tiles, self.offs = tiles, offs
                self.n, self.acc, self.out = 0, None, []

            def items(self, n, pace=None):
                for it in range(self.n, min(self.n + n, 64 * len(self.tiles))):
                    c, i = divmod(it, 64)
                    w = wmodv[self.tiles[c], i * 8:(i + 1) * 8, :]
                    if pace is not None:
                        w = w | pace
                    v = (pltpu.bitcast(w << 16, F32) * scol[0, i * 8:(i + 1) * 8, :]
                         + pltpu.bitcast(w & HI, F32) * scol[1, i * 8:(i + 1) * 8, :])
                    self.acc = v if i == 0 else self.acc + v
                    if i == 63:
                        m = jnp.broadcast_to(
                            jnp.sum(self.acc, axis=0, keepdims=True) + self.offs[c],
                            (8, 128))
                        modv[self.tiles[c]] = m
                        self.out.append(m)
                self.n += n

        def h_lead(n, b, sa, ca):
            rep = lambda m: jnp.concatenate([m, m], axis=0)
            y = _pack(xn[n, 16 * b:16 * b + 16, :] * rep(ca) + rep(sa))
            hn[8 * b:8 * b + 8, :] = y
            hv0[n, 8 * b:8 * b + 8, :] = y

        def relayout(par, g, p0, n, pace=None):
            base = g * (8 * SL)
            mask = jnp.uint32(0xFFFF0000 if par else 0xFFFF)
            if pace is not None:
                mask = pace | mask
            for u in range(n):
                a = st[g, 2 * (p0 + u)]
                b = st[g, 2 * (p0 + u) + 1]
                if par == 0:
                    w = (a & mask) | (b << 16)
                else:
                    w = (a >> 16) | (b & mask)
                wq2[par][pl.ds(base + p0 + u, 8, stride=SL), :] = w

        def to_ring(y, par, s0, b0):
            for u in range(y.shape[1] // 128):
                row = pl.multiple_of((2 * (s0 + u) + par) * 8, 8)
                for b in range(y.shape[0] // 8):
                    ring[b0 + b, pl.ds(row, 8), :] = (
                        y[b * 8:(b + 1) * 8, u * 128:(u + 1) * 128])

        def k_body(n, _):
            @pl.when(n < 2)
            def _():
                wait(pair_cps(n, SEM_M + n))
                md = Mod([n, 8 + n], [0.0, 1.0])
                md.items(128)
                for b in range(32):
                    h_lead(n, b, *md.out)

            wait(k_cps(n))

            @pl.when((n > 0) & (n < 7))
            def _():
                wait(pair_cps(n + 1, SEM_K + n))

            nn = jnp.where(n == 0, 0, jnp.minimum(n + 1, 7))
            md = Mod([nn, 8 + nn], [0.0, 1.0])
            zero = zt[0:8, :]
            order = [(0, 0), (1, 0), (0, 1), (1, 1)]
            relayout(0, 0, n * 64, 64)
            for i, (par, g) in enumerate(order):
                for hq in range(2):
                    s0 = g * 8 + hq * 4
                    w = jnp.concatenate(
                        [_unpack(wq2[par][pl.ds(pl.multiple_of(
                            (s0 + u) * SL + n * 64, 4), 64), :])
                         for u in range(4)], axis=1)
                    m = LQ if par else LEAD
                    y = _dot(_unpack(hn[0:m // 2, :]), w) + acc[2 * i + hq, 0:m, :]
                    acc[2 * i + hq, 0:m, :] = y
                    y = _pack(y)
                    to_ring(y, par, s0, 0)
                    tiles = [y[8 * b:8 * b + 8, 0:128] & zero for b in range(m // 16)]
                    tiles = [tiles[b * len(tiles) // 32] for b in range(32)]
                    for b in range(32):
                        pace = tiles[b]
                        if hq == 0 and i < 3:
                            relayout(*order[i + 1], n * 64 + 2 * b, 2, pace)
                        elif hq == 1 and i < 3:
                            md.items(2 - b % 2, pace)
                        elif hq == 1:
                            sa, ca = md.out
                            ca = ca + pltpu.bitcast(tiles[max(b - 3, 0)], F32)
                            h_lead(nn, b, sa, ca)
            return 0

        with scope("ksteps"):
            lax.fori_loop(0, 8, k_body, 0)

        start(mod_cps(4) + mod_cps(5) + wo_cps + late_cps)
        for c in range(8):
            hl = hv0[c, LQ // 2:LEAD // 2, :]
            us[0, :, c * 128:(c + 1) * 128] = hl
            gsb[0, :, c * 128:(c + 1) * 128] = hl
        wait([st_cp(2), xw_cp])

        def rl_body(i, _):
            relayout(0, 2, i * 64, 64)
            return 0

        lax.fori_loop(0, 8, rl_body, 0)

        def lead_proj(par, s0, n, rc, rl):
            w = jnp.concatenate(
                [_unpack(wq2[par][pl.ds(pl.multiple_of((s0 + u) * SL, 4), 512), :])
                 for u in range(n)], axis=1)
            lhs = jnp.concatenate(
                [_unpack(hv0[q, rc * 128:(rc + 1) * 128, :]) for q in range(8)],
                axis=1)
            y = _pack(_dot(lhs, w))
            to_ring(y, par, s0, rc * 16)
            zero = zt[0:8, :]
            for u in range(n):
                for b in range(16):
                    k = min(3, 512 - rl[2])
                    if k > 0:
                        relayout(rl[0], rl[1], rl[2], k,
                                 y[b * 8:(b + 1) * 8, u * 128:(u + 1) * 128] & zero)
                        rl[2] += k
            return y

        def group_body(g, _):
            rl = [1, g, 0]
            for k in range(16):
                lead_proj(0, g * 8 + k // 2, 1, k % 2, rl)

            @pl.when(g < NG - 1)
            def _():
                cp(st_src(1), st.at[g + 1], SEM_G + g).wait()

            for gg in (3, 4, 5):
                @pl.when(g == gg)
                def _(gg=gg):
                    wait(mod_cps(gg))

            gn = jnp.minimum(g + 1, NG - 1)
            t0 = jnp.where(g == 2, 0, jnp.minimum(11 * g - 17, 37))
            part = [lax.shift_right_logical(t0 + c, 3) for c in range(11)]
            md = Mod([t0 + c for c in range(11)],
                     [jnp.where((p == 1) | (p == 4), 1.0, 0.0).astype(F32)
                      for p in part])
            rl = [0, gn, 0]
            for k in range(16):
                y = lead_proj(1, g * 8 + k // 2, 1, k % 2, rl)
                for b in range(16):
                    md.items(3, y[8 * b:8 * b + 8] & zt[0:8, :])
                if k == 11:
                    t = [y[0:8], y[64:72]]
                    for i in range(3):
                        t = h_next(LEAD, i, t)
            assert len(md.out) == 11
            return 0

        with scope("groups"):
            lax.fori_loop(2, NG, group_body, 0)

    pl.run_scoped(
        prologue,
        pltpu.VMEM((NG, D, 8, E), U32),
        pltpu.VMEM((8, LEAD, 128), F32),
        pltpu.VMEM((8, LEAD, 512), F32),
        pltpu.VMEM((2, D // 2, 128), F32),
        pltpu.VMEM((LEAD // 2, 128), U32),
    )

    def main(w3v, w4v, zv, ttv):
        w34_cps = col_copies(w3_hbm, w3v, SEM_B) + col_copies(w4_hbm, w4v, SEM_B)
        start(w34_cps)
        zv[0:HALO, :] = jnp.zeros((HALO, D), F32)
        wait(wo_cps)

        scale = float(E) ** -0.5

        def segment(lhs, ro, store_tok, wo_lhs, extras):
            fill = fillv[...]
            keep = fill == 0.0
            NP = H // 2
            qkv, probs, blocks = {}, {}, []

            def proj(hp):
                slots = [t * H + 2 * hp + par for t in range(3) for par in range(2)]
                wt = [jnp.concatenate(
                    [_unpack(wq2[sl % 2][pl.ds((sl // 2) * SL, 512), :])
                     for sl in slots[2 * t:2 * t + 2]], axis=1) for t in range(3)]
                if hp == 0:
                    w = jnp.concatenate(wt, axis=1)
                    y = _dot(lhs[:, :512], w[:512])
                    y = _dot(lhs[:, 512:], w[512:]) + y
                else:
                    y = jnp.concatenate([_dot(lhs, w) for w in wt], axis=1)
                for u, sl in enumerate(slots):
                    store_tok(sl, y[8:32, u * 128:(u + 1) * 128])
                ops = []
                for t in range(3):
                    ym = jnp.concatenate(
                        [y[0:8, (2 * t) * 128:(2 * t + 1) * 128],
                         y[0:8, (2 * t + 1) * 128:(2 * t + 2) * 128]], axis=0)
                    ops.append(jnp.concatenate(
                        [ym.astype(BF16)]
                        + [_unpack(ring[ro + b, sl * 8:(sl + 1) * 8, :])
                           for sl in slots[2 * t:2 * t + 2] for b in range(2)]
                        + ([jnp.zeros((48, 128), BF16)] if t else []),
                        axis=0))
                qkv[hp] = ops

            def scores(hp):
                q, kk, _ = qkv[hp]
                s = lax.dot_general(q, kk, (((1,), (1,)), ((), ())),
                                    preferred_element_type=F32)
                s = jnp.where(keep, s * scale, fill)
                mx = jnp.max(s, axis=-1, keepdims=True)
                p = jnp.exp(s - mx)
                l = jnp.sum(p, axis=-1, keepdims=True)
                rl = pl.reciprocal(l, approx=True)
                rl = rl * (2.0 - l * rl)
                probs[hp] = (p * rl).astype(BF16)

            def pv(hp):
                o = _dot(probs[hp], qkv[hp][2])
                blocks.append(wo_lhs(2 * hp, o[0:8], o[16:48]).astype(BF16))
                blocks.append(wo_lhs(2 * hp + 1, o[8:16], o[48:80]).astype(BF16))

            def wo_part(h0, h1, acc=None):
                lw = jnp.concatenate(blocks[h0:h1], axis=1)
                y = _dot(lw, _cols(wov, 0, 8, E * h0, E * h1))
                return y if acc is None else y + acc

            def attend(i):
                scores(i - 1)
                if i >= 3:
                    pv(i - 3)

            def fillers(key):
                for thunk in extras.get(key, ()):
                    thunk()

            for i in range(NP):
                proj(i)
                if i > 0:
                    attend(i)
                fillers(i)
            acc = wo_part(0, 4)
            attend(NP)
            fillers(NP)
            acc = wo_part(4, 10, acc)
            pv(NP - 2)
            pv(NP - 1)
            fillers(NP + 1)
            acc = wo_part(10, 20, acc)
            fillers(NP + 2)
            return wo_part(20, 32, acc)

        def put_x2(r0, lo, a):
            n = a.shape[0]
            x2 = (xv[pl.ds(pl.multiple_of(r0 + lo, 8), n), :].astype(F32)
                  + mod_rows(2, n) * a)
            zv[pl.ds(pl.multiple_of(HALO + r0 + lo, 8), n), :] = x2
            sums[lo:lo + n, :] = functools.reduce(
                jnp.add, [x2[:, c * 128:(c + 1) * 128] for c in range(8)])

        def p1_front(r0, sb=3):
            x2 = zv[pl.ds(pl.multiple_of(HALO + r0, 16), 64), :]
            h2 = _ln(x2, sums[...]) * mod_rows(4, 64) + mod_rows(sb, 64)
            return h2, _ln(h2)

        def w12(i):
            return jnp.concatenate(
                [_unpack(wqb[pl.ds(WB + (8 * i + c) * 512, 512), :]) for c in range(8)],
                axis=1)

        def p1_store(y, c, live):
            g = _gelu(y)
            if live is not None:
                g = jnp.where(live, g, y)
            ring[GB, c * 96 + 24:c * 96 + 88, :] = pltpu.bitcast(g, U32)

        def half_dots(lhs, i, live, done):
            part = {}

            def run(c, kh):
                row = jnp.where(live, WB + (8 * i + c) * 512, (8 * i + c) * SL)
                w = wqb[pl.ds(pl.multiple_of(row + kh * 256, 4), 256), :]
                y = _dot(lhs(kh), _unpack(w))
                if kh == 0:
                    part[c] = y
                else:
                    done(y + part[c], c)

            return [functools.partial(run, c, kh) for c in range(8) for kh in range(2)]

        def p2_front(n):
            return jnp.concatenate(
                [pltpu.bitcast(ring[GB, pl.ds(c * 96 + 8 + SHIFTS[c], n), :], F32)
                 for c in range(8)], axis=1)

        def p2_x1(h2, hs, row, gb=5):
            n = hs.shape[0]
            x1 = jnp.concatenate([h2t[...], h2[0:n - 16]], axis=0) + hs
            rows = pl.ds(pl.multiple_of(row, 16), n)
            zv[rows, :] = zv[rows, :] + mod_rows(gb, n) * x1
            return x1

        def p2_norm(x1, row, t):
            for g in range(x1.shape[0] // 16):
                y = _ln(paced(x1[16 * g:16 * g + 16, :], t))
                ttv[pl.ds(pl.multiple_of(row // 2 + 8 * g, 8), 8), :] = _pack(y)
                t = [y[0:8, 896:1024], y[8:16, 896:1024]]

        def a_body(j, mem):
            @pl.when(j == 1)
            def _():
                wait(late_cps)
                for k in range(16):
                    if k < 8:
                        q = pltpu.bitcast(ring[GB, k * 96 + 24:k * 96 + 88, :], F32)
                        ring[GB, k * 96 + 16:k * 96 + 24, :] = zt[0:8, :]
                    else:
                        q = zv[0:64, (k - 8) * 128:(k - 7) * 128]
                    q = _pack(q)
                    for b in range(4):
                        ring[LQ // 16 + b, (2 * k + 1) * 8:(2 * k + 2) * 8, :] = (
                            q[8 * b:8 * b + 8])

            hcur[...] = hnext[...]
            hb = _unpack(hcur[0:8, :])
            hac = _unpack(hcur[8:16, :]).astype(F32)
            hd = _unpack(hcur[16:24, :])
            wr = [lax.rem(LEAD // 16 + 3 * j + i, RING) for i in range(3)]
            ro0 = lax.rem(4 * j, RING)
            ro1 = ro0 + 2

            live = j > 0
            dead = jnp.where(live, 0, 1)
            h2, u = p1_front(64 * (j - 1), 3 + 3 * dead)
            us[dead] = _pack(u)

            lhs = jnp.concatenate(
                [jnp.concatenate([mem, hac[0:8]], axis=0).astype(BF16), hb], axis=0)
            tok_a = {}

            def store0(c, y):
                tok_a[c] = y[0:8]
                ring[wr[0], c * 8:(c + 1) * 8, :] = _pack(y[8:24])

            deferred = {}

            def wo_lhs0(h, om, ot):
                deferred[h] = ot[24:32]
                return jnp.concatenate([om, ot[0:24]], axis=0)

            pend = []

            def flush():
                while pend:
                    p1_store(*pend.pop(), live)

            th = half_dots(lambda kh: _unpack(us[0, :, kh * 512:(kh + 1) * 512]), 0,
                           live, lambda y, c: pend.append((y, c)))
            extras = {i: [flush, th[i - 2]] for i in range(2, 18)}
            out = segment(lhs, ro0, store0, wo_lhs0, extras)
            flush()
            mem = out[0:8]
            put_x2(64 * j, 0, out[8:32])

            lhs = jnp.concatenate(
                [jnp.concatenate([mem, hac[8:16]], axis=0).astype(BF16), hd], axis=0)

            def store1(c, y):
                ring[wr[1], c * 8:(c + 1) * 8, :] = _pack(
                    jnp.concatenate([tok_a[c], y[0:8]], axis=0))
                ring[wr[2], c * 8:(c + 1) * 8, :] = _pack(y[8:24])

            def wo_lhs1(h, om, ot):
                return jnp.concatenate([om, deferred[h], ot], axis=0)

            gsb[dead] = _pack(p2_front(64))
            for c in range(8):
                ring[GB, c * 96:c * 96 + 24, :] = ring[GB, c * 96 + 64:c * 96 + 88, :]
            hs = []

            def p2_fin():
                t = [hs[7][0:8], hs[7][0:8]]
                for g in range(3):
                    t = h_next(rn, g, t)
                x1 = p2_x1(h2, jnp.concatenate(hs, axis=1), 64 * j, 5 + 2 * dead)
                p2_norm(x1, 64 * j, t)
                h2t[...] = h2[48:64]

            th = half_dots(lambda kh: _unpack(gsb[0, :, kh * 512:(kh + 1) * 512]), 1, live,
                           lambda y, c: hs.append(y))
            extras = {i: [th[i]] for i in range(16)}
            extras[18] = [p2_fin]
            rn = LEAD + 48 * jnp.minimum(j + 1, NPAIR - 1)
            out = segment(lhs, ro1, store1, wo_lhs1, extras)
            put_x2(64 * j, 24, out[8:48])
            return out[0:8]

        if "A" in phases:
            with scope("aloop"):
                lax.fori_loop(0, NPAIR, a_body, memv[...].astype(F32))
        else:
            zv[...] = jnp.zeros(zv.shape, F32)
            ttv[...] = jnp.zeros(ttv.shape, U32)

        wait(w34_cps)

        def out_cp(i, slot):
            return cp(outv.at[slot], out_hbm.at[pl.ds(i * RB, RB), :],
                      SEM_OUT + slot)

        def p3_body(i, _):
            slot = i % 2

            @pl.when(i >= 2)
            def _():
                out_cp(i - 2, slot).wait()

            @pl.when(i == 1)
            def _():
                y = _dot(_unpack(us[0]), w12(0))
                for c in range(8):
                    p1_store(y[:, c * 128:(c + 1) * 128], c, None)
                hs = _dot(p2_front(80).astype(BF16), w12(1))
                x1l[...] = p2_x1(h2l, hs, S)

            r0 = HALO + i * RB
            tt = _unpack(ttv[pl.ds(pl.multiple_of(r0 // 2, 8), RB // 2), :])
            ys = [_dot(tt, _cols(w3v, 4 * q, 4 * q + 4)) for q in range(FF // 512)]
            ff = jnp.concatenate([_gelu(y).astype(BF16) for y in ys], axis=1)
            t = [ys[-1][240:248, 384:512], ys[-1][248:256, 384:512]]
            for g in range(4):
                rows = slice(16 * g, 16 * g + 16)
                x2 = zv[HALO + S - 64 + 16 * g:HALO + S - 48 + 16 * g, :]
                h2 = (_ln(x2, paced(sums[rows, :], t)) * mod_rows(4, 16)
                      + mod_rows(3, 16))
                h2l[rows, :] = h2
                u = _ln(h2)
                us[0, 8 * g:8 * g + 8, :] = _pack(u)
                t = [u[0:8, 896:1024], u[8:16, 896:1024]]
            p2_norm(x1l, S, t)
            gb = mod_rows(5, RB)
            for c0, c1 in ((0, 7), (7, 8)):
                cols = slice(c0 * 128, c1 * 128)
                y = _dot(ff, _cols(w4v, c0, c1))
                res = zv[pl.ds(pl.multiple_of(r0, 16), RB), cols] + gb[:, cols] * y
                outv[slot, :, cols] = res.astype(BF16)
                cp(outv.at[slot, :, cols], out_hbm.at[pl.ds(i * RB, RB), cols],
                   SEM_OUT + slot).start()
            return 0

        nb = S // RB
        if "B" in phases:
            with scope("p3"):
                lax.fori_loop(0, nb, p3_body, 0)
            out_cp(nb - 2, 0).wait()
            out_cp(nb - 1, 1).wait()
        else:
            outv[0] = zv[pl.ds(HALO, RB), :].astype(BF16)
            out_cp(0, 0).start()
            out_cp(0, 0).wait()

    pl.run_scoped(
        main,
        pltpu.VMEM((FF // 128, D // 2, 128), U32),
        pltpu.VMEM((8, FF // 2, 128), U32),
        pltpu.VMEM((S + HALO, D), F32),
        pltpu.VMEM(((S + HALO) // 2, D), U32),
    )


def _call(A_x, A_mem0, A_Wq, A_Wk, A_Wv, A_Wo, B_w1, B_w2, B_w3, B_w4, c, w_mod,
          phases="AB"):
    any_spec = pl.BlockSpec(memory_space=pl.ANY)
    scratch = [
        pltpu.VMEM((S, D), BF16),
        pltpu.VMEM((M, D), BF16),
        pltpu.VMEM((48, D // 2, 128), U32),
        pltpu.VMEM((64, 8, 128), F32),
        pltpu.VMEM((WB, E), U32),
        pltpu.VMEM((WB + 16 * 512, E), U32),
        pltpu.VMEM((8, H * E // 2, 128), U32),
        pltpu.VMEM((2, 32, D), U32),
        pltpu.VMEM((2, 32, D), U32),
        pltpu.VMEM((8, LEAD // 2, 128), U32),
        pltpu.VMEM((24, D), U32),
        pltpu.VMEM((24, D), U32),
        pltpu.VMEM((RING + 1, 3 * H * 8, E), U32),
        pltpu.VMEM((64, 128), F32),
        pltpu.VMEM((16, D), F32),
        pltpu.VMEM((64, D), F32),
        pltpu.VMEM((80, D), F32),
        pltpu.VMEM((32, 128), U32),
        pltpu.VMEM((2, RB, D), BF16),
        pltpu.VMEM((80, 128), F32),
        pltpu.VMEM((1, D), BF16),
        pltpu.SemaphoreType.DMA((NSEM,)),
    ]
    out = pl.pallas_call(
        functools.partial(_kernel, phases=phases),
        in_specs=[any_spec] * 12,
        out_specs=any_spec,
        out_shape=jax.ShapeDtypeStruct((S, D), BF16),
        scratch_shapes=scratch,
        compiler_params=pltpu.CompilerParams(
            vmem_limit_bytes=126 * 1024 * 1024,
            disable_bounds_checks=True, disable_semaphore_checks=True),
    )(A_x.reshape(S, D), A_mem0.reshape(M, D), A_Wq, A_Wk, A_Wv,
      A_Wo.reshape(H * E, D), B_w1, B_w2, B_w3, B_w4, c, w_mod)
    return out.reshape(1, S, D)


def pallas_adaLN_cond__memory_aug_recurrent_mem_tr__mixer_s_mlp__prompt_kernel(
    A_x, A_mem0, A_Wq, A_Wk, A_Wv, A_Wo, A_seg_len, B_x, B_w1, B_w2, B_w3, B_w4,
    c, w_mod,
):
    if isinstance(A_seg_len, int):
        assert A_seg_len == SEG
    del B_x
    return _call(A_x, A_mem0, A_Wq, A_Wk, A_Wv, A_Wo, B_w1, B_w2, B_w3, B_w4,
                 c, w_mod)
```

```python
import contextlib
import functools

import jax
import jax.numpy as jnp
from jax import lax
import jax.experimental.pallas as pl
import jax.experimental.pallas.tpu as pltpu

F32 = jnp.float32
BF16 = jnp.bfloat16
U32 = jnp.uint32

S = 2048
D = 1024
H = 32
E = 128
M = 8
SEG = 32
FF = 3584
EPS = 1e-5

LEAD = 512
RING = 36
GB = RING
SL = 516
WB = 3 * H // 2 * SL + 544
LQ = LEAD - 64
HG = 16
NG = 3 * H // HG
NPAIR = S // (2 * SEG)
HALO = 80
RB = 256
SHIFTS = (-1, -1, 1, 1, -2, -2, 2, 2)

SEM_C = 0
SEM_X = 1
SEM_A = 2
SEM_B = 3
SEM_XR = 4
SEM_M = 5
SEM_K = 7
SEM_G = 14
SEM_OUT = 20
NSEM = 22


def _ln(x, part=None):
    if part is None:
        mu = jnp.mean(x, axis=-1, keepdims=True)
    else:
        mu = jnp.sum(part, axis=-1, keepdims=True) * (1.0 / x.shape[-1])
    xc = x - mu
    var = jnp.mean(xc * xc, axis=-1, keepdims=True)
    return xc * lax.rsqrt(var + EPS)


def _gelu(x):
    return jax.nn.gelu(x, approximate=True)


def _pack(x):
    return pltpu.bitcast(x.astype(BF16), U32)


def _unpack(x):
    return pltpu.bitcast(x, BF16)


def _dot(a, b):
    return jnp.dot(a, b, preferred_element_type=F32)


def _cols(ref, lo, hi, k0=0, k1=None):
    k1 = 2 * ref.shape[1] if k1 is None else k1
    return jnp.concatenate(
        [_unpack(ref[c, k0 // 2:k1 // 2, :]) for c in range(lo, hi)], axis=1)


def _kernel(x_hbm, mem_hbm, wq_hbm, wk_hbm, wv_hbm, wo_hbm, w1_hbm, w2_hbm,
            w3_hbm, w4_hbm, c_hbm, wmod_hbm, out_hbm,
            xv, memv, wmodv, modv, wqa, wqb, wov, us, gsb,
            hv0, hv1, hcur, ring, sums, h2t, h2l, x1l, zt, outv, fillv, cv, sems, *, phases):
    def scope(name):
        return jax.named_scope(name) if "s" in phases else contextlib.nullcontext()

    def cp(src, dst, s):
        return pltpu.make_async_copy(src, dst, sems.at[s])

    def col_copies(w_hbm, w_v, s, lo=0, hi=None):
        w32 = w_hbm.bitcast(U32)
        hi = w_v.shape[0] if hi is None else hi
        return [cp(w32.at[:, pl.ds(c * 128, 128)], w_v.at[c], s)
                for c in range(lo, hi)]

    def start(cps):
        for q in cps:
            q.start()

    def wait(cps):
        for q in cps:
            q.wait()

    def x_cp(r0, n, s):
        return cp(x_hbm.at[pl.ds(r0, n)], xv.at[pl.ds(r0, n)], s)

    c_cps = [cp(c_hbm, cv, SEM_C), cp(mem_hbm, memv, SEM_C)]
    x0_cp = x_cp(0, LEAD, SEM_X)
    wo_cps = col_copies(wo_hbm, wov, SEM_A)
    late_cps = [
        cp(w.bitcast(U32).at[:, pl.ds(c * 128, 128)],
           wqb.at[pl.ds(WB + (8 * i + c) * 512, 512)], SEM_XR)
        for i, w in enumerate((w1_hbm, w2_hbm)) for c in range(8)]

    def mod_rows(i, n):
        m = jnp.concatenate([modv[8 * i + c] for c in range(8)], axis=1)
        return jnp.concatenate([m] * (n // 8), axis=0)

    HI = jnp.uint32(0xFFFF0000)
    wq2 = (wqa, wqb)

    def paced(x, tiles):
        z = [pltpu.bitcast((t if t.dtype == U32 else pltpu.bitcast(t, U32))
                           & zt[0:8, :], F32) for t in tiles]
        z = jnp.concatenate(z, axis=0)
        if x.shape[1] == 128:
            return x + z
        return jnp.concatenate([x[:, 0:128] + z, x[:, 128:]], axis=1)

    def h_rest(k, t):
        xf = xv[pl.ds(pl.multiple_of(LEAD + 16 * k, 16), 16), :].astype(F32)
        y = _ln(paced(xf, t)) * mod_rows(1, 16) + mod_rows(0, 16)
        hv1[pl.ds(pl.multiple_of(8 * k, 8), 8), :] = _pack(y)
        return [y[0:8, 896:1024], y[8:16, 896:1024]]

    def prologue(st, xn, acc, scol, hn):
        w_hbms = (wq_hbm, wk_hbm, wv_hbm)

        def st_src(i):
            return w_hbms[i // 2].bitcast(U32).at[:, pl.ds((i % 2) * 8, 8), :]

        def pair_cps(n, s):
            w32 = wmod_hbm.bitcast(U32)
            return [cp(w32.at[:, pl.ds(pl.multiple_of(c * 128, 128), 128)],
                       wmodv.at[c], s) for c in (n, 8 + n)]

        def k_cps(n):
            return [cp(st_src(i).at[pl.ds(n * 128, 128)],
                       st.at[i, pl.ds(n * 128, 128)], SEM_K + n) for i in range(2)]

        def g_cps(g, src):
            return [cp(st_src(src), st.at[g], SEM_G + g - 1),
                    x_cp(pl.multiple_of(LEAD + 384 * (g - 2), 128), 384,
                         SEM_G + g - 1)]

        def mod_cps(g):
            lo, hi = {3: (16, 27), 4: (27, 38), 5: (38, 48)}[g]
            return col_copies(wmod_hbm, wmodv, SEM_G + g, lo, hi)

        with scope("first"):
            start(c_cps + [x0_cp])
        for n in range(8):
            start((pair_cps(n, SEM_M + n) if n < 2 else []) + k_cps(n)
                  + (pair_cps(n + 1, SEM_K + n) if 0 < n < 7 else []))
        start(g_cps(2, 2) + g_cps(3, 3) + g_cps(4, 4) + mod_cps(3) + g_cps(5, 5))

        r = lax.broadcasted_iota(jnp.int32, (80, 128), 0)
        k = lax.broadcasted_iota(jnp.int32, (80, 128), 1)

        def head_of(i):
            return jnp.where(i < 16, i // 8, (i - 16) // 32)

        def pos_of(i):
            return jnp.where(i < 16, i % 8, 8 + (i - 16) % 32)

        same = head_of(r) == head_of(k)
        vis = (pos_of(r) < M) | (pos_of(r) >= pos_of(k))
        fillv[...] = jnp.where(same, jnp.where(vis, 0.0, -1e9), -jnp.inf).astype(F32)
        sums[...] = jnp.zeros(sums.shape, F32)
        modv[48:56] = jnp.zeros((8, 8, 128), F32)
        modv[56:64] = jnp.ones((8, 8, 128), F32)
        ring[GB] = jnp.zeros(ring.shape[1:], U32)
        zt[...] = jnp.zeros(zt.shape, U32)
        h2t[...] = jnp.zeros(h2t.shape, F32)
        x1l[...] = jnp.zeros(x1l.shape, F32)


        def zero_body(i, _):
            rows = pl.ds(pl.multiple_of((i & 3) * 128, 128), 128)
            acc[lax.shift_right_logical(i, 2), rows, :] = jnp.zeros((128, 512), F32)
            return 0

        lax.fori_loop(0, 32, zero_body, 0)

        wait(c_cps)
        cf = cv[...].astype(F32)
        sil = cf * jax.nn.sigmoid(cf)
        for c in range(8):
            sw = _pack(jnp.broadcast_to(sil[:, c * 128:(c + 1) * 128], (128, 128)).T)
            scol[0, c * 64:(c + 1) * 64, :] = pltpu.bitcast(sw << 16, F32)
            scol[1, c * 64:(c + 1) * 64, :] = pltpu.bitcast(sw & HI, F32)

        x0_cp.wait()

        def ln_body(i, _):
            r0 = pl.multiple_of(i * 64, 64)
            y = _ln(xv[pl.ds(r0, 64), :].astype(F32))
            for q in range(8):
                xn[q, pl.ds(r0, 64), :] = y[:, q * 128:(q + 1) * 128]
            return 0

        lax.fori_loop(0, LEAD // 64, ln_body, 0)

        class Mod:
            def __init__(self, tiles, offs):
                self.tiles, self.offs = tiles, offs
                self.n, self.acc, self.out = 0, None, []

            def items(self, n, pace=None):
                for it in range(self.n, min(self.n + n, 64 * len(self.tiles))):
                    c, i = divmod(it, 64)
                    w = wmodv[self.tiles[c], i * 8:(i + 1) * 8, :]
                    if pace is not None:
                        w = w | pace
                    v = (pltpu.bitcast(w << 16, F32) * scol[0, i * 8:(i + 1) * 8, :]
                         + pltpu.bitcast(w & HI, F32) * scol[1, i * 8:(i + 1) * 8, :])
                    self.acc = v if i == 0 else self.acc + v
                    if i == 63:
                        m = jnp.broadcast_to(
                            jnp.sum(self.acc, axis=0, keepdims=True) + self.offs[c],
                            (8, 128))
                        modv[self.tiles[c]] = m
                        self.out.append(m)
                self.n += n

        def h_lead(n, b, sa, ca):
            rep = lambda m: jnp.concatenate([m, m], axis=0)
            y = _pack(xn[n, 16 * b:16 * b + 16, :] * rep(ca) + rep(sa))
            hn[8 * b:8 * b + 8, :] = y
            hv0[n, 8 * b:8 * b + 8, :] = y

        def relayout(par, g, p0, n, pace=None):
            base = g * (8 * SL)
            mask = jnp.uint32(0xFFFF0000 if par else 0xFFFF)
            if pace is not None:
                mask = pace | mask
            for u in range(n):
                a = st[g, 2 * (p0 + u)]
                b = st[g, 2 * (p0 + u) + 1]
                if par == 0:
                    w = (a & mask) | (b << 16)
                else:
                    w = (a >> 16) | (b & mask)
                wq2[par][pl.ds(base + p0 + u, 8, stride=SL), :] = w

        def to_ring(y, par, s0, b0):
            for u in range(y.shape[1] // 128):
                row = pl.multiple_of((2 * (s0 + u) + par) * 8, 8)
                for b in range(y.shape[0] // 8):
                    ring[b0 + b, pl.ds(row, 8), :] = (
                        y[b * 8:(b + 1) * 8, u * 128:(u + 1) * 128])

        def k_body(n, _):
            @pl.when(n < 2)
            def _():
                wait(pair_cps(n, SEM_M + n))
                md = Mod([n, 8 + n], [0.0, 1.0])
                md.items(128)
                for b in range(32):
                    h_lead(n, b, *md.out)

            wait(k_cps(n))

            @pl.when((n > 0) & (n < 7))
            def _():
                wait(pair_cps(n + 1, SEM_K + n))

            nn = jnp.where(n == 0, 0, jnp.minimum(n + 1, 7))
            md = Mod([nn, 8 + nn], [0.0, 1.0])
            zero = zt[0:8, :]
            order = [(0, 0), (1, 0), (0, 1), (1, 1)]
            relayout(0, 0, n * 64, 64)
            for i, (par, g) in enumerate(order):
                for hq in range(2):
                    s0 = g * 8 + hq * 4
                    w = jnp.concatenate(
                        [_unpack(wq2[par][pl.ds(pl.multiple_of(
                            (s0 + u) * SL + n * 64, 4), 64), :])
                         for u in range(4)], axis=1)
                    m = LQ if par else LEAD
                    y = _dot(_unpack(hn[0:m // 2, :]), w) + acc[2 * i + hq, 0:m, :]
                    acc[2 * i + hq, 0:m, :] = y
                    y = _pack(y)
                    to_ring(y, par, s0, 0)
                    tiles = [y[8 * b:8 * b + 8, 0:128] & zero for b in range(m // 16)]
                    tiles = [tiles[b * len(tiles) // 32] for b in range(32)]
                    for b in range(32):
                        pace = tiles[b]
                        if hq == 0 and i < 3:
                            relayout(*order[i + 1], n * 64 + 2 * b, 2, pace)
                        elif hq == 1 and i < 3:
                            md.items(2 - b % 2, pace)
                        elif hq == 1:
                            sa, ca = md.out
                            ca = ca + pltpu.bitcast(tiles[max(b - 3, 0)], F32)
                            h_lead(nn, b, sa, ca)
            return 0

        with scope("ksteps"):
            lax.fori_loop(0, 8, k_body, 0)

        start(mod_cps(4) + mod_cps(5) + wo_cps + late_cps)
        for c in range(8):
            hl = hv0[c, LQ // 2:LEAD // 2, :]
            us[0, :, c * 128:(c + 1) * 128] = hl
            gsb[0, :, c * 128:(c + 1) * 128] = hl
        wait(g_cps(2, 2))

        def rl_body(i, _):
            relayout(0, 2, i * 64, 64)
            return 0

        lax.fori_loop(0, 8, rl_body, 0)

        def lead_proj(par, s0, n, rc, rl, mp=128):
            w = jnp.concatenate(
                [_unpack(wq2[par][pl.ds(pl.multiple_of((s0 + u) * SL, 4), 512), :])
                 for u in range(n)], axis=1)
            lhs = jnp.concatenate(
                [_unpack(hv0[q, rc * mp:(rc + 1) * mp, :]) for q in range(8)],
                axis=1)
            y = _pack(_dot(lhs, w))
            to_ring(y, par, s0, rc * mp // 8)
            zero = zt[0:8, :]
            for u in range(n):
                for b in range(mp // 8):
                    k = min(3, 512 - rl[2])
                    if k > 0:
                        relayout(rl[0], rl[1], rl[2], k,
                                 y[b * 8:(b + 1) * 8, u * 128:(u + 1) * 128] & zero)
                        rl[2] += k
            return y

        def group_body(g, _):
            rl = [1, g, 0]
            for k in range(32):
                y = lead_proj(0, g * 8 + k // 4, 1, k % 4, rl, 64)
                if k == 12:
                    ts = [[y[0:8], y[16:24]], [y[40:48], y[56:64]]]
                    for i in range(24):
                        ts[i % 2] = h_rest(24 * (g - 2) + i, ts[i % 2])

            @pl.when(g < NG - 1)
            def _():
                wait(g_cps(g + 1, 0))

            for gg in (3, 4, 5):
                @pl.when(g == gg)
                def _(gg=gg):
                    wait(mod_cps(gg))

            gn = jnp.minimum(g + 1, NG - 1)
            t0 = jnp.where(g == 2, 0, jnp.minimum(11 * g - 17, 37))
            part = [lax.shift_right_logical(t0 + c, 3) for c in range(11)]
            md = Mod([t0 + c for c in range(11)],
                     [jnp.where((p == 1) | (p == 4), 1.0, 0.0).astype(F32)
                      for p in part])
            rl = [0, gn, 0]
            for k in range(16):
                y = lead_proj(1, g * 8 + k // 2, 1, k % 2, rl)
                for b in range(16):
                    md.items(3, y[8 * b:8 * b + 8] & zt[0:8, :])
            assert len(md.out) == 11
            return 0

        with scope("groups"):
            lax.fori_loop(2, NG, group_body, 0)

    pl.run_scoped(
        prologue,
        pltpu.VMEM((NG, D, 8, E), U32),
        pltpu.VMEM((8, LEAD, 128), F32),
        pltpu.VMEM((8, LEAD, 512), F32),
        pltpu.VMEM((2, D // 2, 128), F32),
        pltpu.VMEM((LEAD // 2, 128), U32),
    )

    def main(w3v, w4v, zv, ttv):
        w34_cps = col_copies(w3_hbm, w3v, SEM_B) + col_copies(w4_hbm, w4v, SEM_B)
        start(w34_cps)
        zv[0:HALO, :] = jnp.zeros((HALO, D), F32)
        wait(wo_cps)

        scale = float(E) ** -0.5

        def segment(lhs, ro, store_tok, wo_lhs, extras):
            fill = fillv[...]
            keep = fill == 0.0
            NP = H // 2
            qkv, probs, blocks = {}, {}, []

            def proj(hp):
                slots = [t * H + 2 * hp + par for t in range(3) for par in range(2)]
                wt = [jnp.concatenate(
                    [_unpack(wq2[sl % 2][pl.ds((sl // 2) * SL, 512), :])
                     for sl in slots[2 * t:2 * t + 2]], axis=1) for t in range(3)]
                if hp == 0:
                    w = jnp.concatenate(wt, axis=1)
                    y = _dot(lhs[:, :512], w[:512])
                    y = _dot(lhs[:, 512:], w[512:]) + y
                else:
                    y = jnp.concatenate([_dot(lhs, w) for w in wt], axis=1)
                for u, sl in enumerate(slots):
                    store_tok(sl, y[8:32, u * 128:(u + 1) * 128])
                ops = []
                for t in range(3):
                    ym = jnp.concatenate(
                        [y[0:8, (2 * t) * 128:(2 * t + 1) * 128],
                         y[0:8, (2 * t + 1) * 128:(2 * t + 2) * 128]], axis=0)
                    ops.append(jnp.concatenate(
                        [ym.astype(BF16)]
                        + [_unpack(ring[ro + b, sl * 8:(sl + 1) * 8, :])
                           for sl in slots[2 * t:2 * t + 2] for b in range(2)]
                        + ([jnp.zeros((48, 128), BF16)] if t else []),
                        axis=0))
                qkv[hp] = ops

            def scores(hp):
                q, kk, _ = qkv[hp]
                s = lax.dot_general(q, kk, (((1,), (1,)), ((), ())),
                                    preferred_element_type=F32)
                s = jnp.where(keep, s * scale, fill)
                mx = jnp.max(s, axis=-1, keepdims=True)
                p = jnp.exp(s - mx)
                l = jnp.sum(p, axis=-1, keepdims=True)
                rl = pl.reciprocal(l, approx=True)
                rl = rl * (2.0 - l * rl)
                probs[hp] = (p * rl).astype(BF16)

            def pv(hp):
                o = _dot(probs[hp], qkv[hp][2])
                blocks.append(wo_lhs(2 * hp, o[0:8], o[16:48]).astype(BF16))
                blocks.append(wo_lhs(2 * hp + 1, o[8:16], o[48:80]).astype(BF16))

            def wo_part(h0, h1, acc=None):
                lw = jnp.concatenate(blocks[h0:h1], axis=1)
                y = _dot(lw, _cols(wov, 0, 8, E * h0, E * h1))
                return y if acc is None else y + acc

            def attend(i):
                scores(i - 1)
                if i >= 3:
                    pv(i - 3)

            def fillers(key):
                for thunk in extras.get(key, ()):
                    thunk()

            for i in range(NP):
                proj(i)
                if i > 0:
                    attend(i)
                fillers(i)
            acc = wo_part(0, 4)
            attend(NP)
            fillers(NP)
            acc = wo_part(4, 10, acc)
            pv(NP - 2)
            pv(NP - 1)
            fillers(NP + 1)
            acc = wo_part(10, 20, acc)
            fillers(NP + 2)
            return wo_part(20, 32, acc)

        def put_x2(r0, lo, a):
            n = a.shape[0]
            x2 = (xv[pl.ds(pl.multiple_of(r0 + lo, 8), n), :].astype(F32)
                  + mod_rows(2, n) * a)
            zv[pl.ds(pl.multiple_of(HALO + r0 + lo, 8), n), :] = x2
            sums[lo:lo + n, :] = functools.reduce(
                jnp.add, [x2[:, c * 128:(c + 1) * 128] for c in range(8)])

        def p1_front(r0, sb=3):
            x2 = zv[pl.ds(pl.multiple_of(HALO + r0, 16), 64), :]
            h2 = _ln(x2, sums[...]) * mod_rows(4, 64) + mod_rows(sb, 64)
            return h2, _ln(h2)

        def w12(i):
            return jnp.concatenate(
                [_unpack(wqb[pl.ds(WB + (8 * i + c) * 512, 512), :]) for c in range(8)],
                axis=1)

        def p1_store(y, c, live):
            g = _gelu(y)
            if live is not None:
                g = jnp.where(live, g, y)
            ring[GB, c * 96 + 24:c * 96 + 88, :] = pltpu.bitcast(g, U32)

        def half_dots(lhs, i, live, done):
            part = {}

            def run(c, kh):
                row = jnp.where(live, WB + (8 * i + c) * 512, (8 * i + c) * SL)
                w = wqb[pl.ds(pl.multiple_of(row + kh * 256, 4), 256), :]
                y = _dot(lhs(kh), _unpack(w))
                if kh == 0:
                    part[c] = y
                else:
                    done(y + part[c], c)

            return [functools.partial(run, c, kh) for c in range(8) for kh in range(2)]

        def p2_front(n):
            return jnp.concatenate(
                [pltpu.bitcast(ring[GB, pl.ds(c * 96 + 8 + SHIFTS[c], n), :], F32)
                 for c in range(8)], axis=1)

        def p2_x1(h2, hs, row, gb=5):
            n = hs.shape[0]
            x1 = jnp.concatenate([h2t[...], h2[0:n - 16]], axis=0) + hs
            rows = pl.ds(pl.multiple_of(row, 16), n)
            zv[rows, :] = zv[rows, :] + mod_rows(gb, n) * x1
            return x1

        def p2_norm(x1, row, t):
            for g in range(x1.shape[0] // 16):
                y = _ln(paced(x1[16 * g:16 * g + 16, :], t))
                ttv[pl.ds(pl.multiple_of(row // 2 + 8 * g, 8), 8), :] = _pack(y)
                t = [y[0:8, 896:1024], y[8:16, 896:1024]]

        def a_body(j, mem):
            @pl.when(j == 1)
            def _():
                wait(late_cps)
                for k in range(16):
                    if k < 8:
                        q = pltpu.bitcast(ring[GB, k * 96 + 24:k * 96 + 88, :], F32)
                        ring[GB, k * 96 + 16:k * 96 + 24, :] = zt[0:8, :]
                    else:
                        q = zv[0:64, (k - 8) * 128:(k - 7) * 128]
                    q = _pack(q)
                    for b in range(4):
                        ring[LQ // 16 + b, (2 * k + 1) * 8:(2 * k + 2) * 8, :] = (
                            q[8 * b:8 * b + 8])

            hcur[...] = hv1[pl.ds(pl.multiple_of(24 * j, 8), 24), :]
            hb = _unpack(hcur[0:8, :])
            hac = _unpack(hcur[8:16, :]).astype(F32)
            hd = _unpack(hcur[16:24, :])
            wr = [lax.rem(LEAD // 16 + 3 * j + i, RING) for i in range(3)]
            ro0 = lax.rem(4 * j, RING)
            ro1 = ro0 + 2

            live = j > 0
            dead = jnp.where(live, 0, 1)
            h2, u = p1_front(64 * (j - 1), 3 + 3 * dead)
            us[dead] = _pack(u)

            lhs = jnp.concatenate(
                [jnp.concatenate([mem, hac[0:8]], axis=0).astype(BF16), hb], axis=0)
            tok_a = {}

            def store0(c, y):
                tok_a[c] = y[0:8]
                ring[wr[0], c * 8:(c + 1) * 8, :] = _pack(y[8:24])

            deferred = {}

            def wo_lhs0(h, om, ot):
                deferred[h] = ot[24:32]
                return jnp.concatenate([om, ot[0:24]], axis=0)

            pend = []

            def flush():
                while pend:
                    p1_store(*pend.pop(), live)

            th = half_dots(lambda kh: _unpack(us[0, :, kh * 512:(kh + 1) * 512]), 0,
                           live, lambda y, c: pend.append((y, c)))
            extras = {i: [flush, th[i - 2]] for i in range(2, 18)}
            out = segment(lhs, ro0, store0, wo_lhs0, extras)
            flush()
            mem = out[0:8]
            put_x2(64 * j, 0, out[8:32])

            lhs = jnp.concatenate(
                [jnp.concatenate([mem, hac[8:16]], axis=0).astype(BF16), hd], axis=0)

            def store1(c, y):
                ring[wr[1], c * 8:(c + 1) * 8, :] = _pack(
                    jnp.concatenate([tok_a[c], y[0:8]], axis=0))
                ring[wr[2], c * 8:(c + 1) * 8, :] = _pack(y[8:24])

            def wo_lhs1(h, om, ot):
                return jnp.concatenate([om, deferred[h], ot], axis=0)

            gsb[dead] = _pack(p2_front(64))
            for c in range(8):
                ring[GB, c * 96:c * 96 + 24, :] = ring[GB, c * 96 + 64:c * 96 + 88, :]
            hs = []

            def p2_fin():
                t = [hs[7][0:8], hs[7][0:8]]
                x1 = p2_x1(h2, jnp.concatenate(hs, axis=1), 64 * j, 5 + 2 * dead)
                p2_norm(x1, 64 * j, t)
                h2t[...] = h2[48:64]

            th = half_dots(lambda kh: _unpack(gsb[0, :, kh * 512:(kh + 1) * 512]), 1, live,
                           lambda y, c: hs.append(y))
            extras = {i: [th[i]] for i in range(16)}
            extras[18] = [p2_fin]
            out = segment(lhs, ro1, store1, wo_lhs1, extras)
            put_x2(64 * j, 24, out[8:48])
            return out[0:8]

        if "A" in phases:
            with scope("aloop"):
                lax.fori_loop(0, NPAIR, a_body, memv[...].astype(F32))
        else:
            zv[...] = jnp.zeros(zv.shape, F32)
            ttv[...] = jnp.zeros(ttv.shape, U32)

        wait(w34_cps)

        def out_cp(i, slot):
            return cp(outv.at[slot], out_hbm.at[pl.ds(i * RB, RB), :],
                      SEM_OUT + slot)

        def p3_body(i, _):
            slot = i % 2

            @pl.when(i >= 2)
            def _():
                out_cp(i - 2, slot).wait()

            @pl.when(i == 1)
            def _():
                y = _dot(_unpack(us[0]), w12(0))
                for c in range(8):
                    p1_store(y[:, c * 128:(c + 1) * 128], c, None)
                hs = _dot(p2_front(80).astype(BF16), w12(1))
                x1l[...] = p2_x1(h2l, hs, S)

            r0 = HALO + i * RB
            tt = _unpack(ttv[pl.ds(pl.multiple_of(r0 // 2, 8), RB // 2), :])
            ys = [_dot(tt, _cols(w3v, 4 * q, 4 * q + 4)) for q in range(FF // 512)]
            ff = jnp.concatenate([_gelu(y).astype(BF16) for y in ys], axis=1)
            t = [ys[-1][240:248, 384:512], ys[-1][248:256, 384:512]]
            for g in range(4):
                rows = slice(16 * g, 16 * g + 16)
                x2 = zv[HALO + S - 64 + 16 * g:HALO + S - 48 + 16 * g, :]
                h2 = (_ln(x2, paced(sums[rows, :], t)) * mod_rows(4, 16)
                      + mod_rows(3, 16))
                h2l[rows, :] = h2
                u = _ln(h2)
                us[0, 8 * g:8 * g + 8, :] = _pack(u)
                t = [u[0:8, 896:1024], u[8:16, 896:1024]]
            p2_norm(x1l, S, t)
            gb = mod_rows(5, RB)
            for c0, c1 in ((0, 7), (7, 8)):
                cols = slice(c0 * 128, c1 * 128)
                y = _dot(ff, _cols(w4v, c0, c1))
                res = zv[pl.ds(pl.multiple_of(r0, 16), RB), cols] + gb[:, cols] * y
                outv[slot, :, cols] = res.astype(BF16)
                cp(outv.at[slot, :, cols], out_hbm.at[pl.ds(i * RB, RB), cols],
                   SEM_OUT + slot).start()
            return 0

        nb = S // RB
        if "B" in phases:
            with scope("p3"):
                lax.fori_loop(0, nb, p3_body, 0)
            out_cp(nb - 2, 0).wait()
            out_cp(nb - 1, 1).wait()
        else:
            outv[0] = zv[pl.ds(HALO, RB), :].astype(BF16)
            out_cp(0, 0).start()
            out_cp(0, 0).wait()

    pl.run_scoped(
        main,
        pltpu.VMEM((FF // 128, D // 2, 128), U32),
        pltpu.VMEM((8, FF // 2, 128), U32),
        pltpu.VMEM((S + HALO, D), F32),
        pltpu.VMEM(((S + HALO) // 2, D), U32),
    )


def _call(A_x, A_mem0, A_Wq, A_Wk, A_Wv, A_Wo, B_w1, B_w2, B_w3, B_w4, c, w_mod,
          phases="AB"):
    any_spec = pl.BlockSpec(memory_space=pl.ANY)
    scratch = [
        pltpu.VMEM((S, D), BF16),
        pltpu.VMEM((M, D), BF16),
        pltpu.VMEM((48, D // 2, 128), U32),
        pltpu.VMEM((64, 8, 128), F32),
        pltpu.VMEM((WB, E), U32),
        pltpu.VMEM((WB + 16 * 512, E), U32),
        pltpu.VMEM((8, H * E // 2, 128), U32),
        pltpu.VMEM((2, 32, D), U32),
        pltpu.VMEM((2, 32, D), U32),
        pltpu.VMEM((8, LEAD // 2, 128), U32),
        pltpu.VMEM(((S - LEAD) // 2, D), U32),
        pltpu.VMEM((24, D), U32),
        pltpu.VMEM((RING + 1, 3 * H * 8, E), U32),
        pltpu.VMEM((64, 128), F32),
        pltpu.VMEM((16, D), F32),
        pltpu.VMEM((64, D), F32),
        pltpu.VMEM((80, D), F32),
        pltpu.VMEM((32, 128), U32),
        pltpu.VMEM((2, RB, D), BF16),
        pltpu.VMEM((80, 128), F32),
        pltpu.VMEM((1, D), BF16),
        pltpu.SemaphoreType.DMA((NSEM,)),
    ]
    out = pl.pallas_call(
        functools.partial(_kernel, phases=phases),
        in_specs=[any_spec] * 12,
        out_specs=any_spec,
        out_shape=jax.ShapeDtypeStruct((S, D), BF16),
        scratch_shapes=scratch,
        compiler_params=pltpu.CompilerParams(
            vmem_limit_bytes=126 * 1024 * 1024,
            disable_bounds_checks=True, disable_semaphore_checks=True),
    )(A_x.reshape(S, D), A_mem0.reshape(M, D), A_Wq, A_Wk, A_Wv,
      A_Wo.reshape(H * E, D), B_w1, B_w2, B_w3, B_w4, c, w_mod)
    return out.reshape(1, S, D)


def pallas_adaLN_cond__memory_aug_recurrent_mem_tr__mixer_s_mlp__prompt_kernel(
    A_x, A_mem0, A_Wq, A_Wk, A_Wv, A_Wo, A_seg_len, B_x, B_w1, B_w2, B_w3, B_w4,
    c, w_mod,
):
    if isinstance(A_seg_len, int):
        assert A_seg_len == SEG
    del B_x
    return _call(A_x, A_mem0, A_Wq, A_Wk, A_Wv, A_Wo, B_w1, B_w2, B_w3, B_w4,
                 c, w_mod)
```

```python
import contextlib
import functools

import jax
import jax.numpy as jnp
from jax import lax
import jax.experimental.pallas as pl
import jax.experimental.pallas.tpu as pltpu

F32 = jnp.float32
BF16 = jnp.bfloat16
U32 = jnp.uint32

S = 2048
D = 1024
H = 32
E = 128
M = 8
SEG = 32
FF = 3584
EPS = 1e-5
SCALE = float(E) ** -0.5
LOG2E = 1.4426950408889634

LEAD = 512
RING = 36
GB = RING
SL = 516
WB = 3 * H // 2 * SL + 544
LQ = LEAD - 64
HG = 16
NG = 3 * H // HG
NPAIR = S // (2 * SEG)
HALO = 80
RB = 256
SHIFTS = (-1, -1, 1, 1, -2, -2, 2, 2)

SEM_C = 0
SEM_X = 1
SEM_A = 2
SEM_B = 3
SEM_XR = 4
SEM_M = 5
SEM_K = 7
SEM_G = 14
SEM_OUT = 20
NSEM = 22


def _ln(x, part=None):
    if part is None:
        mu = jnp.mean(x, axis=-1, keepdims=True)
    else:
        mu = jnp.sum(part, axis=-1, keepdims=True) * (1.0 / x.shape[-1])
    xc = x - mu
    var = jnp.mean(xc * xc, axis=-1, keepdims=True)
    return xc * lax.rsqrt(var + EPS)


def _gelu(x):
    return jax.nn.gelu(x, approximate=True)


def _pack(x):
    return pltpu.bitcast(x.astype(BF16), U32)


def _unpack(x):
    return pltpu.bitcast(x, BF16)


def _dot(a, b):
    return jnp.dot(a, b, preferred_element_type=F32)


def _cols(ref, lo, hi, k0=0, k1=None):
    k1 = 2 * ref.shape[1] if k1 is None else k1
    return jnp.concatenate(
        [_unpack(ref[c, k0 // 2:k1 // 2, :]) for c in range(lo, hi)], axis=1)


def _kernel(x_hbm, mem_hbm, wq_hbm, wk_hbm, wv_hbm, wo_hbm, w1_hbm, w2_hbm,
            w3_hbm, w4_hbm, c_hbm, wmod_hbm, out_hbm,
            xv, memv, wmodv, modv, wqa, wqb, wov, us, gsb,
            hv0, hv1, hcur, ring, sums, h2t, h2l, x1l, zt, outv, fillv, cv, sems, *, phases):
    def scope(name):
        return jax.named_scope(name) if "s" in phases else contextlib.nullcontext()

    def cp(src, dst, s):
        return pltpu.make_async_copy(src, dst, sems.at[s])

    def col_copies(w_hbm, w_v, s, lo=0, hi=None):
        w32 = w_hbm.bitcast(U32)
        hi = w_v.shape[0] if hi is None else hi
        return [cp(w32.at[:, pl.ds(c * 128, 128)], w_v.at[c], s)
                for c in range(lo, hi)]

    def start(cps):
        for q in cps:
            q.start()

    def wait(cps):
        for q in cps:
            q.wait()

    def x_cp(r0, n, s):
        return cp(x_hbm.at[pl.ds(r0, n)], xv.at[pl.ds(r0, n)], s)

    c_cps = [cp(c_hbm, cv, SEM_C), cp(mem_hbm, memv, SEM_C)]
    x0_cp = x_cp(0, LEAD, SEM_X)
    wo_cps = col_copies(wo_hbm, wov, SEM_A)
    late_cps = [
        cp(w.bitcast(U32).at[:, pl.ds(c * 128, 128)],
           wqb.at[pl.ds(WB + (8 * i + c) * 512, 512)], SEM_XR)
        for i, w in enumerate((w1_hbm, w2_hbm)) for c in range(8)]

    def mod_rows(i, n):
        m = jnp.concatenate([modv[8 * i + c] for c in range(8)], axis=1)
        return jnp.concatenate([m] * (n // 8), axis=0)

    HI = jnp.uint32(0xFFFF0000)
    wq2 = (wqa, wqb)

    def paced(x, tiles):
        z = [pltpu.bitcast((t if t.dtype == U32 else pltpu.bitcast(t, U32))
                           & zt[0:8, :], F32) for t in tiles]
        z = jnp.concatenate(z, axis=0)
        if x.shape[1] == 128:
            return x + z
        return jnp.concatenate([x[:, 0:128] + z, x[:, 128:]], axis=1)

    def h_rest(k, t):
        xf = xv[pl.ds(pl.multiple_of(LEAD + 16 * k, 16), 16), :].astype(F32)
        y = _ln(paced(xf, t)) * mod_rows(1, 16) + mod_rows(0, 16)
        hv1[pl.ds(pl.multiple_of(8 * k, 8), 8), :] = _pack(y)
        return [y[0:8, 896:1024], y[8:16, 896:1024]]

    def prologue(st, xn, acc, scol, hn):
        w_hbms = (wq_hbm, wk_hbm, wv_hbm)

        def st_src(i):
            return w_hbms[i // 2].bitcast(U32).at[:, pl.ds((i % 2) * 8, 8), :]

        def pair_cps(n, s):
            w32 = wmod_hbm.bitcast(U32)
            return [cp(w32.at[:, pl.ds(pl.multiple_of(c * 128, 128), 128)],
                       wmodv.at[c], s) for c in (n, 8 + n)]

        def k_cps(n):
            return [cp(st_src(i).at[pl.ds(n * 128, 128)],
                       st.at[i, pl.ds(n * 128, 128)], SEM_K + n) for i in range(2)]

        def g_cps(g, src):
            return [cp(st_src(src), st.at[g], SEM_G + g - 1),
                    x_cp(pl.multiple_of(LEAD + 384 * (g - 2), 128), 384,
                         SEM_G + g - 1)]

        def mod_cps(g):
            lo, hi = {3: (16, 27), 4: (27, 38), 5: (38, 48)}[g]
            return col_copies(wmod_hbm, wmodv, SEM_G + g, lo, hi)

        with scope("first"):
            start(c_cps + [x0_cp])
        for n in range(8):
            start((pair_cps(n, SEM_M + n) if n < 2 else []) + k_cps(n)
                  + (pair_cps(n + 1, SEM_K + n) if 0 < n < 7 else []))
        start(g_cps(2, 2) + g_cps(3, 3) + g_cps(4, 4) + mod_cps(3) + g_cps(5, 5))

        r = lax.broadcasted_iota(jnp.int32, (80, 128), 0)
        k = lax.broadcasted_iota(jnp.int32, (80, 128), 1)

        def head_of(i):
            return jnp.where(i < 16, i // 8, (i - 16) // 32)

        def pos_of(i):
            return jnp.where(i < 16, i % 8, 8 + (i - 16) % 32)

        same = head_of(r) == head_of(k)
        vis = (pos_of(r) < M) | (pos_of(r) >= pos_of(k))
        fillv[...] = jnp.where(same, jnp.where(vis, 0.0, -1e9 / SCALE), -jnp.inf).astype(F32)
        sums[...] = jnp.zeros(sums.shape, F32)
        modv[48:56] = jnp.zeros((8, 8, 128), F32)
        modv[56:64] = jnp.ones((8, 8, 128), F32)
        ring[GB] = jnp.zeros(ring.shape[1:], U32)
        zt[...] = jnp.zeros(zt.shape, U32)
        h2t[...] = jnp.zeros(h2t.shape, F32)
        x1l[...] = jnp.zeros(x1l.shape, F32)


        def zero_body(i, _):
            rows = pl.ds(pl.multiple_of((i & 3) * 128, 128), 128)
            acc[lax.shift_right_logical(i, 2), rows, :] = jnp.zeros((128, 512), F32)
            return 0

        lax.fori_loop(0, 32, zero_body, 0)

        wait(c_cps)
        cf = cv[...].astype(F32)
        sil = cf * jax.nn.sigmoid(cf)
        for c in range(8):
            sw = _pack(jnp.broadcast_to(sil[:, c * 128:(c + 1) * 128], (128, 128)).T)
            scol[0, c * 64:(c + 1) * 64, :] = pltpu.bitcast(sw << 16, F32)
            scol[1, c * 64:(c + 1) * 64, :] = pltpu.bitcast(sw & HI, F32)

        x0_cp.wait()

        def ln_body(i, _):
            r0 = pl.multiple_of(i * 64, 64)
            y = _ln(xv[pl.ds(r0, 64), :].astype(F32))
            for q in range(8):
                xn[q, pl.ds(r0, 64), :] = y[:, q * 128:(q + 1) * 128]
            return 0

        lax.fori_loop(0, LEAD // 64, ln_body, 0)

        class Mod:
            def __init__(self, tiles, offs):
                self.tiles, self.offs = tiles, offs
                self.n, self.acc, self.out = 0, None, []

            def items(self, n, pace=None):
                for it in range(self.n, min(self.n + n, 64 * len(self.tiles))):
                    c, i = divmod(it, 64)
                    w = wmodv[self.tiles[c], i * 8:(i + 1) * 8, :]
                    if pace is not None:
                        w = w | pace
                    v = (pltpu.bitcast(w << 16, F32) * scol[0, i * 8:(i + 1) * 8, :]
                         + pltpu.bitcast(w & HI, F32) * scol[1, i * 8:(i + 1) * 8, :])
                    self.acc = v if i == 0 else self.acc + v
                    if i == 63:
                        m = jnp.broadcast_to(
                            jnp.sum(self.acc, axis=0, keepdims=True) + self.offs[c],
                            (8, 128))
                        modv[self.tiles[c]] = m
                        self.out.append(m)
                self.n += n

        def h_lead(n, b, sa, ca):
            rep = lambda m: jnp.concatenate([m, m], axis=0)
            y = _pack(xn[n, 16 * b:16 * b + 16, :] * rep(ca) + rep(sa))
            hn[8 * b:8 * b + 8, :] = y
            hv0[n, 8 * b:8 * b + 8, :] = y

        def relayout(par, g, p0, n, pace=None):
            base = g * (8 * SL)
            mask = jnp.uint32(0xFFFF0000 if par else 0xFFFF)
            if pace is not None:
                mask = pace | mask
            for u in range(n):
                a = st[g, 2 * (p0 + u)]
                b = st[g, 2 * (p0 + u) + 1]
                if par == 0:
                    w = (a & mask) | (b << 16)
                else:
                    w = (a >> 16) | (b & mask)
                wq2[par][pl.ds(base + p0 + u, 8, stride=SL), :] = w

        def to_ring(y, par, s0, b0):
            for u in range(y.shape[1] // 128):
                row = pl.multiple_of((2 * (s0 + u) + par) * 8, 8)
                for b in range(y.shape[0] // 8):
                    ring[b0 + b, pl.ds(row, 8), :] = (
                        y[b * 8:(b + 1) * 8, u * 128:(u + 1) * 128])

        def k_body(n, _):
            @pl.when(n < 2)
            def _():
                wait(pair_cps(n, SEM_M + n))
                md = Mod([n, 8 + n], [0.0, 1.0])
                md.items(128)
                for b in range(32):
                    h_lead(n, b, *md.out)

            wait(k_cps(n))

            @pl.when((n > 0) & (n < 7))
            def _():
                wait(pair_cps(n + 1, SEM_K + n))

            nn = jnp.where(n == 0, 0, jnp.minimum(n + 1, 7))
            md = Mod([nn, 8 + nn], [0.0, 1.0])
            zero = zt[0:8, :]
            order = [(0, 0), (1, 0), (0, 1), (1, 1)]
            relayout(0, 0, n * 64, 64)
            for i, (par, g) in enumerate(order):
                for hq in range(2):
                    s0 = g * 8 + hq * 4
                    w = jnp.concatenate(
                        [_unpack(wq2[par][pl.ds(pl.multiple_of(
                            (s0 + u) * SL + n * 64, 4), 64), :])
                         for u in range(4)], axis=1)
                    m = LQ if par else LEAD
                    y = _dot(_unpack(hn[0:m // 2, :]), w) + acc[2 * i + hq, 0:m, :]
                    acc[2 * i + hq, 0:m, :] = y
                    y = _pack(y)
                    to_ring(y, par, s0, 0)
                    tiles = [y[8 * b:8 * b + 8, 0:128] & zero for b in range(m // 16)]
                    tiles = [tiles[b * len(tiles) // 32] for b in range(32)]
                    for b in range(32):
                        pace = tiles[b]
                        if hq == 0 and i < 3:
                            relayout(*order[i + 1], n * 64 + 2 * b, 2, pace)
                        elif hq == 1 and i < 3:
                            md.items(2 - b % 2, pace)
                        elif hq == 1:
                            sa, ca = md.out
                            ca = ca + pltpu.bitcast(tiles[max(b - 3, 0)], F32)
                            h_lead(nn, b, sa, ca)
            return 0

        with scope("ksteps"):
            lax.fori_loop(0, 8, k_body, 0)

        start(mod_cps(4) + mod_cps(5) + wo_cps + late_cps)
        for c in range(8):
            hl = hv0[c, LQ // 2:LEAD // 2, :]
            us[0, :, c * 128:(c + 1) * 128] = hl
            gsb[0, :, c * 128:(c + 1) * 128] = hl
        wait(g_cps(2, 2))

        def rl_body(i, _):
            relayout(0, 2, i * 64, 64)
            return 0

        lax.fori_loop(0, 8, rl_body, 0)

        def lead_proj(par, s0, n, rc, rl, mp=128):
            w = jnp.concatenate(
                [_unpack(wq2[par][pl.ds(pl.multiple_of((s0 + u) * SL, 4), 512), :])
                 for u in range(n)], axis=1)
            lhs = jnp.concatenate(
                [_unpack(hv0[q, rc * mp:(rc + 1) * mp, :]) for q in range(8)],
                axis=1)
            y = _pack(_dot(lhs, w))
            to_ring(y, par, s0, rc * mp // 8)
            zero = zt[0:8, :]
            for u in range(n):
                for b in range(mp // 8):
                    k = min(3, 512 - rl[2])
                    if k > 0:
                        relayout(rl[0], rl[1], rl[2], k,
                                 y[b * 8:(b + 1) * 8, u * 128:(u + 1) * 128] & zero)
                        rl[2] += k
            return y

        def group_body(g, _):
            rl = [1, g, 0]
            for k in range(32):
                y = lead_proj(0, g * 8 + k // 4, 1, k % 4, rl, 64)
                if k == 12:
                    ts = [[y[0:8], y[16:24]], [y[40:48], y[56:64]]]
                    for i in range(24):
                        ts[i % 2] = h_rest(24 * (g - 2) + i, ts[i % 2])

            @pl.when(g < NG - 1)
            def _():
                wait(g_cps(g + 1, 0))

            for gg in (3, 4, 5):
                @pl.when(g == gg)
                def _(gg=gg):
                    wait(mod_cps(gg))

            gn = jnp.minimum(g + 1, NG - 1)
            t0 = jnp.where(g == 2, 0, jnp.minimum(11 * g - 17, 37))
            part = [lax.shift_right_logical(t0 + c, 3) for c in range(11)]
            md = Mod([t0 + c for c in range(11)],
                     [jnp.where((p == 1) | (p == 4), 1.0, 0.0).astype(F32)
                      for p in part])
            rl = [0, gn, 0]
            for k in range(16):
                y = lead_proj(1, g * 8 + k // 2, 1, k % 2, rl)
                for b in range(16):
                    md.items(3, y[8 * b:8 * b + 8] & zt[0:8, :])
            assert len(md.out) == 11
            return 0

        with scope("groups"):
            lax.fori_loop(2, NG, group_body, 0)

    pl.run_scoped(
        prologue,
        pltpu.VMEM((NG, D, 8, E), U32),
        pltpu.VMEM((8, LEAD, 128), F32),
        pltpu.VMEM((8, LEAD, 512), F32),
        pltpu.VMEM((2, D // 2, 128), F32),
        pltpu.VMEM((LEAD // 2, 128), U32),
    )

    def main(w3v, w4v, zv, ttv):
        w34_cps = col_copies(w3_hbm, w3v, SEM_B) + col_copies(w4_hbm, w4v, SEM_B)
        start(w34_cps)
        zv[0:HALO, :] = jnp.zeros((HALO, D), F32)
        wait(wo_cps)

        def segment(lhs, ro, store_tok, wo_lhs, extras, cut):
            fill = fillv[...]
            keep = fill == 0.0
            NP = H // 2
            qkv, probs, blocks = {}, {}, []

            def proj(hp):
                slots = [t * H + 2 * hp + par for t in range(3) for par in range(2)]
                wt = [jnp.concatenate(
                    [_unpack(wq2[sl % 2][pl.ds((sl // 2) * SL, 512), :])
                     for sl in slots[2 * t:2 * t + 2]], axis=1) for t in range(3)]
                if hp == 0:
                    w = jnp.concatenate(wt, axis=1)
                    y = _dot(lhs[:, :512], w[:512])
                    y = _dot(lhs[:, 512:], w[512:]) + y
                else:
                    ys = [_dot(lhs, wt[0]), _dot(lhs, wt[1])]
                    attend(hp)
                    y = jnp.concatenate(ys + [_dot(lhs, wt[2])], axis=1)
                for u, sl in enumerate(slots):
                    store_tok(sl, y[8:32, u * 128:(u + 1) * 128])
                ops = []
                for t in range(3):
                    ym = jnp.concatenate(
                        [y[0:8, (2 * t) * 128:(2 * t + 1) * 128],
                         y[0:8, (2 * t + 1) * 128:(2 * t + 2) * 128]], axis=0)
                    ops.append(jnp.concatenate(
                        [ym.astype(BF16)]
                        + [_unpack(ring[ro + b, sl * 8:(sl + 1) * 8, :])
                           for sl in slots[2 * t:2 * t + 2] for b in range(2)]
                        + ([jnp.zeros((48, 128), BF16)] if t else []),
                        axis=0))
                qkv[hp] = ops

            def scores(hp):
                q, kk, _ = qkv[hp]
                s = lax.dot_general(q, kk, (((1,), (1,)), ((), ())),
                                    preferred_element_type=F32)
                s = jnp.where(keep, s, fill)
                mx = jnp.max(s, axis=-1, keepdims=True)
                p = jnp.exp2((s - mx) * (SCALE * LOG2E))
                l = jnp.sum(p, axis=-1, keepdims=True)
                rl = pl.reciprocal(l, approx=True)
                rl = rl * (2.0 - l * rl)
                probs[hp] = (p * rl).astype(BF16)

            def pv(hp):
                o = _dot(probs[hp], qkv[hp][2])
                blocks.append(wo_lhs(2 * hp, o[0:8], o[16:48]).astype(BF16))
                blocks.append(wo_lhs(2 * hp + 1, o[8:16], o[48:80]).astype(BF16))

            def wo_part(h0, h1, acc=None):
                lw = jnp.concatenate(blocks[h0:h1], axis=1)
                y = _dot(lw, _cols(wov, 0, 8, E * h0, E * h1))
                return y if acc is None else y + acc

            def attend(i):
                scores(i - 1)
                if i >= 3:
                    pv(i - 3)

            def fillers(key):
                for thunk in extras.get(key, ()):
                    thunk()

            for i in range(NP):
                proj(i)
                fillers(i)
            acc = wo_part(0, 4)
            attend(NP)
            fillers(NP)
            acc = wo_part(4, cut, acc)
            pv(NP - 2)
            pv(NP - 1)
            fillers(NP + 1)
            acc = wo_part(cut, 22, acc)
            fillers(NP + 2)
            return wo_part(22, 32, acc)

        def put_x2(r0, lo, a):
            n = a.shape[0]
            x2 = (xv[pl.ds(pl.multiple_of(r0 + lo, 8), n), :].astype(F32)
                  + mod_rows(2, n) * a)
            zv[pl.ds(pl.multiple_of(HALO + r0 + lo, 8), n), :] = x2
            sums[lo:lo + n, :] = functools.reduce(
                jnp.add, [x2[:, c * 128:(c + 1) * 128] for c in range(8)])

        def p1_front(r0, sb=3):
            x2 = zv[pl.ds(pl.multiple_of(HALO + r0, 16), 64), :]
            h2 = _ln(x2, sums[...]) * mod_rows(4, 64) + mod_rows(sb, 64)
            return h2, _ln(h2)

        def w12(i):
            return jnp.concatenate(
                [_unpack(wqb[pl.ds(WB + (8 * i + c) * 512, 512), :]) for c in range(8)],
                axis=1)

        def p1_store(y, c, live):
            g = _gelu(y)
            if live is not None:
                g = jnp.where(live, g, y)
            ring[GB, c * 96 + 24:c * 96 + 88, :] = pltpu.bitcast(g, U32)

        def half_dots(lhs, i, live, done):
            part = {}

            def run(c, kh):
                row = jnp.where(live, WB + (8 * i + c) * 512, (8 * i + c) * SL)
                w = wqb[pl.ds(pl.multiple_of(row + kh * 256, 4), 256), :]
                y = _dot(lhs(kh), _unpack(w))
                if kh == 0:
                    part[c] = y
                else:
                    done(y + part[c], c)

            return [functools.partial(run, c, kh) for c in range(8) for kh in range(2)]

        def p2_front(n):
            return jnp.concatenate(
                [pltpu.bitcast(ring[GB, pl.ds(c * 96 + 8 + SHIFTS[c], n), :], F32)
                 for c in range(8)], axis=1)

        def p2_x1(h2, hs, row, gb=5):
            n = hs.shape[0]
            x1 = jnp.concatenate([h2t[...], h2[0:n - 16]], axis=0) + hs
            rows = pl.ds(pl.multiple_of(row, 16), n)
            zv[rows, :] = zv[rows, :] + mod_rows(gb, n) * x1
            return x1

        def p2_norm(x1, row, t):
            for g in range(x1.shape[0] // 16):
                y = _ln(paced(x1[16 * g:16 * g + 16, :], t))
                ttv[pl.ds(pl.multiple_of(row // 2 + 8 * g, 8), 8), :] = _pack(y)
                t = [y[0:8, 896:1024], y[8:16, 896:1024]]

        def a_body(j, mem):
            hcur[...] = hv1[pl.ds(pl.multiple_of(24 * j, 8), 24), :]
            hb = _unpack(hcur[0:8, :])
            hac = _unpack(hcur[8:16, :]).astype(F32)
            hd = _unpack(hcur[16:24, :])
            wr = [lax.rem(LEAD // 16 + 3 * j + i, RING) for i in range(3)]
            ro0 = lax.rem(4 * j, RING)
            ro1 = ro0 + 2

            live = j > 0
            dead = jnp.where(live, 0, 1)
            h2, u = p1_front(64 * (j - 1), 3 + 3 * dead)
            us[dead] = _pack(u)

            lhs = jnp.concatenate(
                [jnp.concatenate([mem, hac[0:8]], axis=0).astype(BF16), hb], axis=0)
            tok_a = {}

            def store0(c, y):
                tok_a[c] = y[0:8]
                ring[wr[0], c * 8:(c + 1) * 8, :] = _pack(y[8:24])

            deferred = {}

            def wo_lhs0(h, om, ot):
                deferred[h] = ot[24:32]
                return jnp.concatenate([om, ot[0:24]], axis=0)

            pend = []

            def flush():
                while pend:
                    p1_store(*pend.pop(), live)

            th = half_dots(lambda kh: _unpack(us[0, :, kh * 512:(kh + 1) * 512]), 0,
                           live, lambda y, c: pend.append((y, c)))
            extras = {i: [flush, th[i - 2]] for i in range(2, 18)}
            out = segment(lhs, ro0, store0, wo_lhs0, extras, 11)
            flush()
            mem = out[0:8]
            put_x2(64 * j, 0, out[8:32])

            lhs = jnp.concatenate(
                [jnp.concatenate([mem, hac[8:16]], axis=0).astype(BF16), hd], axis=0)

            def store1(c, y):
                ring[wr[1], c * 8:(c + 1) * 8, :] = _pack(
                    jnp.concatenate([tok_a[c], y[0:8]], axis=0))
                ring[wr[2], c * 8:(c + 1) * 8, :] = _pack(y[8:24])

            def wo_lhs1(h, om, ot):
                return jnp.concatenate([om, deferred[h], ot], axis=0)

            gsb[dead] = _pack(p2_front(64))
            for c in range(8):
                ring[GB, c * 96:c * 96 + 24, :] = ring[GB, c * 96 + 64:c * 96 + 88, :]
            hs = []

            def p2_fin():
                t = [hs[7][0:8], hs[7][0:8]]
                x1 = p2_x1(h2, jnp.concatenate(hs, axis=1), 64 * j, 5 + 2 * dead)
                p2_norm(x1, 64 * j, t)
                h2t[...] = h2[48:64]

            th = half_dots(lambda kh: _unpack(gsb[0, :, kh * 512:(kh + 1) * 512]), 1, live,
                           lambda y, c: hs.append(y))
            extras = {i: [th[i]] for i in range(16)}
            extras[18] = [p2_fin]
            out = segment(lhs, ro1, store1, wo_lhs1, extras, 12)
            put_x2(64 * j, 24, out[8:48])
            return out[0:8]

        def a_phase(ph, mem):
            mem = lax.fori_loop(ph, 1 + ph * (NPAIR - 1), a_body, mem)

            @pl.when(ph == 0)
            def _():
                wait(late_cps)
                for k in range(16):
                    if k < 8:
                        q = pltpu.bitcast(ring[GB, k * 96 + 24:k * 96 + 88, :], F32)
                        ring[GB, k * 96 + 16:k * 96 + 24, :] = zt[0:8, :]
                    else:
                        q = zv[0:64, (k - 8) * 128:(k - 7) * 128]
                    q = _pack(q)
                    for b in range(4):
                        ring[LQ // 16 + b, (2 * k + 1) * 8:(2 * k + 2) * 8, :] = (
                            q[8 * b:8 * b + 8])

            return mem

        if "A" in phases:
            with scope("aloop"):
                lax.fori_loop(0, 2, a_phase, memv[...].astype(F32))
        else:
            zv[...] = jnp.zeros(zv.shape, F32)
            ttv[...] = jnp.zeros(ttv.shape, U32)

        wait(w34_cps)

        def out_cp(i, slot):
            return cp(outv.at[slot], out_hbm.at[pl.ds(i * RB, RB), :],
                      SEM_OUT + slot)

        def p3_body(i, _):
            slot = i % 2

            @pl.when(i >= 2)
            def _():
                out_cp(i - 2, slot).wait()

            @pl.when(i == 1)
            def _():
                y = _dot(_unpack(us[0]), w12(0))
                for c in range(8):
                    p1_store(y[:, c * 128:(c + 1) * 128], c, None)
                hs = _dot(p2_front(80).astype(BF16), w12(1))
                x1l[...] = p2_x1(h2l, hs, S)

            r0 = HALO + i * RB
            tt = _unpack(ttv[pl.ds(pl.multiple_of(r0 // 2, 8), RB // 2), :])
            ys = [_dot(tt, _cols(w3v, 4 * q, 4 * q + 4)) for q in range(FF // 512)]
            ff = jnp.concatenate([_gelu(y).astype(BF16) for y in ys], axis=1)
            t = [ys[-1][240:248, 384:512], ys[-1][248:256, 384:512]]
            for g in range(4):
                rows = slice(16 * g, 16 * g + 16)
                x2 = zv[HALO + S - 64 + 16 * g:HALO + S - 48 + 16 * g, :]
                h2 = (_ln(x2, paced(sums[rows, :], t)) * mod_rows(4, 16)
                      + mod_rows(3, 16))
                h2l[rows, :] = h2
                u = _ln(h2)
                us[0, 8 * g:8 * g + 8, :] = _pack(u)
                t = [u[0:8, 896:1024], u[8:16, 896:1024]]
            p2_norm(x1l, S, t)
            gb = mod_rows(5, RB)
            for c0, c1 in ((0, 7), (7, 8)):
                cols = slice(c0 * 128, c1 * 128)
                y = _dot(ff, _cols(w4v, c0, c1))
                res = zv[pl.ds(pl.multiple_of(r0, 16), RB), cols] + gb[:, cols] * y
                outv[slot, :, cols] = res.astype(BF16)
                cp(outv.at[slot, :, cols], out_hbm.at[pl.ds(i * RB, RB), cols],
                   SEM_OUT + slot).start()
            return 0

        nb = S // RB
        if "B" in phases:
            with scope("p3"):
                lax.fori_loop(0, nb, p3_body, 0)
            out_cp(nb - 2, 0).wait()
            out_cp(nb - 1, 1).wait()
        else:
            outv[0] = zv[pl.ds(HALO, RB), :].astype(BF16)
            out_cp(0, 0).start()
            out_cp(0, 0).wait()

    pl.run_scoped(
        main,
        pltpu.VMEM((FF // 128, D // 2, 128), U32),
        pltpu.VMEM((8, FF // 2, 128), U32),
        pltpu.VMEM((S + HALO, D), F32),
        pltpu.VMEM(((S + HALO) // 2, D), U32),
    )


def _call(A_x, A_mem0, A_Wq, A_Wk, A_Wv, A_Wo, B_w1, B_w2, B_w3, B_w4, c, w_mod,
          phases="AB"):
    any_spec = pl.BlockSpec(memory_space=pl.ANY)
    scratch = [
        pltpu.VMEM((S, D), BF16),
        pltpu.VMEM((M, D), BF16),
        pltpu.VMEM((48, D // 2, 128), U32),
        pltpu.VMEM((64, 8, 128), F32),
        pltpu.VMEM((WB, E), U32),
        pltpu.VMEM((WB + 16 * 512, E), U32),
        pltpu.VMEM((8, H * E // 2, 128), U32),
        pltpu.VMEM((2, 32, D), U32),
        pltpu.VMEM((2, 32, D), U32),
        pltpu.VMEM((8, LEAD // 2, 128), U32),
        pltpu.VMEM(((S - LEAD) // 2, D), U32),
        pltpu.VMEM((24, D), U32),
        pltpu.VMEM((RING + 1, 3 * H * 8, E), U32),
        pltpu.VMEM((64, 128), F32),
        pltpu.VMEM((16, D), F32),
        pltpu.VMEM((64, D), F32),
        pltpu.VMEM((80, D), F32),
        pltpu.VMEM((32, 128), U32),
        pltpu.VMEM((2, RB, D), BF16),
        pltpu.VMEM((80, 128), F32),
        pltpu.VMEM((1, D), BF16),
        pltpu.SemaphoreType.DMA((NSEM,)),
    ]
    out = pl.pallas_call(
        functools.partial(_kernel, phases=phases),
        in_specs=[any_spec] * 12,
        out_specs=any_spec,
        out_shape=jax.ShapeDtypeStruct((S, D), BF16),
        scratch_shapes=scratch,
        compiler_params=pltpu.CompilerParams(
            vmem_limit_bytes=126 * 1024 * 1024,
            disable_bounds_checks=True, disable_semaphore_checks=True),
    )(A_x.reshape(S, D), A_mem0.reshape(M, D), A_Wq, A_Wk, A_Wv,
      A_Wo.reshape(H * E, D), B_w1, B_w2, B_w3, B_w4, c, w_mod)
    return out.reshape(1, S, D)


def pallas_adaLN_cond__memory_aug_recurrent_mem_tr__mixer_s_mlp__prompt_kernel(
    A_x, A_mem0, A_Wq, A_Wk, A_Wv, A_Wo, A_seg_len, B_x, B_w1, B_w2, B_w3, B_w4,
    c, w_mod,
):
    if isinstance(A_seg_len, int):
        assert A_seg_len == SEG
    del B_x
    return _call(A_x, A_mem0, A_Wq, A_Wk, A_Wv, A_Wo, B_w1, B_w2, B_w3, B_w4,
                 c, w_mod)
```

```python
import contextlib
import functools

import jax
import jax.numpy as jnp
from jax import lax
import jax.experimental.pallas as pl
import jax.experimental.pallas.tpu as pltpu

F32 = jnp.float32
BF16 = jnp.bfloat16
U32 = jnp.uint32

S = 2048
D = 1024
H = 32
E = 128
M = 8
SEG = 32
FF = 3584
EPS = 1e-5
SCALE = float(E) ** -0.5
LOG2E = 1.4426950408889634

LEAD = 512
RING = 36
GB = RING
SL = 516
WB = 3 * H // 2 * SL + 544
LQ = LEAD - 64
HG = 16
NG = 3 * H // HG
NPAIR = S // (2 * SEG)
HALO = 80
RB = 256
SHIFTS = (-1, -1, 1, 1, -2, -2, 2, 2)

SEM_C = 0
SEM_X = 1
SEM_A = 2
SEM_B = 3
SEM_XR = 4
SEM_M = 5
SEM_K = 7
SEM_G = 14
SEM_OUT = 20
NSEM = 22


def _ln(x, part=None):
    if part is None:
        mu = jnp.mean(x, axis=-1, keepdims=True)
    else:
        mu = jnp.sum(part, axis=-1, keepdims=True) * (1.0 / x.shape[-1])
    xc = x - mu
    var = jnp.mean(xc * xc, axis=-1, keepdims=True)
    return xc * lax.rsqrt(var + EPS)


def _gelu(x):
    return jax.nn.gelu(x, approximate=True)


def _pack(x):
    return pltpu.bitcast(x.astype(BF16), U32)


def _unpack(x):
    return pltpu.bitcast(x, BF16)


def _dot(a, b):
    return jnp.dot(a, b, preferred_element_type=F32)


def _cols(ref, lo, hi, k0=0, k1=None):
    k1 = 2 * ref.shape[1] if k1 is None else k1
    return jnp.concatenate(
        [_unpack(ref[c, k0 // 2:k1 // 2, :]) for c in range(lo, hi)], axis=1)


def _kernel(x_hbm, mem_hbm, wq_hbm, wk_hbm, wv_hbm, wo_hbm, w1_hbm, w2_hbm,
            w3_hbm, w4_hbm, c_hbm, wmod_hbm, out_hbm,
            xv, memv, wmodv, modv, wqa, wqb, wov, us, gsb, hv0, hv1, hcur, ring,
            sums, h2t, h2l, x1l, zt, outv, fillv, cv, sems, *, scopes):
    def scope(name):
        return jax.named_scope(name) if scopes else contextlib.nullcontext()

    def cp(src, dst, s):
        return pltpu.make_async_copy(src, dst, sems.at[s])

    def col_copies(w_hbm, w_v, s, lo=0, hi=None):
        w32 = w_hbm.bitcast(U32)
        hi = w_v.shape[0] if hi is None else hi
        return [cp(w32.at[:, pl.ds(c * 128, 128)], w_v.at[c], s)
                for c in range(lo, hi)]

    def start(cps):
        for q in cps:
            q.start()

    def wait(cps):
        for q in cps:
            q.wait()

    def x_cp(r0, n, s):
        return cp(x_hbm.at[pl.ds(r0, n)], xv.at[pl.ds(r0, n)], s)

    c_cps = [cp(c_hbm, cv, SEM_C), cp(mem_hbm, memv, SEM_C)]
    x0_cp = x_cp(0, LEAD, SEM_X)
    wo_cps = col_copies(wo_hbm, wov, SEM_A)
    late_cps = [
        cp(w.bitcast(U32).at[:, pl.ds(c * 128, 128)],
           wqb.at[pl.ds(WB + (8 * i + c) * 512, 512)], SEM_XR)
        for i, w in enumerate((w1_hbm, w2_hbm)) for c in range(8)]

    def mod_rows(i, n):
        m = jnp.concatenate([modv[8 * i + c] for c in range(8)], axis=1)
        return jnp.concatenate([m] * (n // 8), axis=0)

    HI = jnp.uint32(0xFFFF0000)
    wq2 = (wqa, wqb)

    def paced(x, tiles):
        z = [pltpu.bitcast((t if t.dtype == U32 else pltpu.bitcast(t, U32))
                           & zt[0:8, :], F32) for t in tiles]
        z = jnp.concatenate(z, axis=0)
        if x.shape[1] == 128:
            return x + z
        return jnp.concatenate([x[:, 0:128] + z, x[:, 128:]], axis=1)

    def h_rest(k, t):
        xf = xv[pl.ds(pl.multiple_of(LEAD + 16 * k, 16), 16), :].astype(F32)
        y = _ln(paced(xf, t)) * mod_rows(1, 16) + mod_rows(0, 16)
        hv1[pl.ds(pl.multiple_of(8 * k, 8), 8), :] = _pack(y)
        return [y[0:8, 896:1024], y[8:16, 896:1024]]

    def prologue(st, xn, acc, scol, hn):
        w_hbms = (wq_hbm, wk_hbm, wv_hbm)

        def st_src(i):
            return w_hbms[i // 2].bitcast(U32).at[:, pl.ds((i % 2) * 8, 8), :]

        def pair_cps(n, s):
            w32 = wmod_hbm.bitcast(U32)
            return [cp(w32.at[:, pl.ds(pl.multiple_of(c * 128, 128), 128)],
                       wmodv.at[c], s) for c in (n, 8 + n)]

        def k_cps(n):
            return [cp(st_src(i).at[pl.ds(n * 128, 128)],
                       st.at[i, pl.ds(n * 128, 128)], SEM_K + n) for i in range(2)]

        def g_cps(g, src):
            return [cp(st_src(src), st.at[g], SEM_G + g - 1),
                    x_cp(pl.multiple_of(LEAD + 384 * (g - 2), 128), 384,
                         SEM_G + g - 1)]

        def mod_cps(g):
            lo, hi = {3: (16, 27), 4: (27, 38), 5: (38, 48)}[g]
            return col_copies(wmod_hbm, wmodv, SEM_G + g, lo, hi)

        with scope("first"):
            start(c_cps + [x0_cp])
        for n in range(8):
            start((pair_cps(n, SEM_M + n) if n < 2 else []) + k_cps(n)
                  + (pair_cps(n + 1, SEM_K + n) if 0 < n < 7 else []))
        start(g_cps(2, 2) + g_cps(3, 3) + g_cps(4, 4) + mod_cps(3) + g_cps(5, 5))

        r = lax.broadcasted_iota(jnp.int32, (80, 128), 0)
        k = lax.broadcasted_iota(jnp.int32, (80, 128), 1)

        def head_of(i):
            return jnp.where(i < 16, i // 8, (i - 16) // 32)

        def pos_of(i):
            return jnp.where(i < 16, i % 8, 8 + (i - 16) % 32)

        same = head_of(r) == head_of(k)
        vis = (pos_of(r) < M) | (pos_of(r) >= pos_of(k))
        fillv[...] = jnp.where(same, jnp.where(vis, 0.0, -1e9 / SCALE),
                               -jnp.inf).astype(F32)
        sums[...] = jnp.zeros(sums.shape, F32)
        modv[48:56] = jnp.zeros((8, 8, 128), F32)
        modv[56:64] = jnp.ones((8, 8, 128), F32)
        ring[GB] = jnp.zeros(ring.shape[1:], U32)
        zt[...] = jnp.zeros(zt.shape, U32)
        h2t[...] = jnp.zeros(h2t.shape, F32)
        x1l[...] = jnp.zeros(x1l.shape, F32)

        def zero_body(i, _):
            rows = pl.ds(pl.multiple_of((i & 3) * 128, 128), 128)
            acc[lax.shift_right_logical(i, 2), rows, :] = jnp.zeros((128, 512), F32)
            return 0

        lax.fori_loop(0, 32, zero_body, 0)

        wait(c_cps)
        cf = cv[...].astype(F32)
        sil = cf * jax.nn.sigmoid(cf)
        for c in range(8):
            sw = _pack(jnp.broadcast_to(sil[:, c * 128:(c + 1) * 128], (128, 128)).T)
            scol[0, c * 64:(c + 1) * 64, :] = pltpu.bitcast(sw << 16, F32)
            scol[1, c * 64:(c + 1) * 64, :] = pltpu.bitcast(sw & HI, F32)

        x0_cp.wait()

        def ln_body(i, _):
            r0 = pl.multiple_of(i * 64, 64)
            y = _ln(xv[pl.ds(r0, 64), :].astype(F32))
            for q in range(8):
                xn[q, pl.ds(r0, 64), :] = y[:, q * 128:(q + 1) * 128]
            return 0

        lax.fori_loop(0, LEAD // 64, ln_body, 0)

        class Mod:
            def __init__(self, tiles, offs):
                self.tiles, self.offs = tiles, offs
                self.n, self.acc, self.out = 0, None, []

            def items(self, n, pace=None):
                for it in range(self.n, min(self.n + n, 64 * len(self.tiles))):
                    c, i = divmod(it, 64)
                    w = wmodv[self.tiles[c], i * 8:(i + 1) * 8, :]
                    if pace is not None:
                        w = w | pace
                    v = (pltpu.bitcast(w << 16, F32) * scol[0, i * 8:(i + 1) * 8, :]
                         + pltpu.bitcast(w & HI, F32) * scol[1, i * 8:(i + 1) * 8, :])
                    self.acc = v if i == 0 else self.acc + v
                    if i == 63:
                        m = jnp.broadcast_to(
                            jnp.sum(self.acc, axis=0, keepdims=True) + self.offs[c],
                            (8, 128))
                        modv[self.tiles[c]] = m
                        self.out.append(m)
                self.n += n

        def h_lead(n, b, sa, ca):
            rep = lambda m: jnp.concatenate([m, m], axis=0)
            y = _pack(xn[n, 16 * b:16 * b + 16, :] * rep(ca) + rep(sa))
            hn[8 * b:8 * b + 8, :] = y
            hv0[n, 8 * b:8 * b + 8, :] = y

        def relayout(par, g, p0, n, pace=None):
            base = g * (8 * SL)
            mask = jnp.uint32(0xFFFF0000 if par else 0xFFFF)
            if pace is not None:
                mask = pace | mask
            for u in range(n):
                a = st[g, 2 * (p0 + u)]
                b = st[g, 2 * (p0 + u) + 1]
                if par == 0:
                    w = (a & mask) | (b << 16)
                else:
                    w = (a >> 16) | (b & mask)
                wq2[par][pl.ds(base + p0 + u, 8, stride=SL), :] = w

        def to_ring(y, par, s0, b0):
            for u in range(y.shape[1] // 128):
                row = pl.multiple_of((2 * (s0 + u) + par) * 8, 8)
                for b in range(y.shape[0] // 8):
                    ring[b0 + b, pl.ds(row, 8), :] = (
                        y[b * 8:(b + 1) * 8, u * 128:(u + 1) * 128])

        def k_body(n, _):
            @pl.when(n < 2)
            def _():
                wait(pair_cps(n, SEM_M + n))
                md = Mod([n, 8 + n], [0.0, 1.0])
                md.items(128)
                for b in range(32):
                    h_lead(n, b, *md.out)

            wait(k_cps(n))

            @pl.when((n > 0) & (n < 7))
            def _():
                wait(pair_cps(n + 1, SEM_K + n))

            nn = jnp.where(n == 0, 0, jnp.minimum(n + 1, 7))
            md = Mod([nn, 8 + nn], [0.0, 1.0])
            zero = zt[0:8, :]
            order = [(0, 0), (1, 0), (0, 1), (1, 1)]
            relayout(0, 0, n * 64, 64)
            for i, (par, g) in enumerate(order):
                for hq in range(2):
                    s0 = g * 8 + hq * 4
                    w = jnp.concatenate(
                        [_unpack(wq2[par][pl.ds(pl.multiple_of(
                            (s0 + u) * SL + n * 64, 4), 64), :])
                         for u in range(4)], axis=1)
                    m = LQ if par else LEAD
                    y = _dot(_unpack(hn[0:m // 2, :]), w) + acc[2 * i + hq, 0:m, :]
                    acc[2 * i + hq, 0:m, :] = y
                    y = _pack(y)
                    to_ring(y, par, s0, 0)
                    tiles = [y[8 * b:8 * b + 8, 0:128] & zero for b in range(m // 16)]
                    tiles = [tiles[b * len(tiles) // 32] for b in range(32)]
                    for b in range(32):
                        pace = tiles[b]
                        if hq == 0 and i < 3:
                            relayout(*order[i + 1], n * 64 + 2 * b, 2, pace)
                        elif hq == 1 and i < 3:
                            md.items(2 - b % 2, pace)
                        elif hq == 1:
                            sa, ca = md.out
                            ca = ca + pltpu.bitcast(tiles[max(b - 3, 0)], F32)
                            h_lead(nn, b, sa, ca)
            return 0

        with scope("ksteps"):
            lax.fori_loop(0, 8, k_body, 0)

        start(mod_cps(4) + mod_cps(5) + wo_cps + late_cps)
        for c in range(8):
            hl = hv0[c, LQ // 2:LEAD // 2, :]
            us[0, :, c * 128:(c + 1) * 128] = hl
            gsb[0, :, c * 128:(c + 1) * 128] = hl
        wait(g_cps(2, 2))

        def rl_body(i, _):
            relayout(0, 2, i * 64, 64)
            return 0

        lax.fori_loop(0, 8, rl_body, 0)

        def lead_proj(par, s0, n, rc, rl, mp=128):
            w = jnp.concatenate(
                [_unpack(wq2[par][pl.ds(pl.multiple_of((s0 + u) * SL, 4), 512), :])
                 for u in range(n)], axis=1)
            lhs = jnp.concatenate(
                [_unpack(hv0[q, rc * mp:(rc + 1) * mp, :]) for q in range(8)],
                axis=1)
            y = _pack(_dot(lhs, w))
            to_ring(y, par, s0, rc * mp // 8)
            zero = zt[0:8, :]
            for u in range(n):
                for b in range(mp // 8):
                    k = min(3, 512 - rl[2])
                    if k > 0:
                        relayout(rl[0], rl[1], rl[2], k,
                                 y[b * 8:(b + 1) * 8, u * 128:(u + 1) * 128] & zero)
                        rl[2] += k
            return y

        def group_body(g, _):
            rl = [1, g, 0]
            for k in range(32):
                y = lead_proj(0, g * 8 + k // 4, 1, k % 4, rl, 64)
                if k == 12:
                    ts = [[y[0:8], y[16:24]], [y[40:48], y[56:64]]]
                    for i in range(24):
                        ts[i % 2] = h_rest(24 * (g - 2) + i, ts[i % 2])

            @pl.when(g < NG - 1)
            def _():
                wait(g_cps(g + 1, 0))

            for gg in (3, 4, 5):
                @pl.when(g == gg)
                def _(gg=gg):
                    wait(mod_cps(gg))

            gn = jnp.minimum(g + 1, NG - 1)
            t0 = jnp.where(g == 2, 0, jnp.minimum(11 * g - 17, 37))
            part = [lax.shift_right_logical(t0 + c, 3) for c in range(11)]
            md = Mod([t0 + c for c in range(11)],
                     [jnp.where((p == 1) | (p == 4), 1.0, 0.0).astype(F32)
                      for p in part])
            rl = [0, gn, 0]
            for k in range(16):
                y = lead_proj(1, g * 8 + k // 2, 1, k % 2, rl)
                for b in range(16):
                    md.items(3, y[8 * b:8 * b + 8] & zt[0:8, :])
            assert len(md.out) == 11
            return 0

        with scope("groups"):
            lax.fori_loop(2, NG, group_body, 0)

    pl.run_scoped(
        prologue,
        pltpu.VMEM((NG, D, 8, E), U32),
        pltpu.VMEM((8, LEAD, 128), F32),
        pltpu.VMEM((8, LEAD, 512), F32),
        pltpu.VMEM((2, D // 2, 128), F32),
        pltpu.VMEM((LEAD // 2, 128), U32),
    )

    def main(w3v, w4v, zv, ttv):
        w34_cps = col_copies(w3_hbm, w3v, SEM_B) + col_copies(w4_hbm, w4v, SEM_B)
        start(w34_cps)
        zv[0:HALO, :] = jnp.zeros((HALO, D), F32)
        wait(wo_cps)

        def segment(lhs, ro, store_tok, wo_lhs, extras, cut):
            fill = fillv[...]
            keep = fill == 0.0
            NP = H // 2
            qkv, probs, blocks = {}, {}, []

            def proj(hp):
                slots = [t * H + 2 * hp + par for t in range(3) for par in range(2)]
                wt = [jnp.concatenate(
                    [_unpack(wq2[sl % 2][pl.ds((sl // 2) * SL, 512), :])
                     for sl in slots[2 * t:2 * t + 2]], axis=1) for t in range(3)]
                if hp == 0:
                    w = jnp.concatenate(wt, axis=1)
                    y = _dot(lhs[:, :512], w[:512])
                    y = _dot(lhs[:, 512:], w[512:]) + y
                else:
                    ys = [_dot(lhs, wt[0]), _dot(lhs, wt[1])]
                    attend(hp)
                    y = jnp.concatenate(ys + [_dot(lhs, wt[2])], axis=1)
                for u, sl in enumerate(slots):
                    store_tok(sl, y[8:32, u * 128:(u + 1) * 128])
                ops = []
                for t in range(3):
                    ym = jnp.concatenate(
                        [y[0:8, (2 * t) * 128:(2 * t + 1) * 128],
                         y[0:8, (2 * t + 1) * 128:(2 * t + 2) * 128]], axis=0)
                    ops.append(jnp.concatenate(
                        [ym.astype(BF16)]
                        + [_unpack(ring[ro + b, sl * 8:(sl + 1) * 8, :])
                           for sl in slots[2 * t:2 * t + 2] for b in range(2)]
                        + ([jnp.zeros((48, 128), BF16)] if t else []),
                        axis=0))
                qkv[hp] = ops

            def scores(hp):
                q, kk, _ = qkv[hp]
                s = lax.dot_general(q, kk, (((1,), (1,)), ((), ())),
                                    preferred_element_type=F32)
                s = jnp.where(keep, s, fill)
                mx = jnp.max(s, axis=-1, keepdims=True)
                p = jnp.exp2((s - mx) * (SCALE * LOG2E))
                l = jnp.sum(p, axis=-1, keepdims=True)
                rl = pl.reciprocal(l, approx=True)
                rl = rl * (2.0 - l * rl)
                probs[hp] = (p * rl).astype(BF16)

            def pv(hp):
                o = _dot(probs[hp], qkv[hp][2])
                blocks.append(wo_lhs(2 * hp, o[0:8], o[16:48]).astype(BF16))
                blocks.append(wo_lhs(2 * hp + 1, o[8:16], o[48:80]).astype(BF16))

            def wo_part(h0, h1, acc=None):
                lw = jnp.concatenate(blocks[h0:h1], axis=1)
                y = _dot(lw, _cols(wov, 0, 8, E * h0, E * h1))
                return y if acc is None else y + acc

            def attend(i):
                scores(i - 1)
                if i >= 3:
                    pv(i - 3)

            def fillers(key):
                for thunk in extras.get(key, ()):
                    thunk()

            for i in range(NP):
                proj(i)
                fillers(i)
            acc = wo_part(0, 4)
            attend(NP)
            fillers(NP)
            acc = wo_part(4, cut, acc)
            pv(NP - 2)
            pv(NP - 1)
            fillers(NP + 1)
            acc = wo_part(cut, 22, acc)
            fillers(NP + 2)
            return wo_part(22, 32, acc)

        def put_x2(r0, lo, a):
            n = a.shape[0]
            x2 = (xv[pl.ds(pl.multiple_of(r0 + lo, 8), n), :].astype(F32)
                  + mod_rows(2, n) * a)
            zv[pl.ds(pl.multiple_of(HALO + r0 + lo, 8), n), :] = x2
            sums[lo:lo + n, :] = functools.reduce(
                jnp.add, [x2[:, c * 128:(c + 1) * 128] for c in range(8)])

        def p1_front(r0, sb=3):
            x2 = zv[pl.ds(pl.multiple_of(HALO + r0, 16), 64), :]
            h2 = _ln(x2, sums[...]) * mod_rows(4, 64) + mod_rows(sb, 64)
            return h2, _ln(h2)

        def w12(i):
            return jnp.concatenate(
                [_unpack(wqb[pl.ds(WB + (8 * i + c) * 512, 512), :]) for c in range(8)],
                axis=1)

        def p1_store(y, c, live):
            g = _gelu(y)
            if live is not None:
                g = jnp.where(live, g, y)
            ring[GB, c * 96 + 24:c * 96 + 88, :] = pltpu.bitcast(g, U32)

        def half_dots(lhs, i, live, done):
            part = {}

            def run(c, kh):
                row = jnp.where(live, WB + (8 * i + c) * 512, (8 * i + c) * SL)
                w = wqb[pl.ds(pl.multiple_of(row + kh * 256, 4), 256), :]
                y = _dot(lhs(kh), _unpack(w))
                if kh == 0:
                    part[c] = y
                else:
                    done(y + part[c], c)

            return [functools.partial(run, c, kh) for c in range(8) for kh in range(2)]

        def p2_front(n):
            return jnp.concatenate(
                [pltpu.bitcast(ring[GB, pl.ds(c * 96 + 8 + SHIFTS[c], n), :], F32)
                 for c in range(8)], axis=1)

        def p2_x1(h2, hs, row, gb=5):
            n = hs.shape[0]
            x1 = jnp.concatenate([h2t[...], h2[0:n - 16]], axis=0) + hs
            rows = pl.ds(pl.multiple_of(row, 16), n)
            zv[rows, :] = zv[rows, :] + mod_rows(gb, n) * x1
            return x1

        def p2_norm(x1, row, t):
            for g in range(x1.shape[0] // 16):
                y = _ln(paced(x1[16 * g:16 * g + 16, :], t))
                ttv[pl.ds(pl.multiple_of(row // 2 + 8 * g, 8), 8), :] = _pack(y)
                t = [y[0:8, 896:1024], y[8:16, 896:1024]]

        def a_body(j, mem):
            hcur[...] = hv1[pl.ds(pl.multiple_of(24 * j, 8), 24), :]
            hb = _unpack(hcur[0:8, :])
            hac = _unpack(hcur[8:16, :]).astype(F32)
            hd = _unpack(hcur[16:24, :])
            wr = [lax.rem(LEAD // 16 + 3 * j + i, RING) for i in range(3)]
            ro0 = lax.rem(4 * j, RING)
            ro1 = ro0 + 2

            live = j > 0
            dead = jnp.where(live, 0, 1)
            h2, u = p1_front(64 * (j - 1), 3 + 3 * dead)
            us[dead] = _pack(u)

            lhs = jnp.concatenate(
                [jnp.concatenate([mem, hac[0:8]], axis=0).astype(BF16), hb], axis=0)
            tok_a = {}

            def store0(c, y):
                tok_a[c] = y[0:8]
                ring[wr[0], c * 8:(c + 1) * 8, :] = _pack(y[8:24])

            deferred = {}

            def wo_lhs0(h, om, ot):
                deferred[h] = ot[24:32]
                return jnp.concatenate([om, ot[0:24]], axis=0)

            pend = []

            def flush():
                while pend:
                    p1_store(*pend.pop(), live)

            th = half_dots(lambda kh: _unpack(us[0, :, kh * 512:(kh + 1) * 512]), 0,
                           live, lambda y, c: pend.append((y, c)))
            extras = {i: [flush, th[i - 2]] for i in range(2, 18)}
            out = segment(lhs, ro0, store0, wo_lhs0, extras, 11)
            flush()
            mem = out[0:8]
            put_x2(64 * j, 0, out[8:32])

            lhs = jnp.concatenate(
                [jnp.concatenate([mem, hac[8:16]], axis=0).astype(BF16), hd], axis=0)

            def store1(c, y):
                ring[wr[1], c * 8:(c + 1) * 8, :] = _pack(
                    jnp.concatenate([tok_a[c], y[0:8]], axis=0))
                ring[wr[2], c * 8:(c + 1) * 8, :] = _pack(y[8:24])

            def wo_lhs1(h, om, ot):
                return jnp.concatenate([om, deferred[h], ot], axis=0)

            gsb[dead] = _pack(p2_front(64))
            for c in range(8):
                ring[GB, c * 96:c * 96 + 24, :] = ring[GB, c * 96 + 64:c * 96 + 88, :]
            hs = []

            def p2_fin():
                t = [hs[7][0:8], hs[7][0:8]]
                x1 = p2_x1(h2, jnp.concatenate(hs, axis=1), 64 * j, 5 + 2 * dead)
                p2_norm(x1, 64 * j, t)
                h2t[...] = h2[48:64]

            th = half_dots(lambda kh: _unpack(gsb[0, :, kh * 512:(kh + 1) * 512]), 1,
                           live, lambda y, c: hs.append(y))
            extras = {i: [th[i]] for i in range(16)}
            extras[18] = [p2_fin]
            out = segment(lhs, ro1, store1, wo_lhs1, extras, 12)
            put_x2(64 * j, 24, out[8:48])
            return out[0:8]

        def a_phase(ph, mem):
            mem = lax.fori_loop(ph, 1 + ph * (NPAIR - 1), a_body, mem)

            @pl.when(ph == 0)
            def _():
                wait(late_cps)
                for k in range(16):
                    if k < 8:
                        q = pltpu.bitcast(ring[GB, k * 96 + 24:k * 96 + 88, :], F32)
                        ring[GB, k * 96 + 16:k * 96 + 24, :] = zt[0:8, :]
                    else:
                        q = zv[0:64, (k - 8) * 128:(k - 7) * 128]
                    q = _pack(q)
                    for b in range(4):
                        ring[LQ // 16 + b, (2 * k + 1) * 8:(2 * k + 2) * 8, :] = (
                            q[8 * b:8 * b + 8])

            return mem

        with scope("aloop"):
            lax.fori_loop(0, 2, a_phase, memv[...].astype(F32))

        wait(w34_cps)

        def out_cp(i, slot):
            return cp(outv.at[slot], out_hbm.at[pl.ds(i * RB, RB), :],
                      SEM_OUT + slot)

        def p3_body(i, _):
            slot = i % 2

            @pl.when(i >= 2)
            def _():
                out_cp(i - 2, slot).wait()

            @pl.when(i == 1)
            def _():
                y = _dot(_unpack(us[0]), w12(0))
                for c in range(8):
                    p1_store(y[:, c * 128:(c + 1) * 128], c, None)
                hs = _dot(p2_front(80).astype(BF16), w12(1))
                x1l[...] = p2_x1(h2l, hs, S)

            r0 = HALO + i * RB
            tt = _unpack(ttv[pl.ds(pl.multiple_of(r0 // 2, 8), RB // 2), :])
            ys = [_dot(tt, _cols(w3v, 4 * q, 4 * q + 4)) for q in range(FF // 512)]
            ff = jnp.concatenate([_gelu(y).astype(BF16) for y in ys], axis=1)
            t = [ys[-1][240:248, 384:512], ys[-1][248:256, 384:512]]
            for g in range(4):
                rows = slice(16 * g, 16 * g + 16)
                x2 = zv[HALO + S - 64 + 16 * g:HALO + S - 48 + 16 * g, :]
                h2 = (_ln(x2, paced(sums[rows, :], t)) * mod_rows(4, 16)
                      + mod_rows(3, 16))
                h2l[rows, :] = h2
                u = _ln(h2)
                us[0, 8 * g:8 * g + 8, :] = _pack(u)
                t = [u[0:8, 896:1024], u[8:16, 896:1024]]
            p2_norm(x1l, S, t)
            gb = mod_rows(5, RB)
            for c0, c1 in ((0, 7), (7, 8)):
                cols = slice(c0 * 128, c1 * 128)
                y = _dot(ff, _cols(w4v, c0, c1))
                res = zv[pl.ds(pl.multiple_of(r0, 16), RB), cols] + gb[:, cols] * y
                outv[slot, :, cols] = res.astype(BF16)
                cp(outv.at[slot, :, cols], out_hbm.at[pl.ds(i * RB, RB), cols],
                   SEM_OUT + slot).start()
            return 0

        nb = S // RB
        with scope("p3"):
            lax.fori_loop(0, nb, p3_body, 0)
        out_cp(nb - 2, 0).wait()
        out_cp(nb - 1, 1).wait()

    pl.run_scoped(
        main,
        pltpu.VMEM((FF // 128, D // 2, 128), U32),
        pltpu.VMEM((8, FF // 2, 128), U32),
        pltpu.VMEM((S + HALO, D), F32),
        pltpu.VMEM(((S + HALO) // 2, D), U32),
    )


def _call(A_x, A_mem0, A_Wq, A_Wk, A_Wv, A_Wo, B_w1, B_w2, B_w3, B_w4, c, w_mod,
          scopes=False):
    any_spec = pl.BlockSpec(memory_space=pl.ANY)
    scratch = [
        pltpu.VMEM((S, D), BF16),
        pltpu.VMEM((M, D), BF16),
        pltpu.VMEM((48, D // 2, 128), U32),
        pltpu.VMEM((64, 8, 128), F32),
        pltpu.VMEM((WB, E), U32),
        pltpu.VMEM((WB + 16 * 512, E), U32),
        pltpu.VMEM((8, H * E // 2, 128), U32),
        pltpu.VMEM((2, 32, D), U32),
        pltpu.VMEM((2, 32, D), U32),
        pltpu.VMEM((8, LEAD // 2, 128), U32),
        pltpu.VMEM(((S - LEAD) // 2, D), U32),
        pltpu.VMEM((24, D), U32),
        pltpu.VMEM((RING + 1, 3 * H * 8, E), U32),
        pltpu.VMEM((64, 128), F32),
        pltpu.VMEM((16, D), F32),
        pltpu.VMEM((64, D), F32),
        pltpu.VMEM((80, D), F32),
        pltpu.VMEM((32, 128), U32),
        pltpu.VMEM((2, RB, D), BF16),
        pltpu.VMEM((80, 128), F32),
        pltpu.VMEM((1, D), BF16),
        pltpu.SemaphoreType.DMA((NSEM,)),
    ]
    out = pl.pallas_call(
        functools.partial(_kernel, scopes=scopes),
        in_specs=[any_spec] * 12,
        out_specs=any_spec,
        out_shape=jax.ShapeDtypeStruct((S, D), BF16),
        scratch_shapes=scratch,
        compiler_params=pltpu.CompilerParams(
            vmem_limit_bytes=126 * 1024 * 1024,
            disable_bounds_checks=True, disable_semaphore_checks=True),
    )(A_x.reshape(S, D), A_mem0.reshape(M, D), A_Wq, A_Wk, A_Wv,
      A_Wo.reshape(H * E, D), B_w1, B_w2, B_w3, B_w4, c, w_mod)
    return out.reshape(1, S, D)


def pallas_adaLN_cond__memory_aug_recurrent_mem_tr__mixer_s_mlp__prompt_kernel(
    A_x, A_mem0, A_Wq, A_Wk, A_Wv, A_Wo, A_seg_len, B_x, B_w1, B_w2, B_w3, B_w4,
    c, w_mod,
):
    if isinstance(A_seg_len, int):
        assert A_seg_len == SEG
    del B_x
    return _call(A_x, A_mem0, A_Wq, A_Wk, A_Wv, A_Wo, B_w1, B_w2, B_w3, B_w4,
                 c, w_mod)
```

```python
import contextlib
import functools

import jax
import jax.numpy as jnp
from jax import lax
import jax.experimental.pallas as pl
import jax.experimental.pallas.tpu as pltpu

F32 = jnp.float32
BF16 = jnp.bfloat16
U32 = jnp.uint32

S = 2048
D = 1024
H = 32
E = 128
M = 8
SEG = 32
FF = 3584
EPS = 1e-5
SCALE = float(E) ** -0.5
LOG2E = 1.4426950408889634

LEAD = 512
RING = 36
GB = RING
SL = 516
WB = 3 * H // 2 * SL + 544
LQ = LEAD - 64
HG = 16
NG = 3 * H // HG
NPAIR = S // (2 * SEG)
HALO = 80
RB = 256
SHIFTS = (-1, -1, 1, 1, -2, -2, 2, 2)

SEM_C = 0
SEM_X = 1
SEM_A = 2
SEM_B = 3
SEM_XR = 4
SEM_M = 5
SEM_K = 7
SEM_G = 14
SEM_OUT = 20
NSEM = 22


def _ln(x, part=None):
    if part is None:
        mu = jnp.mean(x, axis=-1, keepdims=True)
    else:
        mu = jnp.sum(part, axis=-1, keepdims=True) * (1.0 / x.shape[-1])
    xc = x - mu
    var = jnp.mean(xc * xc, axis=-1, keepdims=True)
    return xc * lax.rsqrt(var + EPS)


def _gelu(x):
    return jax.nn.gelu(x, approximate=True)


def _pack(x):
    return pltpu.bitcast(x.astype(BF16), U32)


def _unpack(x):
    return pltpu.bitcast(x, BF16)


def _dot(a, b):
    return jnp.dot(a, b, preferred_element_type=F32)


def _cols(ref, lo, hi, k0=0, k1=None):
    k1 = 2 * ref.shape[1] if k1 is None else k1
    return jnp.concatenate(
        [_unpack(ref[c, k0 // 2:k1 // 2, :]) for c in range(lo, hi)], axis=1)


def _kernel(x_hbm, mem_hbm, wq_hbm, wk_hbm, wv_hbm, wo_hbm, w1_hbm, w2_hbm,
            w3_hbm, w4_hbm, c_hbm, wmod_hbm, out_hbm,
            xv, memv, wmodv, modv, wqa, wqb, wov, us, gsb, hv0, hv1, hcur, ring,
            sums, h2t, h2l, x1l, zt, outv, fillv, cv, sems, *, scopes):
    def scope(name):
        return jax.named_scope(name) if scopes else contextlib.nullcontext()

    def cp(src, dst, s):
        return pltpu.make_async_copy(src, dst, sems.at[s])

    def col_copies(w_hbm, w_v, s, lo=0, hi=None):
        w32 = w_hbm.bitcast(U32)
        hi = w_v.shape[0] if hi is None else hi
        return [cp(w32.at[:, pl.ds(c * 128, 128)], w_v.at[c], s)
                for c in range(lo, hi)]

    def start(cps):
        for q in cps:
            q.start()

    def wait(cps):
        for q in cps:
            q.wait()

    def x_cp(r0, n, s):
        return cp(x_hbm.at[pl.ds(r0, n)], xv.at[pl.ds(r0, n)], s)

    c_cps = [cp(c_hbm, cv, SEM_C), cp(mem_hbm, memv, SEM_C)]
    x0_cp = x_cp(0, LEAD, SEM_X)
    wo_cps = col_copies(wo_hbm, wov, SEM_A)
    late_cps = [
        cp(w.bitcast(U32).at[:, pl.ds(c * 128, 128)],
           wqb.at[pl.ds(WB + (8 * i + c) * 512, 512)], SEM_XR)
        for i, w in enumerate((w1_hbm, w2_hbm)) for c in range(8)]

    def mod_rows(i, n):
        m = jnp.concatenate([modv[8 * i + c] for c in range(8)], axis=1)
        return jnp.concatenate([m] * (n // 8), axis=0)

    HI = jnp.uint32(0xFFFF0000)
    wq2 = (wqa, wqb)

    def paced(x, tiles):
        z = [pltpu.bitcast((t if t.dtype == U32 else pltpu.bitcast(t, U32))
                           & zt[0:8, :], F32) for t in tiles]
        z = jnp.concatenate(z, axis=0)
        if x.shape[1] == 128:
            return x + z
        return jnp.concatenate([x[:, 0:128] + z, x[:, 128:]], axis=1)

    def h_rest(k, t):
        xf = xv[pl.ds(pl.multiple_of(LEAD + 16 * k, 16), 16), :].astype(F32)
        y = _ln(paced(xf, t)) * mod_rows(1, 16) + mod_rows(0, 16)
        hv1[pl.ds(pl.multiple_of(8 * k, 8), 8), :] = _pack(y)
        return [y[0:8, 896:1024], y[8:16, 896:1024]]

    def prologue(st, xn, acc, scol, hn):
        w_hbms = (wq_hbm, wk_hbm, wv_hbm)

        def st_src(i):
            return w_hbms[i // 2].bitcast(U32).at[:, pl.ds((i % 2) * 8, 8), :]

        def pair_cps(n, s):
            w32 = wmod_hbm.bitcast(U32)
            return [cp(w32.at[:, pl.ds(pl.multiple_of(c * 128, 128), 128)],
                       wmodv.at[c], s) for c in (n, 8 + n)]

        def k_cps(n):
            return [cp(st_src(i).at[pl.ds(n * 128, 128)],
                       st.at[i, pl.ds(n * 128, 128)], SEM_K + n) for i in range(2)]

        def g_cps(g, src):
            return [cp(st_src(src), st.at[g], SEM_G + g - 1),
                    x_cp(pl.multiple_of(LEAD + 384 * (g - 2), 128), 384,
                         SEM_G + g - 1)]

        def mod_cps(g):
            lo, hi = {3: (16, 27), 4: (27, 38), 5: (38, 48)}[g]
            return col_copies(wmod_hbm, wmodv, SEM_G + g, lo, hi)

        with scope("first"):
            start(c_cps + [x0_cp])
        for n in range(8):
            start((pair_cps(n, SEM_M + n) if n < 2 else []) + k_cps(n)
                  + (pair_cps(n + 1, SEM_K + n) if 0 < n < 7 else []))
        start(g_cps(2, 2) + g_cps(3, 3) + g_cps(4, 4) + mod_cps(3) + g_cps(5, 5))

        r = lax.broadcasted_iota(jnp.int32, (80, 128), 0)
        k = lax.broadcasted_iota(jnp.int32, (80, 128), 1)

        def head_of(i):
            return jnp.where(i < 16, i // 8, (i - 16) // 32)

        def pos_of(i):
            return jnp.where(i < 16, i % 8, 8 + (i - 16) % 32)

        same = head_of(r) == head_of(k)
        vis = (pos_of(r) < M) | (pos_of(r) >= pos_of(k))
        fillv[...] = jnp.where(same, jnp.where(vis, 0.0, -1e9 / SCALE),
                               -jnp.inf).astype(F32)
        sums[...] = jnp.zeros(sums.shape, F32)
        modv[48:56] = jnp.zeros((8, 8, 128), F32)
        modv[56:64] = jnp.ones((8, 8, 128), F32)
        ring[GB] = jnp.zeros(ring.shape[1:], U32)
        zt[...] = jnp.zeros(zt.shape, U32)
        h2t[...] = jnp.zeros(h2t.shape, F32)
        x1l[...] = jnp.zeros(x1l.shape, F32)

        def zero_body(i, _):
            rows = pl.ds(pl.multiple_of((i & 3) * 128, 128), 128)
            acc[lax.shift_right_logical(i, 2), rows, :] = jnp.zeros((128, 512), F32)
            return 0

        lax.fori_loop(0, 32, zero_body, 0)

        wait(c_cps)
        cf = cv[...].astype(F32)
        sil = cf * jax.nn.sigmoid(cf)
        for c in range(8):
            sw = _pack(jnp.broadcast_to(sil[:, c * 128:(c + 1) * 128], (128, 128)).T)
            scol[0, c * 64:(c + 1) * 64, :] = pltpu.bitcast(sw << 16, F32)
            scol[1, c * 64:(c + 1) * 64, :] = pltpu.bitcast(sw & HI, F32)

        x0_cp.wait()

        def ln_body(i, _):
            r0 = pl.multiple_of(i * 64, 64)
            y = _ln(xv[pl.ds(r0, 64), :].astype(F32))
            for q in range(8):
                xn[q, pl.ds(r0, 64), :] = y[:, q * 128:(q + 1) * 128]
            return 0

        lax.fori_loop(0, LEAD // 64, ln_body, 0)

        class Mod:
            def __init__(self, tiles, offs):
                self.tiles, self.offs = tiles, offs
                self.n, self.acc, self.out = 0, None, []

            def items(self, n, pace=None):
                for it in range(self.n, min(self.n + n, 64 * len(self.tiles))):
                    c, i = divmod(it, 64)
                    w = wmodv[self.tiles[c], i * 8:(i + 1) * 8, :]
                    if pace is not None:
                        w = w | pace
                    v = (pltpu.bitcast(w << 16, F32) * scol[0, i * 8:(i + 1) * 8, :]
                         + pltpu.bitcast(w & HI, F32) * scol[1, i * 8:(i + 1) * 8, :])
                    self.acc = v if i == 0 else self.acc + v
                    if i == 63:
                        m = jnp.broadcast_to(
                            jnp.sum(self.acc, axis=0, keepdims=True) + self.offs[c],
                            (8, 128))
                        modv[self.tiles[c]] = m
                        self.out.append(m)
                self.n += n

        def h_lead(n, b, sa, ca):
            rep = lambda m: jnp.concatenate([m, m], axis=0)
            y = _pack(xn[n, 16 * b:16 * b + 16, :] * rep(ca) + rep(sa))
            hn[8 * b:8 * b + 8, :] = y
            hv0[n, 8 * b:8 * b + 8, :] = y

        def relayout(par, g, p0, n, pace=None):
            base = g * (8 * SL)
            mask = jnp.uint32(0xFFFF0000 if par else 0xFFFF)
            if pace is not None:
                mask = pace | mask
            for u in range(n):
                a = st[g, 2 * (p0 + u)]
                b = st[g, 2 * (p0 + u) + 1]
                if par == 0:
                    w = (a & mask) | (b << 16)
                else:
                    w = (a >> 16) | (b & mask)
                wq2[par][pl.ds(base + p0 + u, 8, stride=SL), :] = w

        def to_ring(y, par, s0, b0):
            for u in range(y.shape[1] // 128):
                row = pl.multiple_of((2 * (s0 + u) + par) * 8, 8)
                for b in range(y.shape[0] // 8):
                    ring[b0 + b, pl.ds(row, 8), :] = (
                        y[b * 8:(b + 1) * 8, u * 128:(u + 1) * 128])

        def k_body(n, _):
            @pl.when(n < 2)
            def _():
                wait(pair_cps(n, SEM_M + n))
                md = Mod([n, 8 + n], [0.0, 1.0])
                md.items(128)
                for b in range(32):
                    h_lead(n, b, *md.out)

            wait(k_cps(n))

            @pl.when((n > 0) & (n < 7))
            def _():
                wait(pair_cps(n + 1, SEM_K + n))

            nn = jnp.where(n == 0, 0, jnp.minimum(n + 1, 7))
            md = Mod([nn, 8 + nn], [0.0, 1.0])
            zero = zt[0:8, :]
            order = [(0, 0), (1, 0), (0, 1), (1, 1)]
            relayout(0, 0, n * 64, 64)
            for i, (par, g) in enumerate(order):
                for hq in range(2):
                    s0 = g * 8 + hq * 4
                    w = jnp.concatenate(
                        [_unpack(wq2[par][pl.ds(pl.multiple_of(
                            (s0 + u) * SL + n * 64, 4), 64), :])
                         for u in range(4)], axis=1)
                    m = LQ if par else LEAD
                    y = _dot(_unpack(hn[0:m // 2, :]), w) + acc[2 * i + hq, 0:m, :]
                    acc[2 * i + hq, 0:m, :] = y
                    y = _pack(y)
                    to_ring(y, par, s0, 0)
                    tiles = [y[8 * b:8 * b + 8, 0:128] & zero for b in range(m // 16)]
                    tiles = [tiles[b * len(tiles) // 32] for b in range(32)]
                    for b in range(32):
                        pace = tiles[b]
                        if hq == 0 and i < 3:
                            relayout(*order[i + 1], n * 64 + 2 * b, 2, pace)
                        elif hq == 1 and i < 3:
                            md.items(2 - b % 2, pace)
                        elif hq == 1:
                            sa, ca = md.out
                            ca = ca + pltpu.bitcast(tiles[max(b - 3, 0)], F32)
                            h_lead(nn, b, sa, ca)
            return 0

        with scope("ksteps"):
            lax.fori_loop(0, 8, k_body, 0)

        start(mod_cps(4) + mod_cps(5) + wo_cps + late_cps)
        for c in range(8):
            hl = hv0[c, LQ // 2:LEAD // 2, :]
            us[0, :, c * 128:(c + 1) * 128] = hl
            gsb[0, :, c * 128:(c + 1) * 128] = hl
        wait(g_cps(2, 2))

        def rl_body(i, _):
            relayout(0, 2, i * 64, 64)
            return 0

        lax.fori_loop(0, 8, rl_body, 0)

        def lead_proj(par, s0, n, rc, rl, mp=128):
            w = jnp.concatenate(
                [_unpack(wq2[par][pl.ds(pl.multiple_of((s0 + u) * SL, 4), 512), :])
                 for u in range(n)], axis=1)
            lhs = jnp.concatenate(
                [_unpack(hv0[q, rc * mp:(rc + 1) * mp, :]) for q in range(8)],
                axis=1)
            y = _pack(_dot(lhs, w))
            to_ring(y, par, s0, rc * mp // 8)
            zero = zt[0:8, :]
            for u in range(n):
                for b in range(mp // 8):
                    k = min(3, 512 - rl[2])
                    if k > 0:
                        relayout(rl[0], rl[1], rl[2], k,
                                 y[b * 8:(b + 1) * 8, u * 128:(u + 1) * 128] & zero)
                        rl[2] += k
            return y

        def group_body(g, _):
            rl = [1, g, 0]
            for k in range(32):
                y = lead_proj(0, g * 8 + k // 4, 1, k % 4, rl, 64)
                if k == 12:
                    ts = [[y[0:8], y[16:24]], [y[40:48], y[56:64]]]
                    for i in range(24):
                        ts[i % 2] = h_rest(24 * (g - 2) + i, ts[i % 2])

            @pl.when(g < NG - 1)
            def _():
                wait(g_cps(g + 1, 0))

            for gg in (3, 4, 5):
                @pl.when(g == gg)
                def _(gg=gg):
                    wait(mod_cps(gg))

            gn = jnp.minimum(g + 1, NG - 1)
            t0 = jnp.where(g == 2, 0, jnp.minimum(11 * g - 17, 37))
            part = [lax.shift_right_logical(t0 + c, 3) for c in range(11)]
            md = Mod([t0 + c for c in range(11)],
                     [jnp.where((p == 1) | (p == 4), 1.0, 0.0).astype(F32)
                      for p in part])
            rl = [0, gn, 0]
            for k in range(16):
                y = lead_proj(1, g * 8 + k // 2, 1, k % 2, rl)
                for b in range(16):
                    md.items(3, y[8 * b:8 * b + 8] & zt[0:8, :])
            assert len(md.out) == 11
            return 0

        with scope("groups"):
            lax.fori_loop(2, NG, group_body, 0)

    pl.run_scoped(
        prologue,
        pltpu.VMEM((NG, D, 8, E), U32),
        pltpu.VMEM((8, LEAD, 128), F32),
        pltpu.VMEM((8, LEAD, 512), F32),
        pltpu.VMEM((2, D // 2, 128), F32),
        pltpu.VMEM((LEAD // 2, 128), U32),
    )

    def main(w3v, w4v, zv, ttv):
        w34_cps = col_copies(w3_hbm, w3v, SEM_B) + col_copies(w4_hbm, w4v, SEM_B)
        start(w34_cps)
        zv[0:HALO, :] = jnp.zeros((HALO, D), F32)
        wait(wo_cps)

        def segment(lhs, ro, store_tok, wo_lhs, extras, cut):
            fill = fillv[...]
            keep = fill == 0.0
            NP = H // 2
            qkv, probs, blocks = {}, {}, []

            def proj(hp):
                slots = [t * H + 2 * hp + par for t in range(3) for par in range(2)]
                wt = [jnp.concatenate(
                    [_unpack(wq2[sl % 2][pl.ds((sl // 2) * SL, 512), :])
                     for sl in slots[2 * t:2 * t + 2]], axis=1) for t in range(3)]
                if hp == 0:
                    w = jnp.concatenate(wt, axis=1)
                    y = _dot(lhs[:, :512], w[:512])
                    y = _dot(lhs[:, 512:], w[512:]) + y
                else:
                    ys = [_dot(lhs, wt[0]), _dot(lhs, wt[1])]
                    attend(hp)
                    y = jnp.concatenate(ys + [_dot(lhs, wt[2])], axis=1)
                for u, sl in enumerate(slots):
                    store_tok(sl, y[8:32, u * 128:(u + 1) * 128])
                ops = []
                for t in range(3):
                    ym = jnp.concatenate(
                        [y[0:8, (2 * t) * 128:(2 * t + 1) * 128],
                         y[0:8, (2 * t + 1) * 128:(2 * t + 2) * 128]], axis=0)
                    ops.append(jnp.concatenate(
                        [ym.astype(BF16)]
                        + [_unpack(ring[ro + b, sl * 8:(sl + 1) * 8, :])
                           for sl in slots[2 * t:2 * t + 2] for b in range(2)]
                        + ([jnp.zeros((48, 128), BF16)] if t else []),
                        axis=0))
                qkv[hp] = ops

            def scores(hp):
                q, kk, _ = qkv[hp]
                s = lax.dot_general(q, kk, (((1,), (1,)), ((), ())),
                                    preferred_element_type=F32)
                s = jnp.where(keep, s, fill)
                mx = jnp.max(s, axis=-1, keepdims=True)
                p = jnp.exp2((s - mx) * (SCALE * LOG2E))
                l = jnp.sum(p, axis=-1, keepdims=True)
                rl = pl.reciprocal(l, approx=True)
                rl = rl * (2.0 - l * rl)
                probs[hp] = (p * rl).astype(BF16)

            def pv(hp):
                o = _dot(probs[hp], qkv[hp][2])
                blocks.append(wo_lhs(2 * hp, o[0:8], o[16:48]).astype(BF16))
                blocks.append(wo_lhs(2 * hp + 1, o[8:16], o[48:80]).astype(BF16))

            def wo_part(h0, h1, acc=None):
                lw = jnp.concatenate(blocks[h0:h1], axis=1)
                y = _dot(lw, _cols(wov, 0, 8, E * h0, E * h1))
                return y if acc is None else y + acc

            def attend(i):
                scores(i - 1)
                if i >= 3:
                    pv(i - 3)

            def fillers(key):
                for thunk in extras.get(key, ()):
                    thunk()

            for i in range(NP):
                proj(i)
                fillers(i)
            acc = wo_part(0, 4)
            attend(NP)
            fillers(NP)
            acc = wo_part(4, cut, acc)
            pv(NP - 2)
            pv(NP - 1)
            fillers(NP + 1)
            acc = wo_part(cut, 22, acc)
            fillers(NP + 2)
            return wo_part(22, 32, acc)

        def put_x2(r0, lo, a):
            n = a.shape[0]
            x2 = (xv[pl.ds(pl.multiple_of(r0 + lo, 8), n), :].astype(F32)
                  + mod_rows(2, n) * a)
            zv[pl.ds(pl.multiple_of(HALO + r0 + lo, 8), n), :] = x2
            sums[lo:lo + n, :] = functools.reduce(
                jnp.add, [x2[:, c * 128:(c + 1) * 128] for c in range(8)])

        def p1_front(r0, sb=3):
            x2 = zv[pl.ds(pl.multiple_of(HALO + r0, 16), 64), :]
            h2 = _ln(x2, sums[...]) * mod_rows(4, 64) + mod_rows(sb, 64)
            return h2, _ln(h2)

        def w12(i):
            return jnp.concatenate(
                [_unpack(wqb[pl.ds(WB + (8 * i + c) * 512, 512), :]) for c in range(8)],
                axis=1)

        def p1_store(y, c, live):
            g = _gelu(y)
            if live is not None:
                g = jnp.where(live, g, y)
            ring[GB, c * 96 + 24:c * 96 + 88, :] = pltpu.bitcast(g, U32)

        def half_dots(lhs, i, live, done):
            part = {}

            def run(c, kh):
                row = jnp.where(live, WB + (8 * i + c) * 512, (8 * i + c) * SL)
                w = wqb[pl.ds(pl.multiple_of(row + kh * 256, 4), 256), :]
                y = _dot(lhs(kh), _unpack(w))
                if kh == 0:
                    part[c] = y
                else:
                    done(y + part[c], c)

            return [functools.partial(run, c, kh) for c in range(8) for kh in range(2)]

        def p2_front(n):
            return jnp.concatenate(
                [pltpu.bitcast(ring[GB, pl.ds(c * 96 + 8 + SHIFTS[c], n), :], F32)
                 for c in range(8)], axis=1)

        def p2_x1(h2, hs, row, gb=5):
            n = hs.shape[0]
            x1 = jnp.concatenate([h2t[...], h2[0:n - 16]], axis=0) + hs
            rows = pl.ds(pl.multiple_of(row, 16), n)
            zv[rows, :] = zv[rows, :] + mod_rows(gb, n) * x1
            return x1

        def p2_norm(x1, row, t):
            for g in range(x1.shape[0] // 16):
                y = _ln(paced(x1[16 * g:16 * g + 16, :], t))
                ttv[pl.ds(pl.multiple_of(row // 2 + 8 * g, 8), 8), :] = _pack(y)
                t = [y[0:8, 896:1024], y[8:16, 896:1024]]

        def a_body(j, mem):
            hcur[...] = hv1[pl.ds(pl.multiple_of(24 * j, 8), 24), :]
            hb = _unpack(hcur[0:8, :])
            hac = _unpack(hcur[8:16, :]).astype(F32)
            hd = _unpack(hcur[16:24, :])
            wr = [lax.rem(LEAD // 16 + 3 * j + i, RING) for i in range(3)]
            ro0 = lax.rem(4 * j, RING)
            ro1 = ro0 + 2

            live = j > 0
            dead = jnp.where(live, 0, 1)
            h2, u = p1_front(64 * (j - 1), 3 + 3 * dead)
            us[dead] = _pack(u)

            lhs = jnp.concatenate(
                [jnp.concatenate([mem, hac[0:8]], axis=0).astype(BF16), hb], axis=0)
            tok_a = {}

            def store0(c, y):
                tok_a[c] = y[0:8]
                ring[wr[0], c * 8:(c + 1) * 8, :] = _pack(y[8:24])

            deferred = {}

            def wo_lhs0(h, om, ot):
                deferred[h] = ot[24:32]
                return jnp.concatenate([om, ot[0:24]], axis=0)

            pend = []

            def flush():
                while pend:
                    p1_store(*pend.pop(), live)

            th = half_dots(lambda kh: _unpack(us[0, :, kh * 512:(kh + 1) * 512]), 0,
                           live, lambda y, c: pend.append((y, c)))
            extras = {i: [flush, th[i - 2]] for i in range(2, 18)}
            out = segment(lhs, ro0, store0, wo_lhs0, extras, 11)
            flush()
            mem = out[0:8]
            put_x2(64 * j, 0, out[8:32])

            lhs = jnp.concatenate(
                [jnp.concatenate([mem, hac[8:16]], axis=0).astype(BF16), hd], axis=0)

            def store1(c, y):
                ring[wr[1], c * 8:(c + 1) * 8, :] = _pack(
                    jnp.concatenate([tok_a[c], y[0:8]], axis=0))
                ring[wr[2], c * 8:(c + 1) * 8, :] = _pack(y[8:24])

            def wo_lhs1(h, om, ot):
                return jnp.concatenate([om, deferred[h], ot], axis=0)

            gsb[dead] = _pack(p2_front(64))
            for c in range(8):
                ring[GB, c * 96:c * 96 + 24, :] = ring[GB, c * 96 + 64:c * 96 + 88, :]
            hs = []

            def p2_fin():
                t = [hs[7][0:8], hs[7][0:8]]
                x1 = p2_x1(h2, jnp.concatenate(hs, axis=1), 64 * j, 5 + 2 * dead)
                p2_norm(x1, 64 * j, t)
                h2t[...] = h2[48:64]

            th = half_dots(lambda kh: _unpack(gsb[0, :, kh * 512:(kh + 1) * 512]), 1,
                           live, lambda y, c: hs.append(y))
            extras = {i: [th[i]] for i in range(16)}
            extras[18] = [p2_fin]
            out = segment(lhs, ro1, store1, wo_lhs1, extras, 12)
            put_x2(64 * j, 24, out[8:48])
            return out[0:8]

        def a_phase(ph, mem):
            mem = lax.fori_loop(ph, 1 + ph * (NPAIR - 1), a_body, mem)

            @pl.when(ph == 0)
            def _():
                wait(late_cps)
                for k in range(16):
                    if k < 8:
                        q = pltpu.bitcast(ring[GB, k * 96 + 24:k * 96 + 88, :], F32)
                        ring[GB, k * 96 + 16:k * 96 + 24, :] = zt[0:8, :]
                    else:
                        q = zv[0:64, (k - 8) * 128:(k - 7) * 128]
                    q = _pack(q)
                    for b in range(4):
                        ring[LQ // 16 + b, (2 * k + 1) * 8:(2 * k + 2) * 8, :] = (
                            q[8 * b:8 * b + 8])

            return mem

        with scope("aloop"):
            lax.fori_loop(0, 2, a_phase, memv[...].astype(F32))

        wait(w34_cps)

        def out_cp(i, slot):
            return cp(outv.at[slot], out_hbm.at[pl.ds(i * RB, RB), :],
                      SEM_OUT + slot)

        def p3_body(i, _):
            slot = i % 2

            @pl.when(i >= 2)
            def _():
                out_cp(i - 2, slot).wait()

            @pl.when(i == 1)
            def _():
                y = _dot(_unpack(us[0]), w12(0))
                for c in range(8):
                    p1_store(y[:, c * 128:(c + 1) * 128], c, None)
                hs = _dot(p2_front(80).astype(BF16), w12(1))
                x1l[...] = p2_x1(h2l, hs, S)

            r0 = HALO + i * RB
            tt = _unpack(ttv[pl.ds(pl.multiple_of(r0 // 2, 8), RB // 2), :])
            ys = [_dot(tt, _cols(w3v, 4 * q, 4 * q + 4)) for q in range(FF // 512)]
            ff = jnp.concatenate([_gelu(y).astype(BF16) for y in ys], axis=1)
            t = [ys[-1][240:248, 384:512], ys[-1][248:256, 384:512]]
            for g in range(4):
                rows = slice(16 * g, 16 * g + 16)
                x2 = zv[HALO + S - 64 + 16 * g:HALO + S - 48 + 16 * g, :]
                h2 = (_ln(x2, paced(sums[rows, :], t)) * mod_rows(4, 16)
                      + mod_rows(3, 16))
                h2l[rows, :] = h2
                u = _ln(h2)
                us[0, 8 * g:8 * g + 8, :] = _pack(u)
                t = [u[0:8, 896:1024], u[8:16, 896:1024]]
            p2_norm(x1l, S, t)
            gb = mod_rows(5, RB)
            for c0, c1 in ((0, 7), (7, 8)):
                cols = slice(c0 * 128, c1 * 128)
                y = _dot(ff, _cols(w4v, c0, c1))
                res = zv[pl.ds(pl.multiple_of(r0, 16), RB), cols] + gb[:, cols] * y
                outv[slot, :, cols] = res.astype(BF16)
                cp(outv.at[slot, :, cols], out_hbm.at[pl.ds(i * RB, RB), cols],
                   SEM_OUT + slot).start()
            return 0

        nb = S // RB
        with scope("p3"):
            lax.fori_loop(0, nb, p3_body, 0)
        out_cp(nb - 2, 0).wait()
        out_cp(nb - 1, 1).wait()

    pl.run_scoped(
        main,
        pltpu.VMEM((FF // 128, D // 2, 128), U32),
        pltpu.VMEM((8, FF // 2, 128), U32),
        pltpu.VMEM((S + HALO, D), F32),
        pltpu.VMEM(((S + HALO) // 2, D), U32),
    )


def _compiler_params():
    vmem = 126 * 1024 * 1024
    try:
        return pltpu.CompilerParams(vmem_limit_bytes=vmem, disable_bounds_checks=True,
                                    disable_semaphore_checks=True)
    except TypeError:
        return pltpu.CompilerParams(vmem_limit_bytes=vmem)


def _call(A_x, A_mem0, A_Wq, A_Wk, A_Wv, A_Wo, B_w1, B_w2, B_w3, B_w4, c, w_mod,
          scopes=False):
    any_spec = pl.BlockSpec(memory_space=pl.ANY)
    scratch = [
        pltpu.VMEM((S, D), BF16),
        pltpu.VMEM((M, D), BF16),
        pltpu.VMEM((48, D // 2, 128), U32),
        pltpu.VMEM((64, 8, 128), F32),
        pltpu.VMEM((WB, E), U32),
        pltpu.VMEM((WB + 16 * 512, E), U32),
        pltpu.VMEM((8, H * E // 2, 128), U32),
        pltpu.VMEM((2, 32, D), U32),
        pltpu.VMEM((2, 32, D), U32),
        pltpu.VMEM((8, LEAD // 2, 128), U32),
        pltpu.VMEM(((S - LEAD) // 2, D), U32),
        pltpu.VMEM((24, D), U32),
        pltpu.VMEM((RING + 1, 3 * H * 8, E), U32),
        pltpu.VMEM((64, 128), F32),
        pltpu.VMEM((16, D), F32),
        pltpu.VMEM((64, D), F32),
        pltpu.VMEM((80, D), F32),
        pltpu.VMEM((32, 128), U32),
        pltpu.VMEM((2, RB, D), BF16),
        pltpu.VMEM((80, 128), F32),
        pltpu.VMEM((1, D), BF16),
        pltpu.SemaphoreType.DMA((NSEM,)),
    ]
    out = pl.pallas_call(
        functools.partial(_kernel, scopes=scopes),
        in_specs=[any_spec] * 12,
        out_specs=any_spec,
        out_shape=jax.ShapeDtypeStruct((S, D), BF16),
        scratch_shapes=scratch,
        compiler_params=_compiler_params(),
    )(A_x.reshape(S, D), A_mem0.reshape(M, D), A_Wq, A_Wk, A_Wv,
      A_Wo.reshape(H * E, D), B_w1, B_w2, B_w3, B_w4, c, w_mod)
    return out.reshape(1, S, D)


def pallas_adaLN_cond__memory_aug_recurrent_mem_tr__mixer_s_mlp__prompt_kernel(
    A_x, A_mem0, A_Wq, A_Wk, A_Wv, A_Wo, A_seg_len, B_x, B_w1, B_w2, B_w3, B_w4,
    c, w_mod,
):
    if isinstance(A_seg_len, int):
        assert A_seg_len == SEG
    del B_x
    return _call(A_x, A_mem0, A_Wq, A_Wk, A_Wv, A_Wo, B_w1, B_w2, B_w3, B_w4,
                 c, w_mod)
```
